```python
import jax
import jax.numpy as jnp

def _softmax(x, axis=-1):
    return jax.nn.softmax(x, axis=axis)
def _gelu(x):
    return jax.nn.gelu(x, approximate=True)
def _silu(x):
    return jax.nn.silu(x)
def _sigmoid(x):
    return jax.nn.sigmoid(x)
def _layernorm(x, axis=-1, eps=1e-5):
    m = jnp.mean(x, axis=axis, keepdims=True)
    v = jnp.var(x, axis=axis, keepdims=True)
    return (x - m) / jnp.sqrt(v + eps)
def _scatter_add(tgt, idx, src, axis=0):
    return tgt.at[idx].add(src)
def _segment_sum(src, seg, n):
    return jax.ops.segment_sum(src, seg, n)
class _Rng:
    def __init__(self, key):
        self._k = key
    def _next(self):
        self._k, sub = jax.random.split(self._k)
        return sub
    def normal(self, shape):
        return jax.random.normal(self._next(), shape, dtype=jnp.bfloat16)
    def randint(self, lo, hi, shape):
        return jax.random.randint(self._next(), shape, lo, hi, dtype=jnp.int32)
    def uniform(self, shape, lo=0.0, hi=1.0):
        return jax.random.uniform(self._next(), shape, jnp.bfloat16, lo, hi)
    def permutation(self, n):
        return jax.random.permutation(self._next(), n)


kernel_name = 'gated_mix__compressed_kv_cla__sliding_local_dilated__prompt'

def setup_inputs():
    _rng = _Rng(jax.random.key(int.from_bytes(__import__("os").urandom(4), "little")))
    _w = (lambda a: (lambda t: t.astype(jnp.bfloat16) if jnp.issubdtype(t.dtype, jnp.floating) else t)(jnp.asarray(a)))
    def _A_setup():
        B, H, Sq, Sk, D, M = 1, 32, 2048, 2048, 128, 1024
        Dc = 4 * D
        return {
            "x": _w((lambda *s: _rng.normal(s) * 0.05)(B, Sq, M)),
            "c_kv": _w((lambda *s: _rng.normal(s) * 0.05)(B, Sk, Dc)),
            "w_q": _w((lambda *s: _rng.normal(s) * 0.05)(M, H, D) * (M ** -0.5)),
            "w_uk": _w((lambda *s: _rng.normal(s) * 0.05)(Dc, H, D) * (Dc ** -0.5)),
            "w_uv": _w((lambda *s: _rng.normal(s) * 0.05)(Dc, H, D) * (Dc ** -0.5)),
            "w_o": _w((lambda *s: _rng.normal(s) * 0.05)(H, D, M) * ((H * D) ** -0.5)),
        }
    _A_in = _A_setup()

    def _B_setup():
        B, S, D = 1, 2048, 1024
        return {
            "x": _w((lambda *s: _rng.normal(s) * 0.05)(B, S, D)),
            "wqkv": _w((lambda *s: _rng.normal(s) * 0.05)(D, 3 * D)),
            "wo": _w((lambda *s: _rng.normal(s) * 0.05)(D, D)),
        }
    _B_in = _B_setup()

    return {
        "A_x": _A_in["x"],
        "A_c_kv": _A_in["c_kv"],
        "A_w_q": _A_in["w_q"],
        "A_w_uk": _A_in["w_uk"],
        "A_w_uv": _A_in["w_uv"],
        "A_w_o": _A_in["w_o"],
        "B_x": _B_in["x"],
        "B_wqkv": _B_in["wqkv"],
        "B_wo": _B_in["wo"],
        "gate_w": _w((lambda *s: _rng.normal(s) * 0.05)(1024)),
    }

def reference(A_x, A_c_kv, A_w_q, A_w_uk, A_w_uv, A_w_o, B_x, B_wqkv, B_wo, gate_w):
    def _A_ref(x, c_kv, w_q, w_uk, w_uv, w_o):
        B, Sq, M = x.shape[0], x.shape[1], x.shape[2]
        Sk = c_kv.shape[1]
        H, D = w_q.shape[1], w_q.shape[2]
        q = jnp.einsum("bqm,mhd->bhqd", x, w_q)
        k = jnp.einsum("bkc,chd->bhkd", c_kv, w_uk)
        v = jnp.einsum("bkc,chd->bhkd", c_kv, w_uv)
        scores = jnp.einsum("bhqd,bhkd->bhqk", q, k) * (D ** -0.5)
        off = Sk - Sq
        qi = jnp.arange(Sq)[:, None]
        kj = jnp.arange(Sk)[None, :]
        cmask = kj <= (qi + off)
        scores = jnp.where(cmask[None, None], scores, -1e9)
        p = _softmax(scores, axis=-1)
        ctx = jnp.einsum("bhqk,bhkd->bhqd", p, v)
        return jnp.einsum("bhqd,hdm->bqm", ctx, w_o)

    def _B_ref(x, wqkv, wo):
        B, S, D = x.shape
        H = 32; Dh = D // H
        W, dil = 8, 2
        qkv = (lambda x, *d: x.transpose(*d))((x @ wqkv).reshape(B, S, 3, H, Dh), 2, 0, 3, 1, 4)
        q, k, v = qkv[0], qkv[1], qkv[2]
        scale = Dh ** -0.5
        pos = jnp.arange(S)
        off = jnp.arange(W) * dil
        idx = pos[:, None] - off[None, :]
        mask = idx >= 0
        idx_c = jnp.where(mask, idx, 0).reshape(-1)
        kg = k[:, :, idx_c, :].reshape(B, H, S, W, Dh)
        vg = v[:, :, idx_c, :].reshape(B, H, S, W, Dh)
        logits = jnp.einsum("bhsd,bhswd->bhsw", q, kg) * scale
        logits = jnp.where(mask[None, None, :, :], logits, -1e9)
        attn = _softmax(logits, axis=-1)
        o = jnp.einsum("bhsw,bhswd->bhsd", attn, vg)
        return (lambda x, *d: x.transpose(*d))(o, 0, 2, 1, 3).reshape(B, S, D) @ wo

    x = A_x
    g = _sigmoid((x * gate_w).sum(-1, keepdims=True))
    a = _A_ref(x, A_c_kv, A_w_q, A_w_uk, A_w_uv, A_w_o)
    b = _B_ref(x, B_wqkv, B_wo)
    return g * a + (1 - g) * b
```

```python
import functools
import math

import jax
import jax.numpy as jnp
from jax import lax
import jax.experimental.pallas as pl
import jax.experimental.pallas.tpu as pltpu

S = 2048
M = 1024
DC = 512
H = 32
D = 128
DH = 32
W = 8
DIL = 2
PAD = 16
TQ = 256
TB = 128
TO = 256
LOG2E = 1.4426950408889634
NEG = -1e9

F32 = jnp.float32
BF16 = jnp.bfloat16
NT = (((1,), (1,)), ((), ()))


def _split_pair(w):
    lo = pltpu.bitcast(w << 16, F32).astype(BF16)
    hi = pltpu.bitcast(w & jnp.uint32(0xFFFF0000), F32).astype(BF16)
    return jnp.concatenate([lo, hi], axis=1)


def _load_pair(w_u, p, n):
    hp = H // 2
    base = pl.multiple_of((p // 4) * 4, 4)
    view = w_u.at[pl.ds(base, n * hp - 12), :]
    r = p % 4
    c = [view[pl.ds(j, n, stride=hp), :] for j in range(4)]
    return jnp.where(r < 2, jnp.where(r == 0, c[0], c[1]), jnp.where(r == 2, c[2], c[3]))


def _kernel(x_hbm, ckv_hbm, wq_hbm, wuk_hbm, wuv_hbm, wo_hbm, bqkv_hbm, bwo_hbm, gate_ref,
            out_hbm,
            x_v, ckv_v, wq_v, wuk_v, wuv_v, wall_v, bqkv_v, bwo_v, wtp_v, tmp_v,
            qb_v, kb_v, vb_v, ctx_v, g_v, q_s, k_s, v_s, o_st, in_sems, out_sems):
    copies = [
        pltpu.make_async_copy(ckv_hbm, ckv_v, in_sems.at[0]),
        pltpu.make_async_copy(wuk_hbm, wuk_v, in_sems.at[1]),
        pltpu.make_async_copy(wuv_hbm, wuv_v, in_sems.at[2]),
        pltpu.make_async_copy(x_hbm, x_v, in_sems.at[3]),
        pltpu.make_async_copy(wq_hbm, wq_v, in_sems.at[4]),
        pltpu.make_async_copy(bqkv_hbm, bqkv_v, in_sems.at[5]),
        pltpu.make_async_copy(bwo_hbm, bwo_v, in_sems.at[6]),
        pltpu.make_async_copy(wo_hbm, wall_v.at[pl.ds(0, H * D), :], in_sems.at[7]),
    ]
    for c in copies:
        c.start()
    for c in copies[:5]:
        c.wait()

    gw = gate_ref[...].astype(F32)

    def gate_body(i, _):
        r = pl.multiple_of(i * 256, 256)
        z = jnp.sum(x_v[pl.ds(r, 256), :].astype(F32) * gw, axis=1, keepdims=True)
        g = 1.0 / (1.0 + jnp.exp(-z))
        g_v[pl.ds(r, 256), :] = jnp.broadcast_to(g, (256, 128))
        return 0

    lax.fori_loop(0, S // 256, gate_body, 0)

    wq_u = wq_v.bitcast(jnp.uint32)
    wuk_u = wuk_v.bitcast(jnp.uint32)
    wuv_u = wuv_v.bitcast(jnp.uint32)
    row = lax.broadcasted_iota(jnp.int32, (TQ, TQ), 0)
    col = lax.broadcasted_iota(jnp.int32, (TQ, TQ), 1)
    causal = col <= row
    qscale = (D ** -0.5) * LOG2E

    def pair_body(p, _):
        wk = _split_pair(_load_pair(wuk_u, p, DC))
        wv = _split_pair(_load_pair(wuv_u, p, DC))
        wq = _split_pair(_load_pair(wq_u, p, M))
        k_s[...] = jnp.dot(ckv_v[...], wk, preferred_element_type=F32).astype(BF16)
        v_s[...] = jnp.dot(ckv_v[...], wv, preferred_element_type=F32).astype(BF16)
        q_s[...] = (jnp.dot(x_v[...], wq, preferred_element_type=F32) * qscale).astype(BF16)
        for hh in range(2):
            cs = slice(hh * D, (hh + 1) * D)
            c0 = pl.multiple_of(p * (2 * D) + hh * D, D)
            for i in reversed(range(S // TQ)):
                rs = slice(i * TQ, (i + 1) * TQ)
                kv = (i + 1) * TQ
                s = lax.dot_general(q_s[rs, cs], k_s[:kv, cs], NT, preferred_element_type=F32)
                sd = jnp.where(causal, s[:, kv - TQ:], NEG)
                s = jnp.concatenate([s[:, :kv - TQ], sd], axis=1) if i > 0 else sd
                m = jnp.max(s, axis=1, keepdims=True)
                e = jnp.exp2(s - m)
                l = jnp.sum(e, axis=1, keepdims=True)
                o = jnp.dot(e.astype(BF16), v_s[:kv, cs], preferred_element_type=F32)
                ctx_v[rs, pl.ds(c0, D)] = (o * (g_v[rs, :] / l)).astype(BF16)
        return 0

    lax.fori_loop(0, H // 2, pair_body, 0)

    for c in copies[5:]:
        c.wait()
    for part in range(3):
        for c in range(M // 128):
            c0 = part * M + c * 128
            for j in range(M // 128):
                tmp_v[j, c * 128:(c + 1) * 128, :] = bqkv_v[j * 128:(j + 1) * 128, c0:c0 + 128].astype(F32).T
        for d in range(DH):
            for j in range(M // 128):
                wtp_v[part * M + d * H: part * M + (d + 1) * H, j * 128:(j + 1) * 128] = (
                    tmp_v[j, pl.ds(d, H, stride=DH), :].astype(BF16))
    for j in range(M // 128):
        tmp_v[j] = bwo_v[:, j * 128:(j + 1) * 128].astype(F32)
    for d in range(DH):
        for j in range(M // 128):
            wall_v[H * D + d * H: H * D + (d + 1) * H, j * 128:(j + 1) * 128] = (
                tmp_v[j, pl.ds(d, H, stride=DH), :].astype(BF16))

    zpad = jnp.zeros((PAD, 128), F32)
    for t in range(M // 128):
        kb_v[t, 0:PAD, :] = zpad
        vb_v[t, 0:PAD, :] = zpad

    bscale = (DH ** -0.5) * LOG2E

    def bproj_body(i, _):
        r = pl.multiple_of(i * 256, 256)
        y = lax.dot_general(x_v[pl.ds(r, 256), :], wtp_v[...], NT, preferred_element_type=F32)
        for t in range(M // 128):
            qb_v[t, pl.ds(r, 256), :] = y[:, t * 128:(t + 1) * 128] * bscale
            kb_v[t, pl.ds(PAD + r, 256), :] = y[:, M + t * 128: M + (t + 1) * 128]
            vb_v[t, pl.ds(PAD + r, 256), :] = y[:, 2 * M + t * 128: 2 * M + (t + 1) * 128]
        return 0

    lax.fori_loop(0, S // 256, bproj_body, 0)

    def battn_body(i, _):
        r = pl.multiple_of(i * TB, TB)
        rowi = r + lax.broadcasted_iota(jnp.int32, (TB, 128), 0)
        logits = []
        for w in range(W):
            acc = None
            for t in range(M // 128):
                pr = qb_v[t, pl.ds(r, TB), :] * kb_v[t, pl.ds(PAD + r - DIL * w, TB), :]
                acc = pr if acc is None else acc + pr
            acc = acc + pltpu.roll(acc, 64, 1)
            acc = acc + pltpu.roll(acc, 32, 1)
            logits.append(jnp.where(rowi >= DIL * w, acc, NEG) if w > 0 else acc)
        m = functools.reduce(jnp.maximum, logits)
        es = [jnp.exp2(lg - m) for lg in logits]
        l = functools.reduce(lambda a, b: a + b, es)
        sc = (1.0 - g_v[pl.ds(r, TB), :]) / l
        for t in range(M // 128):
            acc = None
            for w in range(W):
                pr = es[w] * vb_v[t, pl.ds(PAD + r - DIL * w, TB), :]
                acc = pr if acc is None else acc + pr
            ctx_v[pl.ds(r, TB), H * D + t * 128: H * D + (t + 1) * 128] = (acc * sc).astype(BF16)
        return 0

    lax.fori_loop(0, S // TB, battn_body, 0)

    def out_copy(i, slot):
        return pltpu.make_async_copy(o_st.at[slot], out_hbm.at[pl.ds(i * TO, TO), :], out_sems.at[slot])

    def out_body(i, _):
        slot = i % 2
        r = pl.multiple_of(i * TO, TO)

        @pl.when(i >= 2)
        def _():
            out_copy(i - 2, slot).wait()

        o_st[slot] = jnp.dot(ctx_v[pl.ds(r, TO), :], wall_v[...], preferred_element_type=F32).astype(BF16)
        out_copy(i, slot).start()
        return 0

    n_out = S // TO
    lax.fori_loop(0, n_out, out_body, 0)
    out_copy(n_out - 2, (n_out - 2) % 2).wait()
    out_copy(n_out - 1, (n_out - 1) % 2).wait()


@jax.jit
def pallas_gated_mix__compressed_kv_cla__sliding_local_dilated__prompt_kernel(
    A_x, A_c_kv, A_w_q, A_w_uk, A_w_uv, A_w_o, B_x, B_wqkv, B_wo, gate_w,
):
    del B_x
    x = A_x.reshape(S, M)
    ckv = A_c_kv.reshape(S, DC)
    wq = A_w_q.reshape(M * H, D)
    wuk = A_w_uk.reshape(DC * H, D)
    wuv = A_w_uv.reshape(DC * H, D)
    wo = A_w_o.reshape(H * D, M)
    gate = gate_w.reshape(1, M)
    any_spec = pl.BlockSpec(memory_space=pl.ANY)
    out = pl.pallas_call(
        _kernel,
        out_shape=jax.ShapeDtypeStruct((S, M), BF16),
        in_specs=[any_spec] * 8 + [pl.BlockSpec(memory_space=pltpu.VMEM)],
        out_specs=any_spec,
        scratch_shapes=[
            pltpu.VMEM((S, M), BF16),
            pltpu.VMEM((S, DC), BF16),
            pltpu.VMEM((M * H, D), BF16),
            pltpu.VMEM((DC * H, D), BF16),
            pltpu.VMEM((DC * H, D), BF16),
            pltpu.VMEM((H * D + M, M), BF16),
            pltpu.VMEM((M, 3 * M), BF16),
            pltpu.VMEM((M, M), BF16),
            pltpu.VMEM((3 * M, M), BF16),
            pltpu.VMEM((M // 128, M, 128), F32),
            pltpu.VMEM((M // 128, S, 128), F32),
            pltpu.VMEM((M // 128, S + PAD, 128), F32),
            pltpu.VMEM((M // 128, S + PAD, 128), F32),
            pltpu.VMEM((S, H * D + M), BF16),
            pltpu.VMEM((S, 128), F32),
            pltpu.VMEM((S, 2 * D), BF16),
            pltpu.VMEM((S, 2 * D), BF16),
            pltpu.VMEM((S, 2 * D), BF16),
            pltpu.VMEM((2, TO, M), BF16),
            pltpu.SemaphoreType.DMA((8,)),
            pltpu.SemaphoreType.DMA((2,)),
        ],
        compiler_params=pltpu.CompilerParams(vmem_limit_bytes=120 * 1024 * 1024),
    )(x, ckv, wq, wuk, wuv, wo, B_wqkv, B_wo, gate)
    return out.reshape(1, S, M)
```

```python
import functools

import jax
import jax.numpy as jnp
from jax import lax
import jax.experimental.pallas as pl
import jax.experimental.pallas.tpu as pltpu

S = 2048
M = 1024
DC = 512
H = 32
D = 128
DH = 32
W = 8
DIL = 2
PAD = 16
NT_M = M // 128
TQ = 128
TC = 256
TB = 32
PITCH = 40
LOOK = 2
OLAG = 2
LOG2E = 1.4426950408889634
NEG = -1e9

F32 = jnp.float32
BF16 = jnp.bfloat16
NT = (((1,), (1,)), ((), ()))


def _recip(l):
    r = pl.reciprocal(l, approx=True)
    return r * (2.0 - l * r)


def _split_pair(w):
    lo = pltpu.bitcast(w << 16, F32).astype(BF16)
    hi = pltpu.bitcast(w & jnp.uint32(0xFFFF0000), F32).astype(BF16)
    return jnp.concatenate([lo, hi], axis=1)


def _load_pair(w_u, p, n):
    hp = H // 2
    if isinstance(p, int):
        return w_u[pl.ds(p, n, stride=hp), :]
    base = pl.multiple_of((p // 4) * 4, 4)
    view = w_u.at[pl.ds(base, n * hp - 12), :]
    r = p % 4
    c = [view[pl.ds(j, n, stride=hp), :] for j in range(4)]
    return jnp.where(r < 2, jnp.where(r == 0, c[0], c[1]), jnp.where(r == 2, c[2], c[3]))


def _kernel(x_hbm, ckv_hbm, wq_hbm, wuk_hbm, wuv_hbm, wo_hbm, bqkv_hbm, bwo_hbm, gate_ref,
            out_hbm,
            x_v, ckv_v, wq_v, wuk_v, wuv_v, wo_v, bqkv_v, bwo_v, wtp_v, wop_v, tmp_v,
            qb_v, kb_v, vb_v, acc_v, g_v, q_s, k_s, v_s, o_st, in_sems, out_sems):
    n_chunks = S // TC

    def cp(src, dst, k):
        return pltpu.make_async_copy(src, dst, in_sems.at[k])

    c_bq = [cp(bqkv_hbm.at[:, pl.ds(j * M, M)], bqkv_v.at[:, pl.ds(j * M, M)], j) for j in range(3)]
    x_parts = [(0, TC), (TC, TC), (2 * TC, S - 2 * TC)]
    c_x = [cp(x_hbm.at[pl.ds(r, n), :], x_v.at[pl.ds(r, n), :], 3 + j) for j, (r, n) in enumerate(x_parts)]
    c_bwo = cp(bwo_hbm, bwo_v, 6)
    c_a = [cp(ckv_hbm, ckv_v, 7), cp(wuk_hbm, wuk_v, 8), cp(wuv_hbm, wuv_v, 9), cp(wq_hbm, wq_v, 10),
           cp(wo_hbm, wo_v, 11)]
    for c in [c_bq[0], c_x[0], c_x[1], c_bq[1], c_bq[2], c_x[2], c_bwo] + c_a:
        c.start()

    gw = gate_ref[...].astype(F32)
    bscale = (DH ** -0.5) * LOG2E

    def permute_rows(dst, r0):
        for d in range(DH):
            for j in range(NT_M):
                dst[r0 + d * H: r0 + (d + 1) * H, j * 128:(j + 1) * 128] = (
                    tmp_v[j, pl.ds(d, H, stride=PITCH), :].astype(BF16))

    def prep_qkv(part):
        for j in range(NT_M):
            for c in range(NT_M):
                c0 = part * M + c * 128
                t = bqkv_v[j * 128:(j + 1) * 128, c0:c0 + 128].astype(F32).T
                for hh in range(4):
                    h = 4 * c + hh
                    tmp_v[j, h * PITCH: h * PITCH + DH, :] = t[hh * DH:(hh + 1) * DH, :]
        permute_rows(wtp_v, part * M)

    def prep_wo():
        for j in range(NT_M):
            for h in range(H):
                tmp_v[j, h * PITCH: h * PITCH + DH, :] = (
                    bwo_v[h * DH:(h + 1) * DH, j * 128:(j + 1) * 128].astype(F32))
        permute_rows(wop_v, 0)

    def gate(i):
        r = i * TC
        z = jnp.sum(x_v[r:r + TC, :].astype(F32) * gw, axis=1, keepdims=True)
        g = 1.0 / (1.0 + jnp.exp(-z))
        g_v[r:r + TC, :] = jnp.broadcast_to(g, (TC, 128))

    def bproj(i, part):
        r = i * TC
        y = lax.dot_general(x_v[r:r + TC, :], wtp_v[part * M:(part + 1) * M, :], NT,
                            preferred_element_type=F32)
        for t in range(NT_M):
            yt = y[:, t * 128:(t + 1) * 128]
            if part == 0:
                qb_v[t, r:r + TC, :] = yt * bscale
            elif part == 1:
                kb_v[t, PAD + r:PAD + r + TC, :] = yt
            else:
                vb_v[t, PAD + r:PAD + r + TC, :] = yt

    def local_attn(r):
        logits = []
        for w in range(W):
            a = None
            for t in range(NT_M):
                o = PAD + r - DIL * w
                pr = qb_v[t, r:r + TB, :] * kb_v[t, o:o + TB, :]
                a = pr if a is None else a + pr
            a = a + pltpu.roll(a, 64, 1)
            a = a + pltpu.roll(a, 32, 1)
            if r < DIL * w:
                rowi = r + lax.broadcasted_iota(jnp.int32, (TB, 128), 0)
                a = jnp.where(rowi >= DIL * w, a, NEG)
            logits.append(a)
        m = functools.reduce(jnp.maximum, logits)
        es = [jnp.exp2(lg - m) for lg in logits]
        l = functools.reduce(lambda a, b: a + b, es)
        sc = (1.0 - g_v[r:r + TB, :]) * _recip(l)
        outs = []
        for t in range(NT_M):
            a = None
            for w in range(W):
                o = PAD + r - DIL * w
                pr = es[w] * vb_v[t, o:o + TB, :]
                a = pr if a is None else a + pr
            outs.append((a * sc).astype(BF16))
        return jnp.concatenate(outs, axis=1)

    def bout(i):
        r = i * TC
        ob = jnp.concatenate([local_attn(r + k * TB) for k in range(TC // TB)], axis=0)
        acc_v[r:r + TC, :] = jnp.dot(ob, wop_v[...], preferred_element_type=F32)

    zpad = jnp.zeros((PAD, 128), F32)
    for t in range(NT_M):
        kb_v[t, 0:PAD, :] = zpad
        vb_v[t, 0:PAD, :] = zpad

    c_bq[0].wait()
    prep_qkv(0)
    c_x[0].wait()
    bproj(0, 0)
    gate(0)
    c_x[1].wait()
    c_bq[1].wait()
    bproj(1, 0)
    gate(1)
    prep_qkv(1)
    bproj(0, 1)
    c_bq[2].wait()
    bproj(1, 1)
    prep_qkv(2)
    bproj(0, 2)
    c_x[2].wait()
    c_bwo.wait()
    bproj(1, 2)
    prep_wo()
    for i in range(2, n_chunks):
        gate(i)
        for part in range(3):
            bproj(i, part)
        bout(i - 2)

    for c in c_a:
        c.wait()
    wq_u = wq_v.bitcast(jnp.uint32)
    wuk_u = wuk_v.bitcast(jnp.uint32)
    wuv_u = wuv_v.bitcast(jnp.uint32)
    qscale = (D ** -0.5) * LOG2E

    def proj(p):
        wk = _split_pair(_load_pair(wuk_u, p, DC))
        wv = _split_pair(_load_pair(wuv_u, p, DC))
        wq = _split_pair(_load_pair(wq_u, p, M))
        k_s[...] = jnp.dot(ckv_v[...], wk, preferred_element_type=F32).astype(BF16)
        v_s[...] = jnp.dot(ckv_v[...], wv, preferred_element_type=F32).astype(BF16)
        q_s[...] = (jnp.dot(x_v[...], wq, preferred_element_type=F32) * qscale).astype(BF16)

    def out_copy(k):
        return pltpu.make_async_copy(o_st.at[pl.ds(k * TC, TC), :], out_hbm.at[pl.ds(k * TC, TC), :],
                                     out_sems.at[k])

    def attention(p, last):
        row = lax.broadcasted_iota(jnp.int32, (TQ, TQ), 0)
        col = lax.broadcasted_iota(jnp.int32, (TQ, TQ), 1)
        causal = col <= row
        if isinstance(p, int):
            wo_p = wo_v.at[p * 2 * D:(p + 1) * 2 * D, :]
        else:
            wo_p = wo_v.at[pl.ds(pl.multiple_of(p * (2 * D), 2 * D), 2 * D), :]

        def qk(i, hh):
            cs = slice(hh * D, (hh + 1) * D)
            return lax.dot_general(q_s[i * TQ:(i + 1) * TQ, cs], k_s[:(i + 1) * TQ, cs], NT,
                                   preferred_element_type=F32)

        def softmax_pv(i, hh, s):
            cs = slice(hh * D, (hh + 1) * D)
            r0 = i * TQ
            sd = jnp.where(causal, s[:, r0:], NEG)
            s = jnp.concatenate([s[:, :r0], sd], axis=1) if i > 0 else sd
            m = jnp.max(s, axis=1, keepdims=True)
            e = jnp.exp2(s - m)
            l = jnp.sum(e, axis=1, keepdims=True)
            o = jnp.dot(e.astype(BF16), v_s[:r0 + TQ, cs], preferred_element_type=F32)
            return (o * (g_v[r0:r0 + TQ, :] * _recip(l))).astype(BF16)

        def oproj(i, o0, o1):
            r0 = i * TQ
            y = acc_v[r0:r0 + TQ, :] + jnp.dot(jnp.concatenate([o0, o1], axis=1), wo_p[...],
                                               preferred_element_type=F32)
            if last:
                o_st[r0:r0 + TQ, :] = y.astype(BF16)
                if r0 % TC == 0:
                    out_copy(r0 // TC).start()
            else:
                acc_v[r0:r0 + TQ, :] = y

        items = [(i, hh) for i in reversed(range(S // TQ)) for hh in range(2)]
        n = len(items)
        s_vals, o_vals = {}, {}
        for step in range(n + LOOK + OLAG):
            if step < n:
                s_vals[step] = qk(*items[step])
            b = step - LOOK
            if 0 <= b < n:
                o_vals[b] = softmax_pv(*items[b], s_vals.pop(b))
            c = step - LOOK - OLAG
            if 0 <= c < n and c % 2 == 1:
                oproj(items[c][0], o_vals.pop(c - 1), o_vals.pop(c))

    bout(n_chunks - 2)
    proj(0)
    bout(n_chunks - 1)

    def pair_body(p, _):
        attention(p, False)
        proj(p + 1)
        return 0

    lax.fori_loop(0, H // 2 - 1, pair_body, 0)
    attention(H // 2 - 1, True)
    for k in range(n_chunks):
        out_copy(k).wait()


@jax.jit
def pallas_gated_mix__compressed_kv_cla__sliding_local_dilated__prompt_kernel(
    A_x, A_c_kv, A_w_q, A_w_uk, A_w_uv, A_w_o, B_x, B_wqkv, B_wo, gate_w,
):
    del B_x
    x = A_x.reshape(S, M)
    ckv = A_c_kv.reshape(S, DC)
    wq = A_w_q.reshape(M * H, D)
    wuk = A_w_uk.reshape(DC * H, D)
    wuv = A_w_uv.reshape(DC * H, D)
    wo = A_w_o.reshape(H * D, M)
    gate = gate_w.reshape(1, M)
    any_spec = pl.BlockSpec(memory_space=pl.ANY)
    out = pl.pallas_call(
        _kernel,
        out_shape=jax.ShapeDtypeStruct((S, M), BF16),
        in_specs=[any_spec] * 8 + [pl.BlockSpec(memory_space=pltpu.VMEM)],
        out_specs=any_spec,
        scratch_shapes=[
            pltpu.VMEM((S, M), BF16),
            pltpu.VMEM((S, DC), BF16),
            pltpu.VMEM((M * H, D), BF16),
            pltpu.VMEM((DC * H, D), BF16),
            pltpu.VMEM((DC * H, D), BF16),
            pltpu.VMEM((H * D, M), BF16),
            pltpu.VMEM((M, 3 * M), BF16),
            pltpu.VMEM((M, M), BF16),
            pltpu.VMEM((3 * M, M), BF16),
            pltpu.VMEM((M, M), BF16),
            pltpu.VMEM((NT_M, H * PITCH, 128), F32),
            pltpu.VMEM((NT_M, S, 128), F32),
            pltpu.VMEM((NT_M, S + PAD, 128), F32),
            pltpu.VMEM((NT_M, S + PAD, 128), F32),
            pltpu.VMEM((S, M), F32),
            pltpu.VMEM((S, 128), F32),
            pltpu.VMEM((S, 2 * D), BF16),
            pltpu.VMEM((S, 2 * D), BF16),
            pltpu.VMEM((S, 2 * D), BF16),
            pltpu.VMEM((S, M), BF16),
            pltpu.SemaphoreType.DMA((12,)),
            pltpu.SemaphoreType.DMA((S // TC,)),
        ],
        compiler_params=pltpu.CompilerParams(vmem_limit_bytes=120 * 1024 * 1024),
    )(x, ckv, wq, wuk, wuv, wo, B_wqkv, B_wo, gate)
    return out.reshape(1, S, M)
```

```python
import functools

import jax
import jax.numpy as jnp
from jax import lax
import jax.experimental.pallas as pl
import jax.experimental.pallas.tpu as pltpu

S = 2048
M = 1024
DC = 512
H = 32
HP = H // 2
D = 128
DH = 32
W = 8
DIL = 2
PAD = 16
NT_M = M // 128
TQ = 128
TQP = 256
TC = 512
NC = S // TC
TL = S // HP
TO = 256
GR = 176
PITCH = 40
LOOK = 2
OLAG = 4
LOG2E = 1.4426950408889634
NEG = -1e9

F32 = jnp.float32
BF16 = jnp.bfloat16
U32 = jnp.uint32
NT = (((1,), (1,)), ((), ()))


def _recip(l):
    r = pl.reciprocal(l, approx=True)
    return r * (2.0 - l * r)


def _lo(w):
    return pltpu.bitcast(w << 16, F32).astype(BF16)


def _hi(w):
    return pltpu.bitcast(w & jnp.uint32(0xFFFF0000), F32).astype(BF16)


def _split_pair(w):
    return jnp.concatenate([_lo(w), _hi(w)], axis=1)


def _zero_after(z, *vals):
    acc = None
    for v in vals:
        b = pltpu.bitcast(v, U32)
        for r in range(0, b.shape[0], 8):
            for c in range(0, b.shape[1], 128):
                t = b[r:r + 8, c:c + 128]
                acc = t if acc is None else acc | t
    return acc & z


def _kernel(x_hbm, ckv_hbm, wq_hbm, wuk_hbm, wuv_hbm, wo_hbm, bqkv_hbm, bwo_hbm, gate_ref,
            out_hbm,
            x_v, ckv_v, wq_p, wuk_p, wuv_p, wo_v, bqkv_v, bwo_p, wtp_v, tmp_v,
            qkv_v, acc_v, g_v, z_v, q_s, k_s, v_s, o_st,
            sem_q, sem_x, sem_w, sem_a, sem_o):
    def cp_q(j):
        sl = (pl.ds(j * 128, 128), pl.ds(0, M))
        return pltpu.make_async_copy(bqkv_hbm.at[sl], bqkv_v.at[sl], sem_q.at[j])

    def cp_x(c):
        sl = (pl.ds(c * TC, TC), slice(None))
        return pltpu.make_async_copy(x_hbm.at[sl], x_v.at[sl], sem_x.at[c])

    def cp_w(t):
        sl = (pl.ds((t % 4) * 256, 256), pl.ds((t // 4 + 1) * M, M))
        return pltpu.make_async_copy(bqkv_hbm.at[sl], bqkv_v.at[sl], sem_w.at[t])

    a_copies = [pltpu.make_async_copy(ckv_hbm, ckv_v, sem_a.at[0]),
                pltpu.make_async_copy(wo_hbm, wo_v, sem_a.at[1])]
    for k, (src, dst) in enumerate(((wuk_hbm, wuk_p), (wuv_hbm, wuv_p), (wq_hbm, wq_p), (bwo_hbm, bwo_p))):
        src_u = src.bitcast(U32)
        a_copies += [pltpu.make_async_copy(src_u.at[:, p, :], dst.at[p], sem_a.at[2 + k])
                     for p in range(HP)]

    def cp_o(k):
        sl = (pl.ds(k * TO, TO), slice(None))
        return pltpu.make_async_copy(o_st.at[sl], out_hbm.at[sl], sem_o.at[k])

    for j in range(NT_M):
        cp_q(j).start()
    cp_x(0).start()
    z_v[...] = jnp.zeros((8, 128), U32)
    for part in range(3):
        for t in range(NT_M):
            qkv_v[part, t, 0:PAD, :] = jnp.zeros((PAD, 128), F32)

    def zero_body(i, _):
        acc_v[pl.ds(pl.multiple_of(i * 64, 64), 64), :] = jnp.zeros((64, M), F32)
        return 0

    lax.fori_loop(0, S // 64, zero_body, 0)
    cp_w(0).start()
    for c in range(1, NC):
        cp_x(c).start()
        cp_w(c).start()

    def prep_unit(part, j, buf, z, dep):
        k0 = pl.multiple_of(j * 128, 128)
        p0 = pl.multiple_of(part * M, M)
        for c in range(NT_M):
            src = bqkv_v[pl.ds(k0, 128), pl.ds(p0 + c * 128, 128)]
            if dep is not None:
                top = pltpu.bitcast(pltpu.bitcast(src[:16], U32) | dep, BF16)
                src = jnp.concatenate([top, src[16:]], axis=0)
            t = src.astype(F32).T
            for hh in range(4):
                h = 4 * c + hh
                tmp_v[buf, h * PITCH: h * PITCH + DH, :] = t[hh * DH:(hh + 1) * DH, :]
            if z is not None:
                dep = _zero_after(z, t[120:128])
        outs = []
        for d in range(DH):
            o = tmp_v[buf, pl.ds(d, H, stride=PITCH), :].astype(BF16)
            wtp_v[pl.ds(p0 + d * H, H), pl.ds(k0, 128)] = o
            outs.append(o)
        return None if z is None else _zero_after(z, *outs)

    def prep0_body(j, _):
        cp_q(j).wait()
        prep_unit(0, j, 0, None, None)
        return 0

    lax.fori_loop(0, NT_M, prep0_body, 0)
    for t in range(4, 8):
        cp_w(t).start()
    for c in a_copies:
        c.start()

    def bproj_body(t, _):
        part = t // NC
        c = t % NC

        @pl.when(t < NC)
        def _():
            cp_x(t).wait()

        @pl.when(t < 2 * NC)
        def _():
            cp_w(t).wait()

        r = pl.multiple_of(c * TC, TC)
        y = lax.dot_general(x_v[pl.ds(r, TC), :], wtp_v[pl.ds(pl.multiple_of(part * M, M), M), :], NT,
                            preferred_element_type=F32)
        for tt in range(NT_M):
            qkv_v[part, tt, pl.ds(PAD + r, TC), :] = y[:, tt * 128:(tt + 1) * 128]

        z = z_v[...]
        nxt = (part + 1) % 3
        dep = prep_unit(nxt, 2 * c, 0, z, None)
        dep = prep_unit(nxt, 2 * c + 1, 1, z, dep)
        gw = gate_ref[...].astype(F32)
        g0 = jnp.minimum(t * GR, S - GR)
        for k in range(GR // 16):
            rr = pl.multiple_of(g0 + k * 16, 16)
            xb = pltpu.bitcast(x_v[pl.ds(rr, 16), :], U32)
            xb = xb | jnp.concatenate([dep] * NT_M, axis=1)
            xx = pltpu.bitcast(xb, BF16).astype(F32)
            zz = jnp.sum(xx * gw, axis=1, keepdims=True)
            g = jnp.broadcast_to(1.0 / (1.0 + jnp.exp(-zz)), (16, 128))
            g_v[pl.ds(rr, 16), :] = g
            dep = _zero_after(z, g)
        return 0

    lax.fori_loop(0, 3 * NC, bproj_body, 0)
    for c in a_copies:
        c.wait()

    qscale = (D ** -0.5) * LOG2E
    bscale = (DH ** -0.5) * LOG2E

    def local_attn(r, z, dep):
        sc = jnp.full((8, 128), bscale, F32)
        if dep is not None:
            sc = sc + pltpu.bitcast(dep, F32)
        q = [qkv_v[0, t, pl.ds(PAD + r, 8), :] * sc for t in range(NT_M)]
        rowi = r + lax.broadcasted_iota(jnp.int32, (8, 128), 0)
        logits = []
        for w in range(W):
            a = None if w < 2 else pltpu.bitcast(_zero_after(z, raw[w - 2]), F32)
            if w == 0:
                raw = []
            for t in range(NT_M):
                pr = q[t] * qkv_v[1, t, pl.ds(PAD + r - DIL * w, 8), :]
                a = pr if a is None else a + pr
            raw.append(a)
            a = a + pltpu.roll(a, 64, 1)
            a = a + pltpu.roll(a, 32, 1)
            logits.append(jnp.where(rowi >= DIL * w, a, NEG) if w > 0 else a)
        m = functools.reduce(jnp.maximum, logits)
        es = [jnp.exp2(lg - m) for lg in logits]
        l = functools.reduce(lambda a, b: a + b, es)
        f = (1.0 - g_v[pl.ds(r, 8), :]) * _recip(l)
        es = [e * f for e in es]
        outs = []
        for t in range(NT_M):
            a = None if t < 2 else pltpu.bitcast(_zero_after(z, outs[t - 2]), F32)
            for w in range(W):
                pr = es[w] * qkv_v[2, t, pl.ds(PAD + r - DIL * w, 8), :]
                a = pr if a is None else a + pr
            outs.append(a)
        return jnp.concatenate(outs, axis=1), _zero_after(z, outs[-2], outs[-1])

    def pair_body(p, _):
        z = z_v[...]
        k_s[...] = jnp.dot(ckv_v[...], _split_pair(wuk_p[p]), preferred_element_type=F32).astype(BF16)
        v_s[...] = jnp.dot(ckv_v[...], _split_pair(wuv_p[p]), preferred_element_type=F32).astype(BF16)

        rb = pl.multiple_of(p * TL, TL)
        dep, obs = None, []
        for k in range(TL // 8):
            ob, dep = local_attn(rb + k * 8, z, dep)
            obs.append(ob)
        ob = jnp.concatenate(obs, axis=0).astype(BF16)
        wop = jnp.concatenate([f(bwo_p[dp]) for dp in range(DH // 2) for f in (_lo, _hi)], axis=0)
        acc_v[pl.ds(rb, TL), :] = acc_v[pl.ds(rb, TL), :] + jnp.dot(ob, wop, preferred_element_type=F32)

        wq = _split_pair(wq_p[p])
        wo_p = wo_v.at[pl.ds(pl.multiple_of(p * (2 * D), 2 * D), 2 * D), :]
        row = lax.broadcasted_iota(jnp.int32, (TQ, TQ), 0)
        col = lax.broadcasted_iota(jnp.int32, (TQ, TQ), 1)
        causal = col <= row

        def qproj(c):
            rs = slice(c * TQP, (c + 1) * TQP)
            q_s[rs, :] = (jnp.dot(x_v[rs, :], wq, preferred_element_type=F32) * qscale).astype(BF16)

        def qk(i, hh):
            cs = slice(hh * D, (hh + 1) * D)
            return lax.dot_general(q_s[i * TQ:(i + 1) * TQ, cs], k_s[:(i + 1) * TQ, cs], NT,
                                   preferred_element_type=F32)

        def softmax_pv(i, hh, s):
            cs = slice(hh * D, (hh + 1) * D)
            r0 = i * TQ
            sd = jnp.where(causal, s[:, r0:], NEG)
            s = jnp.concatenate([s[:, :r0], sd], axis=1) if i > 0 else sd
            m = jnp.max(s, axis=1, keepdims=True)
            e = jnp.exp2(s - m)
            l = jnp.sum(e, axis=1, keepdims=True)
            o = jnp.dot(e.astype(BF16), v_s[:r0 + TQ, cs], preferred_element_type=F32)
            return (o * (g_v[r0:r0 + TQ, :] * _recip(l))).astype(BF16)

        def oproj(i, o0, o1):
            r0 = i * TQ
            y = acc_v[r0:r0 + TQ, :] + jnp.dot(jnp.concatenate([o0, o1], axis=1), wo_p[...],
                                               preferred_element_type=F32)
            acc_v[r0:r0 + TQ, :] = y
            o_st[r0:r0 + TQ, :] = y.astype(BF16)
            if r0 % TO == 0:
                @pl.when(p == HP - 1)
                def _():
                    cp_o(r0 // TO).start()

        items = [(i, hh) for i in reversed(range(S // TQ)) for hh in range(2)]
        per_chunk = 2 * (TQP // TQ)
        n_qc = S // TQP
        n = len(items)
        s_vals, o_vals = {}, {}
        qproj(n_qc - 1)
        for step in range(n + LOOK + OLAG):
            if step % per_chunk == 0 and n_qc - 2 - step // per_chunk >= 0:
                qproj(n_qc - 2 - step // per_chunk)
            if step < n:
                s_vals[step] = qk(*items[step])
            b = step - LOOK
            if 0 <= b < n:
                o_vals[b] = softmax_pv(*items[b], s_vals.pop(b))
            c = step - LOOK - OLAG
            if 0 <= c < n and c % 2 == 1:
                oproj(items[c][0], o_vals.pop(c - 1), o_vals.pop(c))
        return 0

    lax.fori_loop(0, HP, pair_body, 0)
    for k in range(S // TO):
        cp_o(k).wait()


@jax.jit
def pallas_gated_mix__compressed_kv_cla__sliding_local_dilated__prompt_kernel(
    A_x, A_c_kv, A_w_q, A_w_uk, A_w_uv, A_w_o, B_x, B_wqkv, B_wo, gate_w,
):
    del B_x
    x = A_x.reshape(S, M)
    ckv = A_c_kv.reshape(S, DC)
    wo = A_w_o.reshape(H * D, M)
    bwo = B_wo.reshape(H, DH, M)
    gate = gate_w.reshape(1, M)
    any_spec = pl.BlockSpec(memory_space=pl.ANY)
    out = pl.pallas_call(
        _kernel,
        out_shape=jax.ShapeDtypeStruct((S, M), BF16),
        in_specs=[any_spec] * 8 + [pl.BlockSpec(memory_space=pltpu.VMEM)],
        out_specs=any_spec,
        scratch_shapes=[
            pltpu.VMEM((S, M), BF16),
            pltpu.VMEM((S, DC), BF16),
            pltpu.VMEM((HP, M, D), U32),
            pltpu.VMEM((HP, DC, D), U32),
            pltpu.VMEM((HP, DC, D), U32),
            pltpu.VMEM((H * D, M), BF16),
            pltpu.VMEM((M, 3 * M), BF16),
            pltpu.VMEM((DH // 2, H, M), U32),
            pltpu.VMEM((3 * M, M), BF16),
            pltpu.VMEM((2, H * PITCH, 128), F32),
            pltpu.VMEM((3, NT_M, S + PAD, 128), F32),
            pltpu.VMEM((S, M), F32),
            pltpu.VMEM((S, 128), F32),
            pltpu.VMEM((8, 128), U32),
            pltpu.VMEM((S, 2 * D), BF16),
            pltpu.VMEM((S, 2 * D), BF16),
            pltpu.VMEM((S, 2 * D), BF16),
            pltpu.VMEM((S, M), BF16),
            pltpu.SemaphoreType.DMA((NT_M,)),
            pltpu.SemaphoreType.DMA((NC,)),
            pltpu.SemaphoreType.DMA((8,)),
            pltpu.SemaphoreType.DMA((6,)),
            pltpu.SemaphoreType.DMA((S // TO,)),
        ],
        compiler_params=pltpu.CompilerParams(vmem_limit_bytes=110 * 1024 * 1024),
    )(x, ckv, A_w_q, A_w_uk, A_w_uv, wo, B_wqkv, bwo, gate)
    return out.reshape(1, S, M)
```

```python
import contextlib
import functools

import jax
import jax.numpy as jnp
from jax import lax
import jax.experimental.pallas as pl
import jax.experimental.pallas.tpu as pltpu

S = 2048
M = 1024
DC = 512
H = 32
HP = H // 2
D = 128
DH = 32
W = 8
DIL = 2
PAD = 16
NT_M = M // 128
TQ = 128
TQP = 256
TC = 512
NC = S // TC
TL = S // HP
TO = 256
GR = 176
PITCH = 40
LOOK = 2
OLAG = 4
LOG2E = 1.4426950408889634
NEG = -1e9

F32 = jnp.float32
BF16 = jnp.bfloat16
U32 = jnp.uint32
NT = (((1,), (1,)), ((), ()))


_PROFILE = False


def _scope(name):
    return jax.named_scope(name) if _PROFILE else contextlib.nullcontext()


def _scoped(name, body):
    def f(i, c):
        with _scope(name):
            return body(i, c)
    return f


def _recip(l):
    r = pl.reciprocal(l, approx=True)
    return r * (2.0 - l * r)


def _lo(w):
    return pltpu.bitcast(w << 16, F32).astype(BF16)


def _hi(w):
    return pltpu.bitcast(w & jnp.uint32(0xFFFF0000), F32).astype(BF16)


def _split_pair(w):
    return jnp.concatenate([_lo(w), _hi(w)], axis=1)


def _zero_after(z, *vals):
    acc = None
    for v in vals:
        b = pltpu.bitcast(v, U32)
        for r in range(0, b.shape[0], 8):
            for c in range(0, b.shape[1], 128):
                t = b[r:r + 8, c:c + 128]
                acc = t if acc is None else acc | t
    return acc & z


def _kernel(x_hbm, ckv_hbm, wq_hbm, wuk_hbm, wuv_hbm, wo_hbm, bqkv_hbm, bwo_hbm, gate_ref,
            out_hbm,
            x_v, ckv_v, wq_p, wuk_p, wuv_p, wo_v, bqkv_v, bwo_p, wcur_v, wnxt_v, tmp_v,
            qkv_v, acc_v, g_v, z_v, q_s, k_s, v_s, o_st,
            sem_q, sem_x, sem_w, sem_a, sem_z, sem_o):
    def cp_q(j):
        sl = (pl.ds(j * 128, 128), pl.ds(0, M))
        return pltpu.make_async_copy(bqkv_hbm.at[sl], bqkv_v.at[sl], sem_q.at[j])

    def cp_x(c):
        sl = (pl.ds(c * TC, TC), slice(None))
        return pltpu.make_async_copy(x_hbm.at[sl], x_v.at[sl], sem_x.at[c])

    def cp_w(t):
        sl = (pl.ds((t % 4) * 256, 256), pl.ds((t // 4 + 1) * M, M))
        return pltpu.make_async_copy(bqkv_hbm.at[sl], bqkv_v.at[sl], sem_w.at[t])

    a_copies = [pltpu.make_async_copy(ckv_hbm, ckv_v, sem_a.at[0]),
                pltpu.make_async_copy(wo_hbm, wo_v, sem_a.at[1])]
    for k, (src, dst) in enumerate(((wuk_hbm, wuk_p), (wuv_hbm, wuv_p), (wq_hbm, wq_p), (bwo_hbm, bwo_p))):
        src_u = src.bitcast(U32)
        a_copies += [pltpu.make_async_copy(src_u.at[:, p, :], dst.at[p], sem_a.at[2 + k])
                     for p in range(HP)]

    def cp_o(k):
        sl = (pl.ds(k * TO, TO), slice(None))
        return pltpu.make_async_copy(o_st.at[sl], out_hbm.at[sl], sem_o.at[k])

    ZR = 64
    z_copies = [pltpu.make_async_copy(acc_v.at[pl.ds(0, ZR), :], acc_v.at[pl.ds(k * ZR, ZR), :], sem_z)
                for k in range(1, S // ZR)]

    for j in range(NT_M):
        cp_q(j).start()
    cp_x(0).start()
    cp_w(0).start()
    z_v[...] = jnp.zeros((8, 128), U32)
    for part in range(3):
        for t in range(NT_M):
            qkv_v[part, t, 0:PAD, :] = jnp.zeros((PAD, 128), F32)
    acc_v[0:ZR, :] = jnp.zeros((ZR, M), F32)

    def prep_unit(dst, part, j, buf, z, dep):
        k0 = pl.multiple_of(j * 128, 128)
        p0 = pl.multiple_of(part * M, M)
        for c in range(NT_M):
            src = bqkv_v[pl.ds(k0, 128), pl.ds(p0 + c * 128, 128)]
            if dep is not None:
                top = pltpu.bitcast(pltpu.bitcast(src[:16], U32) | dep, BF16)
                src = jnp.concatenate([top, src[16:]], axis=0)
            t = src.astype(F32).T
            for hh in range(4):
                h = 4 * c + hh
                tmp_v[buf, h * PITCH: h * PITCH + DH, :] = t[hh * DH:(hh + 1) * DH, :]
            if z is not None:
                dep = _zero_after(z, t[120:128])
        outs = []
        for d in range(DH):
            o = tmp_v[buf, pl.ds(d, H, stride=PITCH), :].astype(BF16)
            dst[d * H:(d + 1) * H, pl.ds(k0, 128)] = o
            outs.append(o)
        return None if z is None else _zero_after(z, *outs)

    def prep0_body(j, _):
        cp_q(2 * j).wait()
        cp_q(2 * j + 1).wait()
        prep_unit(wcur_v, 0, 2 * j, 0, None, None)
        prep_unit(wcur_v, 0, 2 * j + 1, 1, None, None)
        return 0

    lax.fori_loop(0, NT_M // 2, _scoped("prep0", prep0_body), 0)
    for c in range(1, NC):
        cp_x(c).start()
        cp_w(c).start()
    for t in range(4, 8):
        cp_w(t).start()

    def bproj_body(t, _):
        part = t // NC
        c = t % NC

        @pl.when(t < NC)
        def _():
            cp_x(t).wait()

        @pl.when(t < 2 * NC)
        def _():
            cp_w(t).wait()

        @pl.when(t == 2)
        def _():
            for cc in a_copies + z_copies:
                cc.start()

        @pl.when(jnp.logical_and(t > 0, c == 0))
        def _():
            def cpy(i, _):
                rs = pl.ds(pl.multiple_of(i * 128, 128), 128)
                wcur_v[rs, :] = wnxt_v[rs, :]
                return 0
            lax.fori_loop(0, M // 128, cpy, 0)

        r = pl.multiple_of(c * TC, TC)
        y = lax.dot_general(x_v[pl.ds(r, TC), :], wcur_v[...], NT, preferred_element_type=F32)
        for tt in range(NT_M):
            qkv_v[part, tt, pl.ds(PAD + r, TC), :] = y[:, tt * 128:(tt + 1) * 128]

        z = z_v[...]
        nxt = (part + 1) % 3
        dep = prep_unit(wnxt_v, nxt, 2 * c, 0, z, None)
        dep = prep_unit(wnxt_v, nxt, 2 * c + 1, 1, z, dep)
        gw = gate_ref[...].astype(F32)
        g0 = jnp.minimum(t * GR, S - GR)
        for k in range(GR // 16):
            rr = pl.multiple_of(g0 + k * 16, 16)
            xb = pltpu.bitcast(x_v[pl.ds(rr, 16), :], U32)
            xb = xb | jnp.concatenate([dep] * NT_M, axis=1)
            xx = pltpu.bitcast(xb, BF16).astype(F32)
            zz = jnp.sum(xx * gw, axis=1, keepdims=True)
            g = jnp.broadcast_to(1.0 / (1.0 + jnp.exp(-zz)), (16, 128))
            g_v[pl.ds(rr, 16), :] = g
            dep = _zero_after(z, g)
        return 0

    lax.fori_loop(0, 3 * NC, _scoped("bproj", bproj_body), 0)
    for c in a_copies + z_copies:
        c.wait()

    qscale = (D ** -0.5) * LOG2E
    bscale = (DH ** -0.5) * LOG2E

    def local_attn(r, z, dep):
        sc = jnp.full((8, 128), bscale, F32)
        if dep is not None:
            sc = sc + pltpu.bitcast(dep, F32)
        q = [qkv_v[0, t, pl.ds(PAD + r, 8), :] * sc for t in range(NT_M)]
        rowi = r + lax.broadcasted_iota(jnp.int32, (8, 128), 0)
        logits = []
        for w in range(W):
            a = None if w < 2 else pltpu.bitcast(_zero_after(z, raw[w - 2]), F32)
            if w == 0:
                raw = []
            for t in range(NT_M):
                pr = q[t] * qkv_v[1, t, pl.ds(PAD + r - DIL * w, 8), :]
                a = pr if a is None else a + pr
            raw.append(a)
            a = a + pltpu.roll(a, 64, 1)
            a = a + pltpu.roll(a, 32, 1)
            logits.append(jnp.where(rowi >= DIL * w, a, NEG) if w > 0 else a)
        m = functools.reduce(jnp.maximum, logits)
        es = [jnp.exp2(lg - m) for lg in logits]
        l = functools.reduce(lambda a, b: a + b, es)
        f = (1.0 - g_v[pl.ds(r, 8), :]) * _recip(l)
        es = [e * f for e in es]
        outs = []
        for t in range(NT_M):
            a = None if t < 2 else pltpu.bitcast(_zero_after(z, outs[t - 2]), F32)
            for w in range(W):
                pr = es[w] * qkv_v[2, t, pl.ds(PAD + r - DIL * w, 8), :]
                a = pr if a is None else a + pr
            outs.append(a)
        return jnp.concatenate(outs, axis=1), _zero_after(z, outs[-2], outs[-1])

    def pair_body(p, _):
        z = z_v[...]
        k_s[...] = jnp.dot(ckv_v[...], _split_pair(wuk_p[p]), preferred_element_type=F32).astype(BF16)
        v_s[...] = jnp.dot(ckv_v[...], _split_pair(wuv_p[p]), preferred_element_type=F32).astype(BF16)

        rb = pl.multiple_of(p * TL, TL)
        dep, obs = None, []
        for k in range(TL // 8):
            ob, dep = local_attn(rb + k * 8, z, dep)
            obs.append(ob)
        ob = jnp.concatenate(obs, axis=0).astype(BF16)
        wop = jnp.concatenate([f(bwo_p[dp]) for dp in range(DH // 2) for f in (_lo, _hi)], axis=0)
        acc_v[pl.ds(rb, TL), :] = acc_v[pl.ds(rb, TL), :] + jnp.dot(ob, wop, preferred_element_type=F32)

        wq = _split_pair(wq_p[p])
        wo_p = wo_v.at[pl.ds(pl.multiple_of(p * (2 * D), 2 * D), 2 * D), :]
        row = lax.broadcasted_iota(jnp.int32, (TQ, TQ), 0)
        col = lax.broadcasted_iota(jnp.int32, (TQ, TQ), 1)
        causal = col <= row

        def qproj(c):
            rs = slice(c * TQP, (c + 1) * TQP)
            q_s[rs, :] = (jnp.dot(x_v[rs, :], wq, preferred_element_type=F32) * qscale).astype(BF16)

        def qk(i, hh):
            cs = slice(hh * D, (hh + 1) * D)
            return lax.dot_general(q_s[i * TQ:(i + 1) * TQ, cs], k_s[:(i + 1) * TQ, cs], NT,
                                   preferred_element_type=F32)

        def softmax_pv(i, hh, s):
            cs = slice(hh * D, (hh + 1) * D)
            r0 = i * TQ
            sd = jnp.where(causal, s[:, r0:], NEG)
            s = jnp.concatenate([s[:, :r0], sd], axis=1) if i > 0 else sd
            m = jnp.max(s, axis=1, keepdims=True)
            e = jnp.exp2(s - m)
            l = jnp.sum(e, axis=1, keepdims=True)
            o = jnp.dot(e.astype(BF16), v_s[:r0 + TQ, cs], preferred_element_type=F32)
            return (o * (g_v[r0:r0 + TQ, :] * _recip(l))).astype(BF16)

        def oproj(i, o0, o1):
            r0 = i * TQ
            y = acc_v[r0:r0 + TQ, :] + jnp.dot(jnp.concatenate([o0, o1], axis=1), wo_p[...],
                                               preferred_element_type=F32)
            acc_v[r0:r0 + TQ, :] = y
            o_st[r0:r0 + TQ, :] = y.astype(BF16)
            if r0 % TO == 0:
                @pl.when(p == HP - 1)
                def _():
                    cp_o(r0 // TO).start()

        items = [(i, hh) for i in reversed(range(S // TQ)) for hh in range(2)]
        per_chunk = 2 * (TQP // TQ)
        n_qc = S // TQP
        n = len(items)
        s_vals, o_vals = {}, {}
        qproj(n_qc - 1)
        for step in range(n + LOOK + OLAG):
            if step % per_chunk == 0 and n_qc - 2 - step // per_chunk >= 0:
                qproj(n_qc - 2 - step // per_chunk)
            if step < n:
                s_vals[step] = qk(*items[step])
            b = step - LOOK
            if 0 <= b < n:
                o_vals[b] = softmax_pv(*items[b], s_vals.pop(b))
            c = step - LOOK - OLAG
            if 0 <= c < n and c % 2 == 1:
                oproj(items[c][0], o_vals.pop(c - 1), o_vals.pop(c))
        return 0

    lax.fori_loop(0, HP, _scoped("pair", pair_body), 0)
    for k in range(S // TO):
        cp_o(k).wait()


@jax.jit
def pallas_gated_mix__compressed_kv_cla__sliding_local_dilated__prompt_kernel(
    A_x, A_c_kv, A_w_q, A_w_uk, A_w_uv, A_w_o, B_x, B_wqkv, B_wo, gate_w,
):
    del B_x
    x = A_x.reshape(S, M)
    ckv = A_c_kv.reshape(S, DC)
    wo = A_w_o.reshape(H * D, M)
    bwo = B_wo.reshape(H, DH, M)
    gate = gate_w.reshape(1, M)
    any_spec = pl.BlockSpec(memory_space=pl.ANY)
    out = pl.pallas_call(
        _kernel,
        out_shape=jax.ShapeDtypeStruct((S, M), BF16),
        in_specs=[any_spec] * 8 + [pl.BlockSpec(memory_space=pltpu.VMEM)],
        out_specs=any_spec,
        scratch_shapes=[
            pltpu.VMEM((S, M), BF16),
            pltpu.VMEM((S, DC), BF16),
            pltpu.VMEM((HP, M, D), U32),
            pltpu.VMEM((HP, DC, D), U32),
            pltpu.VMEM((HP, DC, D), U32),
            pltpu.VMEM((H * D, M), BF16),
            pltpu.VMEM((M, 3 * M), BF16),
            pltpu.VMEM((DH // 2, H, M), U32),
            pltpu.VMEM((M, M), BF16),
            pltpu.VMEM((M, M), BF16),
            pltpu.VMEM((2, H * PITCH, 128), F32),
            pltpu.VMEM((3, NT_M, S + PAD, 128), F32),
            pltpu.VMEM((S, M), F32),
            pltpu.VMEM((S, 128), F32),
            pltpu.VMEM((8, 128), U32),
            pltpu.VMEM((S, 2 * D), BF16),
            pltpu.VMEM((S, 2 * D), BF16),
            pltpu.VMEM((S, 2 * D), BF16),
            pltpu.VMEM((S, M), BF16),
            pltpu.SemaphoreType.DMA((NT_M,)),
            pltpu.SemaphoreType.DMA((NC,)),
            pltpu.SemaphoreType.DMA((8,)),
            pltpu.SemaphoreType.DMA((6,)),
            pltpu.SemaphoreType.DMA(()),
            pltpu.SemaphoreType.DMA((S // TO,)),
        ],
        compiler_params=pltpu.CompilerParams(vmem_limit_bytes=110 * 1024 * 1024),
    )(x, ckv, A_w_q, A_w_uk, A_w_uv, wo, B_wqkv, bwo, gate)
    return out.reshape(1, S, M)
```

```python
import contextlib
import functools

import jax
import jax.numpy as jnp
from jax import lax
import jax.experimental.pallas as pl
import jax.experimental.pallas.tpu as pltpu

S = 2048
M = 1024
DC = 512
H = 32
HP = H // 2
D = 128
DH = 32
W = 8
DIL = 2
PAD = 16
NT_M = M // 128
TQ = 128
TQP = 256
TC = 512
NC = S // TC
TL = S // HP
TO = 256
GR = 176
PITCH = 40
LOOK = 2
OLAG = 4
LOG2E = 1.4426950408889634
NEG = -1e9

F32 = jnp.float32
BF16 = jnp.bfloat16
U32 = jnp.uint32
NT = (((1,), (1,)), ((), ()))


_PROFILE = False


def _scope(name):
    return jax.named_scope(name) if _PROFILE else contextlib.nullcontext()


def _scoped(name, body):
    def f(i, c):
        with _scope(name):
            return body(i, c)
    return f


def _recip(l):
    r = pl.reciprocal(l, approx=True)
    return r * (2.0 - l * r)


def _lo(w):
    return pltpu.bitcast(w << 16, F32).astype(BF16)


def _hi(w):
    return pltpu.bitcast(w & jnp.uint32(0xFFFF0000), F32).astype(BF16)


def _split_pair(w):
    return jnp.concatenate([_lo(w), _hi(w)], axis=1)


def _zero_after(z, *vals):
    acc = None
    for v in vals:
        b = pltpu.bitcast(v, U32)
        for r in range(0, b.shape[0], 8):
            for c in range(0, b.shape[1], 128):
                t = b[r:r + 8, c:c + 128]
                acc = t if acc is None else acc | t
    return acc & z


def _kernel(x_hbm, ckv_hbm, wq_hbm, wuk_hbm, wuv_hbm, wo_hbm, bqkv_hbm, bwo_hbm, gate_ref,
            out_hbm,
            x_v, ckv_v, wq_p, wuk_p, wuv_p, wo_v, bqkv_v, bwo_p, wcur_v, wnxt_v, tmp_v,
            qkv_v, acc_v, g_v, z_v, q_s, k_s, v_s, o_st,
            sem_q, sem_x, sem_w, sem_a, sem_o):
    def cp_q(j):
        sl = (pl.ds(j * 128, 128), pl.ds(0, M))
        return pltpu.make_async_copy(bqkv_hbm.at[sl], bqkv_v.at[sl], sem_q.at[j])

    def cp_x(c):
        sl = (pl.ds(c * TC, TC), slice(None))
        return pltpu.make_async_copy(x_hbm.at[sl], x_v.at[sl], sem_x.at[c])

    def cp_w(t):
        sl = (pl.ds((t % 4) * 256, 256), pl.ds((t // 4 + 1) * M, M))
        return pltpu.make_async_copy(bqkv_hbm.at[sl], bqkv_v.at[sl], sem_w.at[t])

    a_copies = [pltpu.make_async_copy(ckv_hbm, ckv_v, sem_a.at[0]),
                pltpu.make_async_copy(wo_hbm, wo_v, sem_a.at[1])]
    for k, (src, dst) in enumerate(((wuk_hbm, wuk_p), (wuv_hbm, wuv_p), (wq_hbm, wq_p), (bwo_hbm, bwo_p))):
        src_u = src.bitcast(U32)
        a_copies += [pltpu.make_async_copy(src_u.at[:, p, :], dst.at[p], sem_a.at[2 + k])
                     for p in range(HP)]

    def cp_o(k):
        sl = (pl.ds(k * TO, TO), slice(None))
        return pltpu.make_async_copy(o_st.at[sl], out_hbm.at[sl], sem_o.at[k])

    for j in range(NT_M):
        cp_q(j).start()
    cp_x(0).start()
    cp_w(0).start()
    z_v[...] = jnp.zeros((8, 128), U32)
    for part in range(3):
        for t in range(NT_M):
            qkv_v[part, t, 0:PAD, :] = jnp.zeros((PAD, 128), F32)

    def zero_acc(lo, hi):
        def body(i, _):
            acc_v[pl.ds(pl.multiple_of(i * 64, 64), 64), :] = jnp.zeros((64, M), F32)
            return 0
        lax.fori_loop(lo // 64, hi // 64, body, 0)

    zero_acc(0, S // 2)

    def prep_unit(dst, part, j, buf, z, dep):
        k0 = pl.multiple_of(j * 128, 128)
        p0 = pl.multiple_of(part * M, M)
        for c in range(NT_M):
            src = bqkv_v[pl.ds(k0, 128), pl.ds(p0 + c * 128, 128)]
            if dep is not None:
                top = pltpu.bitcast(pltpu.bitcast(src[:16], U32) | dep, BF16)
                src = jnp.concatenate([top, src[16:]], axis=0)
            t = src.astype(F32).T
            for hh in range(4):
                h = 4 * c + hh
                tmp_v[buf, h * PITCH: h * PITCH + DH, :] = t[hh * DH:(hh + 1) * DH, :]
            if z is not None:
                dep = _zero_after(z, t[120:128])
        outs = []
        for d in range(DH):
            o = tmp_v[buf, pl.ds(d, H, stride=PITCH), :].astype(BF16)
            dst[d * H:(d + 1) * H, pl.ds(k0, 128)] = o
            outs.append(o)
        return None if z is None else _zero_after(z, *outs)

    def prep0_body(j, _):
        cp_q(2 * j).wait()
        cp_q(2 * j + 1).wait()
        prep_unit(wcur_v, 0, 2 * j, 0, None, None)
        prep_unit(wcur_v, 0, 2 * j + 1, 1, None, None)
        return 0

    lax.fori_loop(0, NT_M // 2, _scoped("prep0", prep0_body), 0)
    zero_acc(S // 2, S)

    def bproj_body(t, _):
        part = t // NC
        c = t % NC

        @pl.when(t < NC)
        def _():
            cp_x(t).wait()

        @pl.when(t < 2 * NC)
        def _():
            cp_w(t).wait()

        @pl.when(t == 0)
        def _():
            for cc in range(1, NC):
                cp_x(cc).start()
                cp_w(cc).start()
            for cc in range(4, 8):
                cp_w(cc).start()

        @pl.when(t == 2)
        def _():
            for cc in a_copies:
                cc.start()

        @pl.when(jnp.logical_and(t > 0, c == 0))
        def _():
            def cpy(i, _):
                rs = pl.ds(pl.multiple_of(i * 128, 128), 128)
                wcur_v[rs, :] = wnxt_v[rs, :]
                return 0
            lax.fori_loop(0, M // 128, cpy, 0)

        r = pl.multiple_of(c * TC, TC)
        y = lax.dot_general(x_v[pl.ds(r, TC), :], wcur_v[...], NT, preferred_element_type=F32)
        for tt in range(NT_M):
            qkv_v[part, tt, pl.ds(PAD + r, TC), :] = y[:, tt * 128:(tt + 1) * 128]

        z = z_v[...]
        nxt = (part + 1) % 3
        dep = prep_unit(wnxt_v, nxt, 2 * c, 0, z, None)
        dep = prep_unit(wnxt_v, nxt, 2 * c + 1, 1, z, dep)
        gw = gate_ref[...].astype(F32)
        g0 = jnp.minimum(t * GR, S - GR)
        for k in range(GR // 16):
            rr = pl.multiple_of(g0 + k * 16, 16)
            xb = pltpu.bitcast(x_v[pl.ds(rr, 16), :], U32)
            xb = xb | jnp.concatenate([dep] * NT_M, axis=1)
            xx = pltpu.bitcast(xb, BF16).astype(F32)
            zz = jnp.sum(xx * gw, axis=1, keepdims=True)
            g = jnp.broadcast_to(1.0 / (1.0 + jnp.exp(-zz)), (16, 128))
            g_v[pl.ds(rr, 16), :] = g
            dep = _zero_after(z, g)
        return 0

    lax.fori_loop(0, 3 * NC, _scoped("bproj", bproj_body), 0)
    for c in a_copies:
        c.wait()

    qscale = (D ** -0.5) * LOG2E
    bscale = (DH ** -0.5) * LOG2E

    def local_attn(r, z, dep):
        sc = jnp.full((8, 128), bscale, F32)
        if dep is not None:
            sc = sc + pltpu.bitcast(dep, F32)
        q = [qkv_v[0, t, pl.ds(PAD + r, 8), :] * sc for t in range(NT_M)]
        rowi = r + lax.broadcasted_iota(jnp.int32, (8, 128), 0)
        logits = []
        for w in range(W):
            a = None if w < 2 else pltpu.bitcast(_zero_after(z, raw[w - 2]), F32)
            if w == 0:
                raw = []
            for t in range(NT_M):
                pr = q[t] * qkv_v[1, t, pl.ds(PAD + r - DIL * w, 8), :]
                a = pr if a is None else a + pr
            raw.append(a)
            a = a + pltpu.roll(a, 64, 1)
            a = a + pltpu.roll(a, 32, 1)
            logits.append(jnp.where(rowi >= DIL * w, a, NEG) if w > 0 else a)
        m = functools.reduce(jnp.maximum, logits)
        es = [jnp.exp2(lg - m) for lg in logits]
        l = functools.reduce(lambda a, b: a + b, es)
        f = (1.0 - g_v[pl.ds(r, 8), :]) * _recip(l)
        es = [e * f for e in es]
        outs = []
        for t in range(NT_M):
            a = None if t < 2 else pltpu.bitcast(_zero_after(z, outs[t - 2]), F32)
            for w in range(W):
                pr = es[w] * qkv_v[2, t, pl.ds(PAD + r - DIL * w, 8), :]
                a = pr if a is None else a + pr
            outs.append(a)
        return jnp.concatenate(outs, axis=1), _zero_after(z, outs[-2], outs[-1])

    def pair_body(p, _):
        z = z_v[...]
        k_s[...] = jnp.dot(ckv_v[...], _split_pair(wuk_p[p]), preferred_element_type=F32).astype(BF16)
        v_s[...] = jnp.dot(ckv_v[...], _split_pair(wuv_p[p]), preferred_element_type=F32).astype(BF16)

        rb = pl.multiple_of(p * TL, TL)
        dep, obs = None, []
        for k in range(TL // 8):
            ob, dep = local_attn(rb + k * 8, z, dep)
            obs.append(ob)
        ob = jnp.concatenate(obs, axis=0).astype(BF16)
        wop = jnp.concatenate([f(bwo_p[dp]) for dp in range(DH // 2) for f in (_lo, _hi)], axis=0)
        acc_v[pl.ds(rb, TL), :] = acc_v[pl.ds(rb, TL), :] + jnp.dot(ob, wop, preferred_element_type=F32)

        wq = _split_pair(wq_p[p])
        wo_p = wo_v.at[pl.ds(pl.multiple_of(p * (2 * D), 2 * D), 2 * D), :]
        row = lax.broadcasted_iota(jnp.int32, (TQ, TQ), 0)
        col = lax.broadcasted_iota(jnp.int32, (TQ, TQ), 1)
        causal = col <= row

        def qproj(c):
            rs = slice(c * TQP, (c + 1) * TQP)
            q_s[rs, :] = (jnp.dot(x_v[rs, :], wq, preferred_element_type=F32) * qscale).astype(BF16)

        def qk(i, hh):
            cs = slice(hh * D, (hh + 1) * D)
            return lax.dot_general(q_s[i * TQ:(i + 1) * TQ, cs], k_s[:(i + 1) * TQ, cs], NT,
                                   preferred_element_type=F32)

        def softmax_pv(i, hh, s):
            cs = slice(hh * D, (hh + 1) * D)
            r0 = i * TQ
            sd = jnp.where(causal, s[:, r0:], NEG)
            s = jnp.concatenate([s[:, :r0], sd], axis=1) if i > 0 else sd
            m = jnp.max(s, axis=1, keepdims=True)
            e = jnp.exp2(s - m)
            l = jnp.sum(e, axis=1, keepdims=True)
            o = jnp.dot(e.astype(BF16), v_s[:r0 + TQ, cs], preferred_element_type=F32)
            return (o * (g_v[r0:r0 + TQ, :] * _recip(l))).astype(BF16)

        def oproj(i, o0, o1):
            r0 = i * TQ
            y = acc_v[r0:r0 + TQ, :] + jnp.dot(jnp.concatenate([o0, o1], axis=1), wo_p[...],
                                               preferred_element_type=F32)
            acc_v[r0:r0 + TQ, :] = y
            o_st[r0:r0 + TQ, :] = y.astype(BF16)
            if r0 % TO == 0:
                @pl.when(p == HP - 1)
                def _():
                    cp_o(r0 // TO).start()

        items = [(i, hh) for i in reversed(range(S // TQ)) for hh in range(2)]
        per_chunk = 2 * (TQP // TQ)
        n_qc = S // TQP
        n = len(items)
        s_vals, o_vals = {}, {}
        qproj(n_qc - 1)
        for step in range(n + LOOK + OLAG):
            if step % per_chunk == 0 and n_qc - 2 - step // per_chunk >= 0:
                qproj(n_qc - 2 - step // per_chunk)
            if step < n:
                s_vals[step] = qk(*items[step])
            b = step - LOOK
            if 0 <= b < n:
                o_vals[b] = softmax_pv(*items[b], s_vals.pop(b))
            c = step - LOOK - OLAG
            if 0 <= c < n and c % 2 == 1:
                oproj(items[c][0], o_vals.pop(c - 1), o_vals.pop(c))
        return 0

    lax.fori_loop(0, HP, _scoped("pair", pair_body), 0)
    for k in range(S // TO):
        cp_o(k).wait()


@jax.jit
def pallas_gated_mix__compressed_kv_cla__sliding_local_dilated__prompt_kernel(
    A_x, A_c_kv, A_w_q, A_w_uk, A_w_uv, A_w_o, B_x, B_wqkv, B_wo, gate_w,
):
    del B_x
    x = A_x.reshape(S, M)
    ckv = A_c_kv.reshape(S, DC)
    wo = A_w_o.reshape(H * D, M)
    bwo = B_wo.reshape(H, DH, M)
    gate = gate_w.reshape(1, M)
    any_spec = pl.BlockSpec(memory_space=pl.ANY)
    out = pl.pallas_call(
        _kernel,
        out_shape=jax.ShapeDtypeStruct((S, M), BF16),
        in_specs=[any_spec] * 8 + [pl.BlockSpec(memory_space=pltpu.VMEM)],
        out_specs=any_spec,
        scratch_shapes=[
            pltpu.VMEM((S, M), BF16),
            pltpu.VMEM((S, DC), BF16),
            pltpu.VMEM((HP, M, D), U32),
            pltpu.VMEM((HP, DC, D), U32),
            pltpu.VMEM((HP, DC, D), U32),
            pltpu.VMEM((H * D, M), BF16),
            pltpu.VMEM((M, 3 * M), BF16),
            pltpu.VMEM((DH // 2, H, M), U32),
            pltpu.VMEM((M, M), BF16),
            pltpu.VMEM((M, M), BF16),
            pltpu.VMEM((2, H * PITCH, 128), F32),
            pltpu.VMEM((3, NT_M, S + PAD, 128), F32),
            pltpu.VMEM((S, M), F32),
            pltpu.VMEM((S, 128), F32),
            pltpu.VMEM((8, 128), U32),
            pltpu.VMEM((S, 2 * D), BF16),
            pltpu.VMEM((S, 2 * D), BF16),
            pltpu.VMEM((S, 2 * D), BF16),
            pltpu.VMEM((S, M), BF16),
            pltpu.SemaphoreType.DMA((NT_M,)),
            pltpu.SemaphoreType.DMA((NC,)),
            pltpu.SemaphoreType.DMA((8,)),
            pltpu.SemaphoreType.DMA((6,)),
            pltpu.SemaphoreType.DMA((S // TO,)),
        ],
        compiler_params=pltpu.CompilerParams(vmem_limit_bytes=110 * 1024 * 1024),
    )(x, ckv, A_w_q, A_w_uk, A_w_uv, wo, B_wqkv, bwo, gate)
    return out.reshape(1, S, M)
```

```python
import contextlib
import functools

import jax
import jax.numpy as jnp
from jax import lax
import jax.experimental.pallas as pl
import jax.experimental.pallas.tpu as pltpu

S = 2048
M = 1024
DC = 512
H = 32
HP = H // 2
D = 128
DH = 32
W = 8
DIL = 2
PAD = 16
NT_M = M // 128
TQ = 128
TQP = 256
TC = 512
NC = S // TC
TL = S // HP
TO = 256
GR = 176
PITCH = 40
LOOK = 2
OLAG = 6
SUMG = 32
MAXG = 0
LAP = 2
LAR = 8
LOG2E = 1.4426950408889634
NEG = -1e9

F32 = jnp.float32
BF16 = jnp.bfloat16
U32 = jnp.uint32
NT = (((1,), (1,)), ((), ()))


_PROFILE = False


def _scope(name):
    return jax.named_scope(name) if _PROFILE else contextlib.nullcontext()


def _scoped(name, body):
    def f(i, c):
        with _scope(name):
            return body(i, c)
    return f


def _recip(l):
    r = pl.reciprocal(l, approx=True)
    return r * (2.0 - l * r)


def _lo(w):
    return pltpu.bitcast(w << 16, F32).astype(BF16)


def _hi(w):
    return pltpu.bitcast(w & jnp.uint32(0xFFFF0000), F32).astype(BF16)


def _split_pair(w):
    return jnp.concatenate([_lo(w), _hi(w)], axis=1)


def _ld(ref, r0, n, cols=slice(None)):
    rs = slice(r0 // 2, (r0 + n) // 2) if isinstance(r0, int) else pl.ds(pl.multiple_of(r0 // 2, 8), n // 2)
    return pltpu.bitcast(ref[rs, cols], BF16)


def _st(ref, r0, val, cols=slice(None)):
    ref[r0 // 2:(r0 + val.shape[0]) // 2, cols] = pltpu.bitcast(val, U32)


def _zero_after(z, *vals):
    acc = None
    for v in vals:
        b = pltpu.bitcast(v, U32)
        for r in range(0, b.shape[0], 8):
            for c in range(0, b.shape[1], 128):
                t = b[r:r + 8, c:c + 128]
                acc = t if acc is None else acc | t
    return acc & z


def _chain_reduce(x, op, g, z, dep):
    parts = []
    for r in range(0, x.shape[0], g):
        a = x[r:r + g, 0:128]
        if dep is not None:
            a = pltpu.bitcast(pltpu.bitcast(a, U32) | jnp.concatenate([dep] * (g // 8), axis=0), F32)
        for c in range(128, x.shape[1], 128):
            a = op(a, x[r:r + g, c:c + 128])
        dep = _zero_after(z, a)
        parts.append(a)
    return jnp.concatenate(parts, axis=0), dep


def _kernel(x_hbm, ckv_hbm, wq_hbm, wuk_hbm, wuv_hbm, wo_hbm, bqkv_hbm, bwo_hbm, gate_ref,
            out_hbm,
            x_v, ckv_v, wq_p, wuk_p, wuv_p, wo_v, bqkv_v, bwo_p, wcur_v, wnxt_v, tmp_v,
            qkv_v, acc_v, g_v, z_v, q_s, k_s, v_s, o_st,
            sem_q, sem_x, sem_w, sem_a, sem_o):
    def cp_q(j):
        sl = (pl.ds(j * 128, 128), pl.ds(0, M))
        return pltpu.make_async_copy(bqkv_hbm.at[sl], bqkv_v.at[sl], sem_q.at[j])

    def cp_x(c):
        sl = (pl.ds(c * (TC // 2), TC // 2), slice(None))
        return pltpu.make_async_copy(x_hbm.bitcast(U32).at[sl], x_v.at[sl], sem_x.at[c])

    def cp_w(t):
        sl = (pl.ds((t % 4) * 256, 256), pl.ds((t // 4 + 1) * M, M))
        return pltpu.make_async_copy(bqkv_hbm.at[sl], bqkv_v.at[sl], sem_w.at[t])

    a_copies = [pltpu.make_async_copy(ckv_hbm.bitcast(U32), ckv_v, sem_a.at[0]),
                pltpu.make_async_copy(wo_hbm.bitcast(U32), wo_v, sem_a.at[1])]
    for k, (src, dst) in enumerate(((wuk_hbm, wuk_p), (wuv_hbm, wuv_p), (wq_hbm, wq_p), (bwo_hbm, bwo_p))):
        src_u = src.bitcast(U32)
        a_copies += [pltpu.make_async_copy(src_u.at[:, p, :], dst.at[p], sem_a.at[2 + k])
                     for p in range(HP)]

    def cp_o(k):
        sl = (pl.ds(k * TO, TO), slice(None))
        return pltpu.make_async_copy(o_st.at[sl], out_hbm.at[sl], sem_o.at[k])

    for j in range(NT_M):
        cp_q(j).start()
    cp_x(0).start()
    cp_w(0).start()
    z_v[...] = jnp.zeros((8, 128), U32)
    for part in range(3):
        for t in range(NT_M):
            qkv_v[part, t, 0:PAD, :] = jnp.zeros((PAD, 128), F32)

    def zero_acc(lo, hi):
        def body(i, _):
            acc_v[pl.ds(pl.multiple_of(i * 64, 64), 64), :] = jnp.zeros((64, M), F32)
            return 0
        lax.fori_loop(lo // 64, hi // 64, body, 0)

    zero_acc(0, S // 2)

    def prep_unit(dst, part, j, buf, z, dep):
        k0 = pl.multiple_of(j * 128, 128)
        p0 = pl.multiple_of(part * M, M)
        for c in range(NT_M):
            src = bqkv_v[pl.ds(k0, 128), pl.ds(p0 + c * 128, 128)]
            if dep is not None:
                top = pltpu.bitcast(pltpu.bitcast(src[:16], U32) | dep, BF16)
                src = jnp.concatenate([top, src[16:]], axis=0)
            t = src.astype(F32).T
            for hh in range(4):
                h = 4 * c + hh
                tmp_v[buf, h * PITCH: h * PITCH + DH, :] = t[hh * DH:(hh + 1) * DH, :]
            if z is not None:
                dep = _zero_after(z, t[120:128])
        outs = []
        for d in range(DH):
            o = tmp_v[buf, pl.ds(d, H, stride=PITCH), :].astype(BF16)
            _st(dst, d * H, o, pl.ds(k0, 128))
            outs.append(o)
        return None if z is None else _zero_after(z, *outs)

    def prep0_body(j, _):
        cp_q(2 * j).wait()
        cp_q(2 * j + 1).wait()
        prep_unit(wcur_v, 0, 2 * j, 0, None, None)
        prep_unit(wcur_v, 0, 2 * j + 1, 1, None, None)
        return 0

    lax.fori_loop(0, NT_M // 2, _scoped("prep0", prep0_body), 0)
    zero_acc(S // 2, S)

    def bproj_body(t, _):
        part = t // NC
        c = t % NC

        @pl.when(t < NC)
        def _():
            cp_x(t).wait()

        @pl.when(t < 2 * NC)
        def _():
            cp_w(t).wait()

        @pl.when(t == 0)
        def _():
            for cc in range(1, NC):
                cp_x(cc).start()
                cp_w(cc).start()
            for cc in range(4, 8):
                cp_w(cc).start()

        @pl.when(t == 2)
        def _():
            for cc in a_copies:
                cc.start()

        @pl.when(jnp.logical_and(t > 0, c == 0))
        def _():
            def cpy(i, _):
                rs = pl.ds(pl.multiple_of(i * 64, 64), 64)
                wcur_v[rs, :] = wnxt_v[rs, :]
                return 0
            lax.fori_loop(0, M // 128, cpy, 0)

        r = pl.multiple_of(c * TC, TC)
        y = lax.dot_general(_ld(x_v, r, TC), _ld(wcur_v, 0, M), NT, preferred_element_type=F32)
        for tt in range(NT_M):
            qkv_v[part, tt, pl.ds(PAD + r, TC), :] = y[:, tt * 128:(tt + 1) * 128]

        z = z_v[...]
        nxt = (part + 1) % 3
        dep = prep_unit(wnxt_v, nxt, 2 * c, 0, z, None)
        dep = prep_unit(wnxt_v, nxt, 2 * c + 1, 1, z, dep)
        gw = gate_ref[...].astype(F32)
        g0 = jnp.minimum(t * GR, S - GR)
        for k in range(GR // 16):
            rr = pl.multiple_of(g0 + k * 16, 16)
            xb = x_v[pl.ds(pl.multiple_of(rr // 2, 8), 8), :]
            xb = xb | jnp.concatenate([dep] * NT_M, axis=1)
            xx = pltpu.bitcast(xb, BF16).astype(F32)
            zz = jnp.sum(xx * gw, axis=1, keepdims=True)
            g = jnp.broadcast_to(1.0 / (1.0 + jnp.exp(-zz)), (16, 128))
            g_v[pl.ds(rr, 16), :] = g
            dep = _zero_after(z, g)
        return 0

    lax.fori_loop(0, 3 * NC, _scoped("bproj", bproj_body), 0)
    for c in a_copies:
        c.wait()

    qscale = (D ** -0.5) * LOG2E
    bscale = (DH ** -0.5) * LOG2E

    def local_attn(r, z, dep):
        def zf(*vals):
            return jnp.concatenate([pltpu.bitcast(_zero_after(z, *vals), F32)] * (LAR // 8), axis=0)

        sc = jnp.full((LAR, 128), bscale, F32)
        if dep is not None:
            sc = sc + dep
        q = [qkv_v[0, t, pl.ds(PAD + r, LAR), :] * sc for t in range(NT_M)]
        rowi = r + lax.broadcasted_iota(jnp.int32, (LAR, 128), 0)
        logits, raw = [], []
        for w in range(W):
            a = None if w < LAP else zf(raw[w - LAP])
            for t in range(NT_M):
                pr = q[t] * qkv_v[1, t, pl.ds(PAD + r - DIL * w, LAR), :]
                a = pr if a is None else a + pr
            raw.append(a)
            a = a + pltpu.roll(a, 64, 1)
            a = a + pltpu.roll(a, 32, 1)
            logits.append(jnp.where(rowi >= DIL * w, a, NEG) if w > 0 else a)
        m = functools.reduce(jnp.maximum, logits)
        es = [jnp.exp2(lg - m) for lg in logits]
        l = functools.reduce(lambda a, b: a + b, es)
        f = (1.0 - g_v[pl.ds(r, LAR), :]) * _recip(l)
        es = [e * f for e in es]
        outs = []
        for t in range(NT_M):
            a = None if t < LAP else zf(outs[t - LAP])
            for w in range(W):
                pr = es[w] * qkv_v[2, t, pl.ds(PAD + r - DIL * w, LAR), :]
                a = pr if a is None else a + pr
            outs.append(a)
        return jnp.concatenate(outs, axis=1), zf(*outs[NT_M - LAP:])

    def pair_body(p, _):
        z = z_v[...]
        ckv = _ld(ckv_v, 0, S)
        _st(k_s, 0, jnp.dot(ckv, _split_pair(wuk_p[p]), preferred_element_type=F32).astype(BF16))
        _st(v_s, 0, jnp.dot(ckv, _split_pair(wuv_p[p]), preferred_element_type=F32).astype(BF16))

        rb = pl.multiple_of(p * TL, TL)
        dep, obs = None, []
        for k in range(TL // LAR):
            ob, dep = local_attn(rb + k * LAR, z, dep)
            obs.append(ob)
        ob = jnp.concatenate(obs, axis=0).astype(BF16)
        wop = jnp.concatenate([f(bwo_p[dp]) for dp in range(DH // 2) for f in (_lo, _hi)], axis=0)
        acc_v[pl.ds(rb, TL), :] = acc_v[pl.ds(rb, TL), :] + jnp.dot(ob, wop, preferred_element_type=F32)

        wq = _split_pair(wq_p[p])
        row = lax.broadcasted_iota(jnp.int32, (TQ, TQ), 0)
        col = lax.broadcasted_iota(jnp.int32, (TQ, TQ), 1)
        causal = col <= row

        def qproj(c):
            q = jnp.dot(_ld(x_v, c * TQP, TQP), wq, preferred_element_type=F32) * qscale
            _st(q_s, c * TQP, q.astype(BF16))

        def qk(i, hh):
            cs = slice(hh * D, (hh + 1) * D)
            return lax.dot_general(_ld(q_s, i * TQ, TQ, cs), _ld(k_s, 0, (i + 1) * TQ, cs), NT,
                                   preferred_element_type=F32)

        ldep = [None]

        def softmax_pv(i, hh, s):
            cs = slice(hh * D, (hh + 1) * D)
            r0 = i * TQ
            sd = jnp.where(causal, s[:, r0:], NEG)
            s = jnp.concatenate([s[:, :r0], sd], axis=1) if i > 0 else sd
            if MAXG and i > 1:
                m = jnp.max(_chain_reduce(s, jnp.maximum, MAXG, z, None)[0], axis=1, keepdims=True)
            else:
                m = jnp.max(s, axis=1, keepdims=True)
            e = jnp.exp2(s - m)
            if SUMG and i > 1:
                lp, ldep[0] = _chain_reduce(e, jnp.add, SUMG, z, ldep[0] if hh == 1 else None)
                l = jnp.sum(lp, axis=1, keepdims=True)
            else:
                l = jnp.sum(e, axis=1, keepdims=True)
            o = jnp.dot(e.astype(BF16), _ld(v_s, 0, r0 + TQ, cs), preferred_element_type=F32)
            return (o * (g_v[r0:r0 + TQ, :] * _recip(l))).astype(BF16)

        def oproj(i, o0, o1):
            r0 = i * TQ
            y = acc_v[r0:r0 + TQ, :] + jnp.dot(jnp.concatenate([o0, o1], axis=1),
                                               _ld(wo_v, p * (2 * D), 2 * D), preferred_element_type=F32)
            acc_v[r0:r0 + TQ, :] = y
            o_st[r0:r0 + TQ, :] = y.astype(BF16)
            if r0 % TO == 0:
                @pl.when(p == HP - 1)
                def _():
                    cp_o(r0 // TO).start()

        items = [(i, hh) for i in reversed(range(S // TQ)) for hh in range(2)]
        per_chunk = 2 * (TQP // TQ)
        n_qc = S // TQP
        n = len(items)
        s_vals, o_vals = {}, {}
        qproj(n_qc - 1)
        for step in range(n + LOOK + OLAG):
            if step % per_chunk == 0 and n_qc - 2 - step // per_chunk >= 0:
                qproj(n_qc - 2 - step // per_chunk)
            if step < n:
                s_vals[step] = qk(*items[step])
            b = step - LOOK
            if 0 <= b < n:
                o_vals[b] = softmax_pv(*items[b], s_vals.pop(b))
            c = step - LOOK - OLAG
            if 0 <= c < n and c % 2 == 1:
                oproj(items[c][0], o_vals.pop(c - 1), o_vals.pop(c))
        return 0

    lax.fori_loop(0, HP, _scoped("pair", pair_body), 0)
    for k in range(S // TO):
        cp_o(k).wait()


@jax.jit
def pallas_gated_mix__compressed_kv_cla__sliding_local_dilated__prompt_kernel(
    A_x, A_c_kv, A_w_q, A_w_uk, A_w_uv, A_w_o, B_x, B_wqkv, B_wo, gate_w,
):
    del B_x
    x = A_x.reshape(S, M)
    ckv = A_c_kv.reshape(S, DC)
    wo = A_w_o.reshape(H * D, M)
    bwo = B_wo.reshape(H, DH, M)
    gate = gate_w.reshape(1, M)
    any_spec = pl.BlockSpec(memory_space=pl.ANY)
    out = pl.pallas_call(
        _kernel,
        out_shape=jax.ShapeDtypeStruct((S, M), BF16),
        in_specs=[any_spec] * 8 + [pl.BlockSpec(memory_space=pltpu.VMEM)],
        out_specs=any_spec,
        scratch_shapes=[
            pltpu.VMEM((S // 2, M), U32),
            pltpu.VMEM((S // 2, DC), U32),
            pltpu.VMEM((HP, M, D), U32),
            pltpu.VMEM((HP, DC, D), U32),
            pltpu.VMEM((HP, DC, D), U32),
            pltpu.VMEM((H * D // 2, M), U32),
            pltpu.VMEM((M, 3 * M), BF16),
            pltpu.VMEM((DH // 2, H, M), U32),
            pltpu.VMEM((M // 2, M), U32),
            pltpu.VMEM((M // 2, M), U32),
            pltpu.VMEM((2, H * PITCH, 128), F32),
            pltpu.VMEM((3, NT_M, S + PAD, 128), F32),
            pltpu.VMEM((S, M), F32),
            pltpu.VMEM((S, 128), F32),
            pltpu.VMEM((8, 128), U32),
            pltpu.VMEM((S // 2, 2 * D), U32),
            pltpu.VMEM((S // 2, 2 * D), U32),
            pltpu.VMEM((S // 2, 2 * D), U32),
            pltpu.VMEM((S, M), BF16),
            pltpu.SemaphoreType.DMA((NT_M,)),
            pltpu.SemaphoreType.DMA((NC,)),
            pltpu.SemaphoreType.DMA((8,)),
            pltpu.SemaphoreType.DMA((6,)),
            pltpu.SemaphoreType.DMA((S // TO,)),
        ],
        compiler_params=pltpu.CompilerParams(vmem_limit_bytes=110 * 1024 * 1024),
    )(x, ckv, A_w_q, A_w_uk, A_w_uv, wo, B_wqkv, bwo, gate)
    return out.reshape(1, S, M)
```

```python
import contextlib
import functools

import jax
import jax.numpy as jnp
from jax import lax
import jax.experimental.pallas as pl
import jax.experimental.pallas.tpu as pltpu

S = 2048
M = 1024
DC = 512
H = 32
HP = H // 2
D = 128
DH = 32
W = 8
DIL = 2
PAD = 16
NT_M = M // 128
TQ = 128
TQP = 128
TC = 512
NC = S // TC
TL = S // HP
TO = 256
GR = 176
PITCH = 40
LOOK = 2
OLAG = 6
SUMG = 32
MAXG = 0
LAP = 2
LAR = 8
LOG2E = 1.4426950408889634
NEG = -1e9

F32 = jnp.float32
BF16 = jnp.bfloat16
U32 = jnp.uint32
NT = (((1,), (1,)), ((), ()))


_PROFILE = False


def _scope(name):
    return jax.named_scope(name) if _PROFILE else contextlib.nullcontext()


def _scoped(name, body):
    def f(i, c):
        with _scope(name):
            return body(i, c)
    return f


def _recip(l):
    r = pl.reciprocal(l, approx=True)
    return r * (2.0 - l * r)


def _lo(w):
    return pltpu.bitcast(w << 16, F32)


def _hi(w):
    return pltpu.bitcast(w & jnp.uint32(0xFFFF0000), F32)


def _split_pair(w):
    return jnp.concatenate([_lo(w), _hi(w)], axis=1).astype(BF16)


def _ld(ref, r0, n, cols=slice(None)):
    rs = slice(r0 // 2, (r0 + n) // 2) if isinstance(r0, int) else pl.ds(pl.multiple_of(r0 // 2, 8), n // 2)
    return pltpu.bitcast(ref[rs, cols], BF16)


def _st(ref, r0, val, cols=slice(None)):
    ref[r0 // 2:(r0 + val.shape[0]) // 2, cols] = pltpu.bitcast(val, U32)


def _zero_after(z, *vals):
    acc = None
    for v in vals:
        b = pltpu.bitcast(v, U32)
        for r in range(0, b.shape[0], 8):
            for c in range(0, b.shape[1], 128):
                t = b[r:r + 8, c:c + 128]
                acc = t if acc is None else acc | t
    return acc & z


def _chain_reduce(x, op, g, z, dep):
    parts = []
    for r in range(0, x.shape[0], g):
        a = x[r:r + g, 0:128]
        if dep is not None:
            a = pltpu.bitcast(pltpu.bitcast(a, U32) | jnp.concatenate([dep] * (g // 8), axis=0), F32)
        for c in range(128, x.shape[1], 128):
            a = op(a, x[r:r + g, c:c + 128])
        dep = _zero_after(z, a)
        parts.append(a)
    return jnp.concatenate(parts, axis=0), dep


def _kernel(x_hbm, ckv_hbm, wq_hbm, wuk_hbm, wuv_hbm, wo_hbm, bqkv_hbm, bwo_hbm, gate_ref,
            out_hbm,
            x_v, ckv_v, wq_p, wuk_p, wuv_p, wo_v, bqkv_v, bwo_p, wcur_v, wnxt_v, tmp_v,
            qkv_v, acc_v, g_v, z_v, q_s, k_s, v_s, o_st,
            sem_x, sem_w, sem_a, sem_o):
    def cp_x(c):
        sl = (pl.ds(c * (TC // 2), TC // 2), slice(None))
        return pltpu.make_async_copy(x_hbm.bitcast(U32).at[sl], x_v.at[sl], sem_x.at[c])

    def cp_w(u):
        sl = (pl.ds((u % 4) * 256, 256), pl.ds((u // 4) * M, M))
        return pltpu.make_async_copy(bqkv_hbm.at[sl], bqkv_v.at[sl], sem_w.at[u])

    a_copies = [pltpu.make_async_copy(ckv_hbm.bitcast(U32), ckv_v, sem_a),
                pltpu.make_async_copy(wo_hbm.bitcast(U32), wo_v, sem_a)]
    for src, dst in ((wuk_hbm, wuk_p), (wuv_hbm, wuv_p), (wq_hbm, wq_p), (bwo_hbm, bwo_p)):
        src_u = src.bitcast(U32)
        a_copies += [pltpu.make_async_copy(src_u.at[:, p, :], dst.at[p], sem_a) for p in range(HP)]
    a_waits = [pltpu.make_async_copy(b, b, sem_a) for b in (ckv_v, wo_v, wuk_p, wuv_p, wq_p, bwo_p)]

    def cp_o(r0, n):
        sl = (pl.ds(r0, n), slice(None))
        return pltpu.make_async_copy(o_st.at[sl], out_hbm.at[sl], sem_o)

    for u in range(4):
        cp_w(u).start()
    cp_x(0).start()
    cp_w(4).start()
    z_v[...] = jnp.zeros((8, 128), U32)
    for part in range(3):
        for t in range(NT_M):
            qkv_v[part, t, 0:PAD, :] = jnp.zeros((PAD, 128), F32)

    def zero_acc(lo, hi):
        def body(i, _):
            acc_v[pl.ds(pl.multiple_of(i * 64, 64), 64), :] = jnp.zeros((64, M), F32)
            return 0
        lax.fori_loop(lo // 64, hi // 64, body, 0)

    zero_acc(0, S // 2)

    def prep_unit(dst, part, j, buf, z, dep):
        k0 = pl.multiple_of(j * 128, 128)
        p0 = pl.multiple_of(part * M, M)
        for c in range(NT_M):
            src = bqkv_v[pl.ds(k0, 128), pl.ds(p0 + c * 128, 128)]
            if dep is not None:
                top = pltpu.bitcast(pltpu.bitcast(src[:16], U32) | dep, BF16)
                src = jnp.concatenate([top, src[16:]], axis=0)
            t = src.astype(F32).T
            for hh in range(4):
                h = 4 * c + hh
                tmp_v[buf, h * PITCH: h * PITCH + DH, :] = t[hh * DH:(hh + 1) * DH, :]
            if z is not None:
                dep = _zero_after(z, t[120:128])
        outs = []
        for d in range(DH):
            o = tmp_v[buf, pl.ds(d, H, stride=PITCH), :].astype(BF16)
            _st(dst, d * H, o, pl.ds(k0, 128))
            outs.append(o)
        return None if z is None else _zero_after(z, *outs)

    def prep0_body(j, _):
        cp_w(j).wait()
        prep_unit(wcur_v, 0, 2 * j, 0, None, None)
        prep_unit(wcur_v, 0, 2 * j + 1, 1, None, None)
        return 0

    lax.fori_loop(0, NT_M // 2, _scoped("prep0", prep0_body), 0)
    zero_acc(S // 2, S)

    def bproj_body(t, _):
        part = t // NC
        c = t % NC

        @pl.when(t < NC)
        def _():
            cp_x(t).wait()

        @pl.when(t < 2 * NC)
        def _():
            cp_w(t + 4).wait()

        @pl.when(t == 0)
        def _():
            for k in range(1, NC):
                cp_x(k).start()
                cp_w(4 + k).start()
            for u in range(8, 12):
                cp_w(u).start()

        @pl.when(t == 2)
        def _():
            for cc in a_copies:
                cc.start()

        @pl.when(jnp.logical_and(t > 0, c == 0))
        def _():
            def cpy(i, _):
                rs = pl.ds(pl.multiple_of(i * 64, 64), 64)
                wcur_v[rs, :] = wnxt_v[rs, :]
                return 0
            lax.fori_loop(0, M // 128, cpy, 0)

        r = pl.multiple_of(c * TC, TC)
        y = lax.dot_general(_ld(x_v, r, TC), _ld(wcur_v, 0, M), NT, preferred_element_type=F32)
        for tt in range(NT_M):
            qkv_v[part, tt, pl.ds(PAD + r, TC), :] = y[:, tt * 128:(tt + 1) * 128]

        z = z_v[...]
        nxt = (part + 1) % 3
        dep = prep_unit(wnxt_v, nxt, 2 * c, 0, z, None)
        dep = prep_unit(wnxt_v, nxt, 2 * c + 1, 1, z, dep)
        gw = gate_ref[...].astype(F32).reshape(1, M)
        g0 = jnp.minimum(t * GR, S - GR)
        for k in range(GR // 16):
            rr = pl.multiple_of(g0 + k * 16, 16)
            xb = x_v[pl.ds(pl.multiple_of(rr // 2, 8), 8), :]
            xb = xb | jnp.concatenate([dep] * NT_M, axis=1)
            xx = pltpu.bitcast(xb, BF16).astype(F32)
            zz = jnp.sum(xx * gw, axis=1, keepdims=True)
            g = jnp.broadcast_to(1.0 / (1.0 + jnp.exp(-zz)), (16, 128))
            g_v[pl.ds(rr, 16), :] = g
            dep = _zero_after(z, g)
        return 0

    lax.fori_loop(0, 3 * NC, _scoped("bproj", bproj_body), 0)
    for c in a_waits:
        c.wait()

    qscale = (D ** -0.5) * LOG2E
    bscale = (DH ** -0.5) * LOG2E

    def local_attn(r, z, dep):
        def zf(*vals):
            return jnp.concatenate([pltpu.bitcast(_zero_after(z, *vals), F32)] * (LAR // 8), axis=0)

        sc = jnp.full((LAR, 128), bscale, F32)
        if dep is not None:
            sc = sc + dep
        q = [qkv_v[0, t, pl.ds(PAD + r, LAR), :] * sc for t in range(NT_M)]
        rowi = r + lax.broadcasted_iota(jnp.int32, (LAR, 128), 0)
        logits, raw = [], []
        for w in range(W):
            a = None if w < LAP else zf(raw[w - LAP])
            for t in range(NT_M):
                pr = q[t] * qkv_v[1, t, pl.ds(PAD + r - DIL * w, LAR), :]
                a = pr if a is None else a + pr
            raw.append(a)
            a = a + pltpu.roll(a, 64, 1)
            a = a + pltpu.roll(a, 32, 1)
            logits.append(jnp.where(rowi >= DIL * w, a, NEG) if w > 0 else a)
        m = functools.reduce(jnp.maximum, logits)
        es = [jnp.exp2(lg - m) for lg in logits]
        l = functools.reduce(lambda a, b: a + b, es)
        f = (1.0 - g_v[pl.ds(r, LAR), :]) * _recip(l)
        es = [e * f for e in es]
        outs = []
        for t in range(NT_M):
            a = None if t < LAP else zf(outs[t - LAP])
            for w in range(W):
                pr = es[w] * qkv_v[2, t, pl.ds(PAD + r - DIL * w, LAR), :]
                a = pr if a is None else a + pr
            outs.append(a)
        return jnp.concatenate(outs, axis=1), zf(*outs[NT_M - LAP:])

    def pair_body(p, _):
        z = z_v[...]
        ckv = _ld(ckv_v, 0, S)
        _st(k_s, 0, jnp.dot(ckv, _split_pair(wuk_p[p]), preferred_element_type=F32).astype(BF16))
        _st(v_s, 0, jnp.dot(ckv, _split_pair(wuv_p[p]), preferred_element_type=F32).astype(BF16))

        rb = pl.multiple_of(p * TL, TL)
        dep, obs = None, []
        for k in range(TL // LAR):
            ob, dep = local_attn(rb + k * LAR, z, dep)
            obs.append(ob)
        ob = jnp.concatenate(obs, axis=0).astype(BF16)
        wop = jnp.concatenate([f(bwo_p[dp]) for dp in range(DH // 2) for f in (_lo, _hi)], axis=0).astype(BF16)
        acc_v[pl.ds(rb, TL), :] = acc_v[pl.ds(rb, TL), :] + jnp.dot(ob, wop, preferred_element_type=F32)

        wq = _split_pair(wq_p[p])
        row = lax.broadcasted_iota(jnp.int32, (TQ, TQ), 0)
        col = lax.broadcasted_iota(jnp.int32, (TQ, TQ), 1)
        causal = col <= row

        def qproj(c):
            q = jnp.dot(_ld(x_v, c * TQP, TQP), wq, preferred_element_type=F32) * qscale
            _st(q_s, c * TQP, q.astype(BF16))

        def qk(i, hh):
            cs = slice(hh * D, (hh + 1) * D)
            return lax.dot_general(_ld(q_s, i * TQ, TQ, cs), _ld(k_s, 0, (i + 1) * TQ, cs), NT,
                                   preferred_element_type=F32)

        ldep = [None]

        def softmax_pv(i, hh, s):
            cs = slice(hh * D, (hh + 1) * D)
            r0 = i * TQ
            sd = jnp.where(causal, s[:, r0:], NEG)
            s = jnp.concatenate([s[:, :r0], sd], axis=1) if i > 0 else sd
            if MAXG and i > 1:
                m = jnp.max(_chain_reduce(s, jnp.maximum, MAXG, z, None)[0], axis=1, keepdims=True)
            else:
                m = jnp.max(s, axis=1, keepdims=True)
            e = jnp.exp2(s - m)
            if SUMG and i > 1:
                lp, ldep[0] = _chain_reduce(e, jnp.add, SUMG, z, ldep[0] if hh == 1 else None)
                l = jnp.sum(lp, axis=1, keepdims=True)
            else:
                l = jnp.sum(e, axis=1, keepdims=True)
            o = jnp.dot(e.astype(BF16), _ld(v_s, 0, r0 + TQ, cs), preferred_element_type=F32)
            return o * (g_v[r0:r0 + TQ, :] * _recip(l))

        def oproj(i, o0, o1):
            r0 = i * TQ
            y = acc_v[r0:r0 + TQ, :] + jnp.dot(jnp.concatenate([o0, o1], axis=1).astype(BF16),
                                               _ld(wo_v, p * (2 * D), 2 * D), preferred_element_type=F32)
            acc_v[r0:r0 + TQ, :] = y
            o_st[r0:r0 + TQ, :] = y.astype(BF16)
            if r0 < TO:
                pl.when(p == HP - 1)(cp_o(r0, TQ).start)
            elif r0 % TO == 0:
                pl.when(p == HP - 1)(cp_o(r0, TO).start)

        items = [(i, hh) for i in reversed(range(S // TQ)) for hh in range(2)]
        per_chunk = 2 * (TQP // TQ)
        n_qc = S // TQP
        n = len(items)
        s_vals, o_vals = {}, {}
        qproj(n_qc - 1)
        for step in range(n + LOOK + OLAG):
            if step % per_chunk == 0 and n_qc - 2 - step // per_chunk >= 0:
                qproj(n_qc - 2 - step // per_chunk)
            if step < n:
                s_vals[step] = qk(*items[step])
            b = step - LOOK
            if 0 <= b < n:
                o_vals[b] = softmax_pv(*items[b], s_vals.pop(b))
            c = step - LOOK - OLAG
            if 0 <= c < n and c % 2 == 1:
                oproj(items[c][0], o_vals.pop(c - 1), o_vals.pop(c))
        return 0

    lax.fori_loop(0, HP, _scoped("pair", pair_body), 0)
    cp_o(0, S).wait()


@jax.jit
def pallas_gated_mix__compressed_kv_cla__sliding_local_dilated__prompt_kernel(
    A_x, A_c_kv, A_w_q, A_w_uk, A_w_uv, A_w_o, B_x, B_wqkv, B_wo, gate_w,
):
    del B_x
    x = A_x.reshape(S, M)
    ckv = A_c_kv.reshape(S, DC)
    wo = A_w_o.reshape(H * D, M)
    bwo = B_wo.reshape(H, DH, M)
    any_spec = pl.BlockSpec(memory_space=pl.ANY)
    out = pl.pallas_call(
        _kernel,
        out_shape=jax.ShapeDtypeStruct((S, M), BF16),
        in_specs=[any_spec] * 8 + [pl.BlockSpec(memory_space=pltpu.VMEM)],
        out_specs=any_spec,
        scratch_shapes=[
            pltpu.VMEM((S // 2, M), U32),
            pltpu.VMEM((S // 2, DC), U32),
            pltpu.VMEM((HP, M, D), U32),
            pltpu.VMEM((HP, DC, D), U32),
            pltpu.VMEM((HP, DC, D), U32),
            pltpu.VMEM((H * D // 2, M), U32),
            pltpu.VMEM((M, 3 * M), BF16),
            pltpu.VMEM((DH // 2, H, M), U32),
            pltpu.VMEM((M // 2, M), U32),
            pltpu.VMEM((M // 2, M), U32),
            pltpu.VMEM((2, H * PITCH, 128), F32),
            pltpu.VMEM((3, NT_M, S + PAD, 128), F32),
            pltpu.VMEM((S, M), F32),
            pltpu.VMEM((S, 128), F32),
            pltpu.VMEM((8, 128), U32),
            pltpu.VMEM((S // 2, 2 * D), U32),
            pltpu.VMEM((S // 2, 2 * D), U32),
            pltpu.VMEM((S // 2, 2 * D), U32),
            pltpu.VMEM((S, M), BF16),
            pltpu.SemaphoreType.DMA((NC,)),
            pltpu.SemaphoreType.DMA((12,)),
            pltpu.SemaphoreType.DMA(()),
            pltpu.SemaphoreType.DMA(()),
        ],
        compiler_params=pltpu.CompilerParams(vmem_limit_bytes=110 * 1024 * 1024),
    )(x, ckv, A_w_q, A_w_uk, A_w_uv, wo, B_wqkv, bwo, gate_w)
    return out.reshape(1, S, M)
```

```python
import contextlib
import functools

import jax
import jax.numpy as jnp
from jax import lax
import jax.experimental.pallas as pl
import jax.experimental.pallas.tpu as pltpu

S = 2048
M = 1024
DC = 512
H = 32
HP = H // 2
D = 128
DH = 32
W = 8
DIL = 2
PAD = 16
NT_M = M // 128
TQ = 128
TQP = 128
TC = 512
NC = S // TC
TL = S // HP
TO = 256
GR = 176
PITCH = 40
LOOK = 2
OLAG = 6
SUMG = 32
MAXG = 0
LAP = 2
LAR = 8
NB1 = 4
LOG2E = 1.4426950408889634
NEG = -1e9

F32 = jnp.float32
BF16 = jnp.bfloat16
U32 = jnp.uint32
NT = (((1,), (1,)), ((), ()))


_PROFILE = False


def _scope(name):
    return jax.named_scope(name) if _PROFILE else contextlib.nullcontext()


def _scoped(name, body):
    def f(i, c):
        with _scope(name):
            return body(i, c)
    return f


def _recip(l):
    r = pl.reciprocal(l, approx=True)
    return r * (2.0 - l * r)


def _lo(w):
    return pltpu.bitcast(w << 16, F32)


def _hi(w):
    return pltpu.bitcast(w & jnp.uint32(0xFFFF0000), F32)


def _split_pair(w):
    return jnp.concatenate([_lo(w), _hi(w)], axis=1).astype(BF16)


def _ld(ref, r0, n, cols=slice(None)):
    if isinstance(r0, int):
        rs = slice(r0 // 2, (r0 + n) // 2)
    else:
        rs = pl.ds(pl.multiple_of(lax.shift_right_logical(r0, 1), 8), n // 2)
    return pltpu.bitcast(ref[rs, cols], BF16)


def _st(ref, r0, val, cols=slice(None)):
    ref[r0 // 2:(r0 + val.shape[0]) // 2, cols] = pltpu.bitcast(val, U32)


def _zero_after(z, *vals):
    acc = None
    for v in vals:
        b = pltpu.bitcast(v, U32)
        for r in range(0, b.shape[0], 8):
            for c in range(0, b.shape[1], 128):
                t = b[r:r + 8, c:c + 128]
                acc = t if acc is None else acc | t
    return acc & z


def _chain_reduce(x, op, g, z, dep):
    parts = []
    for r in range(0, x.shape[0], g):
        a = x[r:r + g, 0:128]
        if dep is not None:
            a = pltpu.bitcast(pltpu.bitcast(a, U32) | jnp.concatenate([dep] * (g // 8), axis=0), F32)
        for c in range(128, x.shape[1], 128):
            a = op(a, x[r:r + g, c:c + 128])
        dep = _zero_after(z, a)
        parts.append(a)
    return jnp.concatenate(parts, axis=0), dep


def _kernel(x_hbm, ckv_hbm, wq_hbm, wuk_hbm, wuv_hbm, wo_hbm, bqkv_hbm, bwo_hbm, gate_ref,
            out_hbm,
            x_v, ckv_v, wq_p, wuk_p, wuv_p, wo_v, bqkv_v, bwo_p, wcur_v, wnxt_v, tmp_v,
            qkv_v, acc_v, g_v, z_v, q_s, k_s, v_s, o_st,
            sem_x, sem_w, sem_a, sem_o):
    def cp_x(c):
        sl = (pl.ds(c * (TC // 2), TC // 2), slice(None))
        return pltpu.make_async_copy(x_hbm.bitcast(U32).at[sl], x_v.at[sl], sem_x.at[c])

    def cp_w(u):
        u_lo, u_hi = (u % 4, u // 4) if isinstance(u, int) else (u & 3, lax.shift_right_logical(u, 2))
        sl = (pl.ds(u_lo * 256, 256), pl.ds(u_hi * M, M))
        return pltpu.make_async_copy(bqkv_hbm.at[sl], bqkv_v.at[sl], sem_w.at[u])

    a_copies = [pltpu.make_async_copy(ckv_hbm.bitcast(U32), ckv_v, sem_a),
                pltpu.make_async_copy(wo_hbm.bitcast(U32), wo_v, sem_a)]
    for src, dst in ((wuk_hbm, wuk_p), (wuv_hbm, wuv_p), (wq_hbm, wq_p), (bwo_hbm, bwo_p)):
        src_u = src.bitcast(U32)
        a_copies += [pltpu.make_async_copy(src_u.at[:, p, :], dst.at[p], sem_a) for p in range(HP)]
    a_waits = [pltpu.make_async_copy(b, b, sem_a) for b in (ckv_v, wo_v, wuk_p, wuv_p, wq_p, bwo_p)]

    def cp_o(r0, n):
        sl = (pl.ds(r0, n), slice(None))
        return pltpu.make_async_copy(o_st.at[sl], out_hbm.at[sl], sem_o)

    def cp_x0(half):
        sl = (pl.ds(0, TC // 2), pl.ds(half * (M // 2), M // 2))
        return pltpu.make_async_copy(x_hbm.bitcast(U32).at[sl], x_v.at[sl], sem_x.at[half * NC])

    for cc in (cp_w(0), cp_w(1), cp_x0(0), cp_w(2), cp_w(3), cp_x0(1), cp_w(4)):
        cc.start()
    z_v[...] = jnp.zeros((8, 128), U32)
    for part in range(3):
        for t in range(NT_M):
            qkv_v[part, t, 0:PAD, :] = jnp.zeros((PAD, 128), F32)

    def zero_body(i, _):
        acc_v[pl.ds(pl.multiple_of(i * 64, 64), 64), :] = jnp.zeros((64, M), F32)
        return 0

    with _scope("zero"):
        lax.fori_loop(0, S // 64, zero_body, 0)

    def prep_t(part, units, z, dep=None):
        p0 = part * M if isinstance(part, int) else pl.multiple_of(part * M, M)
        deps = [dep] * len(units)
        for c in range(NT_M):
            for u, (j, buf) in enumerate(units):
                k0 = j * 128 if isinstance(j, int) else pl.multiple_of(j * 128, 128)
                src = bqkv_v[pl.ds(k0, 128), pl.ds(p0 + c * 128, 128)]
                if deps[u] is not None:
                    top = pltpu.bitcast(pltpu.bitcast(src[:16], U32) | deps[u], BF16)
                    src = jnp.concatenate([top, src[16:]], axis=0)
                t = src.T.astype(F32)
                for hh in range(4):
                    h = 4 * c + hh
                    tmp_v[buf, h * PITCH: h * PITCH + DH, :] = t[hh * DH:(hh + 1) * DH, :]
                if z is not None:
                    deps[u] = _zero_after(z, t[120:128])

    def prep_p(dst, j, buf, z):
        k0 = j * 128 if isinstance(j, int) else pl.multiple_of(j * 128, 128)
        outs = []
        for d in range(DH):
            o = tmp_v[buf, pl.ds(d, H, stride=PITCH), :].astype(BF16)
            _st(dst, d * H, o, pl.ds(k0, 128))
            outs.append(o)
        return None if z is None else _zero_after(z, *outs)

    def side_work(t, c, nxt):
        z = z_v[...]
        if isinstance(t, int):
            prep_t(nxt, [(2 * c, 0), (2 * c + 1, 1)], z)
            dep = prep_p(wnxt_v, 2 * c, 0, z) | prep_p(wnxt_v, 2 * c + 1, 1, z)
        else:
            prep_t(nxt, [(2 * c, 0)], z)
            dep = prep_p(wnxt_v, 2 * c, 0, z)
            prep_t(nxt, [(2 * c + 1, 1)], z, dep)
            dep = prep_p(wnxt_v, 2 * c + 1, 1, z)
        gw = gate_ref[...].astype(F32).reshape(1, M)
        g0 = t * GR if isinstance(t, int) else jnp.minimum(t * GR, S - GR)
        for k in range(GR // 16):
            if isinstance(t, int):
                rr, rw = g0 + k * 16, (g0 + k * 16) // 2
            else:
                rr = pl.multiple_of(g0 + k * 16, 16)
                rw = pl.multiple_of(lax.shift_right_logical(rr, 1), 8)
            xb = x_v[pl.ds(rw, 8), :] | jnp.concatenate([dep] * NT_M, axis=1)
            xx = pltpu.bitcast(xb, BF16).astype(F32)
            zz = jnp.sum(xx * gw, axis=1, keepdims=True)
            g = jnp.broadcast_to(1.0 / (1.0 + jnp.exp(-zz)), (16, 128))
            g_v[pl.ds(rr, 16), :] = g
            dep = _zero_after(z, g)

    def prep0_body(j, _):
        cp_w(j).wait()
        prep_t(0, [(2 * j, 0)], None)
        prep_t(0, [(2 * j + 1, 1)], None)
        prep_p(wcur_v, 2 * j, 0, None)
        prep_p(wcur_v, 2 * j + 1, 1, None)
        return 0

    lax.fori_loop(0, 2, _scoped("prep0", prep0_body), 0)

    kh = M // 2

    def first_half(n0, n1):
        y = lax.dot_general(_ld(x_v, 0, TC, slice(0, kh)), _ld(wcur_v, n0 * 128, (n1 - n0) * 128, slice(0, kh)),
                            NT, preferred_element_type=F32)
        for tt in range(n0, n1):
            qkv_v[0, tt, PAD:PAD + TC, :] = y[:, (tt - n0) * 128:(tt - n0 + 1) * 128]

    with _scope("b1"):
        cp_x0(0).wait()
        first_half(0, NB1)
    with _scope("b2"):
        cp_w(2).wait()
        cp_w(3).wait()
        first_half(NB1, NT_M)
        z = z_v[...]
        prep_t(0, [(j, j - 4) for j in range(4, 8)], z)
        for j in range(4, 8):
            prep_p(wcur_v, j, j - 4, None)
    with _scope("b3"):
        cp_x0(1).wait()
        cp_w(4).wait()
        for k in range(1, NC):
            cp_x(k).start()
            cp_w(4 + k).start()
        for u in range(8, 12):
            cp_w(u).start()
        y = lax.dot_general(_ld(x_v, 0, TC, slice(kh, M)), _ld(wcur_v, 0, M, slice(kh, M)),
                            NT, preferred_element_type=F32)
        for tt in range(NT_M):
            qkv_v[0, tt, PAD:PAD + TC, :] = qkv_v[0, tt, PAD:PAD + TC, :] + y[:, tt * 128:(tt + 1) * 128]
        side_work(0, 0, 1)

    def bproj_body(t, _):
        part = lax.shift_right_logical(t, 2)
        c = t & 3

        @pl.when(t < NC)
        def _():
            cp_x(t).wait()

        @pl.when(t < 2 * NC)
        def _():
            cp_w(t + 4).wait()

        @pl.when(jnp.logical_or(t == 2, c == 0))
        def _():
            @pl.when(t == 2)
            def _():
                for cc in a_copies:
                    cc.start()

            @pl.when(t != 2)
            def _():
                def cpy(i, _):
                    rs = pl.ds(pl.multiple_of(i * 64, 64), 64)
                    wcur_v[rs, :] = wnxt_v[rs, :]
                    return 0
                lax.fori_loop(0, M // 128, cpy, 0)

        r = pl.multiple_of(c * TC, TC)
        y = lax.dot_general(_ld(x_v, r, TC), _ld(wcur_v, 0, M), NT, preferred_element_type=F32)
        for tt in range(NT_M):
            qkv_v[part, tt, pl.ds(PAD + r, TC), :] = y[:, tt * 128:(tt + 1) * 128]
        side_work(t, c, jnp.where(part == 2, 0, part + 1))
        return 0

    lax.fori_loop(1, 3 * NC, _scoped("bproj", bproj_body), 0)
    for c in a_waits:
        c.wait()

    qscale = (D ** -0.5) * LOG2E
    bscale = (DH ** -0.5) * LOG2E

    def local_attn(r, z, dep):
        def zf(*vals):
            return jnp.concatenate([pltpu.bitcast(_zero_after(z, *vals), F32)] * (LAR // 8), axis=0)

        sc = jnp.full((LAR, 128), bscale, F32)
        if dep is not None:
            sc = sc + dep
        q = [qkv_v[0, t, pl.ds(PAD + r, LAR), :] * sc for t in range(NT_M)]
        rowi = r + lax.broadcasted_iota(jnp.int32, (LAR, 128), 0)
        logits, raw = [], []
        for w in range(W):
            a = None if w < LAP else zf(raw[w - LAP])
            for t in range(NT_M):
                pr = q[t] * qkv_v[1, t, pl.ds(PAD + r - DIL * w, LAR), :]
                a = pr if a is None else a + pr
            raw.append(a)
            a = a + pltpu.roll(a, 64, 1)
            a = a + pltpu.roll(a, 32, 1)
            logits.append(jnp.where(rowi >= DIL * w, a, NEG) if w > 0 else a)
        m = functools.reduce(jnp.maximum, logits)
        es = [jnp.exp2(lg - m) for lg in logits]
        l = functools.reduce(lambda a, b: a + b, es)
        f = (1.0 - g_v[pl.ds(r, LAR), :]) * _recip(l)
        es = [e * f for e in es]
        outs = []
        for t in range(NT_M):
            a = None if t < LAP else zf(outs[t - LAP])
            for w in range(W):
                pr = es[w] * qkv_v[2, t, pl.ds(PAD + r - DIL * w, LAR), :]
                a = pr if a is None else a + pr
            outs.append(a)
        return jnp.concatenate(outs, axis=1), zf(*outs[NT_M - LAP:])

    def pair_body(p, _):
        z = z_v[...]
        ckv = _ld(ckv_v, 0, S)
        _st(k_s, 0, jnp.dot(ckv, _split_pair(wuk_p[p]), preferred_element_type=F32).astype(BF16))
        _st(v_s, 0, jnp.dot(ckv, _split_pair(wuv_p[p]), preferred_element_type=F32).astype(BF16))

        rb = pl.multiple_of(p * TL, TL)
        dep, obs = None, []
        for k in range(TL // LAR):
            ob, dep = local_attn(rb + k * LAR, z, dep)
            obs.append(ob)
        ob = jnp.concatenate(obs, axis=0).astype(BF16)
        wop = jnp.concatenate([f(bwo_p[dp]) for dp in range(DH // 2) for f in (_lo, _hi)], axis=0).astype(BF16)
        acc_v[pl.ds(rb, TL), :] = acc_v[pl.ds(rb, TL), :] + jnp.dot(ob, wop, preferred_element_type=F32)

        wq = _split_pair(wq_p[p])
        row = lax.broadcasted_iota(jnp.int32, (TQ, TQ), 0)
        col = lax.broadcasted_iota(jnp.int32, (TQ, TQ), 1)
        causal = col <= row

        def qproj(c):
            q = jnp.dot(_ld(x_v, c * TQP, TQP), wq, preferred_element_type=F32) * qscale
            _st(q_s, c * TQP, q.astype(BF16))

        def qk(i, hh):
            cs = slice(hh * D, (hh + 1) * D)
            return lax.dot_general(_ld(q_s, i * TQ, TQ, cs), _ld(k_s, 0, (i + 1) * TQ, cs), NT,
                                   preferred_element_type=F32)

        ldep = [None]

        def softmax_pv(i, hh, s):
            cs = slice(hh * D, (hh + 1) * D)
            r0 = i * TQ
            sd = jnp.where(causal, s[:, r0:], NEG)
            s = jnp.concatenate([s[:, :r0], sd], axis=1) if i > 0 else sd
            if MAXG and i > 1:
                m = jnp.max(_chain_reduce(s, jnp.maximum, MAXG, z, None)[0], axis=1, keepdims=True)
            else:
                m = jnp.max(s, axis=1, keepdims=True)
            e = jnp.exp2(s - m)
            if SUMG and i > 1:
                lp, ldep[0] = _chain_reduce(e, jnp.add, SUMG, z, ldep[0] if hh == 1 else None)
                l = jnp.sum(lp, axis=1, keepdims=True)
            else:
                l = jnp.sum(e, axis=1, keepdims=True)
            o = jnp.dot(e.astype(BF16), _ld(v_s, 0, r0 + TQ, cs), preferred_element_type=F32)
            return o * (g_v[r0:r0 + TQ, :] * _recip(l))

        def oproj(i, o0, o1):
            r0 = i * TQ
            y = acc_v[r0:r0 + TQ, :] + jnp.dot(jnp.concatenate([o0, o1], axis=1).astype(BF16),
                                               _ld(wo_v, p * (2 * D), 2 * D), preferred_element_type=F32)
            acc_v[r0:r0 + TQ, :] = y
            o_st[r0:r0 + TQ, :] = y.astype(BF16)
            if r0 < TO:
                pl.when(p == HP - 1)(cp_o(r0, TQ).start)
            elif r0 % TO == 0:
                pl.when(p == HP - 1)(cp_o(r0, TO).start)

        items = [(i, hh) for i in reversed(range(S // TQ)) for hh in range(2)]
        per_chunk = 2 * (TQP // TQ)
        n_qc = S // TQP
        n = len(items)
        s_vals, o_vals = {}, {}
        qproj(n_qc - 1)
        for step in range(n + LOOK + OLAG):
            if step % per_chunk == 0 and n_qc - 2 - step // per_chunk >= 0:
                qproj(n_qc - 2 - step // per_chunk)
            if step < n:
                s_vals[step] = qk(*items[step])
            b = step - LOOK
            if 0 <= b < n:
                o_vals[b] = softmax_pv(*items[b], s_vals.pop(b))
            c = step - LOOK - OLAG
            if 0 <= c < n and c % 2 == 1:
                oproj(items[c][0], o_vals.pop(c - 1), o_vals.pop(c))
        return 0

    lax.fori_loop(0, HP, _scoped("pair", pair_body), 0)
    cp_o(0, S).wait()


@jax.jit
def pallas_gated_mix__compressed_kv_cla__sliding_local_dilated__prompt_kernel(
    A_x, A_c_kv, A_w_q, A_w_uk, A_w_uv, A_w_o, B_x, B_wqkv, B_wo, gate_w,
):
    del B_x
    x = A_x.reshape(S, M)
    ckv = A_c_kv.reshape(S, DC)
    wo = A_w_o.reshape(H * D, M)
    bwo = B_wo.reshape(H, DH, M)
    any_spec = pl.BlockSpec(memory_space=pl.ANY)
    out = pl.pallas_call(
        _kernel,
        out_shape=jax.ShapeDtypeStruct((S, M), BF16),
        in_specs=[any_spec] * 8 + [pl.BlockSpec(memory_space=pltpu.VMEM)],
        out_specs=any_spec,
        scratch_shapes=[
            pltpu.VMEM((S // 2, M), U32),
            pltpu.VMEM((S // 2, DC), U32),
            pltpu.VMEM((HP, M, D), U32),
            pltpu.VMEM((HP, DC, D), U32),
            pltpu.VMEM((HP, DC, D), U32),
            pltpu.VMEM((H * D // 2, M), U32),
            pltpu.VMEM((M, 3 * M), BF16),
            pltpu.VMEM((DH // 2, H, M), U32),
            pltpu.VMEM((M // 2, M), U32),
            pltpu.VMEM((M // 2, M), U32),
            pltpu.VMEM((4, H * PITCH, 128), F32),
            pltpu.VMEM((3, NT_M, S + PAD, 128), F32),
            pltpu.VMEM((S, M), F32),
            pltpu.VMEM((S, 128), F32),
            pltpu.VMEM((8, 128), U32),
            pltpu.VMEM((S // 2, 2 * D), U32),
            pltpu.VMEM((S // 2, 2 * D), U32),
            pltpu.VMEM((S // 2, 2 * D), U32),
            pltpu.VMEM((S, M), BF16),
            pltpu.SemaphoreType.DMA((NC + 1,)),
            pltpu.SemaphoreType.DMA((12,)),
            pltpu.SemaphoreType.DMA(()),
            pltpu.SemaphoreType.DMA(()),
        ],
        compiler_params=pltpu.CompilerParams(vmem_limit_bytes=110 * 1024 * 1024),
    )(x, ckv, A_w_q, A_w_uk, A_w_uv, wo, B_wqkv, bwo, gate_w)
    return out.reshape(1, S, M)
```

```python
import contextlib
import functools

import jax
import jax.numpy as jnp
from jax import lax
import jax.experimental.pallas as pl
import jax.experimental.pallas.tpu as pltpu

S = 2048
M = 1024
DC = 512
H = 32
HP = H // 2
D = 128
DH = 32
W = 8
DIL = 2
PAD = 16
NT_M = M // 128
TQ = 128
TQP = 128
TC = 512
NC = S // TC
KB = 256
NK = M // KB
R1 = 640
TL = S // HP
TO = 128
GR = 192
PITCH = 40
LOOK = 2
OLAG = 6
SUMG = 32
MAXG = 0
LAP = 2
LAR = 8
LOG2E = 1.4426950408889634
NEG = -1e9

F32 = jnp.float32
BF16 = jnp.bfloat16
U32 = jnp.uint32
NT = (((1,), (1,)), ((), ()))


_PROFILE = False


def _scope(name):
    return jax.named_scope(name) if _PROFILE else contextlib.nullcontext()


def _scoped(name, body):
    def f(i, c):
        with _scope(name):
            return body(i, c)
    return f


def _recip(l):
    r = pl.reciprocal(l, approx=True)
    return r * (2.0 - l * r)


def _lo(w):
    return pltpu.bitcast(w << 16, F32)


def _hi(w):
    return pltpu.bitcast(w & jnp.uint32(0xFFFF0000), F32)


def _split_pair(w):
    return jnp.concatenate([_lo(w), _hi(w)], axis=1).astype(BF16)


def _ld(ref, r0, n, cols=slice(None)):
    if isinstance(r0, int):
        rs = slice(r0 // 2, (r0 + n) // 2)
    else:
        rs = pl.ds(pl.multiple_of(lax.shift_right_logical(r0, 1), 8), n // 2)
    return pltpu.bitcast(ref[rs, cols], BF16)


def _st(ref, r0, val, cols=slice(None)):
    ref[r0 // 2:(r0 + val.shape[0]) // 2, cols] = pltpu.bitcast(val, U32)


def _zero_after(z, *vals):
    acc = None
    for v in vals:
        b = pltpu.bitcast(v, U32)
        for r in range(0, b.shape[0], 8):
            for c in range(0, b.shape[1], 128):
                t = b[r:r + 8, c:c + 128]
                acc = t if acc is None else acc | t
    return acc & z


def _chain_reduce(x, op, g, z, dep):
    parts = []
    for r in range(0, x.shape[0], g):
        a = x[r:r + g, 0:128]
        if dep is not None:
            a = pltpu.bitcast(pltpu.bitcast(a, U32) | jnp.concatenate([dep] * (g // 8), axis=0), F32)
        for c in range(128, x.shape[1], 128):
            a = op(a, x[r:r + g, c:c + 128])
        dep = _zero_after(z, a)
        parts.append(a)
    return jnp.concatenate(parts, axis=0), dep


def _kernel(x_hbm, ckv_hbm, wq_hbm, wuk_hbm, wuv_hbm, wo_hbm, bqkv_hbm, bwo_hbm, gate_hbm,
            out_hbm,
            x_v, ckv_v, wq_p, wuk_p, wuv_p, wo_v, bqkv_v, bwo_p, wcur_v, wnxt_v, tmp_v,
            qkv_v, acc_v, g_v, z_v, q_s, k_s, v_s, o_st, gate_v,
            sem_x, sem_w, sem_a, sem_o):
    x_parts = [(0, R1, 0), (R1, S, 0), (0, S, 1), (0, TC, 2), (0, TC, 3), (TC, S, 2), (TC, S, 3)]

    def cp_x(i):
        r0, r1, k = x_parts[i]
        rs = pl.ds(r0 // 2, (r1 - r0) // 2)
        return pltpu.make_async_copy(x_hbm.bitcast(U32).at[rs, pl.ds(k * KB, KB)], x_v.at[k, rs], sem_x.at[i])

    def cp_w(u):
        u_lo, u_hi = (u % NK, u // NK) if isinstance(u, int) else (u & 3, lax.shift_right_logical(u, 2))
        sl = (pl.ds(u_lo * KB, KB), pl.ds(u_hi * M, M))
        return pltpu.make_async_copy(bqkv_hbm.at[sl], bqkv_v.at[sl], sem_w.at[u])

    def cp_w0(j):
        sl = (pl.ds(j * 128, 128), pl.ds(0, M))
        return pltpu.make_async_copy(bqkv_hbm.at[sl], bqkv_v.at[sl], sem_w.at[j * 3 * NK])

    cp_g = pltpu.make_async_copy(gate_hbm, gate_v, sem_x.at[len(x_parts)])

    a_copies = [pltpu.make_async_copy(ckv_hbm.bitcast(U32), ckv_v, sem_a),
                pltpu.make_async_copy(wo_hbm.bitcast(U32), wo_v, sem_a)]
    for src, dst in ((wuk_hbm, wuk_p), (wuv_hbm, wuv_p), (wq_hbm, wq_p), (bwo_hbm, bwo_p)):
        src_u = src.bitcast(U32)
        a_copies += [pltpu.make_async_copy(src_u.at[:, p, :], dst.at[p], sem_a) for p in range(HP)]
    a_waits = [pltpu.make_async_copy(b, b, sem_a) for b in (ckv_v, wo_v, wuk_p, wuv_p, wq_p, bwo_p)]

    def cp_o(r0, n):
        sl = (pl.ds(r0, n), slice(None))
        return pltpu.make_async_copy(o_st.at[sl], out_hbm.at[sl], sem_o)

    for cc in (cp_w0(0), cp_w0(1), cp_x(0), cp_x(1), cp_w(1), cp_g):
        cc.start()
    z_v[...] = jnp.zeros((8, 128), U32)
    for part in range(3):
        for t in range(NT_M):
            qkv_v[part, t, 0:PAD, :] = jnp.zeros((PAD, 128), F32)

    def prep_t(part, units, z, dep=None):
        p0 = part * M if isinstance(part, int) else pl.multiple_of(part * M, M)
        deps = [dep] * len(units)
        for c in range(NT_M):
            for u, (j, buf) in enumerate(units):
                k0 = j * 128 if isinstance(j, int) else pl.multiple_of(j * 128, 128)
                src = bqkv_v[pl.ds(k0, 128), pl.ds(p0 + c * 128, 128)]
                if deps[u] is not None:
                    top = pltpu.bitcast(pltpu.bitcast(src[:16], U32) | deps[u], BF16)
                    src = jnp.concatenate([top, src[16:]], axis=0)
                t = src.T.astype(F32)
                for hh in range(4):
                    h = 4 * c + hh
                    tmp_v[buf, h * PITCH: h * PITCH + DH, :] = t[hh * DH:(hh + 1) * DH, :]
                if z is not None:
                    deps[u] = _zero_after(z, t[120:128])

    def prep_p(dst, j, buf, z):
        k0 = j * 128 if isinstance(j, int) else pl.multiple_of(j * 128, 128)
        outs = []
        for d in range(DH):
            o = tmp_v[buf, pl.ds(d, H, stride=PITCH), :].astype(BF16)
            _st(dst, d * H, o, pl.ds(k0, 128))
            outs.append(o)
        return None if z is None else _zero_after(z, *outs)

    def prep_next(u, z):
        part, kq = (u // NK, u % NK) if isinstance(u, int) else (lax.shift_right_logical(u, 2), u & 3)
        prep_t(part, [(2 * kq, 0)], z)
        dep = prep_p(wnxt_v, 0, 0, z)
        prep_t(part, [(2 * kq + 1, 1)], z, dep)
        return prep_p(wnxt_v, 1, 1, z)

    def gate_rows(t, z, dep):
        gw = gate_v[...].astype(F32).reshape(1, M)
        g0 = jnp.minimum((t - 1) * GR, S - GR)
        for k in range(GR // 16):
            rr = pl.multiple_of(g0 + k * 16, 16)
            rw = pl.multiple_of(lax.shift_right_logical(rr, 1), 8)
            xb = jnp.concatenate([x_v[q, pl.ds(rw, 8), :] for q in range(NK)], axis=1)
            xb = xb | jnp.concatenate([dep] * NT_M, axis=1)
            xx = pltpu.bitcast(xb, BF16).astype(F32)
            zz = jnp.sum(xx * gw, axis=1, keepdims=True)
            g = jnp.broadcast_to(1.0 / (1.0 + jnp.exp(-zz)), (16, 128))
            g_v[pl.ds(rr, 16), :] = g
            acc_v[pl.ds(rr, 16), :] = jnp.zeros((16, M), F32)
            dep = _zero_after(z, g)

    def prep0_body(j, _):
        cp_w0(j).wait()
        prep_t(0, [(j, 0)], None)
        prep_p(wcur_v, j, 0, None)
        return 0

    lax.fori_loop(0, 2, _scoped("prep0", prep0_body), 0)

    def first(r0, r1):
        y = lax.dot_general(_ld(x_v.at[0], r0, r1 - r0), _ld(wcur_v, 0, M), NT, preferred_element_type=F32)
        for tt in range(NT_M):
            qkv_v[0, tt, PAD + r0:PAD + r1, :] = y[:, tt * 128:(tt + 1) * 128]

    with _scope("b1"):
        cp_x(0).wait()
        for cc in (cp_x(2), cp_w(2), cp_x(3), cp_x(4)):
            cc.start()
        first(0, R1)
    with _scope("b2"):
        cp_x(1).wait()
        cp_w(1).wait()
        cp_x(5).start()
        cp_x(6).start()
        for u in range(3, 3 * NK):
            cp_w(u).start()
        cuts = [R1] + [c for c in range(TC, S + 1, TC) if c > R1 + 128]
        for r0, r1 in zip(cuts[:-1], cuts[1:]):
            first(r0, r1)
        prep_next(1, z_v[...])
        wcur_v[...] = wnxt_v[...]
        for cc in a_copies[2:] + a_copies[:2]:
            cc.start()
    cp_x(2).wait()
    cp_x(3).wait()
    cp_x(4).wait()
    cp_g.wait()

    def bproj_body(t, _):
        part = lax.shift_right_logical(t, 2)
        kq = t & 3

        @pl.when(t < 3 * NK - 1)
        def _():
            cp_w(t + 1).wait()

        @pl.when(t == 2)
        def _():
            cp_x(5).wait()
            cp_x(6).wait()

        w = _ld(wcur_v, 0, M)
        for c in range(NC):
            y = lax.dot_general(_ld(x_v.at[kq], c * TC, TC), w, NT, preferred_element_type=F32)
            rs = slice(PAD + c * TC, PAD + (c + 1) * TC)
            for tt in range(NT_M):
                yt = y[:, tt * 128:(tt + 1) * 128]
                qkv_v[part, tt, rs, :] = jnp.where(kq == 0, yt, qkv_v[part, tt, rs, :] + yt)
        z = z_v[...]
        dep = prep_next(jnp.minimum(t + 1, 3 * NK - 1), z)
        gate_rows(t, z, dep)
        wcur_v[...] = wnxt_v[...]
        return 0

    lax.fori_loop(1, 3 * NK, _scoped("bproj", bproj_body), 0)
    for c in a_waits:
        c.wait()

    qscale = (D ** -0.5) * LOG2E
    bscale = (DH ** -0.5) * LOG2E

    def local_attn(r, z, dep):
        def zf(*vals):
            return jnp.concatenate([pltpu.bitcast(_zero_after(z, *vals), F32)] * (LAR // 8), axis=0)

        sc = jnp.full((LAR, 128), bscale, F32)
        if dep is not None:
            sc = sc + dep
        q = [qkv_v[0, t, pl.ds(PAD + r, LAR), :] * sc for t in range(NT_M)]
        rowi = r + lax.broadcasted_iota(jnp.int32, (LAR, 128), 0)
        logits, raw = [], []
        for w in range(W):
            a = None if w < LAP else zf(raw[w - LAP])
            for t in range(NT_M):
                pr = q[t] * qkv_v[1, t, pl.ds(PAD + r - DIL * w, LAR), :]
                a = pr if a is None else a + pr
            raw.append(a)
            a = a + pltpu.roll(a, 64, 1)
            a = a + pltpu.roll(a, 32, 1)
            logits.append(jnp.where(rowi >= DIL * w, a, NEG) if w > 0 else a)
        m = functools.reduce(jnp.maximum, logits)
        es = [jnp.exp2(lg - m) for lg in logits]
        l = functools.reduce(lambda a, b: a + b, es)
        f = (1.0 - g_v[pl.ds(r, LAR), :]) * _recip(l)
        es = [e * f for e in es]
        outs = []
        for t in range(NT_M):
            a = None if t < LAP else zf(outs[t - LAP])
            for w in range(W):
                pr = es[w] * qkv_v[2, t, pl.ds(PAD + r - DIL * w, LAR), :]
                a = pr if a is None else a + pr
            outs.append(a)
        return jnp.concatenate(outs, axis=1), zf(*outs[NT_M - LAP:])

    def pair_body(p, _):
        z = z_v[...]
        ckv = _ld(ckv_v, 0, S)
        _st(k_s, 0, jnp.dot(ckv, _split_pair(wuk_p[p]), preferred_element_type=F32).astype(BF16))
        _st(v_s, 0, jnp.dot(ckv, _split_pair(wuv_p[p]), preferred_element_type=F32).astype(BF16))

        rb = pl.multiple_of(p * TL, TL)
        dep, obs = None, []
        for k in range(TL // LAR):
            ob, dep = local_attn(rb + k * LAR, z, dep)
            obs.append(ob)
        ob = jnp.concatenate(obs, axis=0).astype(BF16)
        wop = jnp.concatenate([f(bwo_p[dp]) for dp in range(DH // 2) for f in (_lo, _hi)], axis=0).astype(BF16)
        acc_v[pl.ds(rb, TL), :] = acc_v[pl.ds(rb, TL), :] + jnp.dot(ob, wop, preferred_element_type=F32)

        wq = _split_pair(wq_p[p])
        row = lax.broadcasted_iota(jnp.int32, (TQ, TQ), 0)
        col = lax.broadcasted_iota(jnp.int32, (TQ, TQ), 1)
        causal = col <= row

        def qproj(c):
            xc = jnp.concatenate([_ld(x_v.at[k], c * TQP, TQP) for k in range(NK)], axis=1)
            q = jnp.dot(xc, wq, preferred_element_type=F32) * qscale
            _st(q_s, c * TQP, q.astype(BF16))

        def qk(i, hh):
            cs = slice(hh * D, (hh + 1) * D)
            return lax.dot_general(_ld(q_s, i * TQ, TQ, cs), _ld(k_s, 0, (i + 1) * TQ, cs), NT,
                                   preferred_element_type=F32)

        ldep = [None]

        def softmax_pv(i, hh, s):
            cs = slice(hh * D, (hh + 1) * D)
            r0 = i * TQ
            sd = jnp.where(causal, s[:, r0:], NEG)
            s = jnp.concatenate([s[:, :r0], sd], axis=1) if i > 0 else sd
            if MAXG and i > 1:
                m = jnp.max(_chain_reduce(s, jnp.maximum, MAXG, z, None)[0], axis=1, keepdims=True)
            else:
                m = jnp.max(s, axis=1, keepdims=True)
            e = jnp.exp2(s - m)
            if SUMG and i > 1:
                lp, ldep[0] = _chain_reduce(e, jnp.add, SUMG, z, ldep[0] if hh == 1 else None)
                l = jnp.sum(lp, axis=1, keepdims=True)
            else:
                l = jnp.sum(e, axis=1, keepdims=True)
            o = jnp.dot(e.astype(BF16), _ld(v_s, 0, r0 + TQ, cs), preferred_element_type=F32)
            return o * (g_v[r0:r0 + TQ, :] * _recip(l))

        def oproj(i, o0, o1):
            r0 = i * TQ
            y = acc_v[r0:r0 + TQ, :] + jnp.dot(jnp.concatenate([o0, o1], axis=1).astype(BF16),
                                               _ld(wo_v, p * (2 * D), 2 * D), preferred_element_type=F32)
            acc_v[r0:r0 + TQ, :] = y
            o_st[r0:r0 + TQ, :] = y.astype(BF16)
            if r0 < TO:
                pl.when(p == HP - 1)(cp_o(r0, TQ).start)
            elif r0 % TO == 0:
                pl.when(p == HP - 1)(cp_o(r0, TO).start)

        items = [(i, hh) for i in reversed(range(S // TQ)) for hh in range(2)]
        per_chunk = 2 * (TQP // TQ)
        n_qc = S // TQP
        n = len(items)
        s_vals, o_vals = {}, {}
        qproj(n_qc - 1)
        for step in range(n + LOOK + OLAG):
            if step % per_chunk == 0 and n_qc - 2 - step // per_chunk >= 0:
                qproj(n_qc - 2 - step // per_chunk)
            if step < n:
                s_vals[step] = qk(*items[step])
            b = step - LOOK
            if 0 <= b < n:
                o_vals[b] = softmax_pv(*items[b], s_vals.pop(b))
            c = step - LOOK - OLAG
            if 0 <= c < n and c % 2 == 1:
                oproj(items[c][0], o_vals.pop(c - 1), o_vals.pop(c))
        return 0

    lax.fori_loop(0, HP, _scoped("pair", pair_body), 0)
    cp_o(0, S).wait()


@jax.jit
def pallas_gated_mix__compressed_kv_cla__sliding_local_dilated__prompt_kernel(
    A_x, A_c_kv, A_w_q, A_w_uk, A_w_uv, A_w_o, B_x, B_wqkv, B_wo, gate_w,
):
    del B_x
    x = A_x.reshape(S, M)
    ckv = A_c_kv.reshape(S, DC)
    wo = A_w_o.reshape(H * D, M)
    bwo = B_wo.reshape(H, DH, M)
    any_spec = pl.BlockSpec(memory_space=pl.ANY)
    out = pl.pallas_call(
        _kernel,
        out_shape=jax.ShapeDtypeStruct((S, M), BF16),
        in_specs=[any_spec] * 9,
        out_specs=any_spec,
        scratch_shapes=[
            pltpu.VMEM((NK, S // 2, KB), U32),
            pltpu.VMEM((S // 2, DC), U32),
            pltpu.VMEM((HP, M, D), U32),
            pltpu.VMEM((HP, DC, D), U32),
            pltpu.VMEM((HP, DC, D), U32),
            pltpu.VMEM((H * D // 2, M), U32),
            pltpu.VMEM((M, 3 * M), BF16),
            pltpu.VMEM((DH // 2, H, M), U32),
            pltpu.VMEM((M // 2, KB), U32),
            pltpu.VMEM((M // 2, KB), U32),
            pltpu.VMEM((2, H * PITCH, 128), F32),
            pltpu.VMEM((3, NT_M, S + PAD, 128), F32),
            pltpu.VMEM((S, M), F32),
            pltpu.VMEM((S, 128), F32),
            pltpu.VMEM((8, 128), U32),
            pltpu.VMEM((S // 2, 2 * D), U32),
            pltpu.VMEM((S // 2, 2 * D), U32),
            pltpu.VMEM((S // 2, 2 * D), U32),
            pltpu.VMEM((S, M), BF16),
            pltpu.VMEM((M,), BF16),
            pltpu.SemaphoreType.DMA((8,)),
            pltpu.SemaphoreType.DMA((3 * NK + 1,)),
            pltpu.SemaphoreType.DMA(()),
            pltpu.SemaphoreType.DMA(()),
        ],
        compiler_params=pltpu.CompilerParams(vmem_limit_bytes=110 * 1024 * 1024),
    )(x, ckv, A_w_q, A_w_uk, A_w_uv, wo, B_wqkv, bwo, gate_w)
    return out.reshape(1, S, M)
```

```python
import contextlib
import functools

import jax
import jax.numpy as jnp
from jax import lax
import jax.experimental.pallas as pl
import jax.experimental.pallas.tpu as pltpu

S = 2048
M = 1024
DC = 512
H = 32
HP = H // 2
D = 128
DH = 32
W = 8
DIL = 2
PAD = 16
NT_M = M // 128
TQ = 128
TQP = 128
TC = 512
NC = S // TC
KB = 256
NK = M // KB
R1 = 1536
TL = S // HP
TO = 128
GR = 192
PITCH = 40
LOOK = 2
OLAG = 6
SUMG = 32
MAXG = 0
LAP = 2
LAR = 8
B1C = 0
LOG2E = 1.4426950408889634
NEG = -1e9

F32 = jnp.float32
BF16 = jnp.bfloat16
U32 = jnp.uint32
NT = (((1,), (1,)), ((), ()))


_PROFILE = False


def _scope(name):
    return jax.named_scope(name) if _PROFILE else contextlib.nullcontext()


def _scoped(name, body):
    def f(i, c):
        with _scope(name):
            return body(i, c)
    return f


def _recip(l):
    r = pl.reciprocal(l, approx=True)
    return r * (2.0 - l * r)


def _lo(w):
    return pltpu.bitcast(w << 16, F32)


def _hi(w):
    return pltpu.bitcast(w & jnp.uint32(0xFFFF0000), F32)


def _split_pair(w):
    return jnp.concatenate([_lo(w), _hi(w)], axis=1).astype(BF16)


def _ld(ref, r0, n, cols=slice(None)):
    if isinstance(r0, int):
        rs = slice(r0 // 2, (r0 + n) // 2)
    else:
        rs = pl.ds(pl.multiple_of(lax.shift_right_logical(r0, 1), 8), n // 2)
    return pltpu.bitcast(ref[rs, cols], BF16)


def _st(ref, r0, val, cols=slice(None)):
    ref[r0 // 2:(r0 + val.shape[0]) // 2, cols] = pltpu.bitcast(val, U32)


def _zero_after(z, *vals):
    acc = None
    for v in vals:
        b = pltpu.bitcast(v, U32)
        for r in range(0, b.shape[0], 8):
            for c in range(0, b.shape[1], 128):
                t = b[r:r + 8, c:c + 128]
                acc = t if acc is None else acc | t
    return acc & z


def _chain_reduce(x, op, g, z, dep):
    parts = []
    for r in range(0, x.shape[0], g):
        a = x[r:r + g, 0:128]
        if dep is not None:
            a = pltpu.bitcast(pltpu.bitcast(a, U32) | jnp.concatenate([dep] * (g // 8), axis=0), F32)
        for c in range(128, x.shape[1], 128):
            a = op(a, x[r:r + g, c:c + 128])
        dep = _zero_after(z, a)
        parts.append(a)
    return jnp.concatenate(parts, axis=0), dep


def _kernel(x_hbm, ckv_hbm, wq_hbm, wuk_hbm, wuv_hbm, wo_hbm, bqkv_hbm, bwo_hbm, gate_hbm,
            out_hbm,
            x_v, ckv_v, wq_p, wuk_p, wuv_p, wo_v, bqkv_v, bwo_p, wcur_v, wnxt_v, tmp_v,
            qkv_v, acc_v, g_v, z_v, q_s, k_s, v_s, o_st, gate_v,
            sem_x, sem_w, sem_a, sem_o):
    x_parts = [(0, R1, 0, 0, 128), (R1, S, 0, 0, 128), (0, S, 1, 0, KB), (0, TC, 2, 0, KB), (0, TC, 3, 0, KB),
               (TC, S, 2, 0, KB), (TC, S, 3, 0, KB), (0, S, 0, 128, 128)]

    def cp_x(i):
        r0, r1, k, c0, n = x_parts[i]
        rs = pl.ds(r0 // 2, (r1 - r0) // 2)
        return pltpu.make_async_copy(x_hbm.bitcast(U32).at[rs, pl.ds(k * KB + c0, n)], x_v.at[k, rs, pl.ds(c0, n)],
                                     sem_x.at[i])

    def cp_w(u):
        u_lo, u_hi = (u % NK, u // NK) if isinstance(u, int) else (u & 3, lax.shift_right_logical(u, 2))
        sl = (pl.ds(u_lo * KB, KB), pl.ds(u_hi * M, M))
        return pltpu.make_async_copy(bqkv_hbm.at[sl], bqkv_v.at[sl], sem_w.at[u])

    def cp_w0(j):
        sl = (pl.ds(j * 128, 128), pl.ds(0, M))
        return pltpu.make_async_copy(bqkv_hbm.at[sl], bqkv_v.at[sl], sem_w.at[j * 3 * NK])

    cp_g = pltpu.make_async_copy(gate_hbm, gate_v, sem_x.at[len(x_parts)])

    a_copies = [pltpu.make_async_copy(ckv_hbm.bitcast(U32), ckv_v, sem_a),
                pltpu.make_async_copy(wo_hbm.bitcast(U32), wo_v, sem_a)]
    for src, dst in ((wuk_hbm, wuk_p), (wuv_hbm, wuv_p), (wq_hbm, wq_p), (bwo_hbm, bwo_p)):
        src_u = src.bitcast(U32)
        a_copies += [pltpu.make_async_copy(src_u.at[:, p, :], dst.at[p], sem_a) for p in range(HP)]
    a_waits = [pltpu.make_async_copy(b, b, sem_a) for b in (ckv_v, wo_v, wuk_p, wuv_p, wq_p, bwo_p)]

    def cp_o(r0, n):
        sl = (pl.ds(r0, n), slice(None))
        return pltpu.make_async_copy(o_st.at[sl], out_hbm.at[sl], sem_o)

    for cc in (cp_w0(0), cp_x(0), cp_w0(1)):
        cc.start()
    z_v[...] = jnp.zeros((8, 128), U32)
    for part in range(3):
        for t in range(NT_M):
            qkv_v[part, t, 0:PAD, :] = jnp.zeros((PAD, 128), F32)

    def prep_t(part, units, z, dep=None):
        p0 = part * M if isinstance(part, int) else pl.multiple_of(part * M, M)
        deps = [dep] * len(units)
        for c in range(NT_M):
            for u, (j, buf) in enumerate(units):
                k0 = j * 128 if isinstance(j, int) else pl.multiple_of(j * 128, 128)
                src = bqkv_v[pl.ds(k0, 128), pl.ds(p0 + c * 128, 128)]
                if deps[u] is not None:
                    top = pltpu.bitcast(pltpu.bitcast(src[:16], U32) | deps[u], BF16)
                    src = jnp.concatenate([top, src[16:]], axis=0)
                t = src.T.astype(F32)
                for hh in range(4):
                    h = 4 * c + hh
                    tmp_v[buf, h * PITCH: h * PITCH + DH, :] = t[hh * DH:(hh + 1) * DH, :]
                if z is not None:
                    deps[u] = _zero_after(z, t[120:128])

    def prep_p(dst, j, buf, z):
        k0 = j * 128 if isinstance(j, int) else pl.multiple_of(j * 128, 128)
        outs = []
        for d in range(DH):
            o = tmp_v[buf, pl.ds(d, H, stride=PITCH), :].astype(BF16)
            _st(dst, d * H, o, pl.ds(k0, 128))
            outs.append(o)
        return None if z is None else _zero_after(z, *outs)

    def prep_next(u, z):
        part, kq = (u // NK, u % NK) if isinstance(u, int) else (lax.shift_right_logical(u, 2), u & 3)
        prep_t(part, [(2 * kq, 0)], z)
        dep = prep_p(wnxt_v, 0, 0, z)
        prep_t(part, [(2 * kq + 1, 1)], z, dep)
        return prep_p(wnxt_v, 1, 1, z)

    def gate_rows(t, z, dep):
        gw = gate_v[...].astype(F32).reshape(1, M)
        g0 = jnp.minimum((t - 1) * GR, S - GR)
        for k in range(GR // 16):
            rr = pl.multiple_of(g0 + k * 16, 16)
            rw = pl.multiple_of(lax.shift_right_logical(rr, 1), 8)
            xb = jnp.concatenate([x_v[q, pl.ds(rw, 8), :] for q in range(NK)], axis=1)
            xb = xb | jnp.concatenate([dep] * NT_M, axis=1)
            xx = pltpu.bitcast(xb, BF16).astype(F32)
            zz = jnp.sum(xx * gw, axis=1, keepdims=True)
            g = jnp.broadcast_to(1.0 / (1.0 + jnp.exp(-zz)), (16, 128))
            g_v[pl.ds(rr, 16), :] = g
            acc_v[pl.ds(rr, 16), :] = jnp.zeros((16, M), F32)
            dep = _zero_after(z, g)

    with _scope("prep0"):
        cp_w0(0).wait()
        for cc in (cp_x(1), cp_x(7), cp_w(1), cp_g):
            cc.start()
        prep_t(0, [(0, 0)], None)
        prep_p(wcur_v, 0, 0, None)

    def first(j, r0, r1):
        ks = slice(j * 128, (j + 1) * 128)
        y = lax.dot_general(_ld(x_v.at[0], r0, r1 - r0, ks), _ld(wcur_v, 0, M, ks), NT, preferred_element_type=F32)
        for tt in range(NT_M):
            yt = y[:, tt * 128:(tt + 1) * 128]
            qkv_v[0, tt, PAD + r0:PAD + r1, :] = yt if j == 0 else qkv_v[0, tt, PAD + r0:PAD + r1, :] + yt

    with _scope("wx0"):
        cp_x(0).wait()
    with _scope("b1"):
        for cc in (cp_x(2), cp_w(2), cp_x(3), cp_x(4)):
            cc.start()
        first(0, 0, R1)
    with _scope("w2"):
        for cc in (cp_w0(1), cp_x(1), cp_x(7), cp_w(1)):
            cc.wait()
    with _scope("b2"):
        cp_x(5).start()
        cp_x(6).start()
        for u in range(3, 3 * NK):
            cp_w(u).start()
        first(0, R1, S)
        prep_t(0, [(1, 1)], None)
        prep_p(wcur_v, 1, 1, None)
        first(1, 0, S)
        prep_next(1, z_v[...])
        wcur_v[...] = wnxt_v[...]
        for cc in a_copies[2:] + a_copies[:2]:
            cc.start()
    cp_x(2).wait()
    cp_x(3).wait()
    cp_x(4).wait()
    cp_g.wait()

    def bproj_body(t, _):
        part = lax.shift_right_logical(t, 2)
        kq = t & 3

        @pl.when(t < 3 * NK - 1)
        def _():
            cp_w(t + 1).wait()

        @pl.when(t == 2)
        def _():
            cp_x(5).wait()
            cp_x(6).wait()

        w = _ld(wcur_v, 0, M)
        for c in range(NC):
            y = lax.dot_general(_ld(x_v.at[kq], c * TC, TC), w, NT, preferred_element_type=F32)
            rs = slice(PAD + c * TC, PAD + (c + 1) * TC)
            for tt in range(NT_M):
                yt = y[:, tt * 128:(tt + 1) * 128]
                qkv_v[part, tt, rs, :] = jnp.where(kq == 0, yt, qkv_v[part, tt, rs, :] + yt)
        z = z_v[...]
        dep = prep_next(jnp.minimum(t + 1, 3 * NK - 1), z)
        gate_rows(t, z, dep)
        wcur_v[...] = wnxt_v[...]
        return 0

    lax.fori_loop(1, 3 * NK, _scoped("bproj", bproj_body), 0)
    for c in a_waits:
        c.wait()

    qscale = (D ** -0.5) * LOG2E
    bscale = (DH ** -0.5) * LOG2E

    def local_attn(r, z, dep):
        def zf(*vals):
            return jnp.concatenate([pltpu.bitcast(_zero_after(z, *vals), F32)] * (LAR // 8), axis=0)

        sc = jnp.full((LAR, 128), bscale, F32)
        if dep is not None:
            sc = sc + dep
        q = [qkv_v[0, t, pl.ds(PAD + r, LAR), :] * sc for t in range(NT_M)]
        rowi = r + lax.broadcasted_iota(jnp.int32, (LAR, 128), 0)
        logits, raw = [], []
        for w in range(W):
            a = None if w < LAP else zf(raw[w - LAP])
            for t in range(NT_M):
                pr = q[t] * qkv_v[1, t, pl.ds(PAD + r - DIL * w, LAR), :]
                a = pr if a is None else a + pr
            raw.append(a)
            a = a + pltpu.roll(a, 64, 1)
            a = a + pltpu.roll(a, 32, 1)
            logits.append(jnp.where(rowi >= DIL * w, a, NEG) if w > 0 else a)
        m = functools.reduce(jnp.maximum, logits)
        es = [jnp.exp2(lg - m) for lg in logits]
        l = functools.reduce(lambda a, b: a + b, es)
        f = (1.0 - g_v[pl.ds(r, LAR), :]) * _recip(l)
        es = [e * f for e in es]
        outs = []
        for t in range(NT_M):
            a = None if t < LAP else zf(outs[t - LAP])
            for w in range(W):
                pr = es[w] * qkv_v[2, t, pl.ds(PAD + r - DIL * w, LAR), :]
                a = pr if a is None else a + pr
            outs.append(a)
        return jnp.concatenate(outs, axis=1), zf(*outs[NT_M - LAP:])

    def pair_body(p, _):
        z = z_v[...]
        ckv = _ld(ckv_v, 0, S)
        _st(k_s, 0, jnp.dot(ckv, _split_pair(wuk_p[p]), preferred_element_type=F32).astype(BF16))
        _st(v_s, 0, jnp.dot(ckv, _split_pair(wuv_p[p]), preferred_element_type=F32).astype(BF16))

        rb = pl.multiple_of(p * TL, TL)
        dep, obs = None, []
        for k in range(TL // LAR):
            ob, dep = local_attn(rb + k * LAR, z, dep)
            obs.append(ob)
        ob = jnp.concatenate(obs, axis=0).astype(BF16)
        wop = jnp.concatenate([f(bwo_p[dp]) for dp in range(DH // 2) for f in (_lo, _hi)], axis=0).astype(BF16)
        acc_v[pl.ds(rb, TL), :] = acc_v[pl.ds(rb, TL), :] + jnp.dot(ob, wop, preferred_element_type=F32)

        wq = _split_pair(wq_p[p])
        row = lax.broadcasted_iota(jnp.int32, (TQ, TQ), 0)
        col = lax.broadcasted_iota(jnp.int32, (TQ, TQ), 1)
        causal = col <= row

        def qproj(c):
            xc = jnp.concatenate([_ld(x_v.at[k], c * TQP, TQP) for k in range(NK)], axis=1)
            q = jnp.dot(xc, wq, preferred_element_type=F32) * qscale
            _st(q_s, c * TQP, q.astype(BF16))

        def qk(i, hh):
            cs = slice(hh * D, (hh + 1) * D)
            return lax.dot_general(_ld(q_s, i * TQ, TQ, cs), _ld(k_s, 0, (i + 1) * TQ, cs), NT,
                                   preferred_element_type=F32)

        ldep = [None]

        def softmax_pv(i, hh, s):
            cs = slice(hh * D, (hh + 1) * D)
            r0 = i * TQ
            sd = jnp.where(causal, s[:, r0:], NEG)
            s = jnp.concatenate([s[:, :r0], sd], axis=1) if i > 0 else sd
            if MAXG and i > 1:
                m = jnp.max(_chain_reduce(s, jnp.maximum, MAXG, z, None)[0], axis=1, keepdims=True)
            else:
                m = jnp.max(s, axis=1, keepdims=True)
            e = jnp.exp2(s - m)
            if SUMG and i > 1:
                lp, ldep[0] = _chain_reduce(e, jnp.add, SUMG, z, ldep[0] if hh == 1 else None)
                l = jnp.sum(lp, axis=1, keepdims=True)
            else:
                l = jnp.sum(e, axis=1, keepdims=True)
            o = jnp.dot(e.astype(BF16), _ld(v_s, 0, r0 + TQ, cs), preferred_element_type=F32)
            return o * (g_v[r0:r0 + TQ, :] * _recip(l))

        def oproj(i, o0, o1):
            r0 = i * TQ
            y = acc_v[r0:r0 + TQ, :] + jnp.dot(jnp.concatenate([o0, o1], axis=1).astype(BF16),
                                               _ld(wo_v, p * (2 * D), 2 * D), preferred_element_type=F32)
            acc_v[r0:r0 + TQ, :] = y
            o_st[r0:r0 + TQ, :] = y.astype(BF16)
            if r0 < TO:
                pl.when(p == HP - 1)(cp_o(r0, TQ).start)
            elif r0 % TO == 0:
                pl.when(p == HP - 1)(cp_o(r0, TO).start)

        items = [(i, hh) for i in reversed(range(S // TQ)) for hh in range(2)]
        per_chunk = 2 * (TQP // TQ)
        n_qc = S // TQP
        n = len(items)
        s_vals, o_vals = {}, {}
        qproj(n_qc - 1)
        for step in range(n + LOOK + OLAG):
            if step % per_chunk == 0 and n_qc - 2 - step // per_chunk >= 0:
                qproj(n_qc - 2 - step // per_chunk)
            if step < n:
                s_vals[step] = qk(*items[step])
            b = step - LOOK
            if 0 <= b < n:
                o_vals[b] = softmax_pv(*items[b], s_vals.pop(b))
            c = step - LOOK - OLAG
            if 0 <= c < n and c % 2 == 1:
                oproj(items[c][0], o_vals.pop(c - 1), o_vals.pop(c))
        return 0

    lax.fori_loop(0, HP, _scoped("pair", pair_body), 0)
    cp_o(0, S).wait()


@jax.jit
def pallas_gated_mix__compressed_kv_cla__sliding_local_dilated__prompt_kernel(
    A_x, A_c_kv, A_w_q, A_w_uk, A_w_uv, A_w_o, B_x, B_wqkv, B_wo, gate_w,
):
    del B_x
    x = A_x.reshape(S, M)
    ckv = A_c_kv.reshape(S, DC)
    wo = A_w_o.reshape(H * D, M)
    bwo = B_wo.reshape(H, DH, M)
    any_spec = pl.BlockSpec(memory_space=pl.ANY)
    out = pl.pallas_call(
        _kernel,
        out_shape=jax.ShapeDtypeStruct((S, M), BF16),
        in_specs=[any_spec] * 9,
        out_specs=any_spec,
        scratch_shapes=[
            pltpu.VMEM((NK, S // 2, KB), U32),
            pltpu.VMEM((S // 2, DC), U32),
            pltpu.VMEM((HP, M, D), U32),
            pltpu.VMEM((HP, DC, D), U32),
            pltpu.VMEM((HP, DC, D), U32),
            pltpu.VMEM((H * D // 2, M), U32),
            pltpu.VMEM((M, 3 * M), BF16),
            pltpu.VMEM((DH // 2, H, M), U32),
            pltpu.VMEM((M // 2, KB), U32),
            pltpu.VMEM((M // 2, KB), U32),
            pltpu.VMEM((2, H * PITCH, 128), F32),
            pltpu.VMEM((3, NT_M, S + PAD, 128), F32),
            pltpu.VMEM((S, M), F32),
            pltpu.VMEM((S, 128), F32),
            pltpu.VMEM((8, 128), U32),
            pltpu.VMEM((S // 2, 2 * D), U32),
            pltpu.VMEM((S // 2, 2 * D), U32),
            pltpu.VMEM((S // 2, 2 * D), U32),
            pltpu.VMEM((S, M), BF16),
            pltpu.VMEM((M,), BF16),
            pltpu.SemaphoreType.DMA((9,)),
            pltpu.SemaphoreType.DMA((3 * NK + 1,)),
            pltpu.SemaphoreType.DMA(()),
            pltpu.SemaphoreType.DMA(()),
        ],
        compiler_params=pltpu.CompilerParams(vmem_limit_bytes=110 * 1024 * 1024),
    )(x, ckv, A_w_q, A_w_uk, A_w_uv, wo, B_wqkv, bwo, gate_w)
    return out.reshape(1, S, M)
```

```python
import contextlib
import functools

import jax
import jax.numpy as jnp
from jax import lax
import jax.experimental.pallas as pl
import jax.experimental.pallas.tpu as pltpu

S = 2048
M = 1024
DC = 512
H = 32
HP = H // 2
D = 128
DH = 32
W = 8
DIL = 2
PAD = 16
NT_M = M // 128
TQ = 128
TQP = 128
TC = 512
NC = S // TC
KB = 256
NK = M // KB
R1 = 1536
TL = S // HP
OCUT = (0, 512, 768, M)
GR = 192
PITCH = 40
LOOK = 2
OLAG = 10
SUMG = 16
MAXG = 0
LAP = 1
LAR = 8
KVC = 2048
KVI = 0
BPOS = 99
SUMT = 2
QAH = 1
ORD = 0
SCH = 2
ROLL3 = 0
LAQ = 2
LFIRST = 1
KVM = 0
MSK = 0
DEPQ = 0
LOG2E = 1.4426950408889634
NEG = -1e9

F32 = jnp.float32
BF16 = jnp.bfloat16
U32 = jnp.uint32
NT = (((1,), (1,)), ((), ()))


_PROFILE = False


def _scope(name):
    return jax.named_scope(name) if _PROFILE else contextlib.nullcontext()


def _scoped(name, body):
    def f(i, c):
        with _scope(name):
            return body(i, c)
    return f


def _recip(l):
    r = pl.reciprocal(l, approx=True)
    return r * (2.0 - l * r)


def _lo(w):
    return pltpu.bitcast(w << 16, F32)


def _hi(w):
    return pltpu.bitcast(w & jnp.uint32(0xFFFF0000), F32)


def _split_pair(w):
    return jnp.concatenate([_lo(w), _hi(w)], axis=1).astype(BF16)


def _ld(ref, r0, n, cols=slice(None)):
    if isinstance(r0, int):
        rs = slice(r0 // 2, (r0 + n) // 2)
    else:
        rs = pl.ds(pl.multiple_of(lax.shift_right_logical(r0, 1), 8), n // 2)
    return pltpu.bitcast(ref[rs, cols], BF16)


def _st(ref, r0, val, cols=slice(None)):
    ref[r0 // 2:(r0 + val.shape[0]) // 2, cols] = pltpu.bitcast(val, U32)


def _zero_after(z, *vals):
    acc = None
    for v in vals:
        b = pltpu.bitcast(v, U32)
        for r in range(0, b.shape[0], 8):
            for c in range(0, b.shape[1], 128):
                t = b[r:r + 8, c:c + 128]
                acc = t if acc is None else acc | t
    return acc & z


def _chain_reduce(x, op, g, z, dep):
    parts = []
    for r in range(0, x.shape[0], g):
        a = x[r:r + g, 0:128]
        if dep is not None:
            a = pltpu.bitcast(pltpu.bitcast(a, U32) | jnp.concatenate([dep] * (g // 8), axis=0), F32)
        for c in range(128, x.shape[1], 128):
            a = op(a, x[r:r + g, c:c + 128])
        dep = _zero_after(z, a)
        parts.append(a)
    return jnp.concatenate(parts, axis=0), dep


def _body(x_hbm, ckv_hbm, wq_hbm, wuk_hbm, wuv_hbm, wo_hbm, bqkv_hbm, bwo_hbm, gate_hbm,
            out_hbm,
            x_v, ckv_v, wq_p, wuk_p, wuv_p, wo_v, bqkv_v, bwo_p, wcur_v, wnxt_v, tmp_v,
            qkv_v, acc_v, g_v, z_v, q_s, k_s, v_s, o_st, gate_v,
            sem_x, sem_w, sem_a, sem_o):
    x_parts = [(0, R1, 0, 0, 128), (R1, S, 0, 0, 128), (0, S, 1, 0, KB), (0, TC, 2, 0, KB), (0, TC, 3, 0, KB),
               (TC, S, 2, 0, KB), (TC, S, 3, 0, KB), (0, S, 0, 128, 128)]

    def cp_x(i):
        r0, r1, k, c0, n = x_parts[i]
        rs = pl.ds(r0 // 2, (r1 - r0) // 2)
        return pltpu.make_async_copy(x_hbm.bitcast(U32).at[rs, pl.ds(k * KB + c0, n)], x_v.at[k, rs, pl.ds(c0, n)],
                                     sem_x.at[i])

    def cp_w(u):
        u_lo, u_hi = (u % NK, u // NK) if isinstance(u, int) else (u & 3, lax.shift_right_logical(u, 2))
        sl = (pl.ds(u_lo * KB, KB), pl.ds(u_hi * M, M))
        return pltpu.make_async_copy(bqkv_hbm.at[sl], bqkv_v.at[sl], sem_w.at[u])

    def cp_w0(j):
        sl = (pl.ds(j * 128, 128), pl.ds(0, M))
        return pltpu.make_async_copy(bqkv_hbm.at[sl], bqkv_v.at[sl], sem_w.at[j * 3 * NK])

    cp_g = pltpu.make_async_copy(gate_hbm, gate_v, sem_x.at[len(x_parts)])

    a_copies = [pltpu.make_async_copy(ckv_hbm.bitcast(U32), ckv_v, sem_a),
                pltpu.make_async_copy(wo_hbm.bitcast(U32), wo_v, sem_a)]
    for src, dst in ((wuk_hbm, wuk_p), (wuv_hbm, wuv_p), (wq_hbm, wq_p), (bwo_hbm, bwo_p)):
        src_u = src.bitcast(U32)
        a_copies += [pltpu.make_async_copy(src_u.at[:, p, :], dst.at[p], sem_a) for p in range(HP)]
    a_waits = [pltpu.make_async_copy(b, b, sem_a) for b in (ckv_v, wo_v, wuk_p, wuv_p, wq_p, bwo_p)]

    def cp_o(r0, n, c0=0, c1=M):
        sl = (pl.ds(r0, n), pl.ds(c0, c1 - c0))
        return pltpu.make_async_copy(o_st.at[sl], out_hbm.at[sl], sem_o)

    for cc in (cp_w0(0), cp_x(0), cp_w0(1)):
        cc.start()
    z_v[...] = jnp.zeros((8, 128), U32)
    for part in range(3):
        for t in range(NT_M):
            qkv_v[part, t, 0:PAD, :] = jnp.zeros((PAD, 128), F32)

    def prep_t(part, units, z, dep=None):
        p0 = part * M if isinstance(part, int) else pl.multiple_of(part * M, M)
        deps = [dep] * len(units)
        for c in range(NT_M):
            for u, (j, buf) in enumerate(units):
                k0 = j * 128 if isinstance(j, int) else pl.multiple_of(j * 128, 128)
                src = bqkv_v[pl.ds(k0, 128), pl.ds(p0 + c * 128, 128)]
                if deps[u] is not None:
                    top = pltpu.bitcast(pltpu.bitcast(src[:16], U32) | deps[u], BF16)
                    src = jnp.concatenate([top, src[16:]], axis=0)
                t = src.T.astype(F32)
                for hh in range(4):
                    h = 4 * c + hh
                    tmp_v[buf, h * PITCH: h * PITCH + DH, :] = t[hh * DH:(hh + 1) * DH, :]
                if z is not None:
                    deps[u] = _zero_after(z, t[120:128])

    def prep_p(dst, j, buf, z):
        k0 = j * 128 if isinstance(j, int) else pl.multiple_of(j * 128, 128)
        outs = []
        for d in range(DH):
            o = tmp_v[buf, pl.ds(d, H, stride=PITCH), :].astype(BF16)
            _st(dst, d * H, o, pl.ds(k0, 128))
            outs.append(o)
        return None if z is None else _zero_after(z, *outs)

    def prep_next(u, z):
        part, kq = (u // NK, u % NK) if isinstance(u, int) else (lax.shift_right_logical(u, 2), u & 3)
        prep_t(part, [(2 * kq, 0)], z)
        dep = prep_p(wnxt_v, 0, 0, z)
        prep_t(part, [(2 * kq + 1, 1)], z, dep)
        return prep_p(wnxt_v, 1, 1, z)

    def gate_rows(t, z, dep):
        gw = gate_v[...].astype(F32).reshape(1, M)
        g0 = jnp.minimum((t - 1) * GR, S - GR)
        for k in range(GR // 16):
            rr = pl.multiple_of(g0 + k * 16, 16)
            rw = pl.multiple_of(lax.shift_right_logical(rr, 1), 8)
            xb = jnp.concatenate([x_v[q, pl.ds(rw, 8), :] for q in range(NK)], axis=1)
            xb = xb | jnp.concatenate([dep] * NT_M, axis=1)
            xx = pltpu.bitcast(xb, BF16).astype(F32)
            zz = jnp.sum(xx * gw, axis=1, keepdims=True)
            g = jnp.broadcast_to(1.0 / (1.0 + jnp.exp(-zz)), (16, 128))
            g_v[pl.ds(rr, 16), :] = g
            acc_v[pl.ds(rr, 16), :] = jnp.zeros((16, M), F32)
            dep = _zero_after(z, g)

    with _scope("prep0"):
        cp_w0(0).wait()
        for cc in (cp_x(1), cp_x(7), cp_w(1), cp_g):
            cc.start()
        prep_t(0, [(0, 0)], None)
        prep_p(wcur_v, 0, 0, None)

    def first(j, r0, r1):
        ks = slice(j * 128, (j + 1) * 128)
        y = lax.dot_general(_ld(x_v.at[0], r0, r1 - r0, ks), _ld(wcur_v, 0, M, ks), NT, preferred_element_type=F32)
        for tt in range(NT_M):
            yt = y[:, tt * 128:(tt + 1) * 128]
            qkv_v[0, tt, PAD + r0:PAD + r1, :] = yt if j == 0 else qkv_v[0, tt, PAD + r0:PAD + r1, :] + yt

    with _scope("wx0"):
        cp_x(0).wait()
    with _scope("b1"):
        for cc in (cp_x(2), cp_w(2), cp_x(3), cp_x(4)):
            cc.start()
        first(0, 0, R1)
    with _scope("w2"):
        for cc in (cp_w0(1), cp_x(1), cp_x(7), cp_w(1)):
            cc.wait()
    with _scope("b2"):
        cp_x(5).start()
        cp_x(6).start()
        for u in range(3, 3 * NK):
            cp_w(u).start()
        first(0, R1, S)
        prep_t(0, [(1, 1)], None)
        prep_p(wcur_v, 1, 1, None)
        first(1, 0, S)
        prep_next(1, z_v[...])
        wcur_v[...] = wnxt_v[...]
        for cc in a_copies[2:] + a_copies[:2]:
            cc.start()
    cp_x(2).wait()
    cp_x(3).wait()
    cp_x(4).wait()
    cp_g.wait()

    def bproj_body(t, _):
        part = lax.shift_right_logical(t, 2)
        kq = t & 3

        @pl.when(t < 3 * NK - 1)
        def _():
            cp_w(t + 1).wait()

        @pl.when(t == 2)
        def _():
            cp_x(5).wait()
            cp_x(6).wait()

        w = _ld(wcur_v, 0, M)
        for c in range(NC):
            y = lax.dot_general(_ld(x_v.at[kq], c * TC, TC), w, NT, preferred_element_type=F32)
            rs = slice(PAD + c * TC, PAD + (c + 1) * TC)
            for tt in range(NT_M):
                yt = y[:, tt * 128:(tt + 1) * 128]
                qkv_v[part, tt, rs, :] = jnp.where(kq == 0, yt, qkv_v[part, tt, rs, :] + yt)
        z = z_v[...]
        dep = prep_next(jnp.minimum(t + 1, 3 * NK - 1), z)
        gate_rows(t, z, dep)
        wcur_v[...] = wnxt_v[...]
        return 0

    lax.fori_loop(1, 3 * NK, _scoped("bproj", bproj_body), 0)
    with _scope("aw"):
        for c in a_waits:
            c.wait()

    qscale = (D ** -0.5) * LOG2E
    bscale = (DH ** -0.5) * LOG2E

    def local_attn(r, z, dep, masked):
        def zf(*vals):
            return jnp.concatenate([pltpu.bitcast(_zero_after(z, *vals), F32)] * (LAR // 8), axis=0)

        sc = jnp.full((LAR, 128), bscale, F32)
        if dep is not None:
            sc = sc + dep
        q = [qkv_v[0, t, pl.ds(PAD + r, LAR), :] * sc for t in range(NT_M)]
        rowi = r + lax.broadcasted_iota(jnp.int32, (LAR, 128), 0)
        logits, raw = [], []
        for w in range(W):
            a = None if w < LAQ else zf(raw[w - LAQ])
            for t in range(NT_M):
                pr = q[t] * qkv_v[1, t, pl.ds(PAD + r - DIL * w, LAR), :]
                a = pr if a is None else a + pr
            raw.append(a)
            if ROLL3:
                a = (a + pltpu.roll(a, 64, 1)) + (pltpu.roll(a, 32, 1) + pltpu.roll(a, 96, 1))
            else:
                a = a + pltpu.roll(a, 64, 1)
                a = a + pltpu.roll(a, 32, 1)
            logits.append(jnp.where(rowi >= DIL * w, a, NEG) if w > 0 and masked else a)
        m = functools.reduce(jnp.maximum, logits)
        es = [jnp.exp2(lg - m) for lg in logits]
        l = functools.reduce(lambda a, b: a + b, es)
        f = (1.0 - g_v[pl.ds(r, LAR), :]) * _recip(l)
        es = [e * f for e in es]
        outs = []
        for t in range(NT_M):
            a = None if t < LAP else zf(outs[t - LAP])
            for w in range(W):
                pr = es[w] * qkv_v[2, t, pl.ds(PAD + r - DIL * w, LAR), :]
                a = pr if a is None else a + pr
            outs.append(a)
        return jnp.concatenate(outs, axis=1), zf(*outs[NT_M - LAP:])

    def pair_body(p, _):
        z = z_v[...]
        def kvproj():
            wk, wv = _split_pair(wuk_p[p]), _split_pair(wuv_p[p])
            if KVM:
                for r in range(0, S, KVC):
                    kv = jnp.dot(_ld(ckv_v, r, KVC), jnp.concatenate([wk, wv], axis=1), preferred_element_type=F32).astype(BF16)
                    _st(k_s, r, kv[:, :2 * D])
                    _st(v_s, r, kv[:, 2 * D:])
                return
            jobs = [(k_s, wk, r) for r in range(0, S, KVC)] + [(v_s, wv, r) for r in range(0, S, KVC)]
            if KVI:
                jobs = [j for r in range(0, S, KVC) for j in ((k_s, wk, r), (v_s, wv, r))]
            for dst, w, r in jobs:
                _st(dst, r, jnp.dot(_ld(ckv_v, r, KVC), w, preferred_element_type=F32).astype(BF16))

        if not LFIRST:
            kvproj()
        rb = pl.multiple_of(p * TL, TL)
        dep, obs = None, []
        for k in range(TL // LAR):
            ob, dep = local_attn(rb + k * LAR, z, dep, k * LAR < PAD or not MSK)
            obs.append(ob)
        ob = jnp.concatenate(obs, axis=0).astype(BF16)
        if LFIRST:
            kvproj()

        def bout():
            wop = jnp.concatenate([f(bwo_p[dp]) for dp in range(DH // 2) for f in (_lo, _hi)], axis=0).astype(BF16)
            y = acc_v[pl.ds(rb, TL), :] + jnp.dot(ob, wop, preferred_element_type=F32)
            acc_v[pl.ds(rb, TL), :] = y
            if BPOS == 99:
                for c0, c1 in zip(OCUT[:-1], OCUT[1:]):
                    o_st[S - TL:S, c0:c1] = y[:, c0:c1].astype(BF16)
                    pl.when(p == HP - 1)(cp_o(S - TL, TL, c0, c1).start)

        if BPOS < 0:
            bout()

        wqw = wq_p[p]
        if BPOS == 99 and not DEPQ:
            wqw = jnp.concatenate([wqw[:8] | _zero_after(z, ob[TL - 16:]), wqw[8:]], axis=0)
        wq = _split_pair(wqw)
        row = lax.broadcasted_iota(jnp.int32, (TQ, TQ), 0)
        col = lax.broadcasted_iota(jnp.int32, (TQ, TQ), 1)
        causal = col <= row

        def qproj(c):
            xc = jnp.concatenate([_ld(x_v.at[k], c * TQP, TQP) for k in range(NK)], axis=1)
            if BPOS == 99 and DEPQ and c == order[DEPQ]:
                top = pltpu.bitcast(pltpu.bitcast(xc[:16, :128], U32) | _zero_after(z, ob[TL - 16:]), BF16)
                xc = jnp.concatenate([jnp.concatenate([top, xc[:16, 128:]], axis=1), xc[16:]], axis=0)
            q = jnp.dot(xc, wq, preferred_element_type=F32) * qscale
            _st(q_s, c * TQP, q.astype(BF16))

        def qk(i, hh):
            cs = slice(hh * D, (hh + 1) * D)
            return lax.dot_general(_ld(q_s, i * TQ, TQ, cs), _ld(k_s, 0, (i + 1) * TQ, cs), NT,
                                   preferred_element_type=F32)

        ldep = [None]

        def softmax_pv(i, hh, s):
            cs = slice(hh * D, (hh + 1) * D)
            r0 = i * TQ
            sd = jnp.where(causal, s[:, r0:], NEG)
            s = jnp.concatenate([s[:, :r0], sd], axis=1) if i > 0 else sd
            if MAXG and i > 1:
                m = jnp.max(_chain_reduce(s, jnp.maximum, MAXG, z, None)[0], axis=1, keepdims=True)
            else:
                m = jnp.max(s, axis=1, keepdims=True)
            e = jnp.exp2(s - m)
            if SUMG and i > SUMT:
                lp, ldep[0] = _chain_reduce(e, jnp.add, SUMG, z, (ldep[0] if hh == 1 else None) if SCH == 1 else (ldep[0] if SCH == 2 else None))
                l = jnp.sum(lp, axis=1, keepdims=True)
            else:
                l = jnp.sum(e, axis=1, keepdims=True)
            o = jnp.dot(e.astype(BF16), _ld(v_s, 0, r0 + TQ, cs), preferred_element_type=F32)
            return o * (g_v[r0:r0 + TQ, :] * _recip(l))

        def oproj(i, o0, o1):
            r0 = i * TQ
            y = acc_v[r0:r0 + TQ, :] + jnp.dot(jnp.concatenate([o0, o1], axis=1).astype(BF16),
                                               _ld(wo_v, p * (2 * D), 2 * D), preferred_element_type=F32)
            acc_v[r0:r0 + TQ, :] = y
            cuts = OCUT if i == order[-1] else (0, M)
            if BPOS == 99:
                cuts = (0, M) if r0 != S - TL else (0,)
            for c0, c1 in zip(cuts[:-1], cuts[1:]):
                o_st[r0:r0 + TQ, c0:c1] = y[:, c0:c1].astype(BF16)
                pl.when(p == HP - 1)(cp_o(r0, TQ, c0, c1).start)

        desc = list(reversed(range(S // TQ)))
        order = {0: desc, 1: [13, 15, 14] + desc[3:], 2: [8] + [i for i in desc if i != 8],
                 3: [4] + [i for i in desc if i != 4], 4: [0] + desc[:-1], 5: [12, 15, 14, 13] + desc[4:],
                 6: [1] + [i for i in desc if i != 1], 7: [10, 15, 14, 13, 12, 11] + desc[6:],
                 8: [15, 3, 14, 2, 13, 1, 12, 11, 10, 9, 8, 7, 6, 5, 4, 0],
                 9: [15, 0, 14, 1, 13, 2, 12, 3, 11, 4, 10, 5, 9, 6, 8, 7],
                 10: [15, 14, 13, 12, 3, 11, 2, 10, 1, 9, 8, 7, 6, 5, 4, 0]}[ORD]
        items = [(i, hh) for i in order for hh in range(2)]
        n = len(items)
        s_vals, o_vals = {}, {}
        for a in range(QAH):
            qproj(order[a])
        for step in range(n + LOOK + OLAG):
            if step == BPOS:
                bout()
            if step % 2 == 0 and QAH + step // 2 < len(order):
                qproj(order[QAH + step // 2])
            if step < n:
                s_vals[step] = qk(*items[step])
            b = step - LOOK
            if 0 <= b < n:
                o_vals[b] = softmax_pv(*items[b], s_vals.pop(b))
            c = step - LOOK - OLAG
            if 0 <= c < n and c % 2 == 1:
                oproj(items[c][0], o_vals.pop(c - 1), o_vals.pop(c))
        if BPOS == 99:
            bout()
        return 0

    lax.fori_loop(0, HP, _scoped("pair", pair_body), 0)
    with _scope("ow"):
        cp_o(0, S).wait()


def _kernel(*refs):
    dma = pltpu.SemaphoreType.DMA
    pl.run_scoped(functools.partial(_body, *refs), dma((9,)), dma((3 * NK + 1,)), dma(()), dma(()))


@jax.jit
def pallas_gated_mix__compressed_kv_cla__sliding_local_dilated__prompt_kernel(
    A_x, A_c_kv, A_w_q, A_w_uk, A_w_uv, A_w_o, B_x, B_wqkv, B_wo, gate_w,
):
    del B_x
    x = A_x.reshape(S, M)
    ckv = A_c_kv.reshape(S, DC)
    wo = A_w_o.reshape(H * D, M)
    bwo = B_wo.reshape(H, DH, M)
    any_spec = pl.BlockSpec(memory_space=pl.ANY)
    out = pl.pallas_call(
        _kernel,
        out_shape=jax.ShapeDtypeStruct((S, M), BF16),
        in_specs=[any_spec] * 9,
        out_specs=any_spec,
        scratch_shapes=[
            pltpu.VMEM((NK, S // 2, KB), U32),
            pltpu.VMEM((S // 2, DC), U32),
            pltpu.VMEM((HP, M, D), U32),
            pltpu.VMEM((HP, DC, D), U32),
            pltpu.VMEM((HP, DC, D), U32),
            pltpu.VMEM((H * D // 2, M), U32),
            pltpu.VMEM((M, 3 * M), BF16),
            pltpu.VMEM((DH // 2, H, M), U32),
            pltpu.VMEM((M // 2, KB), U32),
            pltpu.VMEM((M // 2, KB), U32),
            pltpu.VMEM((2, H * PITCH, 128), F32),
            pltpu.VMEM((3, NT_M, S + PAD, 128), F32),
            pltpu.VMEM((S, M), F32),
            pltpu.VMEM((S, 128), F32),
            pltpu.VMEM((8, 128), U32),
            pltpu.VMEM((S // 2, 2 * D), U32),
            pltpu.VMEM((S // 2, 2 * D), U32),
            pltpu.VMEM((S // 2, 2 * D), U32),
            pltpu.VMEM((S, M), BF16),
            pltpu.VMEM((M,), BF16),
        ],
        compiler_params=pltpu.CompilerParams(vmem_limit_bytes=110 * 1024 * 1024),
    )(x, ckv, A_w_q, A_w_uk, A_w_uv, wo, B_wqkv, bwo, gate_w)
    return out.reshape(1, S, M)
```

```python
import contextlib
import functools

import jax
import jax.numpy as jnp
from jax import lax
import jax.experimental.pallas as pl
import jax.experimental.pallas.tpu as pltpu

S = 2048
M = 1024
DC = 512
H = 32
HP = H // 2
D = 128
DH = 32
W = 8
DIL = 2
PAD = 16
NT_M = M // 128
TQ = 128
TQP = 128
TC = 512
NC = S // TC
KB = 256
NK = M // KB
R1 = 768
TL = S // HP
OCUT = (0, 512, 768, M)
GR = 192
PITCH = 17
LOOK = 2
OLAG = 10
SUMG = 16
MAXG = 0
LAP = 1
LAR = 8
KVC = 2048
KVI = 0
BPOS = 99
SUMT = 2
QAH = 1
ORD = 0
SCH = 2
ROLL3 = 0
LAQ = 2
LFIRST = 1
KVM = 0
MSK = 0
DEPQ = 0
B1C = 0
B2C = 1
LOG2E = 1.4426950408889634
NEG = -1e9

F32 = jnp.float32
BF16 = jnp.bfloat16
U32 = jnp.uint32
NT = (((1,), (1,)), ((), ()))


_PROFILE = False


def _scope(name):
    return jax.named_scope(name) if _PROFILE else contextlib.nullcontext()


def _scoped(name, body):
    def f(i, c):
        with _scope(name):
            return body(i, c)
    return f


def _recip(l):
    r = pl.reciprocal(l, approx=True)
    return r * (2.0 - l * r)


def _lo(w):
    return pltpu.bitcast(w << 16, F32)


def _hi(w):
    return pltpu.bitcast(w & jnp.uint32(0xFFFF0000), F32)


def _split_pair(w):
    return jnp.concatenate([_lo(w), _hi(w)], axis=1).astype(BF16)


def _ld(ref, r0, n, cols=slice(None)):
    if isinstance(r0, int):
        rs = slice(r0 // 2, (r0 + n) // 2)
    else:
        rs = pl.ds(pl.multiple_of(lax.shift_right_logical(r0, 1), 8), n // 2)
    return pltpu.bitcast(ref[rs, cols], BF16)


def _st(ref, r0, val, cols=slice(None)):
    ref[r0 // 2:(r0 + val.shape[0]) // 2, cols] = pltpu.bitcast(val, U32)


def _zero_after(z, *vals):
    acc = None
    for v in vals:
        b = pltpu.bitcast(v, U32)
        for r in range(0, b.shape[0], 8):
            for c in range(0, b.shape[1], 128):
                t = b[r:r + 8, c:c + 128]
                acc = t if acc is None else acc | t
    return acc & z


def _chain_reduce(x, op, g, z, dep):
    parts = []
    for r in range(0, x.shape[0], g):
        a = x[r:r + g, 0:128]
        if dep is not None:
            a = pltpu.bitcast(pltpu.bitcast(a, U32) | jnp.concatenate([dep] * (g // 8), axis=0), F32)
        for c in range(128, x.shape[1], 128):
            a = op(a, x[r:r + g, c:c + 128])
        dep = _zero_after(z, a)
        parts.append(a)
    return jnp.concatenate(parts, axis=0), dep


def _body(x_hbm, ckv_hbm, wq_hbm, wuk_hbm, wuv_hbm, wo_hbm, bqkv_hbm, bwo_hbm, gate_hbm,
            out_hbm,
            x_v, ckv_v, wq_p, wuk_p, wuv_p, wo_v, bqkv_v, bwo_p, wcur_v, wnxt_v, wfst_v,
            qkv_v, acc_v, g_v, z_v, q_s, k_s, v_s, o_st, gate_v,
            sem_x, sem_w, sem_a, sem_o):
    x_parts = [(0, R1, 0, 0, 128), (R1, S, 0, 0, 128), (0, S, 1, 0, KB), (0, TC, 2, 0, KB), (0, TC, 3, 0, KB),
               (TC, S, 2, 0, KB), (TC, S, 3, 0, KB), (0, S, 0, 128, 128)]

    def cp_x(i):
        r0, r1, k, c0, n = x_parts[i]
        rs = pl.ds(r0 // 2, (r1 - r0) // 2)
        return pltpu.make_async_copy(x_hbm.bitcast(U32).at[rs, pl.ds(k * KB + c0, n)], x_v.at[k, rs, pl.ds(c0, n)],
                                     sem_x.at[i])

    def cp_w(u):
        u_lo, u_hi = (u % NK, u // NK) if isinstance(u, int) else (u & 3, lax.shift_right_logical(u, 2))
        sl = (pl.ds(u_lo * KB, KB), pl.ds(u_hi * M, M))
        return pltpu.make_async_copy(bqkv_hbm.at[sl], bqkv_v.at[sl], sem_w.at[u])

    def cp_w0(j):
        sl = (pl.ds(j * 128, 128), pl.ds(0, M))
        return pltpu.make_async_copy(bqkv_hbm.at[sl], bqkv_v.at[sl], sem_w.at[j * 3 * NK])

    cp_g = pltpu.make_async_copy(gate_hbm, gate_v, sem_x.at[len(x_parts)])

    a_copies = [pltpu.make_async_copy(ckv_hbm.bitcast(U32), ckv_v, sem_a),
                pltpu.make_async_copy(wo_hbm.bitcast(U32), wo_v, sem_a)]
    for src, dst in ((wuk_hbm, wuk_p), (wuv_hbm, wuv_p), (wq_hbm, wq_p), (bwo_hbm, bwo_p)):
        src_u = src.bitcast(U32)
        a_copies += [pltpu.make_async_copy(src_u.at[:, p, :], dst.at[p], sem_a) for p in range(HP)]
    a_waits = [pltpu.make_async_copy(b, b, sem_a) for b in (ckv_v, wo_v, wuk_p, wuv_p, wq_p, bwo_p)]

    def cp_o(r0, n, c0=0, c1=M):
        sl = (pl.ds(r0, n), pl.ds(c0, c1 - c0))
        return pltpu.make_async_copy(o_st.at[sl], out_hbm.at[sl], sem_o)

    for cc in (cp_w0(0), cp_x(0), cp_w0(1)):
        cc.start()
    z_v[...] = jnp.zeros((8, 128), U32)
    for part in range(3):
        for t in range(NT_M):
            qkv_v[part, t, 0:PAD, :] = jnp.zeros((PAD, 128), F32)

    def prep(dst, part, j, slot, z, dep=None):
        p0 = part * M if isinstance(part, int) else pl.multiple_of(part * M, M)
        k0 = j * 128 if isinstance(j, int) else pl.multiple_of(j * 128, 128)
        for c in range(NT_M):
            src = bqkv_v[pl.ds(k0, 128), pl.ds(p0 + c * 128, 128)]
            if dep is not None:
                top = pltpu.bitcast(pltpu.bitcast(src[:16], U32) | dep, BF16)
                src = jnp.concatenate([top, src[16:]], axis=0)
            t = pltpu.bitcast(src.T, U32)
            for hp in range(2):
                a, b = t[32 * hp:32 * hp + 16], t[32 * hp + 16:32 * hp + 32]
                r = 2 * c + hp
                dst[slot, pl.ds(r, 16, stride=2 * PITCH), :] = (a & jnp.uint32(0xFFFF)) | (b << 16)
                dst[slot, pl.ds(PITCH + r, 16, stride=2 * PITCH), :] = (a >> 16) | (b & jnp.uint32(0xFFFF0000))
            if z is not None:
                dep = _zero_after(z, t[56:64])
        return dep

    def wtile(j):
        return pltpu.bitcast(jnp.concatenate([wcur_v[j, d * PITCH:d * PITCH + HP, :] for d in range(DH)], axis=0), BF16)

    def flip():
        for j in range(2):
            for d in range(DH):
                wcur_v[j, d * PITCH:d * PITCH + HP, :] = wnxt_v[j, d * PITCH:d * PITCH + HP, :]

    def first_tiles():
        for j in range(2):
            for n in range(2):
                w = jnp.concatenate([wnxt_v[j, d * PITCH:d * PITCH + HP, :] for d in range(4 * n, 4 * n + 4)], axis=0)
                _st(wfst_v, j * 128, pltpu.bitcast(w, BF16).T, slice(n * 128, (n + 1) * 128))

    def prep_next(u, z):
        part, kq = (u // NK, u % NK) if isinstance(u, int) else (lax.shift_right_logical(u, 2), u & 3)
        return prep(wnxt_v, part, 2 * kq + 1, 1, z, prep(wnxt_v, part, 2 * kq, 0, z))

    def gate_rows(t, z, dep):
        gw = gate_v[...].astype(F32).reshape(1, M)
        g0 = jnp.minimum((t - 1) * GR, S - GR)
        for k in range(GR // 16):
            rr = pl.multiple_of(g0 + k * 16, 16)
            rw = pl.multiple_of(lax.shift_right_logical(rr, 1), 8)
            xb = jnp.concatenate([x_v[q, pl.ds(rw, 8), :] for q in range(NK)], axis=1)
            xb = xb | jnp.concatenate([dep] * NT_M, axis=1)
            xx = pltpu.bitcast(xb, BF16).astype(F32)
            zz = jnp.sum(xx * gw, axis=1, keepdims=True)
            g = jnp.broadcast_to(1.0 / (1.0 + jnp.exp(-zz)), (16, 128))
            g_v[pl.ds(rr, 16), :] = g
            acc_v[pl.ds(rr, 16), :] = jnp.zeros((16, M), F32)
            dep = _zero_after(z, g)

    def _all(_i, _c):
        with _scope("prep0"):
            cp_w0(0).wait()
            for cc in (cp_x(1), cp_x(7), cp_w(1), cp_g):
                cc.start()
            prep(wcur_v, 0, 0, 0, None)

        def first(j, r0, r1):
            ks = slice(j * 128, (j + 1) * 128)
            y = lax.dot_general(_ld(x_v.at[0], r0, r1 - r0, ks), wtile(j), NT, preferred_element_type=F32)
            for tt in range(NT_M):
                yt = y[:, tt * 128:(tt + 1) * 128]
                qkv_v[0, tt, PAD + r0:PAD + r1, :] = yt if j == 0 else qkv_v[0, tt, PAD + r0:PAD + r1, :] + yt

        with _scope("wx0"):
            cp_x(0).wait()
        with _scope("b1"):
            for cc in (cp_x(2), cp_w(2), cp_x(3), cp_x(4)):
                cc.start()
            first(0, 0, R1)
        with _scope("w2"):
            for cc in (cp_w0(1), cp_x(1)):
                cc.wait()
        with _scope("b1b"):
            first(0, R1, S)
            prep(wcur_v, 0, 1, 1, z_v[...] if B1C else None)
        with _scope("w3"):
            for cc in (cp_x(7), cp_w(1)):
                cc.wait()
        with _scope("b2"):
            cp_x(5).start()
            cp_x(6).start()
            for u in range(3, 3 * NK):
                cp_w(u).start()
            first(1, 0, S)
            prep(wnxt_v, 0, 2, 0, z_v[...] if B2C else None)
            prep(wnxt_v, 0, 3, 1, z_v[...] if B2C else None)
            first_tiles()
            flip()
            for cc in a_copies[2:] + a_copies[:2]:
                cc.start()
        cp_x(2).wait()
        cp_x(3).wait()
        cp_x(4).wait()
        cp_g.wait()

        def bproj_body(t, _):
            part = lax.shift_right_logical(t, 2)
            kq = t & 3

            @pl.when(t < 3 * NK - 1)
            def _():
                cp_w(t + 1).wait()

            @pl.when(t == 2)
            def _():
                cp_x(5).wait()
                cp_x(6).wait()

            w = jnp.concatenate([wtile(0), wtile(1)], axis=1)
            for c in range(NC):
                xc = _ld(x_v.at[kq], c * TC, TC)
                if c == 0:
                    y = jnp.concatenate([jnp.dot(xc, _ld(wfst_v, 0, KB), preferred_element_type=F32),
                                         lax.dot_general(xc, w[256:], NT, preferred_element_type=F32)], axis=1)
                else:
                    y = lax.dot_general(xc, w, NT, preferred_element_type=F32)
                rs = slice(PAD + c * TC, PAD + (c + 1) * TC)
                for tt in range(NT_M):
                    yt = y[:, tt * 128:(tt + 1) * 128]
                    qkv_v[part, tt, rs, :] = jnp.where(kq == 0, yt, qkv_v[part, tt, rs, :] + yt)
            z = z_v[...]
            dep = prep_next(jnp.minimum(t + 1, 3 * NK - 1), z)
            gate_rows(t, z, dep)
            first_tiles()
            flip()
            return 0

        lax.fori_loop(1, 3 * NK, _scoped("bproj", bproj_body), 0)
        with _scope("aw"):
            for c in a_waits:
                c.wait()

        qscale = (D ** -0.5) * LOG2E
        bscale = (DH ** -0.5) * LOG2E

        def local_attn(r, z, dep, masked):
            def zf(*vals):
                return jnp.concatenate([pltpu.bitcast(_zero_after(z, *vals), F32)] * (LAR // 8), axis=0)

            sc = jnp.full((LAR, 128), bscale, F32)
            if dep is not None:
                sc = sc + dep
            q = [qkv_v[0, t, pl.ds(PAD + r, LAR), :] * sc for t in range(NT_M)]
            rowi = r + lax.broadcasted_iota(jnp.int32, (LAR, 128), 0)
            logits, raw = [], []
            for w in range(W):
                a = None if w < LAQ else zf(raw[w - LAQ])
                for t in range(NT_M):
                    pr = q[t] * qkv_v[1, t, pl.ds(PAD + r - DIL * w, LAR), :]
                    a = pr if a is None else a + pr
                raw.append(a)
                if ROLL3:
                    a = (a + pltpu.roll(a, 64, 1)) + (pltpu.roll(a, 32, 1) + pltpu.roll(a, 96, 1))
                else:
                    a = a + pltpu.roll(a, 64, 1)
                    a = a + pltpu.roll(a, 32, 1)
                logits.append(jnp.where(rowi >= DIL * w, a, NEG) if w > 0 and masked else a)
            m = functools.reduce(jnp.maximum, logits)
            es = [jnp.exp2(lg - m) for lg in logits]
            l = functools.reduce(lambda a, b: a + b, es)
            f = (1.0 - g_v[pl.ds(r, LAR), :]) * _recip(l)
            es = [e * f for e in es]
            outs = []
            for t in range(NT_M):
                a = None if t < LAP else zf(outs[t - LAP])
                for w in range(W):
                    pr = es[w] * qkv_v[2, t, pl.ds(PAD + r - DIL * w, LAR), :]
                    a = pr if a is None else a + pr
                outs.append(a)
            return jnp.concatenate(outs, axis=1), zf(*outs[NT_M - LAP:])

        def pair_body(p, _):
            z = z_v[...]
            def kvproj():
                wk, wv = _split_pair(wuk_p[p]), _split_pair(wuv_p[p])
                if KVM:
                    for r in range(0, S, KVC):
                        kv = jnp.dot(_ld(ckv_v, r, KVC), jnp.concatenate([wk, wv], axis=1), preferred_element_type=F32).astype(BF16)
                        _st(k_s, r, kv[:, :2 * D])
                        _st(v_s, r, kv[:, 2 * D:])
                    return
                jobs = [(k_s, wk, r) for r in range(0, S, KVC)] + [(v_s, wv, r) for r in range(0, S, KVC)]
                if KVI:
                    jobs = [j for r in range(0, S, KVC) for j in ((k_s, wk, r), (v_s, wv, r))]
                for dst, w, r in jobs:
                    _st(dst, r, jnp.dot(_ld(ckv_v, r, KVC), w, preferred_element_type=F32).astype(BF16))

            if not LFIRST:
                kvproj()
            rb = pl.multiple_of(p * TL, TL)
            dep, obs = None, []
            for k in range(TL // LAR):
                ob, dep = local_attn(rb + k * LAR, z, dep, k * LAR < PAD or not MSK)
                obs.append(ob)
            ob = jnp.concatenate(obs, axis=0).astype(BF16)
            if LFIRST:
                kvproj()

            def bout():
                wop = jnp.concatenate([f(bwo_p[dp]) for dp in range(DH // 2) for f in (_lo, _hi)], axis=0).astype(BF16)
                y = acc_v[pl.ds(rb, TL), :] + jnp.dot(ob, wop, preferred_element_type=F32)
                acc_v[pl.ds(rb, TL), :] = y
                if BPOS == 99:
                    for c0, c1 in zip(OCUT[:-1], OCUT[1:]):
                        o_st[S - TL:S, c0:c1] = y[:, c0:c1].astype(BF16)
                        pl.when(p == HP - 1)(cp_o(S - TL, TL, c0, c1).start)

            if BPOS < 0:
                bout()

            wqw = wq_p[p]
            if BPOS == 99 and not DEPQ:
                wqw = jnp.concatenate([wqw[:8] | _zero_after(z, ob[TL - 16:]), wqw[8:]], axis=0)
            wq = _split_pair(wqw)
            row = lax.broadcasted_iota(jnp.int32, (TQ, TQ), 0)
            col = lax.broadcasted_iota(jnp.int32, (TQ, TQ), 1)
            causal = col <= row

            def qproj(c):
                xc = jnp.concatenate([_ld(x_v.at[k], c * TQP, TQP) for k in range(NK)], axis=1)
                if BPOS == 99 and DEPQ and c == order[DEPQ]:
                    top = pltpu.bitcast(pltpu.bitcast(xc[:16, :128], U32) | _zero_after(z, ob[TL - 16:]), BF16)
                    xc = jnp.concatenate([jnp.concatenate([top, xc[:16, 128:]], axis=1), xc[16:]], axis=0)
                q = jnp.dot(xc, wq, preferred_element_type=F32) * qscale
                _st(q_s, c * TQP, q.astype(BF16))

            def qk(i, hh):
                cs = slice(hh * D, (hh + 1) * D)
                return lax.dot_general(_ld(q_s, i * TQ, TQ, cs), _ld(k_s, 0, (i + 1) * TQ, cs), NT,
                                       preferred_element_type=F32)

            ldep = [None]

            def softmax_pv(i, hh, s):
                cs = slice(hh * D, (hh + 1) * D)
                r0 = i * TQ
                sd = jnp.where(causal, s[:, r0:], NEG)
                s = jnp.concatenate([s[:, :r0], sd], axis=1) if i > 0 else sd
                if MAXG and i > 1:
                    m = jnp.max(_chain_reduce(s, jnp.maximum, MAXG, z, None)[0], axis=1, keepdims=True)
                else:
                    m = jnp.max(s, axis=1, keepdims=True)
                e = jnp.exp2(s - m)
                if SUMG and i > SUMT:
                    lp, ldep[0] = _chain_reduce(e, jnp.add, SUMG, z, (ldep[0] if hh == 1 else None) if SCH == 1 else (ldep[0] if SCH == 2 else None))
                    l = jnp.sum(lp, axis=1, keepdims=True)
                else:
                    l = jnp.sum(e, axis=1, keepdims=True)
                o = jnp.dot(e.astype(BF16), _ld(v_s, 0, r0 + TQ, cs), preferred_element_type=F32)
                return o * (g_v[r0:r0 + TQ, :] * _recip(l))

            def oproj(i, o0, o1):
                r0 = i * TQ
                y = acc_v[r0:r0 + TQ, :] + jnp.dot(jnp.concatenate([o0, o1], axis=1).astype(BF16),
                                                   _ld(wo_v, p * (2 * D), 2 * D), preferred_element_type=F32)
                acc_v[r0:r0 + TQ, :] = y
                cuts = OCUT if i == order[-1] else (0, M)
                if BPOS == 99:
                    cuts = (0, M) if r0 != S - TL else (0,)
                for c0, c1 in zip(cuts[:-1], cuts[1:]):
                    o_st[r0:r0 + TQ, c0:c1] = y[:, c0:c1].astype(BF16)
                    pl.when(p == HP - 1)(cp_o(r0, TQ, c0, c1).start)

            desc = list(reversed(range(S // TQ)))
            order = {0: desc, 1: [13, 15, 14] + desc[3:], 2: [8] + [i for i in desc if i != 8],
                     3: [4] + [i for i in desc if i != 4], 4: [0] + desc[:-1], 5: [12, 15, 14, 13] + desc[4:],
                     6: [1] + [i for i in desc if i != 1], 7: [10, 15, 14, 13, 12, 11] + desc[6:],
                     8: [15, 3, 14, 2, 13, 1, 12, 11, 10, 9, 8, 7, 6, 5, 4, 0],
                     9: [15, 0, 14, 1, 13, 2, 12, 3, 11, 4, 10, 5, 9, 6, 8, 7],
                     10: [15, 14, 13, 12, 3, 11, 2, 10, 1, 9, 8, 7, 6, 5, 4, 0]}[ORD]
            items = [(i, hh) for i in order for hh in range(2)]
            n = len(items)
            s_vals, o_vals = {}, {}
            for a in range(QAH):
                qproj(order[a])
            for step in range(n + LOOK + OLAG):
                if step == BPOS:
                    bout()
                if step % 2 == 0 and QAH + step // 2 < len(order):
                    qproj(order[QAH + step // 2])
                if step < n:
                    s_vals[step] = qk(*items[step])
                b = step - LOOK
                if 0 <= b < n:
                    o_vals[b] = softmax_pv(*items[b], s_vals.pop(b))
                c = step - LOOK - OLAG
                if 0 <= c < n and c % 2 == 1:
                    oproj(items[c][0], o_vals.pop(c - 1), o_vals.pop(c))
            if BPOS == 99:
                bout()
            return 0

        lax.fori_loop(0, HP, _scoped("pair", pair_body), 0)
        return 0

    lax.fori_loop(0, 1 + pltpu.bitcast(z_v[...], jnp.int32)[0, 0], _all, 0)
    with _scope("ow"):
        cp_o(0, S).wait()


def _kernel(*refs):
    dma = pltpu.SemaphoreType.DMA
    pl.run_scoped(functools.partial(_body, *refs), dma((9,)), dma((3 * NK + 1,)), dma(()), dma(()))


@jax.jit
def pallas_gated_mix__compressed_kv_cla__sliding_local_dilated__prompt_kernel(
    A_x, A_c_kv, A_w_q, A_w_uk, A_w_uv, A_w_o, B_x, B_wqkv, B_wo, gate_w,
):
    del B_x
    x = A_x.reshape(S, M)
    ckv = A_c_kv.reshape(S, DC)
    wo = A_w_o.reshape(H * D, M)
    bwo = B_wo.reshape(H, DH, M)
    any_spec = pl.BlockSpec(memory_space=pl.ANY)
    out = pl.pallas_call(
        _kernel,
        out_shape=jax.ShapeDtypeStruct((S, M), BF16),
        in_specs=[any_spec] * 9,
        out_specs=any_spec,
        scratch_shapes=[
            pltpu.VMEM((NK, S // 2, KB), U32),
            pltpu.VMEM((S // 2, DC), U32),
            pltpu.VMEM((HP, M, D), U32),
            pltpu.VMEM((HP, DC, D), U32),
            pltpu.VMEM((HP, DC, D), U32),
            pltpu.VMEM((H * D // 2, M), U32),
            pltpu.VMEM((M, 3 * M), BF16),
            pltpu.VMEM((DH // 2, H, M), U32),
            pltpu.VMEM((2, DH * 24, 128), U32),
            pltpu.VMEM((2, DH * 24, 128), U32),
            pltpu.VMEM((KB // 2, 256), U32),
            pltpu.VMEM((3, NT_M, S + PAD, 128), F32),
            pltpu.VMEM((S, M), F32),
            pltpu.VMEM((S, 128), F32),
            pltpu.VMEM((8, 128), U32),
            pltpu.VMEM((S // 2, 2 * D), U32),
            pltpu.VMEM((S // 2, 2 * D), U32),
            pltpu.VMEM((S // 2, 2 * D), U32),
            pltpu.VMEM((S, M), BF16),
            pltpu.VMEM((M,), BF16),
        ],
        compiler_params=pltpu.CompilerParams(vmem_limit_bytes=110 * 1024 * 1024),
    )(x, ckv, A_w_q, A_w_uk, A_w_uv, wo, B_wqkv, bwo, gate_w)
    return out.reshape(1, S, M)
```

```python
import contextlib
import functools

import jax
import jax.numpy as jnp
from jax import lax
import jax.experimental.pallas as pl
import jax.experimental.pallas.tpu as pltpu

S = 2048
M = 1024
DC = 512
H = 32
HP = H // 2
D = 128
DH = 32
W = 8
DIL = 2
PAD = 16
NT_M = M // 128
TQ = 128
TL = S // HP
TC = 512
KB = 256
NK = M // KB
NTASK = 3 * NK
R1 = 768
GR = 192
PITCH = 17
NA1 = 36
OCUT = (0, 512, 768, M)
LOOK = 2
OLAG = 10
SUMG = 16
LAQ = 2
LOG2E = 1.4426950408889634
NEG = -1e9

F32 = jnp.float32
BF16 = jnp.bfloat16
U32 = jnp.uint32
NT = (((1,), (1,)), ((), ()))


_PROFILE = False


def _scope(name):
    return jax.named_scope(name) if _PROFILE else contextlib.nullcontext()


def _scoped(name, body):
    def f(i, c):
        with _scope(name):
            return body(i, c)
    return f


def _recip(l):
    r = pl.reciprocal(l, approx=True)
    return r * (2.0 - l * r)


def _lo(w):
    return pltpu.bitcast(w << 16, F32)


def _hi(w):
    return pltpu.bitcast(w & jnp.uint32(0xFFFF0000), F32)


def _split_pair(w):
    return jnp.concatenate([_lo(w), _hi(w)], axis=1).astype(BF16)


def _ld(ref, r0, n, cols=slice(None)):
    if isinstance(r0, int):
        rs = slice(r0 // 2, (r0 + n) // 2)
    else:
        rs = pl.ds(pl.multiple_of(lax.shift_right_logical(r0, 1), 8), n // 2)
    return pltpu.bitcast(ref[rs, cols], BF16)


def _st(ref, r0, val, cols=slice(None)):
    ref[r0 // 2:(r0 + val.shape[0]) // 2, cols] = pltpu.bitcast(val, U32)


def _zero_after(z, *vals):
    acc = None
    for v in vals:
        b = pltpu.bitcast(v, U32)
        for r in range(0, b.shape[0], 8):
            for c in range(0, b.shape[1], 128):
                t = b[r:r + 8, c:c + 128]
                acc = t if acc is None else acc | t
    return acc & z


def _chain_sum(x, z, dep):
    parts = []
    for r in range(0, x.shape[0], SUMG):
        a = x[r:r + SUMG, 0:128]
        if dep is not None:
            a = pltpu.bitcast(pltpu.bitcast(a, U32) | jnp.concatenate([dep] * (SUMG // 8), axis=0), F32)
        for c in range(128, x.shape[1], 128):
            a = a + x[r:r + SUMG, c:c + 128]
        dep = _zero_after(z, a)
        parts.append(a)
    return jnp.concatenate(parts, axis=0), dep


def _body(x_hbm, ckv_hbm, wq_hbm, wuk_hbm, wuv_hbm, wo_hbm, bqkv_hbm, bwo_hbm, gate_hbm,
          out_hbm,
          x_v, ckv_v, wq_p, wuk_p, wuv_p, wo_v, bqkv_v, bwo_p, wcur_v, wnxt_v, wfst_v,
          qkv_v, acc_v, g_v, z_v, q_s, k_s, v_s, o_st, gate_v,
          sem_x, sem_w, sem_a, sem_o):
    x_parts = [(0, R1, 0, 0, 128), (R1, S, 0, 0, 128), (0, S, 0, 128, 128), (0, S, 1, 0, KB),
               (0, TC, 2, 0, KB), (0, TC, 3, 0, KB), (TC, S, 2, 0, KB), (TC, S, 3, 0, KB)]

    def cp_x(i):
        r0, r1, k, c0, n = x_parts[i]
        rs = pl.ds(r0 // 2, (r1 - r0) // 2)
        return pltpu.make_async_copy(x_hbm.bitcast(U32).at[rs, pl.ds(k * KB + c0, n)], x_v.at[k, rs, pl.ds(c0, n)],
                                     sem_x.at[i])

    def cp_w(u):
        u_lo, u_hi = (u % NK, u // NK) if isinstance(u, int) else (u & 3, lax.shift_right_logical(u, 2))
        sl = (pl.ds(u_lo * KB, KB), pl.ds(u_hi * M, M))
        return pltpu.make_async_copy(bqkv_hbm.at[sl], bqkv_v.at[sl], sem_w.at[u])

    def cp_w0(j):
        sl = (pl.ds(j * 128, 128), pl.ds(0, M))
        return pltpu.make_async_copy(bqkv_hbm.at[sl], bqkv_v.at[sl], sem_w.at[j * NTASK])

    cp_g = pltpu.make_async_copy(gate_hbm, gate_v, sem_x.at[len(x_parts)])

    def cp_pairs(src, dst):
        return [pltpu.make_async_copy(src.bitcast(U32).at[:, p, :], dst.at[p], sem_a) for p in range(HP)]

    a_early = cp_pairs(bwo_hbm, bwo_p) + [pltpu.make_async_copy(ckv_hbm.bitcast(U32), ckv_v, sem_a),
                                          pltpu.make_async_copy(wo_hbm.bitcast(U32), wo_v, sem_a)]
    a_late = cp_pairs(wuk_hbm, wuk_p) + cp_pairs(wuv_hbm, wuv_p) + cp_pairs(wq_hbm, wq_p)
    a_waits = [pltpu.make_async_copy(b, b, sem_a) for b in (ckv_v, wo_v, wuk_p, wuv_p, wq_p, bwo_p)]

    def cp_o(r0, n, c0=0, c1=M):
        sl = (pl.ds(r0, n), pl.ds(c0, c1 - c0))
        return pltpu.make_async_copy(o_st.at[sl], out_hbm.at[sl], sem_o)

    def prep(dst, part, j, slot, z, dep=None):
        p0 = part * M if isinstance(part, int) else pl.multiple_of(part * M, M)
        k0 = j * 128 if isinstance(j, int) else pl.multiple_of(j * 128, 128)
        for c in range(NT_M):
            src = bqkv_v[pl.ds(k0, 128), pl.ds(p0 + c * 128, 128)]
            if dep is not None:
                top = pltpu.bitcast(pltpu.bitcast(src[:16], U32) | dep, BF16)
                src = jnp.concatenate([top, src[16:]], axis=0)
            t = pltpu.bitcast(src.T, U32)
            for hp in range(2):
                a, b = t[32 * hp:32 * hp + 16], t[32 * hp + 16:32 * hp + 32]
                r = 2 * c + hp
                dst[slot, pl.ds(r, 16, stride=2 * PITCH), :] = (a & jnp.uint32(0xFFFF)) | (b << 16)
                dst[slot, pl.ds(PITCH + r, 16, stride=2 * PITCH), :] = (a >> 16) | (b & jnp.uint32(0xFFFF0000))
            if z is not None:
                dep = _zero_after(z, t[56:64])
        return dep

    def wrows(ref, j, d0, d1):
        w = jnp.concatenate([ref[j, d * PITCH:d * PITCH + HP, :] for d in range(d0, d1)], axis=0)
        return pltpu.bitcast(w, BF16)

    def flip():
        for j in range(2):
            for n in range(2):
                _st(wfst_v, j * 128, wrows(wnxt_v, j, 4 * n, 4 * n + 4).T, slice(n * 128, (n + 1) * 128))
        for j in range(2):
            for d in range(DH):
                wcur_v[j, d * PITCH:d * PITCH + HP, :] = wnxt_v[j, d * PITCH:d * PITCH + HP, :]

    def gate_rows(t, z, dep):
        gw = gate_v[...].astype(F32).reshape(1, M)
        g0 = jnp.minimum((t - 1) * GR, S - GR)
        for k in range(GR // 16):
            rr = pl.multiple_of(g0 + k * 16, 16)
            rw = pl.multiple_of(lax.shift_right_logical(rr, 1), 8)
            xb = jnp.concatenate([x_v[q, pl.ds(rw, 8), :] for q in range(NK)], axis=1)
            xb = xb | jnp.concatenate([dep] * NT_M, axis=1)
            xx = pltpu.bitcast(xb, BF16).astype(F32)
            zz = jnp.sum(xx * gw, axis=1, keepdims=True)
            g = jnp.broadcast_to(1.0 / (1.0 + jnp.exp(-zz)), (16, 128))
            g_v[pl.ds(rr, 16), :] = g
            acc_v[pl.ds(rr, 16), :] = jnp.zeros((16, M), F32)
            dep = _zero_after(z, g)

    def first_task():
        def piece(j, r0, r1):
            y = lax.dot_general(_ld(x_v.at[0], r0, r1 - r0, slice(j * 128, (j + 1) * 128)), wrows(wcur_v, j, 0, DH),
                                NT, preferred_element_type=F32)
            for tt in range(NT_M):
                yt = y[:, tt * 128:(tt + 1) * 128]
                qkv_v[0, tt, PAD + r0:PAD + r1, :] = yt if j == 0 else qkv_v[0, tt, PAD + r0:PAD + r1, :] + yt

        with _scope("prep0"):
            cp_w0(0).wait()
            prep(wcur_v, 0, 0, 0, None)
        with _scope("b1"):
            cp_x(0).wait()
            piece(0, 0, R1)
        with _scope("b2"):
            cp_w0(1).wait()
            cp_x(1).wait()
            piece(0, R1, S)
            prep(wcur_v, 0, 1, 1, None)
        with _scope("b3"):
            cp_x(2).wait()
            cp_w(1).wait()
            piece(1, 0, S)
            prep(wnxt_v, 0, 2, 0, z_v[...])
            prep(wnxt_v, 0, 3, 1, z_v[...])
            flip()
            for cc in a_late[:NA1]:
                cc.start()
        for cc in (cp_x(3), cp_x(4), cp_x(5), cp_g):
            cc.wait()
        for cc in a_late[NA1:]:
            cc.start()

    def bproj_body(t, _):
        part = lax.shift_right_logical(t, 2)
        kq = t & 3

        @pl.when(t < NTASK - 1)
        def _():
            cp_w(t + 1).wait()

        @pl.when(t == 2)
        def _():
            cp_x(6).wait()
            cp_x(7).wait()

        w = jnp.concatenate([wrows(wcur_v, 0, 0, DH), wrows(wcur_v, 1, 0, DH)], axis=1)
        for c in range(S // TC):
            xc = _ld(x_v.at[kq], c * TC, TC)
            if c == 0:
                y = jnp.concatenate([jnp.dot(xc, _ld(wfst_v, 0, KB), preferred_element_type=F32),
                                     lax.dot_general(xc, w[256:], NT, preferred_element_type=F32)], axis=1)
            else:
                y = lax.dot_general(xc, w, NT, preferred_element_type=F32)
            rs = slice(PAD + c * TC, PAD + (c + 1) * TC)
            for tt in range(NT_M):
                yt = y[:, tt * 128:(tt + 1) * 128]
                qkv_v[part, tt, rs, :] = jnp.where(kq == 0, yt, qkv_v[part, tt, rs, :] + yt)
        z = z_v[...]
        u = jnp.minimum(t + 1, NTASK - 1)
        un, uk = lax.shift_right_logical(u, 2), u & 3
        dep = prep(wnxt_v, un, 2 * uk + 1, 1, z, prep(wnxt_v, un, 2 * uk, 0, z))
        gate_rows(t, z, dep)
        flip()
        return 0

    qscale = (D ** -0.5) * LOG2E
    bscale = (DH ** -0.5) * LOG2E

    def local_attn(r, z, dep):
        def zf(v):
            return pltpu.bitcast(_zero_after(z, v), F32)

        sc = jnp.full((8, 128), bscale, F32)
        if dep is not None:
            sc = sc + dep
        q = [qkv_v[0, t, pl.ds(PAD + r, 8), :] * sc for t in range(NT_M)]
        rowi = r + lax.broadcasted_iota(jnp.int32, (8, 128), 0)
        logits, raw = [], []
        for w in range(W):
            a = None if w < LAQ else zf(raw[w - LAQ])
            for t in range(NT_M):
                pr = q[t] * qkv_v[1, t, pl.ds(PAD + r - DIL * w, 8), :]
                a = pr if a is None else a + pr
            raw.append(a)
            a = a + pltpu.roll(a, 64, 1)
            a = a + pltpu.roll(a, 32, 1)
            logits.append(jnp.where(rowi >= DIL * w, a, NEG) if w > 0 else a)
        m = functools.reduce(jnp.maximum, logits)
        es = [jnp.exp2(lg - m) for lg in logits]
        l = functools.reduce(lambda a, b: a + b, es)
        f = (1.0 - g_v[pl.ds(r, 8), :]) * _recip(l)
        es = [e * f for e in es]
        outs = []
        for t in range(NT_M):
            a = None if t == 0 else zf(outs[t - 1])
            for w in range(W):
                pr = es[w] * qkv_v[2, t, pl.ds(PAD + r - DIL * w, 8), :]
                a = pr if a is None else a + pr
            outs.append(a)
        return jnp.concatenate(outs, axis=1), zf(outs[-1])

    def pair_body(p, _):
        z = z_v[...]
        last = p == HP - 1
        rb = pl.multiple_of(p * TL, TL)
        dep, obs = None, []
        for k in range(TL // 8):
            ob, dep = local_attn(rb + k * 8, z, dep)
            obs.append(ob)
        ob = jnp.concatenate(obs, axis=0).astype(BF16)

        wk, wv = _split_pair(wuk_p[p]), _split_pair(wuv_p[p])
        _st(k_s, 0, jnp.dot(_ld(ckv_v, 0, S), wk, preferred_element_type=F32).astype(BF16))
        _st(v_s, 0, jnp.dot(_ld(ckv_v, 0, S), wv, preferred_element_type=F32).astype(BF16))

        wqw = wq_p[p]
        wq = _split_pair(jnp.concatenate([wqw[:8] | _zero_after(z, ob[TL - 16:]), wqw[8:]], axis=0))
        row = lax.broadcasted_iota(jnp.int32, (TQ, TQ), 0)
        col = lax.broadcasted_iota(jnp.int32, (TQ, TQ), 1)
        causal = col <= row

        def qproj(i):
            xc = jnp.concatenate([_ld(x_v.at[k], i * TQ, TQ) for k in range(NK)], axis=1)
            q = jnp.dot(xc, wq, preferred_element_type=F32) * qscale
            _st(q_s, i * TQ, q.astype(BF16))

        def qk(i, hh):
            cs = slice(hh * D, (hh + 1) * D)
            return lax.dot_general(_ld(q_s, i * TQ, TQ, cs), _ld(k_s, 0, (i + 1) * TQ, cs), NT,
                                   preferred_element_type=F32)

        ldep = [None]

        def softmax_pv(i, hh, s):
            cs = slice(hh * D, (hh + 1) * D)
            r0 = i * TQ
            sd = jnp.where(causal, s[:, r0:], NEG)
            s = jnp.concatenate([s[:, :r0], sd], axis=1) if i > 0 else sd
            e = jnp.exp2(s - jnp.max(s, axis=1, keepdims=True))
            if i > 2:
                lp, ldep[0] = _chain_sum(e, z, ldep[0])
                l = jnp.sum(lp, axis=1, keepdims=True)
            else:
                l = jnp.sum(e, axis=1, keepdims=True)
            o = jnp.dot(e.astype(BF16), _ld(v_s, 0, r0 + TQ, cs), preferred_element_type=F32)
            return o * (g_v[r0:r0 + TQ, :] * _recip(l))

        def oproj(i, o0, o1):
            r0 = i * TQ
            y = acc_v[r0:r0 + TQ, :] + jnp.dot(jnp.concatenate([o0, o1], axis=1).astype(BF16),
                                               _ld(wo_v, p * (2 * D), 2 * D), preferred_element_type=F32)
            acc_v[r0:r0 + TQ, :] = y
            if r0 != S - TL:
                o_st[r0:r0 + TQ, :] = y.astype(BF16)
                pl.when(last)(cp_o(r0, TQ).start)

        nq = S // TQ
        items = [(i, hh) for i in reversed(range(nq)) for hh in range(2)]
        n = len(items)
        s_vals, o_vals = {}, {}
        qproj(nq - 1)
        for step in range(n + LOOK + OLAG):
            if step % 2 == 0 and nq - 2 - step // 2 >= 0:
                qproj(nq - 2 - step // 2)
            if step < n:
                s_vals[step] = qk(*items[step])
            b = step - LOOK
            if 0 <= b < n:
                o_vals[b] = softmax_pv(*items[b], s_vals.pop(b))
            c = step - LOOK - OLAG
            if 0 <= c < n and c % 2 == 1:
                oproj(items[c][0], o_vals.pop(c - 1), o_vals.pop(c))

        wop = jnp.concatenate([f(bwo_p[dp]) for dp in range(DH // 2) for f in (_lo, _hi)], axis=0).astype(BF16)
        y = acc_v[pl.ds(rb, TL), :] + jnp.dot(ob, wop, preferred_element_type=F32)
        acc_v[pl.ds(rb, TL), :] = y
        for c0, c1 in zip(OCUT[:-1], OCUT[1:]):
            o_st[S - TL:S, c0:c1] = y[:, c0:c1].astype(BF16)
            pl.when(last)(cp_o(S - TL, TL, c0, c1).start)
        return 0

    for cc in ([cp_w0(0), cp_x(0), cp_w0(1), cp_x(1), cp_x(2), cp_w(1), cp_g, cp_x(3), cp_w(2)]
               + [cp_x(i) for i in range(4, 8)] + [cp_w(u) for u in range(3, NTASK)] + a_early):
        cc.start()
    z_v[...] = jnp.zeros((8, 128), U32)
    for part in range(3):
        for t in range(NT_M):
            qkv_v[part, t, 0:PAD, :] = jnp.zeros((PAD, 128), F32)

    def phases():
        first_task()
        lax.fori_loop(1, NTASK, _scoped("bproj", bproj_body), 0)
        for cc in a_waits:
            cc.wait()
        lax.fori_loop(0, HP, _scoped("pair", pair_body), 0)

    def once(i, _):
        pl.when(i == 0)(phases)
        return 0

    lax.fori_loop(0, 2, once, 0)
    with _scope("ow"):
        cp_o(0, S).wait()


def _kernel(*refs):
    dma = pltpu.SemaphoreType.DMA
    pl.run_scoped(functools.partial(_body, *refs), dma((9,)), dma((NTASK + 1,)), dma(()), dma(()))


@jax.jit
def pallas_gated_mix__compressed_kv_cla__sliding_local_dilated__prompt_kernel(
    A_x, A_c_kv, A_w_q, A_w_uk, A_w_uv, A_w_o, B_x, B_wqkv, B_wo, gate_w,
):
    del B_x
    x = A_x.reshape(S, M)
    ckv = A_c_kv.reshape(S, DC)
    wo = A_w_o.reshape(H * D, M)
    bwo = B_wo.reshape(H, DH, M)
    any_spec = pl.BlockSpec(memory_space=pl.ANY)
    out = pl.pallas_call(
        _kernel,
        out_shape=jax.ShapeDtypeStruct((S, M), BF16),
        in_specs=[any_spec] * 9,
        out_specs=any_spec,
        scratch_shapes=[
            pltpu.VMEM((NK, S // 2, KB), U32),
            pltpu.VMEM((S // 2, DC), U32),
            pltpu.VMEM((HP, M, D), U32),
            pltpu.VMEM((HP, DC, D), U32),
            pltpu.VMEM((HP, DC, D), U32),
            pltpu.VMEM((H * D // 2, M), U32),
            pltpu.VMEM((M, 3 * M), BF16),
            pltpu.VMEM((DH // 2, H, M), U32),
            pltpu.VMEM((2, DH * 24, 128), U32),
            pltpu.VMEM((2, DH * 24, 128), U32),
            pltpu.VMEM((KB // 2, 256), U32),
            pltpu.VMEM((3, NT_M, S + PAD, 128), F32),
            pltpu.VMEM((S, M), F32),
            pltpu.VMEM((S, 128), F32),
            pltpu.VMEM((8, 128), U32),
            pltpu.VMEM((S // 2, 2 * D), U32),
            pltpu.VMEM((S // 2, 2 * D), U32),
            pltpu.VMEM((S // 2, 2 * D), U32),
            pltpu.VMEM((S, M), BF16),
            pltpu.VMEM((M,), BF16),
        ],
        compiler_params=pltpu.CompilerParams(vmem_limit_bytes=110 * 1024 * 1024),
    )(x, ckv, A_w_q, A_w_uk, A_w_uv, wo, B_wqkv, bwo, gate_w)
    return out.reshape(1, S, M)
```

```python
import contextlib
import functools

import jax
import jax.numpy as jnp
from jax import lax
import jax.experimental.pallas as pl
import jax.experimental.pallas.tpu as pltpu

S = 2048
M = 1024
DC = 512
H = 32
HP = H // 2
D = 128
DH = 32
W = 8
DIL = 2
PAD = 16
NT_M = M // 128
TQ = 128
TL = S // HP
R1 = 768
GR = 304
PITCH = 17
NA1 = 36
OCUT = (0, 512, 768, M)
LOOK = 2
OLAG = 10
SUMG = 16
LAQ = 2
LOG2E = 1.4426950408889634
NEG = -1e9

F32 = jnp.float32
BF16 = jnp.bfloat16
U32 = jnp.uint32
NT = (((1,), (1,)), ((), ()))


_PROFILE = False


def _scope(name):
    return jax.named_scope(name) if _PROFILE else contextlib.nullcontext()


def _scoped(name, body):
    def f(i, c):
        with _scope(name):
            return body(i, c)
    return f


def _recip(l):
    r = pl.reciprocal(l, approx=True)
    return r * (2.0 - l * r)


def _lo(w):
    return pltpu.bitcast(w << 16, F32)


def _hi(w):
    return pltpu.bitcast(w & jnp.uint32(0xFFFF0000), F32)


def _split_pair(w):
    return jnp.concatenate([_lo(w), _hi(w)], axis=1).astype(BF16)


def _ld(ref, r0, n, cols=slice(None)):
    if isinstance(r0, int):
        rs = slice(r0 // 2, (r0 + n) // 2)
    else:
        rs = pl.ds(pl.multiple_of(lax.shift_right_logical(r0, 1), 8), n // 2)
    return pltpu.bitcast(ref[rs, cols], BF16)


def _st(ref, r0, val, cols=slice(None)):
    ref[r0 // 2:(r0 + val.shape[0]) // 2, cols] = pltpu.bitcast(val, U32)


def _zero_after(z, *vals):
    acc = None
    for v in vals:
        b = pltpu.bitcast(v, U32)
        for r in range(0, b.shape[0], 8):
            for c in range(0, b.shape[1], 128):
                t = b[r:r + 8, c:c + 128]
                acc = t if acc is None else acc | t
    return acc & z


def _chain_sum(x, z, dep):
    parts = []
    for r in range(0, x.shape[0], SUMG):
        a = x[r:r + SUMG, 0:128]
        if dep is not None:
            a = pltpu.bitcast(pltpu.bitcast(a, U32) | jnp.concatenate([dep] * (SUMG // 8), axis=0), F32)
        for c in range(128, x.shape[1], 128):
            a = a + x[r:r + SUMG, c:c + 128]
        dep = _zero_after(z, a)
        parts.append(a)
    return jnp.concatenate(parts, axis=0), dep


def _body(x_hbm, ckv_hbm, wq_hbm, wuk_hbm, wuv_hbm, wo_hbm, bqkv_hbm, bwo_hbm, gate_hbm,
          out_hbm,
          x_v, ckv_v, wq_p, wuk_p, wuv_p, wo_v, bqkv_v, bwo_p, wcur_v, wfst_v,
          qkv_v, acc_v, g_v, z_v, q_s, k_s, v_s, o_st, gate_v,
          sem_x, sem_w, sem_a, sem_o):
    def cp_x(sm, r0, r1, c0, c1):
        sl = (pl.ds(r0 // 2, (r1 - r0) // 2), pl.ds(c0, c1 - c0))
        return pltpu.make_async_copy(x_hbm.bitcast(U32).at[sl], x_v.at[sl], sem_x.at[sm])

    def cp_w(k, c0=0, c1=3 * M, sm=None):
        sl = (pl.ds(k * 128, 128), pl.ds(c0, c1 - c0))
        return pltpu.make_async_copy(bqkv_hbm.at[sl], bqkv_v.at[sl], sem_w.at[k if sm is None else sm])

    x0a, x0b, xr = cp_x(0, 0, R1, 0, 128), cp_x(1, R1, S, 0, 128), cp_x(2, 0, S, 128, M)
    w0a, w0b, w0c = cp_w(0, 0, M), cp_w(0, M, 2 * M, NT_M), cp_w(0, 2 * M, 3 * M, NT_M + 1)
    cp_g = pltpu.make_async_copy(gate_hbm, gate_v, sem_x.at[3])

    def cp_pairs(src, dst):
        return [pltpu.make_async_copy(src.bitcast(U32).at[:, p, :], dst.at[p], sem_a) for p in range(HP)]

    a_early = cp_pairs(bwo_hbm, bwo_p) + [pltpu.make_async_copy(ckv_hbm.bitcast(U32), ckv_v, sem_a),
                                          pltpu.make_async_copy(wo_hbm.bitcast(U32), wo_v, sem_a)]
    a_late = cp_pairs(wuk_hbm, wuk_p) + cp_pairs(wuv_hbm, wuv_p) + cp_pairs(wq_hbm, wq_p)
    a_waits = [pltpu.make_async_copy(b, b, sem_a) for b in (ckv_v, wo_v, wuk_p, wuv_p, wq_p, bwo_p)]

    def cp_o(r0, n, c0=0, c1=M):
        sl = (pl.ds(r0, n), pl.ds(c0, c1 - c0))
        return pltpu.make_async_copy(o_st.at[sl], out_hbm.at[sl], sem_o)

    def prep(part, j, z=None, dep=None):
        k0 = j * 128 if isinstance(j, int) else pl.multiple_of(j * 128, 128)
        for c in range(NT_M):
            src = bqkv_v[pl.ds(k0, 128), part * M + c * 128:part * M + (c + 1) * 128]
            if dep is not None:
                top = pltpu.bitcast(pltpu.bitcast(src[:16], U32) | dep, BF16)
                src = jnp.concatenate([top, src[16:]], axis=0)
            t = pltpu.bitcast(src.T, U32)
            for hp in range(2):
                a, b = t[32 * hp:32 * hp + 16], t[32 * hp + 16:32 * hp + 32]
                r = 2 * c + hp
                wcur_v[part, pl.ds(r, 16, stride=2 * PITCH), :] = (a & jnp.uint32(0xFFFF)) | (b << 16)
                wcur_v[part, pl.ds(PITCH + r, 16, stride=2 * PITCH), :] = (a >> 16) | (b & jnp.uint32(0xFFFF0000))
            if z is not None:
                dep = _zero_after(z, t[56:64])
        return dep

    def wrows(part, d0, d1):
        w = jnp.concatenate([wcur_v[part, d * PITCH:d * PITCH + HP, :] for d in range(d0, d1)], axis=0)
        return pltpu.bitcast(w, BF16)

    def first_tiles():
        for n in range(4):
            _st(wfst_v, 0, wrows(0, 4 * n, 4 * n + 4).T, slice(n * 128, (n + 1) * 128))

    def gate_rows(t, z, dep):
        gw = gate_v[...].astype(F32).reshape(1, M)
        g0 = jnp.minimum((t - 1) * GR, S - GR)
        for k in range(GR // 16):
            rr = pl.multiple_of(g0 + k * 16, 16)
            rw = pl.multiple_of(lax.shift_right_logical(rr, 1), 8)
            xb = x_v[pl.ds(rw, 8), :]
            if dep is not None:
                xb = xb | jnp.concatenate([dep] * NT_M, axis=1)
            xx = pltpu.bitcast(xb, BF16).astype(F32)
            zz = jnp.sum(xx * gw, axis=1, keepdims=True)
            g = jnp.broadcast_to(1.0 / (1.0 + jnp.exp(-zz)), (16, 128))
            g_v[pl.ds(rr, 16), :] = g
            acc_v[pl.ds(rr, 16), :] = jnp.zeros((16, M), F32)
            dep = _zero_after(z, g)

    def first_task():
        def piece(part, r0, r1):
            y = lax.dot_general(_ld(x_v, r0, r1 - r0, slice(0, 128)), wrows(part, 0, DH), NT, preferred_element_type=F32)
            for tt in range(NT_M):
                qkv_v[part, tt, PAD + r0:PAD + r1, :] = y[:, tt * 128:(tt + 1) * 128]

        with _scope("prep0"):
            w0a.wait()
            prep(0, 0)
        with _scope("b1"):
            x0a.wait()
            piece(0, 0, R1)
        with _scope("b2"):
            x0b.wait()
            w0b.wait()
            piece(0, R1, S)
            prep(1, 0)
        with _scope("b3"):
            w0c.wait()
            cp_w(1).wait()
            z = z_v[...]
            piece(1, 0, S)
            prep(2, 0)
            dep = prep(0, 1, z)
            first_tiles()
            piece(2, 0, S)
            prep(1, 1, z, dep)
            prep(2, 1)
            for cc in a_late[:NA1]:
                cc.start()
        for cc in (xr, cp_g):
            cc.wait()
        for cc in a_late[NA1:]:
            cc.start()

    def bproj_body(t, _):
        @pl.when(t < NT_M - 1)
        def _():
            cp_w(t + 1).wait()

        z = z_v[...]
        u = jnp.minimum(t + 1, NT_M - 1)
        xw = x_v[:, pl.ds(pl.multiple_of(t * 128, 128), 128)]
        xk = pltpu.bitcast(xw | jnp.concatenate([z] * (S // 16), axis=0), BF16)
        dep = None
        for part in range(3):
            if part == 0:
                y = jnp.concatenate([jnp.dot(xk, _ld(wfst_v, 0, 128), preferred_element_type=F32),
                                     lax.dot_general(xk, wrows(0, DH // 2, DH), NT, preferred_element_type=F32)], axis=1)
            else:
                y = lax.dot_general(xk, wrows(part, 0, DH), NT, preferred_element_type=F32)
            for tt in range(NT_M):
                qkv_v[part, tt, PAD:, :] = qkv_v[part, tt, PAD:, :] + y[:, tt * 128:(tt + 1) * 128]
            dep = prep(part, u, z, dep) if part < 2 else prep(part, u)
            if part == 0:
                first_tiles()
        gate_rows(t, z, None)
        return 0

    qscale = (D ** -0.5) * LOG2E
    bscale = (DH ** -0.5) * LOG2E

    def local_attn(r, z, dep):
        def zf(v):
            return pltpu.bitcast(_zero_after(z, v), F32)

        sc = jnp.full((8, 128), bscale, F32)
        if dep is not None:
            sc = sc + dep
        q = [qkv_v[0, t, pl.ds(PAD + r, 8), :] * sc for t in range(NT_M)]
        rowi = r + lax.broadcasted_iota(jnp.int32, (8, 128), 0)
        logits, raw = [], []
        for w in range(W):
            a = None if w < LAQ else zf(raw[w - LAQ])
            for t in range(NT_M):
                pr = q[t] * qkv_v[1, t, pl.ds(PAD + r - DIL * w, 8), :]
                a = pr if a is None else a + pr
            raw.append(a)
            a = a + pltpu.roll(a, 64, 1)
            a = a + pltpu.roll(a, 32, 1)
            logits.append(jnp.where(rowi >= DIL * w, a, NEG) if w > 0 else a)
        m = functools.reduce(jnp.maximum, logits)
        es = [jnp.exp2(lg - m) for lg in logits]
        l = functools.reduce(lambda a, b: a + b, es)
        f = (1.0 - g_v[pl.ds(r, 8), :]) * _recip(l)
        es = [e * f for e in es]
        outs = []
        for t in range(NT_M):
            a = None if t == 0 else zf(outs[t - 1])
            for w in range(W):
                pr = es[w] * qkv_v[2, t, pl.ds(PAD + r - DIL * w, 8), :]
                a = pr if a is None else a + pr
            outs.append(a)
        return jnp.concatenate(outs, axis=1), zf(outs[-1])

    def pair_body(p, _):
        z = z_v[...]
        last = p == HP - 1
        rb = pl.multiple_of(p * TL, TL)
        dep, obs = None, []
        for k in range(TL // 8):
            ob, dep = local_attn(rb + k * 8, z, dep)
            obs.append(ob)
        ob = jnp.concatenate(obs, axis=0).astype(BF16)

        wk, wv = _split_pair(wuk_p[p]), _split_pair(wuv_p[p])
        _st(k_s, 0, jnp.dot(_ld(ckv_v, 0, S), wk, preferred_element_type=F32).astype(BF16))
        _st(v_s, 0, jnp.dot(_ld(ckv_v, 0, S), wv, preferred_element_type=F32).astype(BF16))

        wqw = wq_p[p]
        wq = _split_pair(jnp.concatenate([wqw[:8] | _zero_after(z, ob[TL - 16:]), wqw[8:]], axis=0))
        row = lax.broadcasted_iota(jnp.int32, (TQ, TQ), 0)
        col = lax.broadcasted_iota(jnp.int32, (TQ, TQ), 1)
        causal = col <= row

        def qproj(i):
            xc = _ld(x_v, i * TQ, TQ)
            q = jnp.dot(xc, wq, preferred_element_type=F32) * qscale
            _st(q_s, i * TQ, q.astype(BF16))

        def qk(i, hh):
            cs = slice(hh * D, (hh + 1) * D)
            return lax.dot_general(_ld(q_s, i * TQ, TQ, cs), _ld(k_s, 0, (i + 1) * TQ, cs), NT,
                                   preferred_element_type=F32)

        ldep = [None]

        def softmax_pv(i, hh, s):
            cs = slice(hh * D, (hh + 1) * D)
            r0 = i * TQ
            sd = jnp.where(causal, s[:, r0:], NEG)
            s = jnp.concatenate([s[:, :r0], sd], axis=1) if i > 0 else sd
            e = jnp.exp2(s - jnp.max(s, axis=1, keepdims=True))
            if i > 2:
                lp, ldep[0] = _chain_sum(e, z, ldep[0])
                l = jnp.sum(lp, axis=1, keepdims=True)
            else:
                l = jnp.sum(e, axis=1, keepdims=True)
            o = jnp.dot(e.astype(BF16), _ld(v_s, 0, r0 + TQ, cs), preferred_element_type=F32)
            return o * (g_v[r0:r0 + TQ, :] * _recip(l))

        def oproj(i, o0, o1):
            r0 = i * TQ
            y = acc_v[r0:r0 + TQ, :] + jnp.dot(jnp.concatenate([o0, o1], axis=1).astype(BF16),
                                               _ld(wo_v, p * (2 * D), 2 * D), preferred_element_type=F32)
            acc_v[r0:r0 + TQ, :] = y
            if r0 != S - TL:
                o_st[r0:r0 + TQ, :] = y.astype(BF16)
                pl.when(last)(cp_o(r0, TQ).start)

        nq = S // TQ
        items = [(i, hh) for i in reversed(range(nq)) for hh in range(2)]
        n = len(items)
        s_vals, o_vals = {}, {}
        qproj(nq - 1)
        for step in range(n + LOOK + OLAG):
            if step % 2 == 0 and nq - 2 - step // 2 >= 0:
                qproj(nq - 2 - step // 2)
            if step < n:
                s_vals[step] = qk(*items[step])
            b = step - LOOK
            if 0 <= b < n:
                o_vals[b] = softmax_pv(*items[b], s_vals.pop(b))
            c = step - LOOK - OLAG
            if 0 <= c < n and c % 2 == 1:
                oproj(items[c][0], o_vals.pop(c - 1), o_vals.pop(c))

        wop = jnp.concatenate([f(bwo_p[dp]) for dp in range(DH // 2) for f in (_lo, _hi)], axis=0).astype(BF16)
        y = acc_v[pl.ds(rb, TL), :] + jnp.dot(ob, wop, preferred_element_type=F32)
        acc_v[pl.ds(rb, TL), :] = y
        for c0, c1 in zip(OCUT[:-1], OCUT[1:]):
            o_st[S - TL:S, c0:c1] = y[:, c0:c1].astype(BF16)
            pl.when(last)(cp_o(S - TL, TL, c0, c1).start)
        return 0

    for cc in [w0a, x0a, x0b, w0b, w0c, cp_w(1), cp_g, xr] + [cp_w(k) for k in range(2, NT_M)] + a_early:
        cc.start()
    z_v[...] = jnp.zeros((8, 128), U32)
    for part in range(3):
        for t in range(NT_M):
            qkv_v[part, t, 0:PAD, :] = jnp.zeros((PAD, 128), F32)

    def phases():
        first_task()
        lax.fori_loop(1, NT_M, _scoped("bproj", bproj_body), 0)
        for cc in a_waits:
            cc.wait()
        lax.fori_loop(0, HP, _scoped("pair", pair_body), 0)

    def once(i, _):
        pl.when(i == 0)(phases)
        return 0

    lax.fori_loop(0, 2, once, 0)
    with _scope("ow"):
        cp_o(0, S).wait()


def _kernel(*refs):
    dma = pltpu.SemaphoreType.DMA
    pl.run_scoped(functools.partial(_body, *refs), dma((4,)), dma((NT_M + 2,)), dma(()), dma(()))


@jax.jit
def pallas_gated_mix__compressed_kv_cla__sliding_local_dilated__prompt_kernel(
    A_x, A_c_kv, A_w_q, A_w_uk, A_w_uv, A_w_o, B_x, B_wqkv, B_wo, gate_w,
):
    del B_x
    x = A_x.reshape(S, M)
    ckv = A_c_kv.reshape(S, DC)
    wo = A_w_o.reshape(H * D, M)
    bwo = B_wo.reshape(H, DH, M)
    any_spec = pl.BlockSpec(memory_space=pl.ANY)
    out = pl.pallas_call(
        _kernel,
        out_shape=jax.ShapeDtypeStruct((S, M), BF16),
        in_specs=[any_spec] * 9,
        out_specs=any_spec,
        scratch_shapes=[
            pltpu.VMEM((S // 2, M), U32),
            pltpu.VMEM((S // 2, DC), U32),
            pltpu.VMEM((HP, M, D), U32),
            pltpu.VMEM((HP, DC, D), U32),
            pltpu.VMEM((HP, DC, D), U32),
            pltpu.VMEM((H * D // 2, M), U32),
            pltpu.VMEM((M, 3 * M), BF16),
            pltpu.VMEM((DH // 2, H, M), U32),
            pltpu.VMEM((3, DH * 24, 128), U32),
            pltpu.VMEM((64, 512), U32),
            pltpu.VMEM((3, NT_M, S + PAD, 128), F32),
            pltpu.VMEM((S, M), F32),
            pltpu.VMEM((S, 128), F32),
            pltpu.VMEM((8, 128), U32),
            pltpu.VMEM((S // 2, 2 * D), U32),
            pltpu.VMEM((S // 2, 2 * D), U32),
            pltpu.VMEM((S // 2, 2 * D), U32),
            pltpu.VMEM((S, M), BF16),
            pltpu.VMEM((M,), BF16),
        ],
        compiler_params=pltpu.CompilerParams(vmem_limit_bytes=110 * 1024 * 1024),
    )(x, ckv, A_w_q, A_w_uk, A_w_uv, wo, B_wqkv, bwo, gate_w)
    return out.reshape(1, S, M)
```

```python
import contextlib
import functools

import jax
import jax.numpy as jnp
from jax import lax
import jax.experimental.pallas as pl
import jax.experimental.pallas.tpu as pltpu

S = 2048
M = 1024
DC = 512
H = 32
HP = H // 2
D = 128
DH = 32
W = 8
DIL = 2
PAD = 16
NT_M = M // 128
TQ = 128
TL = S // HP
R1 = 768
GR = 304
PITCH = 17
NA1 = 44
OCUT = (0, 512, 768, M)
LOOK = 2
OLAG = 10
SUMG = 16
LAQ = 2
LOG2E = 1.4426950408889634
NEG = -1e9

F32 = jnp.float32
BF16 = jnp.bfloat16
U32 = jnp.uint32
NT = (((1,), (1,)), ((), ()))


_PROFILE = False


def _scope(name):
    return jax.named_scope(name) if _PROFILE else contextlib.nullcontext()


def _scoped(name, body):
    def f(i, c):
        with _scope(name):
            return body(i, c)
    return f


def _recip(l):
    r = pl.reciprocal(l, approx=True)
    return r * (2.0 - l * r)


def _lo(w):
    return pltpu.bitcast(w << 16, F32)


def _hi(w):
    return pltpu.bitcast(w & jnp.uint32(0xFFFF0000), F32)


def _split_pair(w):
    return jnp.concatenate([_lo(w), _hi(w)], axis=1).astype(BF16)


def _ld(ref, r0, n, cols=slice(None)):
    if isinstance(r0, int):
        rs = slice(r0 // 2, (r0 + n) // 2)
    else:
        rs = pl.ds(pl.multiple_of(lax.shift_right_logical(r0, 1), 8), n // 2)
    return pltpu.bitcast(ref[rs, cols], BF16)


def _st(ref, r0, val, cols=slice(None)):
    ref[r0 // 2:(r0 + val.shape[0]) // 2, cols] = pltpu.bitcast(val, U32)


def _zero_after(z, *vals):
    acc = None
    for v in vals:
        b = pltpu.bitcast(v, U32)
        for r in range(0, b.shape[0], 8):
            for c in range(0, b.shape[1], 128):
                t = b[r:r + 8, c:c + 128]
                acc = t if acc is None else acc | t
    return acc & z


def _chain_sum(x, z, dep):
    parts = []
    for r in range(0, x.shape[0], SUMG):
        a = x[r:r + SUMG, 0:128]
        if dep is not None:
            a = pltpu.bitcast(pltpu.bitcast(a, U32) | jnp.concatenate([dep] * (SUMG // 8), axis=0), F32)
        for c in range(128, x.shape[1], 128):
            a = a + x[r:r + SUMG, c:c + 128]
        dep = _zero_after(z, a)
        parts.append(a)
    return jnp.concatenate(parts, axis=0), dep


def _body(x_hbm, ckv_hbm, wq_hbm, wuk_hbm, wuv_hbm, wo_hbm, bqkv_hbm, bwo_hbm, gate_hbm,
          out_hbm,
          x_v, ckv_v, wq_p, wuk_p, wuv_p, wo_v, bqkv_v, bwo_p, wcur_v, wfst_v,
          qkv_v, acc_v, g_v, z_v, q_s, k_s, v_s, o_st, gate_v,
          sem_x, sem_w, sem_a, sem_o):
    def cp_x(sm, r0, r1, c0, c1):
        sl = (pl.ds(r0 // 2, (r1 - r0) // 2), pl.ds(c0, c1 - c0))
        return pltpu.make_async_copy(x_hbm.bitcast(U32).at[sl], x_v.at[sl], sem_x.at[sm])

    def cp_w(k, c0=0, c1=3 * M, sm=None):
        sl = (pl.ds(k * 128, 128), pl.ds(c0, c1 - c0))
        return pltpu.make_async_copy(bqkv_hbm.at[sl], bqkv_v.at[sl], sem_w.at[k if sm is None else sm])

    x0a, x0b, xr = cp_x(0, 0, R1, 0, 128), cp_x(1, R1, S, 0, 128), cp_x(2, 0, S, 128, M)
    w0a, w0b, w0c = cp_w(0, 0, M), cp_w(0, M, 2 * M, NT_M), cp_w(0, 2 * M, 3 * M, NT_M + 1)
    cp_g = pltpu.make_async_copy(gate_hbm, gate_v, sem_x.at[3])

    def cp_pairs(src, dst):
        return [pltpu.make_async_copy(src.bitcast(U32).at[:, p, :], dst.at[p], sem_a) for p in range(HP)]

    a_early = cp_pairs(bwo_hbm, bwo_p) + [pltpu.make_async_copy(ckv_hbm.bitcast(U32), ckv_v, sem_a),
                                          pltpu.make_async_copy(wo_hbm.bitcast(U32), wo_v, sem_a)]
    a_late = cp_pairs(wuk_hbm, wuk_p) + cp_pairs(wuv_hbm, wuv_p) + cp_pairs(wq_hbm, wq_p)
    a_waits = [pltpu.make_async_copy(b, b, sem_a) for b in (ckv_v, wo_v, wuk_p, wuv_p, wq_p, bwo_p)]

    def cp_o(r0, n, c0=0, c1=M):
        sl = (pl.ds(r0, n), pl.ds(c0, c1 - c0))
        return pltpu.make_async_copy(o_st.at[sl], out_hbm.at[sl], sem_o)

    def prep(part, j, z=None, dep=None):
        k0 = j * 128 if isinstance(j, int) else pl.multiple_of(j * 128, 128)
        for c in range(NT_M):
            src = bqkv_v[pl.ds(k0, 128), part * M + c * 128:part * M + (c + 1) * 128]
            if dep is not None:
                top = pltpu.bitcast(pltpu.bitcast(src[:16], U32) | dep, BF16)
                src = jnp.concatenate([top, src[16:]], axis=0)
            t = pltpu.bitcast(src.T, U32)
            for hp in range(2):
                a, b = t[32 * hp:32 * hp + 16], t[32 * hp + 16:32 * hp + 32]
                r = 2 * c + hp
                wcur_v[part, pl.ds(r, 16, stride=2 * PITCH), :] = (a & jnp.uint32(0xFFFF)) | (b << 16)
                wcur_v[part, pl.ds(PITCH + r, 16, stride=2 * PITCH), :] = (a >> 16) | (b & jnp.uint32(0xFFFF0000))
            if z is not None:
                dep = _zero_after(z, t[56:64])
        return dep

    def wrows(part, d0, d1):
        w = jnp.concatenate([wcur_v[part, d * PITCH:d * PITCH + HP, :] for d in range(d0, d1)], axis=0)
        return pltpu.bitcast(w, BF16)

    def first_tiles(part):
        for n in range(4):
            _st(wfst_v, 0, wrows(part, 4 * n, 4 * n + 4).T, slice(n * 128, (n + 1) * 128))

    def project(xk, part, first):
        if not first:
            return lax.dot_general(xk, wrows(part, 0, DH), NT, preferred_element_type=F32)
        return jnp.concatenate([jnp.dot(xk, _ld(wfst_v, 0, 128), preferred_element_type=F32),
                                lax.dot_general(xk, wrows(part, DH // 2, DH), NT, preferred_element_type=F32)], axis=1)

    def gate_rows(t, z, dep):
        gw = gate_v[...].astype(F32).reshape(1, M)
        g0 = jnp.minimum((t - 1) * GR, S - GR)
        for k in range(GR // 16):
            rr = pl.multiple_of(g0 + k * 16, 16)
            rw = pl.multiple_of(lax.shift_right_logical(rr, 1), 8)
            xb = x_v[pl.ds(rw, 8), :]
            if dep is not None:
                xb = xb | jnp.concatenate([dep] * NT_M, axis=1)
            xx = pltpu.bitcast(xb, BF16).astype(F32)
            zz = jnp.sum(xx * gw, axis=1, keepdims=True)
            g = jnp.broadcast_to(1.0 / (1.0 + jnp.exp(-zz)), (16, 128))
            g_v[pl.ds(rr, 16), :] = g
            acc_v[pl.ds(rr, 16), :] = jnp.zeros((16, M), F32)
            dep = _zero_after(z, g)

    def first_task():
        def piece(part, r0, r1, first):
            y = project(_ld(x_v, r0, r1 - r0, slice(0, 128)), part, first)
            for tt in range(NT_M):
                qkv_v[part, tt, PAD + r0:PAD + r1, :] = y[:, tt * 128:(tt + 1) * 128]

        with _scope("prep0"):
            w0a.wait()
            prep(0, 0)
        with _scope("b1"):
            x0a.wait()
            piece(0, 0, R1, False)
            first_tiles(0)
        with _scope("b2"):
            x0b.wait()
            w0b.wait()
            piece(0, R1, S, True)
            prep(1, 0)
            first_tiles(1)
        with _scope("b3"):
            w0c.wait()
            cp_w(1).wait()
            z = z_v[...]
            piece(1, 0, S, True)
            prep(2, 0)
            dep = prep(0, 1, z)
            first_tiles(0)
            piece(2, 0, S, False)
            prep(1, 1, z, dep)
            prep(2, 1)
            for cc in a_late[:NA1]:
                cc.start()
        for cc in (xr, cp_g):
            cc.wait()
        for cc in a_late[NA1:]:
            cc.start()

    def bproj_body(t, _):
        @pl.when(t < NT_M - 1)
        def _():
            cp_w(t + 1).wait()

        z = z_v[...]
        u = jnp.minimum(t + 1, NT_M - 1)
        xw = x_v[:, pl.ds(pl.multiple_of(t * 128, 128), 128)]
        xk = pltpu.bitcast(xw | jnp.concatenate([z] * (S // 16), axis=0), BF16)
        dep = None
        for part in range(3):
            y = project(xk, part, part == 0)
            for tt in range(NT_M):
                qkv_v[part, tt, PAD:, :] = qkv_v[part, tt, PAD:, :] + y[:, tt * 128:(tt + 1) * 128]
            dep = prep(part, u, z, dep) if part < 2 else prep(part, u)
            if part == 0:
                first_tiles(0)
        gate_rows(t, z, None)
        return 0

    qscale = (D ** -0.5) * LOG2E
    bscale = (DH ** -0.5) * LOG2E

    def local_attn(r, z, dep):
        def zf(v):
            return pltpu.bitcast(_zero_after(z, v), F32)

        sc = jnp.full((8, 128), bscale, F32)
        if dep is not None:
            sc = sc + dep
        q = [qkv_v[0, t, pl.ds(PAD + r, 8), :] * sc for t in range(NT_M)]
        rowi = r + lax.broadcasted_iota(jnp.int32, (8, 128), 0)
        logits, raw = [], []
        for w in range(W):
            a = None if w < LAQ else zf(raw[w - LAQ])
            for t in range(NT_M):
                pr = q[t] * qkv_v[1, t, pl.ds(PAD + r - DIL * w, 8), :]
                a = pr if a is None else a + pr
            raw.append(a)
            a = a + pltpu.roll(a, 64, 1)
            a = a + pltpu.roll(a, 32, 1)
            logits.append(jnp.where(rowi >= DIL * w, a, NEG) if w > 0 else a)
        m = functools.reduce(jnp.maximum, logits)
        es = [jnp.exp2(lg - m) for lg in logits]
        l = functools.reduce(lambda a, b: a + b, es)
        f = (1.0 - g_v[pl.ds(r, 8), :]) * _recip(l)
        es = [e * f for e in es]
        outs = []
        for t in range(NT_M):
            a = None if t == 0 else zf(outs[t - 1])
            for w in range(W):
                pr = es[w] * qkv_v[2, t, pl.ds(PAD + r - DIL * w, 8), :]
                a = pr if a is None else a + pr
            outs.append(a)
        return jnp.concatenate(outs, axis=1), zf(outs[-1])

    def pair_body(p, _):
        z = z_v[...]
        last = p == HP - 1
        wk, wv = _split_pair(wuk_p[p]), _split_pair(wuv_p[p])
        _st(k_s, 0, jnp.dot(_ld(ckv_v, 0, S), wk, preferred_element_type=F32).astype(BF16))
        _st(v_s, 0, jnp.dot(_ld(ckv_v, 0, S), wv, preferred_element_type=F32).astype(BF16))

        rb = pl.multiple_of(p * TL, TL)
        dep, obs = None, []
        for k in range(TL // 8):
            ob, dep = local_attn(rb + k * 8, z, dep)
            obs.append(ob)
        ob = jnp.concatenate(obs, axis=0).astype(BF16)

        wqw = wq_p[p]
        wq = _split_pair(jnp.concatenate([wqw[:8] | _zero_after(z, ob[TL - 16:]), wqw[8:]], axis=0))
        row = lax.broadcasted_iota(jnp.int32, (TQ, TQ), 0)
        col = lax.broadcasted_iota(jnp.int32, (TQ, TQ), 1)
        causal = col <= row

        def qproj(i):
            xc = _ld(x_v, i * TQ, TQ)
            q = jnp.dot(xc, wq, preferred_element_type=F32) * qscale
            _st(q_s, i * TQ, q.astype(BF16))

        def qk(i, hh):
            cs = slice(hh * D, (hh + 1) * D)
            return lax.dot_general(_ld(q_s, i * TQ, TQ, cs), _ld(k_s, 0, (i + 1) * TQ, cs), NT,
                                   preferred_element_type=F32)

        ldep = [None]

        def softmax_pv(i, hh, s):
            cs = slice(hh * D, (hh + 1) * D)
            r0 = i * TQ
            sd = jnp.where(causal, s[:, r0:], NEG)
            s = jnp.concatenate([s[:, :r0], sd], axis=1) if i > 0 else sd
            e = jnp.exp2(s - jnp.max(s, axis=1, keepdims=True))
            if i > 2:
                lp, ldep[0] = _chain_sum(e, z, ldep[0])
                l = jnp.sum(lp, axis=1, keepdims=True)
            else:
                l = jnp.sum(e, axis=1, keepdims=True)
            o = jnp.dot(e.astype(BF16), _ld(v_s, 0, r0 + TQ, cs), preferred_element_type=F32)
            return o * (g_v[r0:r0 + TQ, :] * _recip(l))

        def oproj(i, o0, o1):
            r0 = i * TQ
            y = acc_v[r0:r0 + TQ, :] + jnp.dot(jnp.concatenate([o0, o1], axis=1).astype(BF16),
                                               _ld(wo_v, p * (2 * D), 2 * D), preferred_element_type=F32)
            acc_v[r0:r0 + TQ, :] = y
            if r0 != S - TL:
                o_st[r0:r0 + TQ, :] = y.astype(BF16)
                pl.when(last)(cp_o(r0, TQ).start)

        nq = S // TQ
        items = [(i, hh) for i in reversed(range(nq)) for hh in range(2)]
        n = len(items)
        s_vals, o_vals = {}, {}
        qproj(nq - 1)
        for step in range(n + LOOK + OLAG):
            if step % 2 == 0 and nq - 2 - step // 2 >= 0:
                qproj(nq - 2 - step // 2)
            if step < n:
                s_vals[step] = qk(*items[step])
            b = step - LOOK
            if 0 <= b < n:
                o_vals[b] = softmax_pv(*items[b], s_vals.pop(b))
            c = step - LOOK - OLAG
            if 0 <= c < n and c % 2 == 1:
                oproj(items[c][0], o_vals.pop(c - 1), o_vals.pop(c))

        wop = jnp.concatenate([f(bwo_p[dp]) for dp in range(DH // 2) for f in (_lo, _hi)], axis=0).astype(BF16)
        y = acc_v[pl.ds(rb, TL), :] + jnp.dot(ob, wop, preferred_element_type=F32)
        acc_v[pl.ds(rb, TL), :] = y
        for c0, c1 in zip(OCUT[:-1], OCUT[1:]):
            o_st[S - TL:S, c0:c1] = y[:, c0:c1].astype(BF16)
            pl.when(last)(cp_o(S - TL, TL, c0, c1).start)
        return 0

    for cc in [w0a, x0a, x0b, w0b, w0c, cp_w(1), cp_g, xr] + [cp_w(k) for k in range(2, NT_M)] + a_early:
        cc.start()
    z_v[...] = jnp.zeros((8, 128), U32)
    for part in range(3):
        for t in range(NT_M):
            qkv_v[part, t, 0:PAD, :] = jnp.zeros((PAD, 128), F32)

    def phases():
        first_task()
        lax.fori_loop(1, NT_M, _scoped("bproj", bproj_body), 0)
        for cc in a_waits:
            cc.wait()
        lax.fori_loop(0, HP, _scoped("pair", pair_body), 0)

    def once(i, _):
        pl.when(i == 0)(phases)
        return 0

    lax.fori_loop(0, 2, once, 0)
    with _scope("ow"):
        cp_o(0, S).wait()


def _kernel(*refs):
    dma = pltpu.SemaphoreType.DMA
    pl.run_scoped(functools.partial(_body, *refs), dma((4,)), dma((NT_M + 2,)), dma(()), dma(()))


@jax.jit
def pallas_gated_mix__compressed_kv_cla__sliding_local_dilated__prompt_kernel(
    A_x, A_c_kv, A_w_q, A_w_uk, A_w_uv, A_w_o, B_x, B_wqkv, B_wo, gate_w,
):
    del B_x
    x = A_x.reshape(S, M)
    ckv = A_c_kv.reshape(S, DC)
    wo = A_w_o.reshape(H * D, M)
    bwo = B_wo.reshape(H, DH, M)
    any_spec = pl.BlockSpec(memory_space=pl.ANY)
    out = pl.pallas_call(
        _kernel,
        out_shape=jax.ShapeDtypeStruct((S, M), BF16),
        in_specs=[any_spec] * 9,
        out_specs=any_spec,
        scratch_shapes=[
            pltpu.VMEM((S // 2, M), U32),
            pltpu.VMEM((S // 2, DC), U32),
            pltpu.VMEM((HP, M, D), U32),
            pltpu.VMEM((HP, DC, D), U32),
            pltpu.VMEM((HP, DC, D), U32),
            pltpu.VMEM((H * D // 2, M), U32),
            pltpu.VMEM((M, 3 * M), BF16),
            pltpu.VMEM((DH // 2, H, M), U32),
            pltpu.VMEM((3, DH * 24, 128), U32),
            pltpu.VMEM((64, 512), U32),
            pltpu.VMEM((3, NT_M, S + PAD, 128), F32),
            pltpu.VMEM((S, M), F32),
            pltpu.VMEM((S, 128), F32),
            pltpu.VMEM((8, 128), U32),
            pltpu.VMEM((S // 2, 2 * D), U32),
            pltpu.VMEM((S // 2, 2 * D), U32),
            pltpu.VMEM((S // 2, 2 * D), U32),
            pltpu.VMEM((S, M), BF16),
            pltpu.VMEM((M,), BF16),
        ],
        compiler_params=pltpu.CompilerParams(vmem_limit_bytes=110 * 1024 * 1024),
    )(x, ckv, A_w_q, A_w_uk, A_w_uv, wo, B_wqkv, bwo, gate_w)
    return out.reshape(1, S, M)
```

```python
import contextlib
import functools
import itertools

import jax
import jax.numpy as jnp
from jax import lax
import jax.experimental.pallas as pl
import jax.experimental.pallas.tpu as pltpu

S = 2048
M = 1024
DC = 512
H = 32
HP = H // 2
D = 128
DH = 32
W = 8
DIL = 2
PAD = 16
NT_M = M // 128
TQ = 128
TL = S // HP
R1 = 768
GR = 304
PITCH = 17
NA1 = 44
OCUT = (0, 512, 768, M)
LOOK = 2
OLAG = 10
SUMG = 16
LAQ = 2
HQ = TQ // 2
BAL = 0
SUMT = 2
LOG2E = 1.4426950408889634
NEG = -1e9

F32 = jnp.float32
BF16 = jnp.bfloat16
U32 = jnp.uint32
NT = (((1,), (1,)), ((), ()))


_PROFILE = False


def _scope(name):
    return jax.named_scope(name) if _PROFILE else contextlib.nullcontext()


def _scoped(name, body):
    def f(i, c):
        with _scope(name):
            return body(i, c)
    return f


def _recip(l):
    r = pl.reciprocal(l, approx=True)
    return r * (2.0 - l * r)


def _lo(w):
    return pltpu.bitcast(w << 16, F32)


def _hi(w):
    return pltpu.bitcast(w & jnp.uint32(0xFFFF0000), F32)


def _split_pair(w):
    return jnp.concatenate([_lo(w), _hi(w)], axis=1).astype(BF16)


def _ld(ref, r0, n, cols=slice(None)):
    if isinstance(r0, int):
        rs = slice(r0 // 2, (r0 + n) // 2)
    else:
        rs = pl.ds(pl.multiple_of(lax.shift_right_logical(r0, 1), 8), n // 2)
    return pltpu.bitcast(ref[rs, cols], BF16)


def _st(ref, r0, val, cols=slice(None)):
    ref[r0 // 2:(r0 + val.shape[0]) // 2, cols] = pltpu.bitcast(val, U32)


def _zero_after(z, *vals):
    acc = None
    for v in vals:
        b = pltpu.bitcast(v, U32)
        for r in range(0, b.shape[0], 8):
            for c in range(0, b.shape[1], 128):
                t = b[r:r + 8, c:c + 128]
                acc = t if acc is None else acc | t
    return acc & z


def _chain_sum(x, z, dep):
    parts = []
    for r in range(0, x.shape[0], SUMG):
        a = x[r:r + SUMG, 0:128]
        if dep is not None:
            a = pltpu.bitcast(pltpu.bitcast(a, U32) | jnp.concatenate([dep] * (SUMG // 8), axis=0), F32)
        for c in range(128, x.shape[1], 128):
            a = a + x[r:r + SUMG, c:c + 128]
        dep = _zero_after(z, a)
        parts.append(a)
    return jnp.concatenate(parts, axis=0), dep


def _plan(groups):
    total = sum(g[1] for g in groups) // 4

    @functools.lru_cache(maxsize=None)
    def go(i, pos, cnt):
        if i == len(groups):
            return ()
        nl, ns, at_end = groups[i]
        n = nl + ns
        slots = list(range(max(n - 4, 0), n)) if at_end else list(range(min(4, n)))
        opts = sorted(itertools.combinations(slots, ns), key=lambda c: sorted(cnt[(pos + k) % 4] for k in c)[::-1])
        for c in opts:
            new = list(cnt)
            for k in c:
                new[(pos + k) % 4] += 1
            if max(new) <= total and max(new) - min(new) <= 2:
                rest = go(i + 1, (pos + n) % 4, tuple(new))
                if rest is not None:
                    return (c,) + rest
        return None

    return go(0, 0, (0, 0, 0, 0))


def _body(x_hbm, ckv_hbm, wq_hbm, wuk_hbm, wuv_hbm, wo_hbm, bqkv_hbm, bwo_hbm, gate_hbm,
          out_hbm,
          x_v, ckv_v, wq_p, wuk_p, wuv_p, wo_v, bqkv_v, bwo_p, wcur_v, wfst_v,
          qkv_v, acc_v, g_v, z_v, q_s, k_s, v_s, o_st, gate_v,
          sem_x, sem_w, sem_a, sem_o):
    def cp_x(sm, r0, r1, c0, c1):
        sl = (pl.ds(r0 // 2, (r1 - r0) // 2), pl.ds(c0, c1 - c0))
        return pltpu.make_async_copy(x_hbm.bitcast(U32).at[sl], x_v.at[sl], sem_x.at[sm])

    def cp_w(k, c0=0, c1=3 * M, sm=None):
        sl = (pl.ds(k * 128, 128), pl.ds(c0, c1 - c0))
        return pltpu.make_async_copy(bqkv_hbm.at[sl], bqkv_v.at[sl], sem_w.at[k if sm is None else sm])

    x0a, x0b, xr = cp_x(0, 0, R1, 0, 128), cp_x(1, R1, S, 0, 128), cp_x(2, 0, S, 128, M)
    w0a, w0b, w0c = cp_w(0, 0, M), cp_w(0, M, 2 * M, NT_M), cp_w(0, 2 * M, 3 * M, NT_M + 1)
    cp_g = pltpu.make_async_copy(gate_hbm, gate_v, sem_x.at[3])

    def cp_pairs(src, dst):
        return [pltpu.make_async_copy(src.bitcast(U32).at[:, p, :], dst.at[p], sem_a) for p in range(HP)]

    a_early = cp_pairs(bwo_hbm, bwo_p) + [pltpu.make_async_copy(ckv_hbm.bitcast(U32), ckv_v, sem_a),
                                          pltpu.make_async_copy(wo_hbm.bitcast(U32), wo_v, sem_a)]
    a_late = cp_pairs(wuk_hbm, wuk_p) + cp_pairs(wuv_hbm, wuv_p) + cp_pairs(wq_hbm, wq_p)
    a_waits = [pltpu.make_async_copy(b, b, sem_a) for b in (ckv_v, wo_v, wuk_p, wuv_p, wq_p, bwo_p)]

    def cp_o(r0, n, c0=0, c1=M):
        sl = (pl.ds(r0, n), pl.ds(c0, c1 - c0))
        return pltpu.make_async_copy(o_st.at[sl], out_hbm.at[sl], sem_o)

    def prep(part, j, z=None, dep=None):
        k0 = j * 128 if isinstance(j, int) else pl.multiple_of(j * 128, 128)
        for c in range(NT_M):
            src = bqkv_v[pl.ds(k0, 128), part * M + c * 128:part * M + (c + 1) * 128]
            if dep is not None:
                top = pltpu.bitcast(pltpu.bitcast(src[:16], U32) | dep, BF16)
                src = jnp.concatenate([top, src[16:]], axis=0)
            t = pltpu.bitcast(src.T, U32)
            for hp in range(2):
                a, b = t[32 * hp:32 * hp + 16], t[32 * hp + 16:32 * hp + 32]
                r = 2 * c + hp
                wcur_v[part, pl.ds(r, 16, stride=2 * PITCH), :] = (a & jnp.uint32(0xFFFF)) | (b << 16)
                wcur_v[part, pl.ds(PITCH + r, 16, stride=2 * PITCH), :] = (a >> 16) | (b & jnp.uint32(0xFFFF0000))
            if z is not None:
                dep = _zero_after(z, t[56:64])
        return dep

    def wrows(part, d0, d1):
        w = jnp.concatenate([wcur_v[part, d * PITCH:d * PITCH + HP, :] for d in range(d0, d1)], axis=0)
        return pltpu.bitcast(w, BF16)

    def first_tiles(part):
        for n in range(4):
            _st(wfst_v, 0, wrows(part, 4 * n, 4 * n + 4).T, slice(n * 128, (n + 1) * 128))

    def project(xk, part, first):
        if not first:
            return lax.dot_general(xk, wrows(part, 0, DH), NT, preferred_element_type=F32)
        return jnp.concatenate([jnp.dot(xk, _ld(wfst_v, 0, 128), preferred_element_type=F32),
                                lax.dot_general(xk, wrows(part, DH // 2, DH), NT, preferred_element_type=F32)], axis=1)

    def gate_rows(t, z, dep):
        gw = gate_v[...].astype(F32).reshape(1, M)
        g0 = jnp.minimum((t - 1) * GR, S - GR)
        for k in range(GR // 16):
            rr = pl.multiple_of(g0 + k * 16, 16)
            rw = pl.multiple_of(lax.shift_right_logical(rr, 1), 8)
            xb = x_v[pl.ds(rw, 8), :]
            if dep is not None:
                xb = xb | jnp.concatenate([dep] * NT_M, axis=1)
            xx = pltpu.bitcast(xb, BF16).astype(F32)
            zz = jnp.sum(xx * gw, axis=1, keepdims=True)
            g = jnp.broadcast_to(1.0 / (1.0 + jnp.exp(-zz)), (16, 128))
            g_v[pl.ds(rr, 16), :] = g
            acc_v[pl.ds(rr, 16), :] = jnp.zeros((16, M), F32)
            dep = _zero_after(z, g)

    def first_task():
        def piece(part, r0, r1, first):
            y = project(_ld(x_v, r0, r1 - r0, slice(0, 128)), part, first)
            for tt in range(NT_M):
                qkv_v[part, tt, PAD + r0:PAD + r1, :] = y[:, tt * 128:(tt + 1) * 128]

        with _scope("prep0"):
            w0a.wait()
            prep(0, 0)
        with _scope("b1"):
            x0a.wait()
            piece(0, 0, R1, False)
            first_tiles(0)
        with _scope("b2"):
            x0b.wait()
            w0b.wait()
            piece(0, R1, S, True)
            prep(1, 0)
            first_tiles(1)
        with _scope("b3"):
            w0c.wait()
            cp_w(1).wait()
            z = z_v[...]
            piece(1, 0, S, True)
            prep(2, 0)
            dep = prep(0, 1, z)
            first_tiles(0)
            piece(2, 0, S, False)
            prep(1, 1, z, dep)
            prep(2, 1)
            for cc in a_late[:NA1]:
                cc.start()
        for cc in (xr, cp_g):
            cc.wait()
        for cc in a_late[NA1:]:
            cc.start()

    def bproj_body(t, _):
        @pl.when(t < NT_M - 1)
        def _():
            cp_w(t + 1).wait()

        z = z_v[...]
        u = jnp.minimum(t + 1, NT_M - 1)
        xw = x_v[:, pl.ds(pl.multiple_of(t * 128, 128), 128)]
        xk = pltpu.bitcast(xw | jnp.concatenate([z] * (S // 16), axis=0), BF16)
        dep = None
        for part in range(3):
            y = project(xk, part, part == 0)
            for tt in range(NT_M):
                qkv_v[part, tt, PAD:, :] = qkv_v[part, tt, PAD:, :] + y[:, tt * 128:(tt + 1) * 128]
            dep = prep(part, u, z, dep) if part < 2 else prep(part, u)
            if part == 0:
                first_tiles(0)
        gate_rows(t, z, None)
        return 0

    qscale = (D ** -0.5) * LOG2E
    bscale = (DH ** -0.5) * LOG2E

    def local_attn(r, z, dep):
        def zf(v):
            return pltpu.bitcast(_zero_after(z, v), F32)

        sc = jnp.full((8, 128), bscale, F32)
        if dep is not None:
            sc = sc + dep
        q = [qkv_v[0, t, pl.ds(PAD + r, 8), :] * sc for t in range(NT_M)]
        rowi = r + lax.broadcasted_iota(jnp.int32, (8, 128), 0)
        logits, raw = [], []
        for w in range(W):
            a = None if w < LAQ else zf(raw[w - LAQ])
            for t in range(NT_M):
                pr = q[t] * qkv_v[1, t, pl.ds(PAD + r - DIL * w, 8), :]
                a = pr if a is None else a + pr
            raw.append(a)
            a = a + pltpu.roll(a, 64, 1)
            a = a + pltpu.roll(a, 32, 1)
            logits.append(jnp.where(rowi >= DIL * w, a, NEG) if w > 0 else a)
        m = functools.reduce(jnp.maximum, logits)
        es = [jnp.exp2(lg - m) for lg in logits]
        l = functools.reduce(lambda a, b: a + b, es)
        f = (1.0 - g_v[pl.ds(r, 8), :]) * _recip(l)
        es = [e * f for e in es]
        outs = []
        for t in range(NT_M):
            a = None if t == 0 else zf(outs[t - 1])
            for w in range(W):
                pr = es[w] * qkv_v[2, t, pl.ds(PAD + r - DIL * w, 8), :]
                a = pr if a is None else a + pr
            outs.append(a)
        return jnp.concatenate(outs, axis=1), zf(outs[-1])

    def pair_body(p, _):
        z = z_v[...]
        last = p == HP - 1
        wk, wv = _split_pair(wuk_p[p]), _split_pair(wuv_p[p])
        _st(k_s, 0, jnp.dot(_ld(ckv_v, 0, S), wk, preferred_element_type=F32).astype(BF16))
        _st(v_s, 0, jnp.dot(_ld(ckv_v, 0, S), wv, preferred_element_type=F32).astype(BF16))

        rb = pl.multiple_of(p * TL, TL)
        dep, obs = None, []
        for k in range(TL // 8):
            ob, dep = local_attn(rb + k * 8, z, dep)
            obs.append(ob)
        ob = jnp.concatenate(obs, axis=0).astype(BF16)

        wqw = wq_p[p]
        wq = _split_pair(jnp.concatenate([wqw[:8] | _zero_after(z, ob[TL - 16:]), wqw[8:]], axis=0))
        row = lax.broadcasted_iota(jnp.int32, (HQ, TQ), 0)
        col = lax.broadcasted_iota(jnp.int32, (HQ, TQ), 1)
        diag = col <= row + HQ

        def rows(j):
            t0 = (j // 2) * 2 * TQ + (j % 2) * HQ
            return t0, t0 + TQ

        def halves(ref, j, ld=lambda ref, r: ref[r:r + HQ, :]):
            return jnp.concatenate([ld(ref, r) for r in rows(j)], axis=0)

        def qproj(j):
            q = jnp.dot(halves(x_v, j, lambda ref, r: _ld(ref, r, HQ)), wq, preferred_element_type=F32) * qscale
            _st(q_s, j * TQ, q.astype(BF16))

        def emit(n_long, slots, long_fn, short_fns):
            longs, shorts, done = [], [], 0
            for k, (slot, fn) in enumerate(zip(slots, short_fns)):
                if slot - k > done:
                    longs.append(long_fn(done, slot - k))
                    done = slot - k
                shorts.append(fn())
            if n_long > done:
                longs.append(long_fn(done, n_long))
            return longs, shorts

        left = {}

        def qk(j, hh, slots):
            cs = slice(hh * D, (hh + 1) * D)
            off = HQ * (1 - j % 2)
            q = _ld(q_s, j * TQ, TQ, cs)
            fns = [lambda: lax.dot_general(q[HQ:], _ld(k_s, off + j * TQ, TQ, cs), NT, preferred_element_type=F32)]
            if off and hh == 0:
                fns += [lambda h=h: lax.dot_general(_ld(k_s, 0, HQ, slice(h * D, (h + 1) * D)),
                                                    _ld(q_s, j * TQ, TQ, slice(h * D, (h + 1) * D)), NT,
                                                    preferred_element_type=F32) for h in range(2)]
            longs, shorts = emit(j, slots, lambda a, b: lax.dot_general(
                q, _ld(k_s, off + a * TQ, (b - a) * TQ, cs), NT, preferred_element_type=F32), fns)
            if len(shorts) > 1:
                left[j] = jnp.concatenate(shorts[1:], axis=0).T
            return longs, shorts[0]

        ldep = [None]

        def softmax(parts):
            s = jnp.concatenate(parts, axis=1)
            e = jnp.exp2(s - jnp.max(s, axis=1, keepdims=True))
            if s.shape[1] > (SUMT + 1) * TQ:
                lp, ldep[0] = _chain_sum(e, z, ldep[0])
                l = jnp.sum(lp, axis=1, keepdims=True)
            else:
                l = jnp.sum(e, axis=1, keepdims=True)
            return e, l

        def softmax_pv(j, hh, sc, slots):
            cs = slice(hh * D, (hh + 1) * D)
            off = HQ * (1 - j % 2)
            longs, extra = sc
            top, bot, vs = [], [], []
            if off:
                mine = (col >= HQ) if hh else (col < HQ)
                top.append(jnp.where(jnp.logical_and(mine, col - hh * HQ <= row) if j == 0 else mine, left[j][:HQ], NEG))
                bot.append(jnp.where(mine, left[j][HQ:], NEG))
                vs += [_ld(v_s, 0, HQ, cs)] * 2
            if j:
                s = jnp.concatenate(longs, axis=1)
                w = (j - 1) * TQ
                top += ([s[:HQ, :w]] if w else []) + [jnp.where(diag, s[:HQ, w:], NEG)]
                bot.append(s[HQ:])
                vs.append(_ld(v_s, off, j * TQ, cs))
            bot.append(jnp.where(diag, extra, NEG))
            (et, lt), (eb, lb) = softmax(top), softmax(bot)
            w = et.shape[1]
            pc = jnp.concatenate([et, eb[:, :w]], axis=0).astype(BF16)
            vc = jnp.concatenate(vs, axis=0)
            longs, (ox,) = emit(w // TQ, slots, lambda a, b: jnp.dot(
                pc[:, a * TQ:b * TQ], vc[a * TQ:b * TQ], preferred_element_type=F32),
                [lambda: jnp.dot(eb[:, w:].astype(BF16), _ld(v_s, off + j * TQ, TQ, cs), preferred_element_type=F32)])
            o = functools.reduce(lambda a, b: a + b, longs)
            o = jnp.concatenate([o[:HQ], o[HQ:] + ox], axis=0)
            return o * (halves(g_v, j) * _recip(jnp.concatenate([lt, lb], axis=0)))

        def oproj(j, o0, o1):
            y = halves(acc_v, j) + jnp.dot(jnp.concatenate([o0, o1], axis=1).astype(BF16),
                                           _ld(wo_v, p * (2 * D), 2 * D), preferred_element_type=F32)
            for r, yh in zip(rows(j), (y[:HQ], y[HQ:])):
                acc_v[r:r + HQ, :] = yh
                if r < S - TL:
                    o_st[r:r + HQ, :] = yh.astype(BF16)
            if j % 2 == 0:
                pl.when(last)(cp_o(j * TQ, min(2 * TQ, S - TL - j * TQ)).start)

        nq = S // TQ
        items = [(j, hh) for j in reversed(range(nq)) for hh in range(2)]
        n = len(items)
        sched = []
        for step in range(n + LOOK):
            if step < n:
                j, hh = items[step]
                sched.append(("qk", step, (j, 3 if j % 2 == 0 and hh == 0 else 1, True)))
            if step >= LOOK:
                j, hh = items[step - LOOK]
                sched.append(("pv", step - LOOK, (j + 1 - j % 2, 1, False)))
        if BAL:
            plan = _plan(tuple(g for _, _, g in sched))
        else:
            plan = [tuple(range(g[0], g[0] + g[1])) for _, _, g in sched]
        slots = {(kind, i): c for (kind, i, _), c in zip(sched, plan)}
        s_vals, o_vals = {}, {}
        qproj(nq - 1)
        for step in range(n + LOOK + OLAG):
            if step % 2 == 0 and nq - 2 - step // 2 >= 0:
                qproj(nq - 2 - step // 2)
            if step < n:
                s_vals[step] = qk(*items[step], slots["qk", step])
            b = step - LOOK
            if 0 <= b < n:
                o_vals[b] = softmax_pv(*items[b], s_vals.pop(b), slots["pv", b])
            c = step - LOOK - OLAG
            if 0 <= c < n and c % 2 == 1:
                oproj(items[c][0], o_vals.pop(c - 1), o_vals.pop(c))

        wop = jnp.concatenate([f(bwo_p[dp]) for dp in range(DH // 2) for f in (_lo, _hi)], axis=0).astype(BF16)
        y = acc_v[pl.ds(rb, TL), :] + jnp.dot(ob, wop, preferred_element_type=F32)
        acc_v[pl.ds(rb, TL), :] = y
        for c0, c1 in zip(OCUT[:-1], OCUT[1:]):
            o_st[S - TL:S, c0:c1] = y[:, c0:c1].astype(BF16)
            pl.when(last)(cp_o(S - TL, TL, c0, c1).start)
        return 0

    for cc in [w0a, x0a, x0b, w0b, w0c, cp_w(1), cp_g, xr] + [cp_w(k) for k in range(2, NT_M)] + a_early:
        cc.start()
    z_v[...] = jnp.zeros((8, 128), U32)
    for part in range(3):
        for t in range(NT_M):
            qkv_v[part, t, 0:PAD, :] = jnp.zeros((PAD, 128), F32)

    def phases():
        first_task()
        lax.fori_loop(1, NT_M, _scoped("bproj", bproj_body), 0)
        for cc in a_waits:
            cc.wait()
        lax.fori_loop(0, HP, _scoped("pair", pair_body), 0)

    def once(i, _):
        pl.when(i == 0)(phases)
        return 0

    lax.fori_loop(0, 2, once, 0)
    with _scope("ow"):
        cp_o(0, S).wait()


def _kernel(*refs):
    dma = pltpu.SemaphoreType.DMA
    pl.run_scoped(functools.partial(_body, *refs), dma((4,)), dma((NT_M + 2,)), dma(()), dma(()))


@jax.jit
def pallas_gated_mix__compressed_kv_cla__sliding_local_dilated__prompt_kernel(
    A_x, A_c_kv, A_w_q, A_w_uk, A_w_uv, A_w_o, B_x, B_wqkv, B_wo, gate_w,
):
    del B_x
    x = A_x.reshape(S, M)
    ckv = A_c_kv.reshape(S, DC)
    wo = A_w_o.reshape(H * D, M)
    bwo = B_wo.reshape(H, DH, M)
    any_spec = pl.BlockSpec(memory_space=pl.ANY)
    out = pl.pallas_call(
        _kernel,
        out_shape=jax.ShapeDtypeStruct((S, M), BF16),
        in_specs=[any_spec] * 9,
        out_specs=any_spec,
        scratch_shapes=[
            pltpu.VMEM((S // 2, M), U32),
            pltpu.VMEM((S // 2, DC), U32),
            pltpu.VMEM((HP, M, D), U32),
            pltpu.VMEM((HP, DC, D), U32),
            pltpu.VMEM((HP, DC, D), U32),
            pltpu.VMEM((H * D // 2, M), U32),
            pltpu.VMEM((M, 3 * M), BF16),
            pltpu.VMEM((DH // 2, H, M), U32),
            pltpu.VMEM((3, DH * 24, 128), U32),
            pltpu.VMEM((64, 512), U32),
            pltpu.VMEM((3, NT_M, S + PAD, 128), F32),
            pltpu.VMEM((S, M), F32),
            pltpu.VMEM((S, 128), F32),
            pltpu.VMEM((8, 128), U32),
            pltpu.VMEM((S // 2, 2 * D), U32),
            pltpu.VMEM((S // 2, 2 * D), U32),
            pltpu.VMEM((S // 2, 2 * D), U32),
            pltpu.VMEM((S, M), BF16),
            pltpu.VMEM((M,), BF16),
        ],
        compiler_params=pltpu.CompilerParams(vmem_limit_bytes=110 * 1024 * 1024),
    )(x, ckv, A_w_q, A_w_uk, A_w_uv, wo, B_wqkv, bwo, gate_w)
    return out.reshape(1, S, M)
```

```python
import contextlib
import functools

import jax
import jax.numpy as jnp
from jax import lax
import jax.experimental.pallas as pl
import jax.experimental.pallas.tpu as pltpu

S = 2048
M = 1024
DC = 512
H = 32
HP = H // 2
D = 128
DH = 32
W = 8
DIL = 2
PAD = 16
NT_M = M // 128
TQ = 128
TL = S // HP
R1 = 768
GR = 304
PITCH = 17
NA1 = 44
OCUT = (0, 512, 768, M)
LOOK = 2
OLAG = 7
SUMG = 8
LAQ = 2
G = 4
RG = TQ // G
QORD = 0
PORD = 0
PACK = 1
SUMT = 2
BSPL = 1
BSW = 128
GORD = 0
QAH = 1
SCH = 2
XREV = 0
BREV = 0
LOG2E = 1.4426950408889634
NEG = -1e9

F32 = jnp.float32
BF16 = jnp.bfloat16
U32 = jnp.uint32
NT = (((1,), (1,)), ((), ()))


_PROFILE = False


def _scope(name):
    return jax.named_scope(name) if _PROFILE else contextlib.nullcontext()


def _scoped(name, body):
    def f(i, c):
        with _scope(name):
            return body(i, c)
    return f


def _recip(l):
    r = pl.reciprocal(l, approx=True)
    return r * (2.0 - l * r)


def _lo(w):
    return pltpu.bitcast(w << 16, F32)


def _hi(w):
    return pltpu.bitcast(w & jnp.uint32(0xFFFF0000), F32)


def _split_pair(w):
    return jnp.concatenate([_lo(w), _hi(w)], axis=1).astype(BF16)


def _ld(ref, r0, n, cols=slice(None)):
    if isinstance(r0, int):
        rs = slice(r0 // 2, (r0 + n) // 2)
    else:
        rs = pl.ds(pl.multiple_of(lax.shift_right_logical(r0, 1), 8), n // 2)
    return pltpu.bitcast(ref[rs, cols], BF16)


def _st(ref, r0, val, cols=slice(None)):
    ref[r0 // 2:(r0 + val.shape[0]) // 2, cols] = pltpu.bitcast(val, U32)


def _zero_after(z, *vals):
    acc = None
    for v in vals:
        b = pltpu.bitcast(v, U32)
        for r in range(0, b.shape[0], 8):
            for c in range(0, b.shape[1], 128):
                t = b[r:r + 8, c:c + 128]
                acc = t if acc is None else acc | t
    return acc & z


def _chain_sum(x, z, dep):
    parts = []
    for r in range(0, x.shape[0], SUMG):
        a = x[r:r + SUMG, 0:128]
        if dep is not None:
            a = pltpu.bitcast(pltpu.bitcast(a, U32) | jnp.concatenate([dep] * (SUMG // 8), axis=0), F32)
        for c in range(128, x.shape[1], 128):
            a = a + x[r:r + SUMG, c:c + 128]
        dep = _zero_after(z, a)
        parts.append(a)
    return jnp.concatenate(parts, axis=0), dep


def _body(x_hbm, ckv_hbm, wq_hbm, wuk_hbm, wuv_hbm, wo_hbm, bqkv_hbm, bwo_hbm, gate_hbm,
          out_hbm,
          x_v, ckv_v, wq_p, wuk_p, wuv_p, wo_v, bqkv_v, bwo_p, wcur_v, wfst_v,
          qkv_v, acc_v, g_v, z_v, q_s, k_s, v_s, o_st, gate_v,
          sem_x, sem_w, sem_a, sem_o):
    def cp_x(sm, r0, r1, c0, c1):
        sl = (pl.ds(r0 // 2, (r1 - r0) // 2), pl.ds(c0, c1 - c0))
        return pltpu.make_async_copy(x_hbm.bitcast(U32).at[sl], x_v.at[sl], sem_x.at[sm])

    def cp_w(k, c0=0, c1=3 * M, sm=None):
        sl = (pl.ds(k * 128, 128), pl.ds(c0, c1 - c0))
        return pltpu.make_async_copy(bqkv_hbm.at[sl], bqkv_v.at[sl], sem_w.at[k if sm is None else sm])

    x0a, x0b, xr = cp_x(0, 0, R1, 0, 128), cp_x(1, R1, S, 0, 128), cp_x(2, 0, S, 128, M)
    w0a, w0b, w0c = cp_w(0, 0, M), cp_w(0, M, 2 * M, NT_M), cp_w(0, 2 * M, 3 * M, NT_M + 1)
    cp_g = pltpu.make_async_copy(gate_hbm, gate_v, sem_x.at[3])

    def cp_pairs(src, dst):
        return [pltpu.make_async_copy(src.bitcast(U32).at[:, p, :], dst.at[p], sem_a) for p in range(HP)]

    a_early = cp_pairs(bwo_hbm, bwo_p) + [pltpu.make_async_copy(ckv_hbm.bitcast(U32), ckv_v, sem_a),
                                          pltpu.make_async_copy(wo_hbm.bitcast(U32), wo_v, sem_a)]
    a_late = cp_pairs(wuk_hbm, wuk_p) + cp_pairs(wuv_hbm, wuv_p) + cp_pairs(wq_hbm, wq_p)
    a_waits = [pltpu.make_async_copy(b, b, sem_a) for b in (ckv_v, wo_v, wuk_p, wuv_p, wq_p, bwo_p)]

    def cp_o(b0, nb, r0, n, c0=0, c1=M):
        sl = (pl.ds(b0, nb), pl.ds(r0, n), pl.ds(c0, c1 - c0))
        return pltpu.make_async_copy(o_st.at[sl], out_hbm.at[sl], sem_o)

    def prep(part, j, z=None, dep=None):
        k0 = j * 128 if isinstance(j, int) else pl.multiple_of(j * 128, 128)
        for c in range(NT_M):
            src = bqkv_v[pl.ds(k0, 128), part * M + c * 128:part * M + (c + 1) * 128]
            if dep is not None:
                top = pltpu.bitcast(pltpu.bitcast(src[:16], U32) | dep, BF16)
                src = jnp.concatenate([top, src[16:]], axis=0)
            t = pltpu.bitcast(src.T, U32)
            for hp in range(2):
                a, b = t[32 * hp:32 * hp + 16], t[32 * hp + 16:32 * hp + 32]
                r = 2 * c + hp
                wcur_v[part, pl.ds(r, 16, stride=2 * PITCH), :] = (a & jnp.uint32(0xFFFF)) | (b << 16)
                wcur_v[part, pl.ds(PITCH + r, 16, stride=2 * PITCH), :] = (a >> 16) | (b & jnp.uint32(0xFFFF0000))
            if z is not None:
                dep = _zero_after(z, t[56:64])
        return dep

    def wrows(part, d0, d1):
        w = jnp.concatenate([wcur_v[part, d * PITCH:d * PITCH + HP, :] for d in range(d0, d1)], axis=0)
        return pltpu.bitcast(w, BF16)

    def first_tiles(part):
        for n in range(4):
            _st(wfst_v, 0, wrows(part, 4 * n, 4 * n + 4).T, slice(n * 128, (n + 1) * 128))

    def project(xk, part, first):
        if not first:
            return lax.dot_general(xk, wrows(part, 0, DH), NT, preferred_element_type=F32)
        return jnp.concatenate([jnp.dot(xk, _ld(wfst_v, 0, 128), preferred_element_type=F32),
                                lax.dot_general(xk, wrows(part, DH // 2, DH), NT, preferred_element_type=F32)], axis=1)

    def gate_rows(t, z, dep):
        gw = gate_v[...].astype(F32).reshape(1, M)
        g0 = jnp.minimum((t - 1) * GR, S - GR)
        for k in range(GR // 16):
            rr = pl.multiple_of(g0 + k * 16, 16)
            rw = pl.multiple_of(lax.shift_right_logical(rr, 1), 8)
            xb = x_v[pl.ds(rw, 8), :]
            if dep is not None:
                xb = xb | jnp.concatenate([dep] * NT_M, axis=1)
            xx = pltpu.bitcast(xb, BF16).astype(F32)
            zz = jnp.sum(xx * gw, axis=1, keepdims=True)
            g = jnp.broadcast_to(1.0 / (1.0 + jnp.exp(-zz)), (16, 128))
            g_v[pl.ds(rr, 16), :] = g
            acc_v[pl.ds(rr, 16), :] = jnp.zeros((16, M), F32)
            dep = _zero_after(z, g)

    def first_task():
        def piece(part, r0, r1, first):
            y = project(_ld(x_v, r0, r1 - r0, slice(0, 128)), part, first)
            for tt in range(NT_M):
                qkv_v[part, tt, PAD + r0:PAD + r1, :] = y[:, tt * 128:(tt + 1) * 128]

        with _scope("prep0"):
            w0a.wait()
            prep(0, 0)
        with _scope("b1"):
            x0a.wait()
            piece(0, 0, R1, False)
            first_tiles(0)
        with _scope("b2"):
            x0b.wait()
            w0b.wait()
            piece(0, R1, S, True)
            prep(1, 0)
            first_tiles(1)
        with _scope("b3"):
            w0c.wait()
            cp_w(1).wait()
            z = z_v[...]
            piece(1, 0, S, True)
            prep(2, 0)
            dep = prep(0, 1, z)
            first_tiles(0)
            piece(2, 0, S, False)
            prep(1, 1, z, dep)
            prep(2, 1)
            for cc in a_late[:NA1]:
                cc.start()
        for cc in (xr, cp_g):
            cc.wait()
        for cc in a_late[NA1:]:
            cc.start()

    def bproj_body(t, _):
        @pl.when(t < NT_M - 1)
        def _():
            cp_w(t + 1).wait()

        z = z_v[...]
        u = jnp.minimum(t + 1, NT_M - 1)
        xw = x_v[:, pl.ds(pl.multiple_of(t * 128, 128), 128)]
        xk = pltpu.bitcast(xw | jnp.concatenate([z] * (S // 16), axis=0), BF16)
        dep = None
        for part in range(3):
            y = project(xk, part, part == 0)
            for tt in range(NT_M):
                qkv_v[part, tt, PAD:, :] = qkv_v[part, tt, PAD:, :] + y[:, tt * 128:(tt + 1) * 128]
            dep = prep(part, u, z, dep) if part < 2 else prep(part, u)
            if part == 0:
                first_tiles(0)
        gate_rows(t, z, None)
        return 0

    qscale = (D ** -0.5) * LOG2E
    bscale = (DH ** -0.5) * LOG2E

    def local_attn(r, z, dep):
        def zf(v):
            return pltpu.bitcast(_zero_after(z, v), F32)

        sc = jnp.full((8, 128), bscale, F32)
        if dep is not None:
            sc = sc + dep
        q = [qkv_v[0, t, pl.ds(PAD + r, 8), :] * sc for t in range(NT_M)]
        rowi = r + lax.broadcasted_iota(jnp.int32, (8, 128), 0)
        logits, raw = [], []
        for w in range(W):
            a = None if w < LAQ else zf(raw[w - LAQ])
            for t in range(NT_M):
                pr = q[t] * qkv_v[1, t, pl.ds(PAD + r - DIL * w, 8), :]
                a = pr if a is None else a + pr
            raw.append(a)
            a = a + pltpu.roll(a, 64, 1)
            a = a + pltpu.roll(a, 32, 1)
            logits.append(jnp.where(rowi >= DIL * w, a, NEG) if w > 0 else a)
        m = functools.reduce(jnp.maximum, logits)
        es = [jnp.exp2(lg - m) for lg in logits]
        l = functools.reduce(lambda a, b: a + b, es)
        f = (1.0 - g_v[pl.ds(r, 8), :]) * _recip(l)
        es = [e * f for e in es]
        outs = []
        for t in range(NT_M):
            a = None if t == 0 else zf(outs[t - 1])
            for w in range(W):
                pr = es[w] * qkv_v[2, t, pl.ds(PAD + r - DIL * w, 8), :]
                a = pr if a is None else a + pr
            outs.append(a)
        return jnp.concatenate(outs, axis=1), zf(outs[-1])

    def pair_body(p, _):
        z = z_v[...]
        last = p == HP - 1
        wk, wv = _split_pair(wuk_p[p]), _split_pair(wuv_p[p])
        _st(k_s, 0, jnp.dot(_ld(ckv_v, 0, S), wk, preferred_element_type=F32).astype(BF16))
        _st(v_s, 0, jnp.dot(_ld(ckv_v, 0, S), wv, preferred_element_type=F32).astype(BF16))

        rb = pl.multiple_of(p * TL, TL)
        dep, obs = None, []
        for k in range(TL // 8):
            ob, dep = local_attn(rb + k * 8, z, dep)
            obs.append(ob)
        ob = jnp.concatenate(obs, axis=0).astype(BF16)

        wqw = wq_p[p]
        wq = _split_pair(jnp.concatenate([wqw[:8] | _zero_after(z, ob[TL - 16:]), wqw[8:]], axis=0))
        row = lax.broadcasted_iota(jnp.int32, (RG, TQ), 0)
        col = lax.broadcasted_iota(jnp.int32, (RG, TQ), 1)
        diag = col <= row + (TQ - RG)

        def rows(j):
            return [(j - j % G + b) * TQ + (j % G) * RG for b in range(G)]

        def geom(j):
            off = (j % G + 1) * RG % TQ
            return off, j - j % G + (0 if off else 1)

        def gather(ref, j, ld=lambda ref, r: ref[r:r + RG, :]):
            return jnp.concatenate([ld(ref, r) for r in rows(j)], axis=0)

        def qproj(j):
            q = jnp.dot(gather(x_v, j, lambda ref, r: _ld(ref, r, RG)), wq, preferred_element_type=F32) * qscale
            _st(q_s, j * TQ, q.astype(BF16))

        def head(h):
            return slice(h * D, (h + 1) * D)

        left = {}

        def qk(j, hh):
            off, nc = geom(j)
            q = _ld(q_s, j * TQ, TQ, head(hh))

            def common():
                return lax.dot_general(q, _ld(k_s, off, nc * TQ, head(hh)), NT, preferred_element_type=F32) if nc else None

            def extras():
                x = {e: lax.dot_general(q[e * RG:], _ld(k_s, off + (nc + e - 1) * TQ, TQ, head(hh)), NT,
                                        preferred_element_type=F32) for e in (reversed(range(1, G)) if XREV else range(1, G))}
                return [x[e] for e in range(1, G)]

            def swapped():
                def st(h):
                    return lax.dot_general(_ld(k_s, 0, off, head(h)), _ld(q_s, j * TQ, TQ, head(h)), NT,
                                           preferred_element_type=F32)
                pad = [jnp.full((TQ // 2 - off, TQ), NEG, F32)] if off < TQ // 2 else []
                if PACK and 0 < off <= TQ // 2:
                    if hh == 0:
                        left[j, 0] = left[j, 1] = jnp.concatenate([st(0)] + pad + [st(1)] + pad, axis=0).T
                elif off:
                    left[j, hh] = jnp.concatenate([st(hh), jnp.full((TQ - off, TQ), NEG, F32)], axis=0).T

            if QORD == 0:
                c = common(); x = extras(); swapped()
            elif QORD == 1:
                swapped(); c = common(); x = extras()
            elif QORD == 2:
                c = common(); swapped(); x = extras()
            elif QORD == 3:
                x = extras(); c = common(); swapped()
            else:
                swapped(); x = extras(); c = common()
            return c, x

        ldep = [None]

        def softmax(parts):
            s = jnp.concatenate(parts, axis=1)
            e = jnp.exp2(s - jnp.max(s, axis=1, keepdims=True))
            if s.shape[1] > (SUMT + 1) * TQ:
                lp, ldep[0] = _chain_sum(e, z, ldep[0])
                l = jnp.sum(lp, axis=1, keepdims=True)
            else:
                l = jnp.sum(e, axis=1, keepdims=True)
            return e, l

        def softmax_pv(j, hh, sc):
            off, nc = geom(j)
            com, ext = sc
            packed = PACK and 0 < off <= TQ // 2
            es, ls = {}, {}
            if SCH == 0 or (SCH == 1 and hh == 0):
                ldep[0] = None
            for b in (reversed(range(G)) if BREV else range(G)):
                rs = slice(b * RG, (b + 1) * RG)
                parts = []
                if off:
                    lf = left[j, hh][rs]
                    c0 = hh * (TQ // 2) if packed else 0
                    if nc + b == 0:
                        keep = col - c0 <= row + (off - RG)
                        lf = jnp.where(jnp.logical_and(keep, col >= c0) if c0 else keep, lf, NEG)
                    elif packed:
                        lf = jnp.where((col >= c0) if hh else (col < TQ // 2), lf, NEG)
                    parts.append(lf)
                parts += [com[rs, t * TQ:(t + 1) * TQ] for t in range(nc)]
                parts += [ext[e - 1][(b - e) * RG:(b - e + 1) * RG] for e in range(1, b + 1)]
                if nc + b:
                    parts[-1] = jnp.where(diag, parts[-1], NEG)
                es[b], ls[b] = softmax(parts)
            es, ls = [es[b] for b in range(G)], [ls[b] for b in range(G)]
            w = es[0].shape[1]
            vs = []
            if off:
                vs = [_ld(v_s, 0, TQ // 2, head(hh))] * 2 if packed else [_ld(v_s, 0, TQ, head(hh))]
            if nc:
                vs.append(_ld(v_s, off, nc * TQ, head(hh)))

            def common():
                return jnp.dot(jnp.concatenate([e[:, :w] for e in es], axis=0).astype(BF16), jnp.concatenate(vs, axis=0),
                               preferred_element_type=F32)

            def extras():
                ord_ = range(1, G) if PORD < 2 else reversed(range(1, G))
                return {e: jnp.dot(jnp.concatenate([x[:, w + (e - 1) * TQ:w + e * TQ] for x in es[e:]], axis=0).astype(BF16),
                                   _ld(v_s, off + (nc + e - 1) * TQ, TQ, head(hh)), preferred_element_type=F32)
                        for e in ord_}

            if PORD in (0, 3):
                o = common(); ox = extras()
            else:
                ox = extras(); o = common()
            o = jnp.concatenate([functools.reduce(lambda a, c: a + c, [o[b * RG:(b + 1) * RG]] + [
                ox[e][(b - e) * RG:(b - e + 1) * RG] for e in range(1, b + 1)]) for b in range(G)], axis=0)
            return o * (gather(g_v, j) * _recip(jnp.concatenate(ls, axis=0)))

        def oproj(j, o0, o1):
            y = gather(acc_v, j) + jnp.dot(jnp.concatenate([o0, o1], axis=1).astype(BF16),
                                           _ld(wo_v, p * (2 * D), 2 * D), preferred_element_type=F32)
            for b, r in enumerate(rows(j)):
                acc_v[r:r + RG, :] = y[b * RG:(b + 1) * RG]
                if r < S - TL:
                    o_st[r // TQ, r % TQ:r % TQ + RG, :] = y[b * RG:(b + 1) * RG].astype(BF16)
            j0 = j - j % G
            if min(G, nq - 1 - j0):
                pl.when(last)(cp_o(j0, min(G, nq - 1 - j0), j % G * RG, RG).start)

        nq = S // TQ
        gs = {0: list(reversed(range(G))), 1: list(range(G)), 2: [G - 1] + list(range(G - 1)),
              3: list(reversed(range(G - 1))) + [G - 1]}[GORD]
        order = [m * G + g for m in reversed(range(nq // G)) for g in gs]
        items = [(j, hh) for j in order for hh in range(2)]
        n = len(items)
        s_vals, o_vals = {}, {}
        for a in range(QAH):
            qproj(order[a])
        for step in range(n + LOOK + OLAG):
            if step % 2 == 0 and QAH + step // 2 < nq:
                qproj(order[QAH + step // 2])
            if step < n:
                s_vals[step] = qk(*items[step])
            b = step - LOOK
            if 0 <= b < n:
                o_vals[b] = softmax_pv(*items[b], s_vals.pop(b))
            c = step - LOOK - OLAG
            if 0 <= c < n and c % 2 == 1:
                oproj(items[c][0], o_vals.pop(c - 1), o_vals.pop(c))

        wop = jnp.concatenate([f(bwo_p[dp]) for dp in range(DH // 2) for f in (_lo, _hi)], axis=0).astype(BF16)
        if BSPL > 1:
            yl = jnp.dot(ob, wop[:, :M - BSW], preferred_element_type=F32)
            yr = jnp.concatenate([jnp.dot(ob[r:r + TL // BSPL], wop[:, M - BSW:], preferred_element_type=F32)
                                  for r in range(0, TL, TL // BSPL)], axis=0)
            y = acc_v[pl.ds(rb, TL), :] + jnp.concatenate([yl, yr], axis=1)
        else:
            y = acc_v[pl.ds(rb, TL), :] + jnp.dot(ob, wop, preferred_element_type=F32)
        acc_v[pl.ds(rb, TL), :] = y
        for c0, c1 in zip(OCUT[:-1], OCUT[1:]):
            o_st[S // TQ - 1, :, c0:c1] = y[:, c0:c1].astype(BF16)
            pl.when(last)(cp_o(S // TQ - 1, 1, 0, TQ, c0, c1).start)
        return 0

    for cc in [w0a, x0a, x0b, w0b, w0c, cp_w(1), cp_g, xr] + [cp_w(k) for k in range(2, NT_M)] + a_early:
        cc.start()
    z_v[...] = jnp.zeros((8, 128), U32)
    for part in range(3):
        for t in range(NT_M):
            qkv_v[part, t, 0:PAD, :] = jnp.zeros((PAD, 128), F32)

    def phases():
        first_task()
        lax.fori_loop(1, NT_M, _scoped("bproj", bproj_body), 0)
        for cc in a_waits:
            cc.wait()
        lax.fori_loop(0, HP, _scoped("pair", pair_body), 0)

    def once(i, _):
        pl.when(i == 0)(phases)
        return 0

    lax.fori_loop(0, 2, once, 0)
    with _scope("ow"):
        cp_o(0, S // TQ, 0, TQ).wait()


def _kernel(*refs):
    dma = pltpu.SemaphoreType.DMA
    pl.run_scoped(functools.partial(_body, *refs), dma((4,)), dma((NT_M + 2,)), dma(()), dma(()))


@jax.jit
def pallas_gated_mix__compressed_kv_cla__sliding_local_dilated__prompt_kernel(
    A_x, A_c_kv, A_w_q, A_w_uk, A_w_uv, A_w_o, B_x, B_wqkv, B_wo, gate_w,
):
    del B_x
    x = A_x.reshape(S, M)
    ckv = A_c_kv.reshape(S, DC)
    wo = A_w_o.reshape(H * D, M)
    bwo = B_wo.reshape(H, DH, M)
    any_spec = pl.BlockSpec(memory_space=pl.ANY)
    out = pl.pallas_call(
        _kernel,
        out_shape=jax.ShapeDtypeStruct((S // TQ, TQ, M), BF16),
        in_specs=[any_spec] * 9,
        out_specs=any_spec,
        scratch_shapes=[
            pltpu.VMEM((S // 2, M), U32),
            pltpu.VMEM((S // 2, DC), U32),
            pltpu.VMEM((HP, M, D), U32),
            pltpu.VMEM((HP, DC, D), U32),
            pltpu.VMEM((HP, DC, D), U32),
            pltpu.VMEM((H * D // 2, M), U32),
            pltpu.VMEM((M, 3 * M), BF16),
            pltpu.VMEM((DH // 2, H, M), U32),
            pltpu.VMEM((3, DH * 24, 128), U32),
            pltpu.VMEM((64, 512), U32),
            pltpu.VMEM((3, NT_M, S + PAD, 128), F32),
            pltpu.VMEM((S, M), F32),
            pltpu.VMEM((S, 128), F32),
            pltpu.VMEM((8, 128), U32),
            pltpu.VMEM((S // 2, 2 * D), U32),
            pltpu.VMEM((S // 2, 2 * D), U32),
            pltpu.VMEM((S // 2, 2 * D), U32),
            pltpu.VMEM((S // TQ, TQ, M), BF16),
            pltpu.VMEM((M,), BF16),
        ],
        compiler_params=pltpu.CompilerParams(vmem_limit_bytes=110 * 1024 * 1024),
    )(x, ckv, A_w_q, A_w_uk, A_w_uv, wo, B_wqkv, bwo, gate_w)
    return out.reshape(1, S, M)
```

```python
import contextlib
import functools

import jax
import jax.numpy as jnp
from jax import lax
import jax.experimental.pallas as pl
import jax.experimental.pallas.tpu as pltpu

S = 2048
M = 1024
DC = 512
H = 32
HP = H // 2
D = 128
DH = 32
W = 8
DIL = 2
PAD = 16
NT_M = M // 128
TQ = 128
TL = S // HP
R1 = 768
GR = 304
PITCH = 17
NA1 = 44
OCUT = (0, 512, 768, M)
LOOK = 2
OLAG = 7
SUMG = 8
SUMT = 3
LAQ = 2
G = 4
RG = TQ // G
LOG2E = 1.4426950408889634
NEG = -1e9

F32 = jnp.float32
BF16 = jnp.bfloat16
U32 = jnp.uint32
NT = (((1,), (1,)), ((), ()))


_PROFILE = False


def _scope(name):
    return jax.named_scope(name) if _PROFILE else contextlib.nullcontext()


def _scoped(name, body):
    def f(i, c):
        with _scope(name):
            return body(i, c)
    return f


def _recip(l):
    r = pl.reciprocal(l, approx=True)
    return r * (2.0 - l * r)


def _lo(w):
    return pltpu.bitcast(w << 16, F32)


def _hi(w):
    return pltpu.bitcast(w & jnp.uint32(0xFFFF0000), F32)


def _split_pair(w):
    return jnp.concatenate([_lo(w), _hi(w)], axis=1).astype(BF16)


def _ld(ref, r0, n, cols=slice(None)):
    if isinstance(r0, int):
        rs = slice(r0 // 2, (r0 + n) // 2)
    else:
        rs = pl.ds(pl.multiple_of(lax.shift_right_logical(r0, 1), 8), n // 2)
    return pltpu.bitcast(ref[rs, cols], BF16)


def _st(ref, r0, val, cols=slice(None)):
    ref[r0 // 2:(r0 + val.shape[0]) // 2, cols] = pltpu.bitcast(val, U32)


def _zero_after(z, *vals):
    acc = None
    for v in vals:
        b = pltpu.bitcast(v, U32)
        for r in range(0, b.shape[0], 8):
            for c in range(0, b.shape[1], 128):
                t = b[r:r + 8, c:c + 128]
                acc = t if acc is None else acc | t
    return acc & z


def _chain_sum(x, z, dep):
    parts = []
    for r in range(0, x.shape[0], SUMG):
        a = x[r:r + SUMG, 0:128]
        if dep is not None:
            a = pltpu.bitcast(pltpu.bitcast(a, U32) | jnp.concatenate([dep] * (SUMG // 8), axis=0), F32)
        for c in range(128, x.shape[1], 128):
            a = a + x[r:r + SUMG, c:c + 128]
        dep = _zero_after(z, a)
        parts.append(a)
    return jnp.concatenate(parts, axis=0), dep


def _body(x_hbm, ckv_hbm, wq_hbm, wuk_hbm, wuv_hbm, wo_hbm, bqkv_hbm, bwo_hbm, gate_hbm,
          out_hbm,
          x_v, ckv_v, wq_p, wuk_p, wuv_p, wo_v, bqkv_v, bwo_p, wcur_v, wfst_v,
          qkv_v, acc_v, g_v, z_v, q_s, k_s, v_s, o_st, gate_v,
          sem_x, sem_w, sem_a, sem_o):
    def cp_x(sm, r0, r1, c0, c1):
        sl = (pl.ds(r0 // 2, (r1 - r0) // 2), pl.ds(c0, c1 - c0))
        return pltpu.make_async_copy(x_hbm.bitcast(U32).at[sl], x_v.at[sl], sem_x.at[sm])

    def cp_w(k, c0=0, c1=3 * M, sm=None):
        sl = (pl.ds(k * 128, 128), pl.ds(c0, c1 - c0))
        return pltpu.make_async_copy(bqkv_hbm.at[sl], bqkv_v.at[sl], sem_w.at[k if sm is None else sm])

    x0a, x0b, xr = cp_x(0, 0, R1, 0, 128), cp_x(1, R1, S, 0, 128), cp_x(2, 0, S, 128, M)
    w0a, w0b, w0c = cp_w(0, 0, M), cp_w(0, M, 2 * M, NT_M), cp_w(0, 2 * M, 3 * M, NT_M + 1)
    cp_g = pltpu.make_async_copy(gate_hbm, gate_v, sem_x.at[3])

    def cp_pairs(src, dst):
        return [pltpu.make_async_copy(src.bitcast(U32).at[:, p, :], dst.at[p], sem_a) for p in range(HP)]

    a_early = cp_pairs(bwo_hbm, bwo_p) + [pltpu.make_async_copy(ckv_hbm.bitcast(U32), ckv_v, sem_a),
                                          pltpu.make_async_copy(wo_hbm.bitcast(U32), wo_v, sem_a)]
    a_late = cp_pairs(wuk_hbm, wuk_p) + cp_pairs(wuv_hbm, wuv_p) + cp_pairs(wq_hbm, wq_p)
    a_waits = [pltpu.make_async_copy(b, b, sem_a) for b in (ckv_v, wo_v, wuk_p, wuv_p, wq_p, bwo_p)]

    def cp_o(b0, nb, r0, n, c0=0, c1=M):
        sl = (pl.ds(b0, nb), pl.ds(r0, n), pl.ds(c0, c1 - c0))
        return pltpu.make_async_copy(o_st.at[sl], out_hbm.at[sl], sem_o)

    def prep(part, j, z=None, dep=None):
        k0 = j * 128 if isinstance(j, int) else pl.multiple_of(j * 128, 128)
        for c in range(NT_M):
            src = bqkv_v[pl.ds(k0, 128), part * M + c * 128:part * M + (c + 1) * 128]
            if dep is not None:
                top = pltpu.bitcast(pltpu.bitcast(src[:16], U32) | dep, BF16)
                src = jnp.concatenate([top, src[16:]], axis=0)
            t = pltpu.bitcast(src.T, U32)
            for hp in range(2):
                a, b = t[32 * hp:32 * hp + 16], t[32 * hp + 16:32 * hp + 32]
                r = 2 * c + hp
                wcur_v[part, pl.ds(r, 16, stride=2 * PITCH), :] = (a & jnp.uint32(0xFFFF)) | (b << 16)
                wcur_v[part, pl.ds(PITCH + r, 16, stride=2 * PITCH), :] = (a >> 16) | (b & jnp.uint32(0xFFFF0000))
            if z is not None:
                dep = _zero_after(z, t[56:64])
        return dep

    def wrows(part, d0, d1):
        w = jnp.concatenate([wcur_v[part, d * PITCH:d * PITCH + HP, :] for d in range(d0, d1)], axis=0)
        return pltpu.bitcast(w, BF16)

    def first_tiles(part):
        for n in range(4):
            _st(wfst_v, 0, wrows(part, 4 * n, 4 * n + 4).T, slice(n * 128, (n + 1) * 128))

    def project(xk, part, first):
        if not first:
            return lax.dot_general(xk, wrows(part, 0, DH), NT, preferred_element_type=F32)
        return jnp.concatenate([jnp.dot(xk, _ld(wfst_v, 0, 128), preferred_element_type=F32),
                                lax.dot_general(xk, wrows(part, DH // 2, DH), NT, preferred_element_type=F32)], axis=1)

    def gate_rows(t, z, dep):
        gw = gate_v[...].astype(F32).reshape(1, M)
        g0 = jnp.minimum((t - 1) * GR, S - GR)
        for k in range(GR // 16):
            rr = pl.multiple_of(g0 + k * 16, 16)
            rw = pl.multiple_of(lax.shift_right_logical(rr, 1), 8)
            xb = x_v[pl.ds(rw, 8), :]
            if dep is not None:
                xb = xb | jnp.concatenate([dep] * NT_M, axis=1)
            xx = pltpu.bitcast(xb, BF16).astype(F32)
            zz = jnp.sum(xx * gw, axis=1, keepdims=True)
            g = jnp.broadcast_to(1.0 / (1.0 + jnp.exp(-zz)), (16, 128))
            g_v[pl.ds(rr, 16), :] = g
            acc_v[pl.ds(rr, 16), :] = jnp.zeros((16, M), F32)
            dep = _zero_after(z, g)

    def first_task():
        def piece(part, r0, r1, first):
            y = project(_ld(x_v, r0, r1 - r0, slice(0, 128)), part, first)
            for tt in range(NT_M):
                qkv_v[part, tt, PAD + r0:PAD + r1, :] = y[:, tt * 128:(tt + 1) * 128]

        with _scope("prep0"):
            w0a.wait()
            prep(0, 0)
        with _scope("b1"):
            x0a.wait()
            piece(0, 0, R1, False)
            first_tiles(0)
        with _scope("b2"):
            x0b.wait()
            w0b.wait()
            piece(0, R1, S, True)
            prep(1, 0)
            first_tiles(1)
        with _scope("b3"):
            w0c.wait()
            cp_w(1).wait()
            z = z_v[...]
            piece(1, 0, S, True)
            prep(2, 0)
            dep = prep(0, 1, z)
            first_tiles(0)
            piece(2, 0, S, False)
            prep(1, 1, z, dep)
            prep(2, 1)
            for cc in a_late[:NA1]:
                cc.start()
        for cc in (xr, cp_g):
            cc.wait()
        for cc in a_late[NA1:]:
            cc.start()

    def bproj_body(t, _):
        @pl.when(t < NT_M - 1)
        def _():
            cp_w(t + 1).wait()

        z = z_v[...]
        u = jnp.minimum(t + 1, NT_M - 1)
        xw = x_v[:, pl.ds(pl.multiple_of(t * 128, 128), 128)]
        xk = pltpu.bitcast(xw | jnp.concatenate([z] * (S // 16), axis=0), BF16)
        dep = None
        for part in range(3):
            y = project(xk, part, part == 0)
            for tt in range(NT_M):
                qkv_v[part, tt, PAD:, :] = qkv_v[part, tt, PAD:, :] + y[:, tt * 128:(tt + 1) * 128]
            dep = prep(part, u, z, dep) if part < 2 else prep(part, u)
            if part == 0:
                first_tiles(0)
        gate_rows(t, z, None)
        return 0

    qscale = (D ** -0.5) * LOG2E
    bscale = (DH ** -0.5) * LOG2E

    def local_attn(r, z, dep):
        def zf(v):
            return pltpu.bitcast(_zero_after(z, v), F32)

        sc = jnp.full((8, 128), bscale, F32)
        if dep is not None:
            sc = sc + dep
        q = [qkv_v[0, t, pl.ds(PAD + r, 8), :] * sc for t in range(NT_M)]
        rowi = r + lax.broadcasted_iota(jnp.int32, (8, 128), 0)
        logits, raw = [], []
        for w in range(W):
            a = None if w < LAQ else zf(raw[w - LAQ])
            for t in range(NT_M):
                pr = q[t] * qkv_v[1, t, pl.ds(PAD + r - DIL * w, 8), :]
                a = pr if a is None else a + pr
            raw.append(a)
            a = a + pltpu.roll(a, 64, 1)
            a = a + pltpu.roll(a, 32, 1)
            logits.append(jnp.where(rowi >= DIL * w, a, NEG) if w > 0 else a)
        m = functools.reduce(jnp.maximum, logits)
        es = [jnp.exp2(lg - m) for lg in logits]
        l = functools.reduce(lambda a, b: a + b, es)
        f = (1.0 - g_v[pl.ds(r, 8), :]) * _recip(l)
        es = [e * f for e in es]
        outs = []
        for t in range(NT_M):
            a = None if t == 0 else zf(outs[t - 1])
            for w in range(W):
                pr = es[w] * qkv_v[2, t, pl.ds(PAD + r - DIL * w, 8), :]
                a = pr if a is None else a + pr
            outs.append(a)
        return jnp.concatenate(outs, axis=1), zf(outs[-1])

    def pair_body(p, _):
        z = z_v[...]
        last = p == HP - 1
        wk, wv = _split_pair(wuk_p[p]), _split_pair(wuv_p[p])
        _st(k_s, 0, jnp.dot(_ld(ckv_v, 0, S), wk, preferred_element_type=F32).astype(BF16))
        _st(v_s, 0, jnp.dot(_ld(ckv_v, 0, S), wv, preferred_element_type=F32).astype(BF16))

        rb = pl.multiple_of(p * TL, TL)
        dep, obs = None, []
        for k in range(TL // 8):
            ob, dep = local_attn(rb + k * 8, z, dep)
            obs.append(ob)
        ob = jnp.concatenate(obs, axis=0).astype(BF16)

        wqw = wq_p[p]
        wq = _split_pair(jnp.concatenate([wqw[:8] | _zero_after(z, ob[TL - 16:]), wqw[8:]], axis=0))
        row = lax.broadcasted_iota(jnp.int32, (RG, TQ), 0)
        col = lax.broadcasted_iota(jnp.int32, (RG, TQ), 1)
        diag = col <= row + (TQ - RG)

        def rows(j):
            return [(j - j % G + b) * TQ + (j % G) * RG for b in range(G)]

        def geom(j):
            off = (j % G + 1) * RG % TQ
            return off, j - j % G + (0 if off else 1)

        def gather(ref, j, ld=lambda ref, r: ref[r:r + RG, :]):
            return jnp.concatenate([ld(ref, r) for r in rows(j)], axis=0)

        def qproj(j):
            q = jnp.dot(gather(x_v, j, lambda ref, r: _ld(ref, r, RG)), wq, preferred_element_type=F32) * qscale
            _st(q_s, j * TQ, q.astype(BF16))

        def head(h):
            return slice(h * D, (h + 1) * D)

        left = {}

        def qk(j, hh):
            off, nc = geom(j)
            q = _ld(q_s, j * TQ, TQ, head(hh))
            com = lax.dot_general(q, _ld(k_s, off, nc * TQ, head(hh)), NT, preferred_element_type=F32) if nc else None
            ext = [lax.dot_general(q[e * RG:], _ld(k_s, off + (nc + e - 1) * TQ, TQ, head(hh)), NT,
                                   preferred_element_type=F32) for e in range(1, G)]

            def st(h):
                return lax.dot_general(_ld(k_s, 0, off, head(h)), _ld(q_s, j * TQ, TQ, head(h)), NT,
                                       preferred_element_type=F32)

            if 0 < off <= TQ // 2:
                if hh == 0:
                    pad = [jnp.full((TQ // 2 - off, TQ), NEG, F32)] if off < TQ // 2 else []
                    left[j, 0] = left[j, 1] = jnp.concatenate([st(0)] + pad + [st(1)] + pad, axis=0).T
            elif off:
                left[j, hh] = jnp.concatenate([st(hh), jnp.full((TQ - off, TQ), NEG, F32)], axis=0).T
            return com, ext

        ldep = [None]

        def softmax(parts):
            s = jnp.concatenate(parts, axis=1)
            e = jnp.exp2(s - jnp.max(s, axis=1, keepdims=True))
            if s.shape[1] > SUMT * TQ:
                lp, ldep[0] = _chain_sum(e, z, ldep[0])
                l = jnp.sum(lp, axis=1, keepdims=True)
            else:
                l = jnp.sum(e, axis=1, keepdims=True)
            return e, l

        def softmax_pv(j, hh, sc):
            off, nc = geom(j)
            com, ext = sc
            packed = 0 < off <= TQ // 2
            es, ls = [], []
            for b in range(G):
                rs = slice(b * RG, (b + 1) * RG)
                parts = []
                if off:
                    lf = left[j, hh][rs]
                    c0 = hh * (TQ // 2) if packed else 0
                    if nc + b == 0:
                        keep = col - c0 <= row + (off - RG)
                        lf = jnp.where(jnp.logical_and(keep, col >= c0) if c0 else keep, lf, NEG)
                    elif packed:
                        lf = jnp.where((col >= c0) if hh else (col < TQ // 2), lf, NEG)
                    parts.append(lf)
                parts += [com[rs, t * TQ:(t + 1) * TQ] for t in range(nc)]
                parts += [ext[e - 1][(b - e) * RG:(b - e + 1) * RG] for e in range(1, b + 1)]
                if nc + b:
                    parts[-1] = jnp.where(diag, parts[-1], NEG)
                e, l = softmax(parts)
                es.append(e)
                ls.append(l)
            w = es[0].shape[1]
            vs = []
            if off:
                vs = [_ld(v_s, 0, TQ // 2, head(hh))] * 2 if packed else [_ld(v_s, 0, TQ, head(hh))]
            if nc:
                vs.append(_ld(v_s, off, nc * TQ, head(hh)))
            o = jnp.dot(jnp.concatenate([e[:, :w] for e in es], axis=0).astype(BF16), jnp.concatenate(vs, axis=0),
                        preferred_element_type=F32)
            ox = [jnp.dot(jnp.concatenate([x[:, w + (e - 1) * TQ:w + e * TQ] for x in es[e:]], axis=0).astype(BF16),
                          _ld(v_s, off + (nc + e - 1) * TQ, TQ, head(hh)), preferred_element_type=F32)
                  for e in range(1, G)]
            o = jnp.concatenate([functools.reduce(lambda a, c: a + c, [o[b * RG:(b + 1) * RG]] + [
                ox[e - 1][(b - e) * RG:(b - e + 1) * RG] for e in range(1, b + 1)]) for b in range(G)], axis=0)
            return o * (gather(g_v, j) * _recip(jnp.concatenate(ls, axis=0)))

        def oproj(j, o0, o1):
            y = gather(acc_v, j) + jnp.dot(jnp.concatenate([o0, o1], axis=1).astype(BF16),
                                           _ld(wo_v, p * (2 * D), 2 * D), preferred_element_type=F32)
            for b, r in enumerate(rows(j)):
                acc_v[r:r + RG, :] = y[b * RG:(b + 1) * RG]
                if r < S - TL:
                    o_st[r // TQ, r % TQ:r % TQ + RG, :] = y[b * RG:(b + 1) * RG].astype(BF16)
            j0 = j - j % G
            pl.when(last)(cp_o(j0, min(G, nq - 1 - j0), j % G * RG, RG).start)

        nq = S // TQ
        order = list(reversed(range(nq)))
        items = [(j, hh) for j in order for hh in range(2)]
        n = len(items)
        s_vals, o_vals = {}, {}
        qproj(order[0])
        for step in range(n + LOOK + OLAG):
            if step % 2 == 0 and 1 + step // 2 < nq:
                qproj(order[1 + step // 2])
            if step < n:
                s_vals[step] = qk(*items[step])
            b = step - LOOK
            if 0 <= b < n:
                o_vals[b] = softmax_pv(*items[b], s_vals.pop(b))
            c = step - LOOK - OLAG
            if 0 <= c < n and c % 2 == 1:
                oproj(items[c][0], o_vals.pop(c - 1), o_vals.pop(c))

        wop = jnp.concatenate([f(bwo_p[dp]) for dp in range(DH // 2) for f in (_lo, _hi)], axis=0).astype(BF16)
        y = acc_v[pl.ds(rb, TL), :] + jnp.dot(ob, wop, preferred_element_type=F32)
        acc_v[pl.ds(rb, TL), :] = y
        for c0, c1 in zip(OCUT[:-1], OCUT[1:]):
            o_st[S // TQ - 1, :, c0:c1] = y[:, c0:c1].astype(BF16)
            pl.when(last)(cp_o(S // TQ - 1, 1, 0, TQ, c0, c1).start)
        return 0

    for cc in [w0a, x0a, x0b, w0b, w0c, cp_w(1), cp_g, xr] + [cp_w(k) for k in range(2, NT_M)] + a_early:
        cc.start()
    z_v[...] = jnp.zeros((8, 128), U32)
    for part in range(3):
        for t in range(NT_M):
            qkv_v[part, t, 0:PAD, :] = jnp.zeros((PAD, 128), F32)

    def phases():
        first_task()
        lax.fori_loop(1, NT_M, _scoped("bproj", bproj_body), 0)
        for cc in a_waits:
            cc.wait()
        lax.fori_loop(0, HP, _scoped("pair", pair_body), 0)

    def once(i, _):
        pl.when(i == 0)(phases)
        return 0

    lax.fori_loop(0, 2, once, 0)
    with _scope("ow"):
        cp_o(0, S // TQ, 0, TQ).wait()


def _kernel(*refs):
    dma = pltpu.SemaphoreType.DMA
    pl.run_scoped(functools.partial(_body, *refs), dma((4,)), dma((NT_M + 2,)), dma(()), dma(()))


@jax.jit
def pallas_gated_mix__compressed_kv_cla__sliding_local_dilated__prompt_kernel(
    A_x, A_c_kv, A_w_q, A_w_uk, A_w_uv, A_w_o, B_x, B_wqkv, B_wo, gate_w,
):
    del B_x
    x = A_x.reshape(S, M)
    ckv = A_c_kv.reshape(S, DC)
    wo = A_w_o.reshape(H * D, M)
    bwo = B_wo.reshape(H, DH, M)
    any_spec = pl.BlockSpec(memory_space=pl.ANY)
    out = pl.pallas_call(
        _kernel,
        out_shape=jax.ShapeDtypeStruct((S // TQ, TQ, M), BF16),
        in_specs=[any_spec] * 9,
        out_specs=any_spec,
        scratch_shapes=[
            pltpu.VMEM((S // 2, M), U32),
            pltpu.VMEM((S // 2, DC), U32),
            pltpu.VMEM((HP, M, D), U32),
            pltpu.VMEM((HP, DC, D), U32),
            pltpu.VMEM((HP, DC, D), U32),
            pltpu.VMEM((H * D // 2, M), U32),
            pltpu.VMEM((M, 3 * M), BF16),
            pltpu.VMEM((DH // 2, H, M), U32),
            pltpu.VMEM((3, DH * 24, 128), U32),
            pltpu.VMEM((64, 512), U32),
            pltpu.VMEM((3, NT_M, S + PAD, 128), F32),
            pltpu.VMEM((S, M), F32),
            pltpu.VMEM((S, 128), F32),
            pltpu.VMEM((8, 128), U32),
            pltpu.VMEM((S // 2, 2 * D), U32),
            pltpu.VMEM((S // 2, 2 * D), U32),
            pltpu.VMEM((S // 2, 2 * D), U32),
            pltpu.VMEM((S // TQ, TQ, M), BF16),
            pltpu.VMEM((M,), BF16),
        ],
        compiler_params=pltpu.CompilerParams(vmem_limit_bytes=110 * 1024 * 1024),
    )(x, ckv, A_w_q, A_w_uk, A_w_uv, wo, B_wqkv, bwo, gate_w)
    return out.reshape(1, S, M)
```

```python
import contextlib
import functools

import jax
import jax.numpy as jnp
from jax import lax
import jax.experimental.pallas as pl
import jax.experimental.pallas.tpu as pltpu

S = 2048
M = 1024
DC = 512
H = 32
HP = H // 2
D = 128
DH = 32
W = 8
DIL = 2
PAD = 16
NT_M = M // 128
TQ = 128
TL = S // HP
R1 = 768
GR = 304
PITCH = 17
NA1 = 44
OCUT = (0, 512, 768, M)
LOOK = 2
OLAG = 7
SUMG = 8
SUMT = 5
LAQ = 2
G = 4
RG = TQ // G
GORD = (2, 1, 0, 3)
NCUT = 4
CUTS = {0: (1,), 1: (1, 2), 5: (1,), 6: (1, 2), 9: (1,), 10: (1,), 11: (1,), 13: (1,), 14: (1,), 16: (1,),
        24: (3,), 26: (3,), 27: (4,)}
LOG2E = 1.4426950408889634
NEG = -1e9

F32 = jnp.float32
BF16 = jnp.bfloat16
U32 = jnp.uint32
NT = (((1,), (1,)), ((), ()))


_PROFILE = False


def _scope(name):
    return jax.named_scope(name) if _PROFILE else contextlib.nullcontext()


def _scoped(name, body):
    def f(i, c):
        with _scope(name):
            return body(i, c)
    return f


def _recip(l):
    r = pl.reciprocal(l, approx=True)
    return r * (2.0 - l * r)


def _lo(w):
    return pltpu.bitcast(w << 16, F32)


def _hi(w):
    return pltpu.bitcast(w & jnp.uint32(0xFFFF0000), F32)


def _split_pair(w):
    return jnp.concatenate([_lo(w), _hi(w)], axis=1).astype(BF16)


def _ld(ref, r0, n, cols=slice(None)):
    if isinstance(r0, int):
        rs = slice(r0 // 2, (r0 + n) // 2)
    else:
        rs = pl.ds(pl.multiple_of(lax.shift_right_logical(r0, 1), 8), n // 2)
    return pltpu.bitcast(ref[rs, cols], BF16)


def _st(ref, r0, val, cols=slice(None)):
    ref[r0 // 2:(r0 + val.shape[0]) // 2, cols] = pltpu.bitcast(val, U32)


def _zero_after(z, *vals):
    acc = None
    for v in vals:
        b = pltpu.bitcast(v, U32)
        for r in range(0, b.shape[0], 8):
            for c in range(0, b.shape[1], 128):
                t = b[r:r + 8, c:c + 128]
                acc = t if acc is None else acc | t
    return acc & z


def _chain_sum(x, z, dep):
    parts = []
    for r in range(0, x.shape[0], SUMG):
        a = x[r:r + SUMG, 0:128]
        if dep is not None:
            a = pltpu.bitcast(pltpu.bitcast(a, U32) | jnp.concatenate([dep] * (SUMG // 8), axis=0), F32)
        for c in range(128, x.shape[1], 128):
            a = a + x[r:r + SUMG, c:c + 128]
        dep = _zero_after(z, a)
        parts.append(a)
    return jnp.concatenate(parts, axis=0), dep


def _body(x_hbm, ckv_hbm, wq_hbm, wuk_hbm, wuv_hbm, wo_hbm, bqkv_hbm, bwo_hbm, gate_hbm,
          out_hbm,
          x_v, ckv_v, wq_p, wuk_p, wuv_p, wo_v, bqkv_v, bwo_p, wcur_v, wfst_v,
          qkv_v, acc_v, g_v, z_v, q_s, k_s, v_s, o_st, gate_v,
          sem_x, sem_w, sem_a, sem_o):
    def cp_x(sm, r0, r1, c0, c1):
        sl = (pl.ds(r0 // 2, (r1 - r0) // 2), pl.ds(c0, c1 - c0))
        return pltpu.make_async_copy(x_hbm.bitcast(U32).at[sl], x_v.at[sl], sem_x.at[sm])

    def cp_w(k, c0=0, c1=3 * M, sm=None):
        sl = (pl.ds(k * 128, 128), pl.ds(c0, c1 - c0))
        return pltpu.make_async_copy(bqkv_hbm.at[sl], bqkv_v.at[sl], sem_w.at[k if sm is None else sm])

    x0a, x0b, xr = cp_x(0, 0, R1, 0, 128), cp_x(1, R1, S, 0, 128), cp_x(2, 0, S, 128, M)
    w0a, w0b, w0c = cp_w(0, 0, M), cp_w(0, M, 2 * M, NT_M), cp_w(0, 2 * M, 3 * M, NT_M + 1)
    cp_g = pltpu.make_async_copy(gate_hbm, gate_v.at[pl.ds(0, M)], sem_x.at[3])

    def cp_pairs(src, dst):
        return [pltpu.make_async_copy(src.bitcast(U32).at[:, p, :], dst.at[p], sem_a) for p in range(HP)]

    a_early = cp_pairs(bwo_hbm, bwo_p) + [pltpu.make_async_copy(ckv_hbm.bitcast(U32), ckv_v, sem_a),
                                          pltpu.make_async_copy(wo_hbm.bitcast(U32), wo_v, sem_a)]
    a_late = cp_pairs(wuk_hbm, wuk_p) + cp_pairs(wuv_hbm, wuv_p) + cp_pairs(wq_hbm, wq_p)
    a_waits = [pltpu.make_async_copy(b, b, sem_a) for b in (ckv_v, wo_v, wuk_p, wuv_p, wq_p, bwo_p)]

    def cp_o(b0, nb, r0, n, c0=0, c1=M):
        sl = (pl.ds(b0, nb), pl.ds(r0, n), pl.ds(c0, c1 - c0))
        return pltpu.make_async_copy(o_st.at[sl], out_hbm.at[sl], sem_o)

    def prep(part, j, z=None, dep=None):
        k0 = j * 128 if isinstance(j, int) else pl.multiple_of(j * 128, 128)
        for c in range(NT_M):
            src = bqkv_v[pl.ds(k0, 128), part * M + c * 128:part * M + (c + 1) * 128]
            if dep is not None:
                top = pltpu.bitcast(pltpu.bitcast(src[:16], U32) | dep, BF16)
                src = jnp.concatenate([top, src[16:]], axis=0)
            t = pltpu.bitcast(src.T, U32)
            for hp in range(2):
                a, b = t[32 * hp:32 * hp + 16], t[32 * hp + 16:32 * hp + 32]
                r = 2 * c + hp
                wcur_v[part, pl.ds(r, 16, stride=2 * PITCH), :] = (a & jnp.uint32(0xFFFF)) | (b << 16)
                wcur_v[part, pl.ds(PITCH + r, 16, stride=2 * PITCH), :] = (a >> 16) | (b & jnp.uint32(0xFFFF0000))
            if z is not None:
                dep = _zero_after(z, t[56:64])
        return dep

    def wrows(part, d0, d1):
        w = jnp.concatenate([wcur_v[part, d * PITCH:d * PITCH + HP, :] for d in range(d0, d1)], axis=0)
        return pltpu.bitcast(w, BF16)

    def first_tiles(part):
        for n in range(4):
            _st(wfst_v, 0, wrows(part, 4 * n, 4 * n + 4).T, slice(n * 128, (n + 1) * 128))

    def project(xk, part, first):
        if not first:
            return lax.dot_general(xk, wrows(part, 0, DH), NT, preferred_element_type=F32)
        return jnp.concatenate([jnp.dot(xk, _ld(wfst_v, 0, 128), preferred_element_type=F32),
                                lax.dot_general(xk, wrows(part, DH // 2, DH), NT, preferred_element_type=F32)], axis=1)

    def gate_rows(t, z, dep):
        gw = gate_v[0:M].astype(F32).reshape(1, M)
        g0 = jnp.minimum((t - 1) * GR, S - GR)
        for k in range(GR // 16):
            rr = pl.multiple_of(g0 + k * 16, 16)
            rw = pl.multiple_of(lax.shift_right_logical(rr, 1), 8)
            xb = x_v[pl.ds(rw, 8), :]
            if dep is not None:
                xb = xb | jnp.concatenate([dep] * NT_M, axis=1)
            xx = pltpu.bitcast(xb, BF16).astype(F32)
            zz = jnp.sum(xx * gw, axis=1, keepdims=True)
            g = jnp.broadcast_to(1.0 / (1.0 + jnp.exp(-zz)), (16, 128))
            g_v[pl.ds(rr, 16), :] = g
            acc_v[pl.ds(rr, 16), :] = jnp.zeros((16, M), F32)
            dep = _zero_after(z, g)

    def first_task():
        def piece(part, r0, r1, first):
            y = project(_ld(x_v, r0, r1 - r0, slice(0, 128)), part, first)
            for tt in range(NT_M):
                qkv_v[part, tt, PAD + r0:PAD + r1, :] = y[:, tt * 128:(tt + 1) * 128]

        with _scope("prep0"):
            w0a.wait()
            prep(0, 0)
        with _scope("b1"):
            x0a.wait()
            piece(0, 0, R1, False)
            first_tiles(0)
        with _scope("b2"):
            x0b.wait()
            w0b.wait()
            piece(0, R1, S, True)
            prep(1, 0)
            first_tiles(1)
        with _scope("b3"):
            w0c.wait()
            cp_w(1).wait()
            z = z_v[...]
            piece(1, 0, S, True)
            prep(2, 0)
            dep = prep(0, 1, z)
            first_tiles(0)
            piece(2, 0, S, False)
            prep(1, 1, z, dep)
            prep(2, 1)
            for cc in a_late[:NA1]:
                cc.start()
        for cc in (xr, cp_g):
            cc.wait()
        for cc in a_late[NA1:]:
            cc.start()

    def bproj_body(t, _):
        @pl.when(t < NT_M - 1)
        def _():
            cp_w(t + 1).wait()

        z = z_v[...]
        u = jnp.minimum(t + 1, NT_M - 1)
        xw = x_v[:, pl.ds(pl.multiple_of(t * 128, 128), 128)]
        xk = pltpu.bitcast(xw | jnp.concatenate([z] * (S // 16), axis=0), BF16)
        dep = None
        for part in range(3):
            y = project(xk, part, part == 0)
            for tt in range(NT_M):
                qkv_v[part, tt, PAD:, :] = qkv_v[part, tt, PAD:, :] + y[:, tt * 128:(tt + 1) * 128]
            dep = prep(part, u, z, dep) if part < 2 else prep(part, u)
            if part == 0:
                first_tiles(0)
        gate_rows(t, z, None)
        return 0

    qscale = (D ** -0.5) * LOG2E
    bscale = (DH ** -0.5) * LOG2E

    def local_attn(r, z, dep):
        def zf(v):
            return pltpu.bitcast(_zero_after(z, v), F32)

        sc = jnp.full((8, 128), bscale, F32)
        if dep is not None:
            sc = sc + dep
        q = [qkv_v[0, t, pl.ds(PAD + r, 8), :] * sc for t in range(NT_M)]
        rowi = r + lax.broadcasted_iota(jnp.int32, (8, 128), 0)
        logits, raw = [], []
        for w in range(W):
            a = None if w < LAQ else zf(raw[w - LAQ])
            for t in range(NT_M):
                pr = q[t] * qkv_v[1, t, pl.ds(PAD + r - DIL * w, 8), :]
                a = pr if a is None else a + pr
            raw.append(a)
            a = a + pltpu.roll(a, 64, 1)
            a = a + pltpu.roll(a, 32, 1)
            logits.append(jnp.where(rowi >= DIL * w, a, NEG) if w > 0 else a)
        m = functools.reduce(jnp.maximum, logits)
        es = [jnp.exp2(lg - m) for lg in logits]
        l = functools.reduce(lambda a, b: a + b, es)
        f = (1.0 - g_v[pl.ds(r, 8), :]) * _recip(l)
        es = [e * f for e in es]
        outs = []
        for t in range(NT_M):
            a = None if t == 0 else zf(outs[t - 1])
            for w in range(W):
                pr = es[w] * qkv_v[2, t, pl.ds(PAD + r - DIL * w, 8), :]
                a = pr if a is None else a + pr
            outs.append(a)
        return jnp.concatenate(outs, axis=1), zf(outs[-1])

    def pair_body(p, _):
        z = z_v[...]
        last = p == HP - 1
        wk, wv = _split_pair(wuk_p[p]), _split_pair(wuv_p[p])
        _st(k_s, 0, jnp.dot(_ld(ckv_v, 0, S), wk, preferred_element_type=F32).astype(BF16))
        _st(v_s, 0, jnp.dot(_ld(ckv_v, 0, S), wv, preferred_element_type=F32).astype(BF16))

        rb = pl.multiple_of(p * TL, TL)
        dep, obs = None, []
        for k in range(TL // 8):
            ob, dep = local_attn(rb + k * 8, z, dep)
            obs.append(ob)
        ob = jnp.concatenate(obs, axis=0).astype(BF16)

        wqw = wq_p[p]
        wq = _split_pair(jnp.concatenate([wqw[:8] | _zero_after(z, ob[TL - 16:]), wqw[8:]], axis=0))
        row = lax.broadcasted_iota(jnp.int32, (RG, TQ), 0)
        col = lax.broadcasted_iota(jnp.int32, (RG, TQ), 1)
        diag = col <= row + (TQ - RG)

        def rows(j):
            return [(j - j % G + b) * TQ + (j % G) * RG for b in range(G)]

        def geom(j):
            off = (j % G + 1) * RG % TQ
            return off, j - j % G + (0 if off else 1)

        def gather(ref, j, ld=lambda ref, r: ref[r:r + RG, :]):
            return jnp.concatenate([ld(ref, r) for r in rows(j)], axis=0)

        def qproj(j):
            q = jnp.dot(gather(x_v, j, lambda ref, r: _ld(ref, r, RG)), wq, preferred_element_type=F32) * qscale
            _st(q_s, j * TQ, q.astype(BF16))

        def head(h):
            return slice(h * D, (h + 1) * D)

        left = {}

        def qk(j, hh):
            off, nc = geom(j)
            q = _ld(q_s, j * TQ, TQ, head(hh))
            com = lax.dot_general(q, _ld(k_s, off, nc * TQ, head(hh)), NT, preferred_element_type=F32) if nc else None
            ext = [lax.dot_general(q[e * RG:], _ld(k_s, off + (nc + e - 1) * TQ, TQ, head(hh)), NT,
                                   preferred_element_type=F32) for e in range(1, G)]

            def st(h):
                return lax.dot_general(_ld(k_s, 0, off, head(h)), _ld(q_s, j * TQ, TQ, head(h)), NT,
                                       preferred_element_type=F32)

            if 0 < off <= TQ // 2:
                if hh == 0:
                    pad = [jnp.full((TQ // 2 - off, TQ), NEG, F32)] if off < TQ // 2 else []
                    left[j, 0] = left[j, 1] = jnp.concatenate([st(0)] + pad + [st(1)] + pad, axis=0).T
            elif off:
                left[j, hh] = jnp.concatenate([st(hh), jnp.full((TQ - off, TQ), NEG, F32)], axis=0).T
            return com, ext

        ldep = [None]

        def softmax(parts):
            s = jnp.concatenate(parts, axis=1)
            e = jnp.exp2(s - jnp.max(s, axis=1, keepdims=True))
            if s.shape[1] > SUMT * TQ:
                lp, ldep[0] = _chain_sum(e, z, ldep[0])
                l = jnp.sum(lp, axis=1, keepdims=True)
            else:
                l = jnp.sum(e, axis=1, keepdims=True)
            return e, l

        def softmax_pv(j, hh, sc):
            off, nc = geom(j)
            com, ext = sc
            packed = 0 < off <= TQ // 2
            es, ls = [None] * G, [None] * G
            for b in reversed(range(G)):
                rs = slice(b * RG, (b + 1) * RG)
                parts = []
                if off:
                    lf = left[j, hh][rs]
                    c0 = hh * (TQ // 2) if packed else 0
                    if nc + b == 0:
                        keep = col - c0 <= row + (off - RG)
                        lf = jnp.where(jnp.logical_and(keep, col >= c0) if c0 else keep, lf, NEG)
                    elif packed:
                        lf = jnp.where((col >= c0) if hh else (col < TQ // 2), lf, NEG)
                    parts.append(lf)
                parts += [com[rs, t * TQ:(t + 1) * TQ] for t in range(nc)]
                parts += [ext[e - 1][(b - e) * RG:(b - e + 1) * RG] for e in range(1, b + 1)]
                if nc + b:
                    parts[-1] = jnp.where(diag, parts[-1], NEG)
                es[b], ls[b] = softmax(parts)
            w = es[0].shape[1]
            vs = []
            if off:
                vs = [_ld(v_s, 0, TQ // 2, head(hh))] * 2 if packed else [_ld(v_s, 0, TQ, head(hh))]
            if nc:
                vs.append(_ld(v_s, off, nc * TQ, head(hh)))
            o = jnp.dot(jnp.concatenate([e[:, :w] for e in es], axis=0).astype(BF16), jnp.concatenate(vs, axis=0),
                        preferred_element_type=F32)
            ox = [jnp.dot(jnp.concatenate([x[:, w + (e - 1) * TQ:w + e * TQ] for x in es[e:]], axis=0).astype(BF16),
                          _ld(v_s, off + (nc + e - 1) * TQ, TQ, head(hh)), preferred_element_type=F32)
                  for e in range(1, G)]
            o = jnp.concatenate([functools.reduce(lambda a, c: a + c, [o[b * RG:(b + 1) * RG]] + [
                ox[e - 1][(b - e) * RG:(b - e + 1) * RG] for e in range(1, b + 1)]) for b in range(G)], axis=0)
            return o * (gather(g_v, j) * _recip(jnp.concatenate(ls, axis=0)))

        def oproj(j, o0, o1):
            y = gather(acc_v, j) + jnp.dot(jnp.concatenate([o0, o1], axis=1).astype(BF16),
                                           _ld(wo_v, p * (2 * D), 2 * D), preferred_element_type=F32)
            for b, r in enumerate(rows(j)):
                acc_v[r:r + RG, :] = y[b * RG:(b + 1) * RG]
                if r < S - TL:
                    o_st[r // TQ, r % TQ:r % TQ + RG, :] = y[b * RG:(b + 1) * RG].astype(BF16)
            j0 = j - j % G
            pl.when(last)(cp_o(j0, min(G, nq - 1 - j0), j % G * RG, RG).start)

        nq = S // TQ
        order = [m * G + g for m in reversed(range(nq // G)) for g in GORD]
        items = [(j, hh) for j in order for hh in range(2)]
        n = len(items)
        s_vals, o_vals = {}, {}
        qproj(order[0])
        for step in range(n + LOOK + OLAG):
            if step % 2 == 0 and 1 + step // 2 < nq:
                qproj(order[1 + step // 2])
            if step < n:
                s_vals[step] = qk(*items[step])
            b = step - LOOK
            if 0 <= b < n:
                o_vals[b] = softmax_pv(*items[b], s_vals.pop(b))
            c = step - LOOK - OLAG
            if 0 <= c < n and c % 2 == 1:
                oproj(items[c][0], o_vals.pop(c - 1), o_vals.pop(c))

        wop = jnp.concatenate([f(bwo_p[dp]) for dp in range(DH // 2) for f in (_lo, _hi)], axis=0).astype(BF16)
        c0 = M - 128 * NCUT
        yl = acc_v[pl.ds(rb, TL), :c0] + jnp.dot(ob, wop[:, :c0], preferred_element_type=F32)
        ya = acc_v[pl.ds(rb, TL), c0:]
        yr = [[ya[r:r + 16, c:c + 128] for r in range(0, TL, 16)] for c in range(0, M - c0, 128)]
        for tile in range(NT_M * NCUT):
            c, k = divmod(tile, NT_M)
            cuts = (0,) + CUTS.get(tile, ()) + (TL // 16,)
            for u0, u1 in zip(cuts[:-1], cuts[1:]):
                t = jnp.dot(ob[u0 * 16:u1 * 16, k * 128:(k + 1) * 128],
                            wop[k * 128:(k + 1) * 128, c0 + c * 128:c0 + (c + 1) * 128], preferred_element_type=F32)
                for u in range(u0, u1):
                    yr[c][u] = yr[c][u] + t[(u - u0) * 16:(u - u0 + 1) * 16]
        y = jnp.concatenate([yl] + [jnp.concatenate(v, axis=0) for v in yr], axis=1)
        acc_v[pl.ds(rb, TL), :] = y
        for c0, c1 in zip(OCUT[:-1], OCUT[1:]):
            o_st[S // TQ - 1, :, c0:c1] = y[:, c0:c1].astype(BF16)
            pl.when(last)(cp_o(S // TQ - 1, 1, 0, TQ, c0, c1).start)
        return 0

    for cc in [w0a, x0a, x0b, w0b, w0c, cp_w(1), cp_g, xr] + [cp_w(k) for k in range(2, NT_M)] + a_early:
        cc.start()
    z_v[...] = jnp.zeros((8, 128), U32)
    for part in range(3):
        for t in range(NT_M):
            qkv_v[part, t, 0:PAD, :] = jnp.zeros((PAD, 128), F32)

    def phases():
        first_task()
        lax.fori_loop(1, NT_M, _scoped("bproj", bproj_body), 0)
        for cc in a_waits:
            cc.wait()
        lax.fori_loop(0, HP, _scoped("pair", pair_body), 0)

    def once(i, _):
        pl.when(i == 0)(phases)
        return 0

    lax.fori_loop(0, 2, once, 0)
    with _scope("ow"):
        cp_o(0, S // TQ, 0, TQ).wait()


def _kernel(*refs):
    dma = pltpu.SemaphoreType.DMA
    pl.run_scoped(functools.partial(_body, *refs), dma((4,)), dma((NT_M + 2,)), dma(()), dma(()))


@jax.jit
def pallas_gated_mix__compressed_kv_cla__sliding_local_dilated__prompt_kernel(
    A_x, A_c_kv, A_w_q, A_w_uk, A_w_uv, A_w_o, B_x, B_wqkv, B_wo, gate_w,
):
    del B_x
    x = A_x.reshape(S, M)
    ckv = A_c_kv.reshape(S, DC)
    wo = A_w_o.reshape(H * D, M)
    bwo = B_wo.reshape(H, DH, M)
    any_spec = pl.BlockSpec(memory_space=pl.ANY)
    out = pl.pallas_call(
        _kernel,
        out_shape=jax.ShapeDtypeStruct((S // TQ, TQ, M), BF16),
        in_specs=[any_spec] * 9,
        out_specs=any_spec,
        scratch_shapes=[
            pltpu.VMEM((S // 2, M), U32),
            pltpu.VMEM((S // 2, DC), U32),
            pltpu.VMEM((HP, M, D), U32),
            pltpu.VMEM((HP, DC, D), U32),
            pltpu.VMEM((HP, DC, D), U32),
            pltpu.VMEM((H * D // 2, M), U32),
            pltpu.VMEM((M, 3 * M), BF16),
            pltpu.VMEM((DH // 2, H, M), U32),
            pltpu.VMEM((3, DH * 24, 128), U32),
            pltpu.VMEM((64, 512), U32),
            pltpu.VMEM((3, NT_M, S + PAD, 128), F32),
            pltpu.VMEM((S, M), F32),
            pltpu.VMEM((S, 128), F32),
            pltpu.VMEM((8, 128), U32),
            pltpu.VMEM((S // 2, 2 * D), U32),
            pltpu.VMEM((S // 2, 2 * D), U32),
            pltpu.VMEM((S // 2, 2 * D), U32),
            pltpu.VMEM((S // TQ, TQ, M), BF16),
            pltpu.VMEM((2 * M,), BF16),
        ],
        compiler_params=pltpu.CompilerParams(vmem_limit_bytes=110 * 1024 * 1024),
    )(x, ckv, A_w_q, A_w_uk, A_w_uv, wo, B_wqkv, bwo, gate_w)
    return out.reshape(1, S, M)
```

```python
import contextlib
import functools

import jax
import jax.numpy as jnp
from jax import lax
import jax.experimental.pallas as pl
import jax.experimental.pallas.tpu as pltpu

S = 2048
M = 1024
DC = 512
H = 32
HP = H // 2
D = 128
DH = 32
W = 8
DIL = 2
PAD = 16
NT_M = M // 128
TQ = 128
TL = S // HP
R1 = 768
GR = 304
PITCH = 17
NA1 = 44
OCUT = (0, 512, 768, M)
LOOK = 2
OLAG = 7
SUMT = 4
MAXT = 3
LAQ = 2
G = 8
RG = TQ // G
NCUT = 4
CUTS = {0: (1,), 1: (1, 2), 5: (1,), 6: (1, 2), 9: (1, 2), 13: (1,), 14: (1,), 17: (1,), 19: (1,), 24: (1,),
        31: (5, 7)}
LOG2E = 1.4426950408889634
NEG = -1e9

F32 = jnp.float32
BF16 = jnp.bfloat16
U32 = jnp.uint32
NT = (((1,), (1,)), ((), ()))


_PROFILE = False


def _scope(name):
    return jax.named_scope(name) if _PROFILE else contextlib.nullcontext()


def _scoped(name, body):
    def f(i, c):
        with _scope(name):
            return body(i, c)
    return f


def _recip(l):
    r = pl.reciprocal(l, approx=True)
    return r * (2.0 - l * r)


def _lo(w):
    return pltpu.bitcast(w << 16, F32)


def _hi(w):
    return pltpu.bitcast(w & jnp.uint32(0xFFFF0000), F32)


def _split_pair(w):
    return jnp.concatenate([_lo(w), _hi(w)], axis=1).astype(BF16)


def _ld(ref, r0, n, cols=slice(None)):
    if isinstance(r0, int):
        rs = slice(r0 // 2, (r0 + n) // 2)
    else:
        rs = pl.ds(pl.multiple_of(lax.shift_right_logical(r0, 1), 8), n // 2)
    return pltpu.bitcast(ref[rs, cols], BF16)


def _st(ref, r0, val, cols=slice(None)):
    ref[r0 // 2:(r0 + val.shape[0]) // 2, cols] = pltpu.bitcast(val, U32)


def _zero_after(z, *vals):
    acc = None
    for v in vals:
        b = pltpu.bitcast(v, U32)
        for r in range(0, b.shape[0], 8):
            for c in range(0, b.shape[1], 128):
                t = b[r:r + 8, c:c + 128]
                acc = t if acc is None else acc | t
    return acc & z


def _chain(op, tiles, z, dep):
    a = tiles[0]
    if dep is not None:
        a = pltpu.bitcast(pltpu.bitcast(a, U32) | jnp.concatenate([dep] * (a.shape[0] // 8), axis=0), F32)
    a = functools.reduce(op, [a] + tiles[1:])
    return a, _zero_after(z, a)


def _body(x_hbm, ckv_hbm, wq_hbm, wuk_hbm, wuv_hbm, wo_hbm, bqkv_hbm, bwo_hbm, gate_hbm,
          out_hbm,
          x_v, ckv_v, wq_p, wuk_p, wuv_p, wo_v, bqkv_v, bwo_p, wcur_v, wfst_v,
          qkv_v, acc_v, g_v, z_v, q_s, k_s, v_s, o_st, gate_v,
          sem_x, sem_w, sem_a, sem_o):
    def cp_x(sm, r0, r1, c0, c1):
        sl = (pl.ds(r0 // 2, (r1 - r0) // 2), pl.ds(c0, c1 - c0))
        return pltpu.make_async_copy(x_hbm.bitcast(U32).at[sl], x_v.at[sl], sem_x.at[sm])

    def cp_w(k, c0=0, c1=3 * M, sm=None):
        sl = (pl.ds(k * 128, 128), pl.ds(c0, c1 - c0))
        return pltpu.make_async_copy(bqkv_hbm.at[sl], bqkv_v.at[sl], sem_w.at[k if sm is None else sm])

    x0a, x0b, xr = cp_x(0, 0, R1, 0, 128), cp_x(1, R1, S, 0, 128), cp_x(2, 0, S, 128, M)
    w0a, w0b, w0c = cp_w(0, 0, M), cp_w(0, M, 2 * M, NT_M), cp_w(0, 2 * M, 3 * M, NT_M + 1)
    cp_g = pltpu.make_async_copy(gate_hbm, gate_v.at[pl.ds(0, M)], sem_x.at[3])

    def cp_pairs(src, dst):
        return [pltpu.make_async_copy(src.bitcast(U32).at[:, p, :], dst.at[p], sem_a) for p in range(HP)]

    a_early = cp_pairs(bwo_hbm, bwo_p) + [pltpu.make_async_copy(ckv_hbm.bitcast(U32), ckv_v, sem_a),
                                          pltpu.make_async_copy(wo_hbm.bitcast(U32), wo_v, sem_a)]
    a_late = cp_pairs(wuk_hbm, wuk_p) + cp_pairs(wuv_hbm, wuv_p) + cp_pairs(wq_hbm, wq_p)
    a_waits = [pltpu.make_async_copy(b, b, sem_a) for b in (ckv_v, wo_v, wuk_p, wuv_p, wq_p, bwo_p)]

    def cp_o(b0, nb, r0, n, c0=0, c1=M):
        sl = (pl.ds(b0, nb), pl.ds(r0, n), pl.ds(c0, c1 - c0))
        return pltpu.make_async_copy(o_st.at[sl], out_hbm.at[sl], sem_o)

    def prep(part, j, z=None, dep=None):
        k0 = j * 128 if isinstance(j, int) else pl.multiple_of(j * 128, 128)
        for c in range(NT_M):
            src = bqkv_v[pl.ds(k0, 128), part * M + c * 128:part * M + (c + 1) * 128]
            if dep is not None:
                top = pltpu.bitcast(pltpu.bitcast(src[:16], U32) | dep, BF16)
                src = jnp.concatenate([top, src[16:]], axis=0)
            t = pltpu.bitcast(src.T, U32)
            for hp in range(2):
                a, b = t[32 * hp:32 * hp + 16], t[32 * hp + 16:32 * hp + 32]
                r = 2 * c + hp
                wcur_v[part, pl.ds(r, 16, stride=2 * PITCH), :] = (a & jnp.uint32(0xFFFF)) | (b << 16)
                wcur_v[part, pl.ds(PITCH + r, 16, stride=2 * PITCH), :] = (a >> 16) | (b & jnp.uint32(0xFFFF0000))
            if z is not None:
                dep = _zero_after(z, t[56:64])
        return dep

    def wrows(part, d0, d1):
        w = jnp.concatenate([wcur_v[part, d * PITCH:d * PITCH + HP, :] for d in range(d0, d1)], axis=0)
        return pltpu.bitcast(w, BF16)

    def first_tiles(part):
        for n in range(4):
            _st(wfst_v, 0, wrows(part, 4 * n, 4 * n + 4).T, slice(n * 128, (n + 1) * 128))

    def project(xk, part, first):
        if not first:
            return lax.dot_general(xk, wrows(part, 0, DH), NT, preferred_element_type=F32)
        return jnp.concatenate([jnp.dot(xk, _ld(wfst_v, 0, 128), preferred_element_type=F32),
                                lax.dot_general(xk, wrows(part, DH // 2, DH), NT, preferred_element_type=F32)], axis=1)

    def gate_rows(t, z, dep):
        gw = gate_v[0:M].astype(F32).reshape(1, M)
        g0 = jnp.minimum((t - 1) * GR, S - GR)
        for k in range(GR // 16):
            rr = pl.multiple_of(g0 + k * 16, 16)
            rw = pl.multiple_of(lax.shift_right_logical(rr, 1), 8)
            xb = x_v[pl.ds(rw, 8), :]
            if dep is not None:
                xb = xb | jnp.concatenate([dep] * NT_M, axis=1)
            xx = pltpu.bitcast(xb, BF16).astype(F32)
            zz = jnp.sum(xx * gw, axis=1, keepdims=True)
            g = jnp.broadcast_to(1.0 / (1.0 + jnp.exp(-zz)), (16, 128))
            g_v[pl.ds(rr, 16), :] = g
            acc_v[pl.ds(rr, 16), :] = jnp.zeros((16, M), F32)
            dep = _zero_after(z, g)

    def first_task():
        def piece(part, r0, r1, first):
            y = project(_ld(x_v, r0, r1 - r0, slice(0, 128)), part, first)
            for tt in range(NT_M):
                qkv_v[part, tt, PAD + r0:PAD + r1, :] = y[:, tt * 128:(tt + 1) * 128]

        with _scope("prep0"):
            w0a.wait()
            prep(0, 0)
        with _scope("b1"):
            x0a.wait()
            piece(0, 0, R1, False)
            first_tiles(0)
        with _scope("b2"):
            x0b.wait()
            w0b.wait()
            piece(0, R1, S, True)
            prep(1, 0)
            first_tiles(1)
        with _scope("b3"):
            w0c.wait()
            cp_w(1).wait()
            z = z_v[...]
            piece(1, 0, S, True)
            prep(2, 0)
            dep = prep(0, 1, z)
            first_tiles(0)
            piece(2, 0, S, False)
            prep(1, 1, z, dep)
            prep(2, 1)
            for cc in a_late[:NA1]:
                cc.start()
        for cc in (xr, cp_g):
            cc.wait()
        for cc in a_late[NA1:]:
            cc.start()

    def bproj_body(t, _):
        @pl.when(t < NT_M - 1)
        def _():
            cp_w(t + 1).wait()

        z = z_v[...]
        u = jnp.minimum(t + 1, NT_M - 1)
        xw = x_v[:, pl.ds(pl.multiple_of(t * 128, 128), 128)]
        xk = pltpu.bitcast(xw | jnp.concatenate([z] * (S // 16), axis=0), BF16)
        dep = None
        for part in range(3):
            y = project(xk, part, part == 0)
            for tt in range(NT_M):
                qkv_v[part, tt, PAD:, :] = qkv_v[part, tt, PAD:, :] + y[:, tt * 128:(tt + 1) * 128]
            dep = prep(part, u, z, dep) if part < 2 else prep(part, u)
            if part == 0:
                first_tiles(0)
        gate_rows(t, z, None)
        return 0

    qscale = (D ** -0.5) * LOG2E
    bscale = (DH ** -0.5) * LOG2E

    def local_attn(r, z, dep):
        def zf(v):
            return pltpu.bitcast(_zero_after(z, v), F32)

        sc = jnp.full((8, 128), bscale, F32)
        if dep is not None:
            sc = sc + dep
        q = [qkv_v[0, t, pl.ds(PAD + r, 8), :] * sc for t in range(NT_M)]
        rowi = r + lax.broadcasted_iota(jnp.int32, (8, 128), 0)
        logits, raw = [], []
        for w in range(W):
            a = None if w < LAQ else zf(raw[w - LAQ])
            for t in range(NT_M):
                pr = q[t] * qkv_v[1, t, pl.ds(PAD + r - DIL * w, 8), :]
                a = pr if a is None else a + pr
            raw.append(a)
            a = a + pltpu.roll(a, 64, 1)
            a = a + pltpu.roll(a, 32, 1)
            logits.append(jnp.where(rowi >= DIL * w, a, NEG) if w > 0 else a)
        m = functools.reduce(jnp.maximum, logits)
        es = [jnp.exp2(lg - m) for lg in logits]
        l = functools.reduce(lambda a, b: a + b, es)
        f = (1.0 - g_v[pl.ds(r, 8), :]) * _recip(l)
        es = [e * f for e in es]
        outs = []
        for t in range(NT_M):
            a = None if t == 0 else zf(outs[t - 1])
            for w in range(W):
                pr = es[w] * qkv_v[2, t, pl.ds(PAD + r - DIL * w, 8), :]
                a = pr if a is None else a + pr
            outs.append(a)
        return jnp.concatenate(outs, axis=1), zf(outs[-1])

    def pair_body(p, _):
        z = z_v[...]
        last = p == HP - 1
        wk, wv = _split_pair(wuk_p[p]), _split_pair(wuv_p[p])
        _st(k_s, 0, jnp.dot(_ld(ckv_v, 0, S), wk, preferred_element_type=F32).astype(BF16))
        _st(v_s, 0, jnp.dot(_ld(ckv_v, 0, S), wv, preferred_element_type=F32).astype(BF16))

        rb = pl.multiple_of(p * TL, TL)
        dep, obs = None, []
        for k in range(TL // 8):
            ob, dep = local_attn(rb + k * 8, z, dep)
            if k == 0:
                v = g_v[pl.ds(rb, 24), :]
                dep = dep + pltpu.bitcast(_zero_after(z, jnp.broadcast_to(v[:, 0:1], v.shape)), F32)
            obs.append(ob)
        ob = jnp.concatenate(obs, axis=0).astype(BF16)

        wqw = wq_p[p]
        wq = _split_pair(jnp.concatenate([wqw[:8] | _zero_after(z, ob[TL - 16:]), wqw[8:]], axis=0))
        row = lax.broadcasted_iota(jnp.int32, (RG, TQ), 0)
        col = lax.broadcasted_iota(jnp.int32, (RG, TQ), 1)
        diag = col <= row + (TQ - RG)

        def rows(j):
            return [(j - j % G + b) * TQ + (j % G) * RG for b in range(G)]

        def geom(j):
            off = (j % G + 1) * RG % TQ
            return off, j - j % G + (0 if off else 1)

        def gather(ref, j, ld=lambda ref, r: ref[r:r + RG, :]):
            return jnp.concatenate([ld(ref, r) for r in rows(j)], axis=0)

        def qproj(j):
            q = jnp.dot(gather(x_v, j, lambda ref, r: _ld(ref, r, RG)), wq, preferred_element_type=F32) * qscale
            _st(q_s, j * TQ, q.astype(BF16))

        def head(h):
            return slice(h * D, (h + 1) * D)

        def qk(j, hh):
            off, nc = geom(j)
            q = _ld(q_s, j * TQ, TQ, head(hh))
            com = lax.dot_general(q, _ld(k_s, off, nc * TQ, head(hh)), NT, preferred_element_type=F32) if nc else None
            ext = {e: lax.dot_general(q[e * RG:], _ld(k_s, off + (nc + e - 1) * TQ, TQ, head(hh)), NT,
                                      preferred_element_type=F32) for e in reversed(range(1, G))}
            left = None
            if off:
                st = lax.dot_general(_ld(k_s, 0, off, head(hh)), q, NT, preferred_element_type=F32)
                left = jnp.concatenate([st, jnp.full((TQ - off, TQ), NEG, F32)], axis=0).T
            return com, ext, left

        deps = {"max": None, "sum": None}

        def softmax(parts):
            if len(parts) > MAXT:
                m, deps["max"] = _chain(jnp.maximum, parts[1:], z, deps["max"])
                m = jnp.maximum(m, parts[0])
            else:
                m = functools.reduce(jnp.maximum, parts[1:] + parts[:1])
            e = jnp.exp2(jnp.concatenate(parts, axis=1) - jnp.max(m, axis=1, keepdims=True))
            l = e
            if len(parts) > SUMT:
                l, deps["sum"] = _chain(jnp.add, [e[:, c:c + TQ] for c in range(0, e.shape[1], TQ)], z, deps["sum"])
            return e, jnp.sum(l, axis=1, keepdims=True)

        def softmax_pv(j, hh, sc):
            off, nc = geom(j)
            com, ext, left = sc
            es, ls = [], []
            for b in range(G):
                rs = slice(b * RG, (b + 1) * RG)
                parts = [left[rs]] if off else []
                parts += [com[rs, t * TQ:(t + 1) * TQ] for t in range(nc)]
                parts += [ext[e][(b - e) * RG:(b - e + 1) * RG] for e in range(1, b + 1)]
                parts[-1] = jnp.where(diag if nc + b else col <= row + (off - RG), parts[-1], NEG)
                e, l = softmax(parts)
                es.append(e)
                ls.append(l)
            w = es[0].shape[1]
            vs = [_ld(v_s, 0, TQ, head(hh))] if off else []
            if nc:
                vs.append(_ld(v_s, off, nc * TQ, head(hh)))
            o = jnp.dot(jnp.concatenate([e[:, :w] for e in es], axis=0).astype(BF16), jnp.concatenate(vs, axis=0),
                        preferred_element_type=F32)
            ox = [jnp.dot(jnp.concatenate([x[:, w + (e - 1) * TQ:w + e * TQ] for x in es[e:]], axis=0).astype(BF16),
                          _ld(v_s, off + (nc + e - 1) * TQ, TQ, head(hh)), preferred_element_type=F32)
                  for e in range(1, G)]
            o = jnp.concatenate([functools.reduce(lambda a, c: a + c, [o[b * RG:(b + 1) * RG]] + [
                ox[e - 1][(b - e) * RG:(b - e + 1) * RG] for e in range(1, b + 1)]) for b in range(G)], axis=0)
            return o * (gather(g_v, j) * _recip(jnp.concatenate(ls, axis=0)))

        def oproj(j, o0, o1):
            y = gather(acc_v, j) + jnp.dot(jnp.concatenate([o0, o1], axis=1).astype(BF16),
                                           _ld(wo_v, p * (2 * D), 2 * D), preferred_element_type=F32)
            for b, r in enumerate(rows(j)):
                acc_v[r:r + RG, :] = y[b * RG:(b + 1) * RG]
                if r < S - TL:
                    o_st[r // TQ, r % TQ:r % TQ + RG, :] = y[b * RG:(b + 1) * RG].astype(BF16)
            j0 = j - j % G
            pl.when(last)(cp_o(j0, min(G, nq - 1 - j0), j % G * RG, RG).start)

        nq = S // TQ
        order = [m * G + g for m in reversed(range(nq // G)) for g in range(G)]
        items = [(j, hh) for j in order for hh in range(2)]
        n = len(items)
        s_vals, o_vals = {}, {}
        qproj(order[0])
        for step in range(n + LOOK + OLAG):
            if step % 2 == 0 and 1 + step // 2 < nq:
                qproj(order[1 + step // 2])
            if step < n:
                s_vals[step] = qk(*items[step])
            b = step - LOOK
            if 0 <= b < n:
                o_vals[b] = softmax_pv(*items[b], s_vals.pop(b))
            c = step - LOOK - OLAG
            if 0 <= c < n and c % 2 == 1:
                oproj(items[c][0], o_vals.pop(c - 1), o_vals.pop(c))

        wop = jnp.concatenate([f(bwo_p[dp]) for dp in range(DH // 2) for f in (_lo, _hi)], axis=0).astype(BF16)
        c0 = M - 128 * NCUT
        yl = acc_v[pl.ds(rb, TL), :c0] + jnp.dot(ob, wop[:, :c0], preferred_element_type=F32)
        ya = acc_v[pl.ds(rb, TL), c0:]
        yr = [[ya[r:r + 16, c:c + 128] for r in range(0, TL, 16)] for c in range(0, M - c0, 128)]
        for tile in range(NT_M * NCUT):
            c, k = divmod(tile, NT_M)
            cuts = (0,) + CUTS.get(tile, ()) + (TL // 16,)
            for u0, u1 in zip(cuts[:-1], cuts[1:]):
                t = jnp.dot(ob[u0 * 16:u1 * 16, k * 128:(k + 1) * 128],
                            wop[k * 128:(k + 1) * 128, c0 + c * 128:c0 + (c + 1) * 128], preferred_element_type=F32)
                for u in range(u0, u1):
                    yr[c][u] = yr[c][u] + t[(u - u0) * 16:(u - u0 + 1) * 16]
        y = jnp.concatenate([yl] + [jnp.concatenate(v, axis=0) for v in yr], axis=1)
        acc_v[pl.ds(rb, TL), :] = y
        for c0, c1 in zip(OCUT[:-1], OCUT[1:]):
            o_st[S // TQ - 1, :, c0:c1] = y[:, c0:c1].astype(BF16)
            pl.when(last)(cp_o(S // TQ - 1, 1, 0, TQ, c0, c1).start)
        return 0

    for cc in [w0a, x0a, x0b, w0b, w0c, cp_w(1), cp_g, xr] + [cp_w(k) for k in range(2, NT_M)] + a_early:
        cc.start()
    z_v[...] = jnp.zeros((8, 128), U32)
    for part in range(3):
        for t in range(NT_M):
            qkv_v[part, t, 0:PAD, :] = jnp.zeros((PAD, 128), F32)

    def phases():
        first_task()
        lax.fori_loop(1, NT_M, _scoped("bproj", bproj_body), 0)
        for cc in a_waits:
            cc.wait()
        lax.fori_loop(0, HP, _scoped("pair", pair_body), 0)

    def once(i, _):
        pl.when(i == 0)(phases)
        return 0

    lax.fori_loop(0, 2, once, 0)
    with _scope("ow"):
        cp_o(0, S // TQ, 0, TQ).wait()


def _kernel(*refs):
    dma = pltpu.SemaphoreType.DMA
    pl.run_scoped(functools.partial(_body, *refs), dma((4,)), dma((NT_M + 2,)), dma(()), dma(()))


@jax.jit
def pallas_gated_mix__compressed_kv_cla__sliding_local_dilated__prompt_kernel(
    A_x, A_c_kv, A_w_q, A_w_uk, A_w_uv, A_w_o, B_x, B_wqkv, B_wo, gate_w,
):
    del B_x
    x = A_x.reshape(S, M)
    ckv = A_c_kv.reshape(S, DC)
    wo = A_w_o.reshape(H * D, M)
    bwo = B_wo.reshape(H, DH, M)
    any_spec = pl.BlockSpec(memory_space=pl.ANY)
    out = pl.pallas_call(
        _kernel,
        out_shape=jax.ShapeDtypeStruct((S // TQ, TQ, M), BF16),
        in_specs=[any_spec] * 9,
        out_specs=any_spec,
        scratch_shapes=[
            pltpu.VMEM((S // 2, M), U32),
            pltpu.VMEM((S // 2, DC), U32),
            pltpu.VMEM((HP, M, D), U32),
            pltpu.VMEM((HP, DC, D), U32),
            pltpu.VMEM((HP, DC, D), U32),
            pltpu.VMEM((H * D // 2, M), U32),
            pltpu.VMEM((M, 3 * M), BF16),
            pltpu.VMEM((DH // 2, H, M), U32),
            pltpu.VMEM((3, DH * 24, 128), U32),
            pltpu.VMEM((64, 512), U32),
            pltpu.VMEM((3, NT_M, S + PAD, 128), F32),
            pltpu.VMEM((S, M), F32),
            pltpu.VMEM((S, 128), F32),
            pltpu.VMEM((8, 128), U32),
            pltpu.VMEM((S // 2, 2 * D), U32),
            pltpu.VMEM((S // 2, 2 * D), U32),
            pltpu.VMEM((S // 2, 2 * D), U32),
            pltpu.VMEM((S // TQ, TQ, M), BF16),
            pltpu.VMEM((2 * M,), BF16),
        ],
        compiler_params=pltpu.CompilerParams(vmem_limit_bytes=110 * 1024 * 1024),
    )(x, ckv, A_w_q, A_w_uk, A_w_uv, wo, B_wqkv, bwo, gate_w)
    return out.reshape(1, S, M)
```

```python
import contextlib
import functools

import jax
import jax.numpy as jnp
from jax import lax
import jax.experimental.pallas as pl
import jax.experimental.pallas.tpu as pltpu

S = 2048
M = 1024
DC = 512
H = 32
HP = H // 2
D = 128
DH = 32
W = 8
DIL = 2
PAD = 16
NT_M = M // 128
TQ = 128
TL = S // HP
R1 = 768
GR = 304
PITCH = 17
NA1 = 44
OCUT = (0, 512, 768, M)
LOOK = 2
OLAG = 7
SUMT = 4
MAXT = 3
LAQ = 2
G = 8
RG = TQ // G
ORDER = (8, 9, 2, 11, 12, 5, 6, 7, 0, 1, 10, 3, 4, 13, 14, 15)
NCUT = 4
CUTS = {0: (1,), 1: (1, 2), 5: (1,), 6: (1, 2), 9: (1, 2), 13: (1,), 14: (1,), 17: (1,), 19: (1,), 24: (1,),
        31: (5, 7)}
LOG2E = 1.4426950408889634
NEG = -1e9

F32 = jnp.float32
BF16 = jnp.bfloat16
U32 = jnp.uint32
NT = (((1,), (1,)), ((), ()))


_PROFILE = False


def _scope(name):
    return jax.named_scope(name) if _PROFILE else contextlib.nullcontext()


def _scoped(name, body):
    def f(i, c):
        with _scope(name):
            return body(i, c)
    return f


def _recip(l):
    r = pl.reciprocal(l, approx=True)
    return r * (2.0 - l * r)


def _lo(w):
    return pltpu.bitcast(w << 16, F32)


def _hi(w):
    return pltpu.bitcast(w & jnp.uint32(0xFFFF0000), F32)


def _split_pair(w):
    return jnp.concatenate([_lo(w), _hi(w)], axis=1).astype(BF16)


def _ld(ref, r0, n, cols=slice(None)):
    if isinstance(r0, int):
        rs = slice(r0 // 2, (r0 + n) // 2)
    else:
        rs = pl.ds(pl.multiple_of(lax.shift_right_logical(r0, 1), 8), n // 2)
    return pltpu.bitcast(ref[rs, cols], BF16)


def _st(ref, r0, val, cols=slice(None)):
    ref[r0 // 2:(r0 + val.shape[0]) // 2, cols] = pltpu.bitcast(val, U32)


def _zero_after(z, *vals):
    acc = None
    for v in vals:
        b = pltpu.bitcast(v, U32)
        for r in range(0, b.shape[0], 8):
            for c in range(0, b.shape[1], 128):
                t = b[r:r + 8, c:c + 128]
                acc = t if acc is None else acc | t
    return acc & z


def _chain(op, tiles, z, dep):
    a = tiles[0]
    if dep is not None:
        a = pltpu.bitcast(pltpu.bitcast(a, U32) | jnp.concatenate([dep] * (a.shape[0] // 8), axis=0), F32)
    a = functools.reduce(op, [a] + tiles[1:])
    return a, _zero_after(z, a)


def _body(x_hbm, ckv_hbm, wq_hbm, wuk_hbm, wuv_hbm, wo_hbm, bqkv_hbm, bwo_hbm, gate_hbm,
          out_hbm,
          x_v, ckv_v, wq_p, wuk_p, wuv_p, wo_v, bqkv_v, bwo_p, wcur_v, wfst_v,
          qkv_v, acc_v, g_v, z_v, q_s, k_s, v_s, o_st, gate_v,
          sem_x, sem_w, sem_a, sem_o):
    def cp_x(sm, r0, r1, c0, c1):
        sl = (pl.ds(r0 // 2, (r1 - r0) // 2), pl.ds(c0, c1 - c0))
        return pltpu.make_async_copy(x_hbm.bitcast(U32).at[sl], x_v.at[sl], sem_x.at[sm])

    def cp_w(k, c0=0, c1=3 * M, sm=None):
        sl = (pl.ds(k * 128, 128), pl.ds(c0, c1 - c0))
        return pltpu.make_async_copy(bqkv_hbm.at[sl], bqkv_v.at[sl], sem_w.at[k if sm is None else sm])

    x0a, x0b, xr = cp_x(0, 0, R1, 0, 128), cp_x(1, R1, S, 0, 128), cp_x(2, 0, S, 128, M)
    w0a, w0b, w0c = cp_w(0, 0, M), cp_w(0, M, 2 * M, NT_M), cp_w(0, 2 * M, 3 * M, NT_M + 1)
    cp_g = pltpu.make_async_copy(gate_hbm, gate_v.at[pl.ds(0, M)], sem_x.at[3])

    def cp_pairs(src, dst):
        return [pltpu.make_async_copy(src.bitcast(U32).at[:, p, :], dst.at[p], sem_a) for p in range(HP)]

    a_early = cp_pairs(bwo_hbm, bwo_p) + [pltpu.make_async_copy(ckv_hbm.bitcast(U32), ckv_v, sem_a),
                                          pltpu.make_async_copy(wo_hbm.bitcast(U32), wo_v, sem_a)]
    a_late = cp_pairs(wuk_hbm, wuk_p) + cp_pairs(wuv_hbm, wuv_p) + cp_pairs(wq_hbm, wq_p)
    a_waits = [pltpu.make_async_copy(b, b, sem_a) for b in (ckv_v, wo_v, wuk_p, wuv_p, wq_p, bwo_p)]

    def cp_o(b0, nb, r0, n, c0=0, c1=M):
        sl = (pl.ds(b0, nb), pl.ds(r0, n), pl.ds(c0, c1 - c0))
        return pltpu.make_async_copy(o_st.at[sl], out_hbm.at[sl], sem_o)

    def prep(part, j, z=None, dep=None):
        k0 = j * 128 if isinstance(j, int) else pl.multiple_of(j * 128, 128)
        for c in range(NT_M):
            src = bqkv_v[pl.ds(k0, 128), part * M + c * 128:part * M + (c + 1) * 128]
            if dep is not None:
                top = pltpu.bitcast(pltpu.bitcast(src[:16], U32) | dep, BF16)
                src = jnp.concatenate([top, src[16:]], axis=0)
            t = pltpu.bitcast(src.T, U32)
            for hp in range(2):
                a, b = t[32 * hp:32 * hp + 16], t[32 * hp + 16:32 * hp + 32]
                r = 2 * c + hp
                wcur_v[part, pl.ds(r, 16, stride=2 * PITCH), :] = (a & jnp.uint32(0xFFFF)) | (b << 16)
                wcur_v[part, pl.ds(PITCH + r, 16, stride=2 * PITCH), :] = (a >> 16) | (b & jnp.uint32(0xFFFF0000))
            if z is not None:
                dep = _zero_after(z, t[56:64])
        return dep

    def wrows(part, d0, d1):
        w = jnp.concatenate([wcur_v[part, d * PITCH:d * PITCH + HP, :] for d in range(d0, d1)], axis=0)
        return pltpu.bitcast(w, BF16)

    def first_tiles(part):
        for n in range(4):
            _st(wfst_v, 0, wrows(part, 4 * n, 4 * n + 4).T, slice(n * 128, (n + 1) * 128))

    def project(xk, part, first):
        if not first:
            return lax.dot_general(xk, wrows(part, 0, DH), NT, preferred_element_type=F32)
        return jnp.concatenate([jnp.dot(xk, _ld(wfst_v, 0, 128), preferred_element_type=F32),
                                lax.dot_general(xk, wrows(part, DH // 2, DH), NT, preferred_element_type=F32)], axis=1)

    def gate_rows(t, z, dep):
        gw = gate_v[0:M].astype(F32).reshape(1, M)
        g0 = jnp.minimum((t - 1) * GR, S - GR)
        for k in range(GR // 16):
            rr = pl.multiple_of(g0 + k * 16, 16)
            rw = pl.multiple_of(lax.shift_right_logical(rr, 1), 8)
            xb = x_v[pl.ds(rw, 8), :]
            if dep is not None:
                xb = xb | jnp.concatenate([dep] * NT_M, axis=1)
            xx = pltpu.bitcast(xb, BF16).astype(F32)
            zz = jnp.sum(xx * gw, axis=1, keepdims=True)
            g = jnp.broadcast_to(1.0 / (1.0 + jnp.exp(-zz)), (16, 128))
            g_v[pl.ds(rr, 16), :] = g
            acc_v[pl.ds(rr, 16), :] = jnp.zeros((16, M), F32)
            dep = _zero_after(z, g)

    def first_task():
        def piece(part, r0, r1, first):
            y = project(_ld(x_v, r0, r1 - r0, slice(0, 128)), part, first)
            for tt in range(NT_M):
                qkv_v[part, tt, PAD + r0:PAD + r1, :] = y[:, tt * 128:(tt + 1) * 128]

        with _scope("prep0"):
            w0a.wait()
            prep(0, 0)
        with _scope("b1"):
            x0a.wait()
            piece(0, 0, R1, False)
            first_tiles(0)
        with _scope("b2"):
            x0b.wait()
            w0b.wait()
            piece(0, R1, S, True)
            prep(1, 0)
            first_tiles(1)
        with _scope("b3"):
            w0c.wait()
            cp_w(1).wait()
            z = z_v[...]
            piece(1, 0, S, True)
            prep(2, 0)
            dep = prep(0, 1, z)
            first_tiles(0)
            piece(2, 0, S, False)
            prep(1, 1, z, dep)
            prep(2, 1)
            for cc in a_late[:NA1]:
                cc.start()
        for cc in (xr, cp_g):
            cc.wait()
        for cc in a_late[NA1:]:
            cc.start()

    def bproj_body(t, _):
        @pl.when(t < NT_M - 1)
        def _():
            cp_w(t + 1).wait()

        z = z_v[...]
        u = jnp.minimum(t + 1, NT_M - 1)
        xw = x_v[:, pl.ds(pl.multiple_of(t * 128, 128), 128)]
        xk = pltpu.bitcast(xw | jnp.concatenate([z] * (S // 16), axis=0), BF16)
        dep = None
        for part in range(3):
            y = project(xk, part, part == 0)
            for tt in range(NT_M):
                qkv_v[part, tt, PAD:, :] = qkv_v[part, tt, PAD:, :] + y[:, tt * 128:(tt + 1) * 128]
            dep = prep(part, u, z, dep) if part < 2 else prep(part, u)
            if part == 0:
                first_tiles(0)
        gate_rows(t, z, None)
        return 0

    qscale = (D ** -0.5) * LOG2E
    bscale = (DH ** -0.5) * LOG2E

    def local_attn(r, z, dep):
        def zf(v):
            return pltpu.bitcast(_zero_after(z, v), F32)

        sc = jnp.full((8, 128), bscale, F32)
        if dep is not None:
            sc = sc + dep
        q = [qkv_v[0, t, pl.ds(PAD + r, 8), :] * sc for t in range(NT_M)]
        rowi = r + lax.broadcasted_iota(jnp.int32, (8, 128), 0)
        logits, raw = [], []
        for w in range(W):
            a = None if w < LAQ else zf(raw[w - LAQ])
            for t in range(NT_M):
                pr = q[t] * qkv_v[1, t, pl.ds(PAD + r - DIL * w, 8), :]
                a = pr if a is None else a + pr
            raw.append(a)
            a = a + pltpu.roll(a, 64, 1)
            a = a + pltpu.roll(a, 32, 1)
            logits.append(jnp.where(rowi >= DIL * w, a, NEG) if w > 0 else a)
        m = functools.reduce(jnp.maximum, logits)
        es = [jnp.exp2(lg - m) for lg in logits]
        l = functools.reduce(lambda a, b: a + b, es)
        f = (1.0 - g_v[pl.ds(r, 8), :]) * _recip(l)
        es = [e * f for e in es]
        outs = []
        for t in range(NT_M):
            a = None if t == 0 else zf(outs[t - 1])
            for w in range(W):
                pr = es[w] * qkv_v[2, t, pl.ds(PAD + r - DIL * w, 8), :]
                a = pr if a is None else a + pr
            outs.append(a)
        return jnp.concatenate(outs, axis=1), zf(outs[-1])

    def pair_body(p, _):
        z = z_v[...]
        last = p == HP - 1
        wk, wv = _split_pair(wuk_p[p]), _split_pair(wuv_p[p])
        _st(k_s, 0, jnp.dot(_ld(ckv_v, 0, S), wk, preferred_element_type=F32).astype(BF16))
        _st(v_s, 0, jnp.dot(_ld(ckv_v, 0, S), wv, preferred_element_type=F32).astype(BF16))

        rb = pl.multiple_of(p * TL, TL)
        dep, obs = None, []
        for k in range(TL // 8):
            ob, dep = local_attn(rb + k * 8, z, dep)
            if k == 0:
                v = g_v[pl.ds(rb, 24), :]
                dep = dep + pltpu.bitcast(_zero_after(z, jnp.broadcast_to(v[:, 0:1], v.shape)), F32)
            obs.append(ob)
        ob = jnp.concatenate(obs, axis=0).astype(BF16)

        wqw = wq_p[p]
        wq = _split_pair(jnp.concatenate([wqw[:8] | _zero_after(z, ob[TL - 16:]), wqw[8:]], axis=0))
        row = lax.broadcasted_iota(jnp.int32, (RG, TQ), 0)
        col = lax.broadcasted_iota(jnp.int32, (RG, TQ), 1)
        diag = col <= row + (TQ - RG)

        def rows(j):
            return [(j - j % G + b) * TQ + (j % G) * RG for b in range(G)]

        def geom(j):
            off = (j % G + 1) * RG % TQ
            return off, j - j % G + (0 if off else 1)

        def gather(ref, j, ld=lambda ref, r: ref[r:r + RG, :]):
            return jnp.concatenate([ld(ref, r) for r in rows(j)], axis=0)

        def qproj(j):
            q = jnp.dot(gather(x_v, j, lambda ref, r: _ld(ref, r, RG)), wq, preferred_element_type=F32) * qscale
            _st(q_s, j * TQ, q.astype(BF16))

        def head(h):
            return slice(h * D, (h + 1) * D)

        def qk(j, hh):
            off, nc = geom(j)
            q = _ld(q_s, j * TQ, TQ, head(hh))
            com = lax.dot_general(q, _ld(k_s, off, nc * TQ, head(hh)), NT, preferred_element_type=F32) if nc else None
            ext = {e: lax.dot_general(q[e * RG:], _ld(k_s, off + (nc + e - 1) * TQ, TQ, head(hh)), NT,
                                      preferred_element_type=F32) for e in reversed(range(1, G))}
            left = None
            if off:
                st = lax.dot_general(_ld(k_s, 0, off, head(hh)), q, NT, preferred_element_type=F32)
                left = jnp.concatenate([st, jnp.full((TQ - off, TQ), NEG, F32)], axis=0).T
            return com, ext, left

        deps = {"max": None, "sum": None}

        def softmax(parts):
            if len(parts) > MAXT:
                m, deps["max"] = _chain(jnp.maximum, parts[1:], z, deps["max"])
                m = jnp.maximum(m, parts[0])
            else:
                m = functools.reduce(jnp.maximum, parts[1:] + parts[:1])
            e = jnp.exp2(jnp.concatenate(parts, axis=1) - jnp.max(m, axis=1, keepdims=True))
            l = e
            if len(parts) > SUMT:
                l, deps["sum"] = _chain(jnp.add, [e[:, c:c + TQ] for c in range(0, e.shape[1], TQ)], z, deps["sum"])
            return e, jnp.sum(l, axis=1, keepdims=True)

        def softmax_pv(j, hh, sc):
            off, nc = geom(j)
            com, ext, left = sc
            es, ls = [], []
            for b in range(G):
                rs = slice(b * RG, (b + 1) * RG)
                parts = [left[rs]] if off else []
                parts += [com[rs, t * TQ:(t + 1) * TQ] for t in range(nc)]
                parts += [ext[e][(b - e) * RG:(b - e + 1) * RG] for e in range(1, b + 1)]
                parts[-1] = jnp.where(diag if nc + b else col <= row + (off - RG), parts[-1], NEG)
                e, l = softmax(parts)
                es.append(e)
                ls.append(l)
            w = es[0].shape[1]
            vs = [_ld(v_s, 0, TQ, head(hh))] if off else []
            if nc:
                vs.append(_ld(v_s, off, nc * TQ, head(hh)))
            o = jnp.dot(jnp.concatenate([e[:, :w] for e in es], axis=0).astype(BF16), jnp.concatenate(vs, axis=0),
                        preferred_element_type=F32)
            ox = [jnp.dot(jnp.concatenate([x[:, w + (e - 1) * TQ:w + e * TQ] for x in es[e:]], axis=0).astype(BF16),
                          _ld(v_s, off + (nc + e - 1) * TQ, TQ, head(hh)), preferred_element_type=F32)
                  for e in range(1, G)]
            o = jnp.concatenate([functools.reduce(lambda a, c: a + c, [o[b * RG:(b + 1) * RG]] + [
                ox[e - 1][(b - e) * RG:(b - e + 1) * RG] for e in range(1, b + 1)]) for b in range(G)], axis=0)
            return o * (gather(g_v, j) * _recip(jnp.concatenate(ls, axis=0)))

        def oproj(j, o0, o1):
            y = gather(acc_v, j) + jnp.dot(jnp.concatenate([o0, o1], axis=1).astype(BF16),
                                           _ld(wo_v, p * (2 * D), 2 * D), preferred_element_type=F32)
            for b, r in enumerate(rows(j)):
                acc_v[r:r + RG, :] = y[b * RG:(b + 1) * RG]
                if r < S - TL:
                    o_st[r // TQ, r % TQ:r % TQ + RG, :] = y[b * RG:(b + 1) * RG].astype(BF16)
            j0 = j - j % G
            pl.when(last)(cp_o(j0, min(G, nq - 1 - j0), j % G * RG, RG).start)

        nq = S // TQ
        items = [(j, hh) for j in ORDER for hh in range(2)]
        n = len(items)
        s_vals, o_vals = {}, {}
        qproj(ORDER[0])
        for step in range(n + LOOK + OLAG):
            if step % 2 == 0 and 1 + step // 2 < nq:
                qproj(ORDER[1 + step // 2])
            if step < n:
                s_vals[step] = qk(*items[step])
            b = step - LOOK
            if 0 <= b < n:
                o_vals[b] = softmax_pv(*items[b], s_vals.pop(b))
            c = step - LOOK - OLAG
            if 0 <= c < n and c % 2 == 1:
                oproj(items[c][0], o_vals.pop(c - 1), o_vals.pop(c))

        wop = jnp.concatenate([f(bwo_p[dp]) for dp in range(DH // 2) for f in (_lo, _hi)], axis=0).astype(BF16)
        c0 = M - 128 * NCUT
        yl = acc_v[pl.ds(rb, TL), :c0] + jnp.dot(ob, wop[:, :c0], preferred_element_type=F32)
        ya = acc_v[pl.ds(rb, TL), c0:]
        yr = [[ya[r:r + 16, c:c + 128] for r in range(0, TL, 16)] for c in range(0, M - c0, 128)]
        for tile in range(NT_M * NCUT):
            c, k = divmod(tile, NT_M)
            cuts = (0,) + CUTS.get(tile, ()) + (TL // 16,)
            for u0, u1 in zip(cuts[:-1], cuts[1:]):
                t = jnp.dot(ob[u0 * 16:u1 * 16, k * 128:(k + 1) * 128],
                            wop[k * 128:(k + 1) * 128, c0 + c * 128:c0 + (c + 1) * 128], preferred_element_type=F32)
                for u in range(u0, u1):
                    yr[c][u] = yr[c][u] + t[(u - u0) * 16:(u - u0 + 1) * 16]
        y = jnp.concatenate([yl] + [jnp.concatenate(v, axis=0) for v in yr], axis=1)
        acc_v[pl.ds(rb, TL), :] = y
        for c0, c1 in zip(OCUT[:-1], OCUT[1:]):
            o_st[S // TQ - 1, :, c0:c1] = y[:, c0:c1].astype(BF16)
            pl.when(last)(cp_o(S // TQ - 1, 1, 0, TQ, c0, c1).start)
        return 0

    for cc in [w0a, x0a, x0b, w0b, w0c, cp_w(1), cp_g, xr] + [cp_w(k) for k in range(2, NT_M)] + a_early:
        cc.start()
    z_v[...] = jnp.zeros((8, 128), U32)
    for part in range(3):
        for t in range(NT_M):
            qkv_v[part, t, 0:PAD, :] = jnp.zeros((PAD, 128), F32)

    def phases():
        first_task()
        lax.fori_loop(1, NT_M, _scoped("bproj", bproj_body), 0)
        for cc in a_waits:
            cc.wait()
        lax.fori_loop(0, HP, _scoped("pair", pair_body), 0)

    def once(i, _):
        pl.when(i == 0)(phases)
        return 0

    lax.fori_loop(0, 2, once, 0)
    with _scope("ow"):
        cp_o(0, S // TQ, 0, TQ).wait()


def _kernel(*refs):
    dma = pltpu.SemaphoreType.DMA
    pl.run_scoped(functools.partial(_body, *refs), dma((4,)), dma((NT_M + 2,)), dma(()), dma(()))


@jax.jit
def pallas_gated_mix__compressed_kv_cla__sliding_local_dilated__prompt_kernel(
    A_x, A_c_kv, A_w_q, A_w_uk, A_w_uv, A_w_o, B_x, B_wqkv, B_wo, gate_w,
):
    del B_x
    x = A_x.reshape(S, M)
    ckv = A_c_kv.reshape(S, DC)
    wo = A_w_o.reshape(H * D, M)
    bwo = B_wo.reshape(H, DH, M)
    any_spec = pl.BlockSpec(memory_space=pl.ANY)
    out = pl.pallas_call(
        _kernel,
        out_shape=jax.ShapeDtypeStruct((S // TQ, TQ, M), BF16),
        in_specs=[any_spec] * 9,
        out_specs=any_spec,
        scratch_shapes=[
            pltpu.VMEM((S // 2, M), U32),
            pltpu.VMEM((S // 2, DC), U32),
            pltpu.VMEM((HP, M, D), U32),
            pltpu.VMEM((HP, DC, D), U32),
            pltpu.VMEM((HP, DC, D), U32),
            pltpu.VMEM((H * D // 2, M), U32),
            pltpu.VMEM((M, 3 * M), BF16),
            pltpu.VMEM((DH // 2, H, M), U32),
            pltpu.VMEM((3, DH * 24, 128), U32),
            pltpu.VMEM((64, 512), U32),
            pltpu.VMEM((3, NT_M, S + PAD, 128), F32),
            pltpu.VMEM((S, M), F32),
            pltpu.VMEM((S, 128), F32),
            pltpu.VMEM((8, 128), U32),
            pltpu.VMEM((S // 2, 2 * D), U32),
            pltpu.VMEM((S // 2, 2 * D), U32),
            pltpu.VMEM((S // 2, 2 * D), U32),
            pltpu.VMEM((S // TQ, TQ, M), BF16),
            pltpu.VMEM((2 * M,), BF16),
        ],
        compiler_params=pltpu.CompilerParams(vmem_limit_bytes=110 * 1024 * 1024),
    )(x, ckv, A_w_q, A_w_uk, A_w_uv, wo, B_wqkv, bwo, gate_w)
    return out.reshape(1, S, M)
```

```python
import contextlib
import functools

import jax
import jax.numpy as jnp
from jax import lax
import jax.experimental.pallas as pl
import jax.experimental.pallas.tpu as pltpu

S = 2048
M = 1024
DC = 512
H = 32
HP = H // 2
D = 128
DH = 32
W = 8
DIL = 2
PAD = 40
NT_M = M // 128
TQ = 128
TL = S // HP
R1 = 768
GR = 304
PITCH = 17
NA1 = 44
OCUT = (0, 512, 768, M)
LOOK = 2
OLAG = 7
SUMT = 4
MAXT = 8
LAQ = 2
G = 8
RG = TQ // G
ORDER = (8, 9, 2, 11, 12, 5, 14, 7, 0, 1, 10, 3, 4, 13, 6, 15)
NCUT = 4
CUTS = {4: (1,), 5: (1, 2), 9: (1,), 10: (1, 2), 13: (1, 2), 17: (1,), 18: (1,), 21: (1,), 23: (1,), 28: (1,),
        31: (5, 7)}
VG = 32
LOG2E = 1.4426950408889634
NEG = -1e9

F32 = jnp.float32
BF16 = jnp.bfloat16
U32 = jnp.uint32
NT = (((1,), (1,)), ((), ()))


_PROFILE = False


def _scope(name):
    return jax.named_scope(name) if _PROFILE else contextlib.nullcontext()


def _scoped(name, body):
    def f(i, c):
        with _scope(name):
            return body(i, c)
    return f


def _recip(l):
    r = pl.reciprocal(l, approx=True)
    return r * (2.0 - l * r)


def _lo(w):
    return pltpu.bitcast(w << 16, F32)


def _hi(w):
    return pltpu.bitcast(w & jnp.uint32(0xFFFF0000), F32)


def _split_pair(w):
    return jnp.concatenate([_lo(w), _hi(w)], axis=1).astype(BF16)


def _ld(ref, r0, n, cols=slice(None)):
    if isinstance(r0, int):
        rs = slice(r0 // 2, (r0 + n) // 2)
    else:
        rs = pl.ds(pl.multiple_of(lax.shift_right_logical(r0, 1), 8), n // 2)
    return pltpu.bitcast(ref[rs, cols], BF16)


def _st(ref, r0, val, cols=slice(None)):
    ref[r0 // 2:(r0 + val.shape[0]) // 2, cols] = pltpu.bitcast(val, U32)


def _zero_after(z, *vals):
    acc = None
    for v in vals:
        b = pltpu.bitcast(v, U32)
        for r in range(0, b.shape[0], 8):
            for c in range(0, b.shape[1], 128):
                t = b[r:r + 8, c:c + 128]
                acc = t if acc is None else acc | t
    return acc & z


def _after(v, dep):
    b = pltpu.bitcast(v, U32)
    return pltpu.bitcast(b | jnp.concatenate([dep] * (b.shape[0] // 8), axis=0), v.dtype)


def _chain(op, tiles, z, dep):
    a = functools.reduce(op, [tiles[0] if dep is None else _after(tiles[0], dep)] + tiles[1:])
    return a, _zero_after(z, a)


def _body(x_hbm, ckv_hbm, wq_hbm, wuk_hbm, wuv_hbm, wo_hbm, bqkv_hbm, bwo_hbm, gate_hbm,
          out_hbm,
          x_v, ckv_v, wq_p, wuk_p, wuv_p, wo_v, bqkv_v, bwo_p, wcur_v, wfst_v,
          qkv_v, acc_v, g_v, z_v, q_s, k_s, v_s, o_st, gate_v,
          sem_x, sem_w, sem_a, sem_o):
    def cp_x(sm, r0, r1, c0, c1):
        sl = (pl.ds(r0 // 2, (r1 - r0) // 2), pl.ds(c0, c1 - c0))
        return pltpu.make_async_copy(x_hbm.bitcast(U32).at[sl], x_v.at[sl], sem_x.at[sm])

    def cp_w(k, c0=0, c1=3 * M, sm=None):
        sl = (pl.ds(k * 128, 128), pl.ds(c0, c1 - c0))
        return pltpu.make_async_copy(bqkv_hbm.at[sl], bqkv_v.at[sl], sem_w.at[k if sm is None else sm])

    x0a, x0b, xr = cp_x(0, 0, R1, 0, 128), cp_x(1, R1, S, 0, 128), cp_x(2, 0, S, 128, M)
    w0a, w0b, w0c = cp_w(0, 0, M), cp_w(0, M, 2 * M, NT_M), cp_w(0, 2 * M, 3 * M, NT_M + 1)
    cp_g = pltpu.make_async_copy(gate_hbm, gate_v.at[pl.ds(0, M)], sem_x.at[3])

    def cp_pairs(src, dst):
        return [pltpu.make_async_copy(src.bitcast(U32).at[:, p, :], dst.at[p], sem_a) for p in range(HP)]

    a_early = cp_pairs(bwo_hbm, bwo_p) + [pltpu.make_async_copy(ckv_hbm.bitcast(U32), ckv_v, sem_a),
                                          pltpu.make_async_copy(wo_hbm.bitcast(U32), wo_v, sem_a)]
    a_late = cp_pairs(wuk_hbm, wuk_p) + cp_pairs(wuv_hbm, wuv_p) + cp_pairs(wq_hbm, wq_p)
    a_waits = [pltpu.make_async_copy(b, b, sem_a) for b in (ckv_v, wo_v, wuk_p, wuv_p, wq_p, bwo_p)]

    def cp_o(b0, nb, r0, n, c0=0, c1=M):
        sl = (pl.ds(b0, nb), pl.ds(r0, n), pl.ds(c0, c1 - c0))
        return pltpu.make_async_copy(o_st.at[sl], out_hbm.at[sl], sem_o)

    def prep(part, j, z=None, dep=None):
        k0 = j * 128 if isinstance(j, int) else pl.multiple_of(j * 128, 128)
        for c in range(NT_M):
            src = bqkv_v[pl.ds(k0, 128), part * M + c * 128:part * M + (c + 1) * 128]
            if dep is not None:
                top = pltpu.bitcast(pltpu.bitcast(src[:16], U32) | dep, BF16)
                src = jnp.concatenate([top, src[16:]], axis=0)
            t = pltpu.bitcast(src.T, U32)
            for hp in range(2):
                a, b = t[32 * hp:32 * hp + 16], t[32 * hp + 16:32 * hp + 32]
                r = 2 * c + hp
                wcur_v[part, pl.ds(r, 16, stride=2 * PITCH), :] = (a & jnp.uint32(0xFFFF)) | (b << 16)
                wcur_v[part, pl.ds(PITCH + r, 16, stride=2 * PITCH), :] = (a >> 16) | (b & jnp.uint32(0xFFFF0000))
            if z is not None:
                dep = _zero_after(z, t[56:64])
        return dep

    def wrows(part, d0, d1):
        w = jnp.concatenate([wcur_v[part, d * PITCH:d * PITCH + HP, :] for d in range(d0, d1)], axis=0)
        return pltpu.bitcast(w, BF16)

    def first_tiles(part):
        for n in range(4):
            _st(wfst_v, 0, wrows(part, 4 * n, 4 * n + 4).T, slice(n * 128, (n + 1) * 128))

    def project(xk, part, first):
        if not first:
            return lax.dot_general(xk, wrows(part, 0, DH), NT, preferred_element_type=F32)
        return jnp.concatenate([jnp.dot(xk, _ld(wfst_v, 0, 128), preferred_element_type=F32),
                                lax.dot_general(xk, wrows(part, DH // 2, DH), NT, preferred_element_type=F32)], axis=1)

    def gate_rows(t, z, dep):
        gw = gate_v[0:M].astype(F32).reshape(1, M)
        g0 = jnp.minimum((t - 1) * GR, S - GR)
        for k in range(GR // 16):
            rr = pl.multiple_of(g0 + k * 16, 16)
            rw = pl.multiple_of(lax.shift_right_logical(rr, 1), 8)
            xb = x_v[pl.ds(rw, 8), :]
            if dep is not None:
                xb = xb | jnp.concatenate([dep] * NT_M, axis=1)
            xx = pltpu.bitcast(xb, BF16).astype(F32)
            zz = jnp.sum(xx * gw, axis=1, keepdims=True)
            g = jnp.broadcast_to(1.0 / (1.0 + jnp.exp(-zz)), (16, 128))
            g_v[pl.ds(rr, 16), :] = g
            acc_v[pl.ds(rr, 16), :] = jnp.zeros((16, M), F32)
            dep = _zero_after(z, g)

    def first_task():
        def piece(part, r0, r1, first):
            y = project(_ld(x_v, r0, r1 - r0, slice(0, 128)), part, first)
            for tt in range(NT_M):
                qkv_v[part, tt, PAD + r0:PAD + r1, :] = y[:, tt * 128:(tt + 1) * 128]

        with _scope("prep0"):
            w0a.wait()
            prep(0, 0)
        with _scope("b1"):
            x0a.wait()
            piece(0, 0, R1, False)
            first_tiles(0)
        with _scope("b2"):
            x0b.wait()
            w0b.wait()
            piece(0, R1, S, True)
            prep(1, 0)
            first_tiles(1)
        with _scope("b3"):
            w0c.wait()
            cp_w(1).wait()
            z = z_v[...]
            piece(1, 0, S, True)
            prep(2, 0)
            dep = prep(0, 1, z)
            first_tiles(0)
            piece(2, 0, S, False)
            prep(1, 1, z, dep)
            prep(2, 1)
            for cc in a_late[:NA1]:
                cc.start()
        for cc in (xr, cp_g):
            cc.wait()
        for cc in a_late[NA1:]:
            cc.start()

    def bproj_body(t, _):
        @pl.when(t < NT_M - 1)
        def _():
            cp_w(t + 1).wait()

        z = z_v[...]
        u = jnp.minimum(t + 1, NT_M - 1)
        xw = x_v[:, pl.ds(pl.multiple_of(t * 128, 128), 128)]
        xk = pltpu.bitcast(xw | jnp.concatenate([z] * (S // 16), axis=0), BF16)
        dep = None
        for part in range(3):
            y = project(xk, part, part == 0)
            for tt in range(NT_M):
                qkv_v[part, tt, PAD:, :] = qkv_v[part, tt, PAD:, :] + y[:, tt * 128:(tt + 1) * 128]
            dep = prep(part, u, z, dep) if part < 2 else prep(part, u)
            if part == 0:
                first_tiles(0)
        gate_rows(t, z, None)
        return 0

    qscale = (D ** -0.5) * LOG2E
    bscale = (DH ** -0.5) * LOG2E

    def local_attn(r, z, dep):
        def zf(v):
            return pltpu.bitcast(_zero_after(z, v), F32)

        sc = jnp.full((8, 128), bscale, F32)
        if dep is not None:
            sc = sc + dep
        q = [qkv_v[0, t, pl.ds(PAD + r, 8), :] * sc for t in range(NT_M)]
        rowi = r + lax.broadcasted_iota(jnp.int32, (8, 128), 0)
        logits, raw = [], []
        for w in range(W):
            a = None if w < LAQ else zf(raw[w - LAQ])
            for t in range(NT_M):
                pr = q[t] * qkv_v[1, t, pl.ds(PAD + r - DIL * w, 8), :]
                a = pr if a is None else a + pr
            raw.append(a)
            a = a + pltpu.roll(a, 64, 1)
            a = a + pltpu.roll(a, 32, 1)
            logits.append(jnp.where(rowi >= DIL * w, a, NEG) if w > 0 else a)
        m = functools.reduce(jnp.maximum, logits)
        es = [jnp.exp2(lg - m) for lg in logits]
        l = functools.reduce(lambda a, b: a + b, es)
        f = (1.0 - g_v[pl.ds(r, 8), :]) * _recip(l)
        es = [e * f for e in es]
        outs = []
        for t in range(NT_M):
            a = None if t == 0 else zf(outs[t - 1])
            for w in range(W):
                pr = es[w] * qkv_v[2, t, pl.ds(PAD + r - DIL * w, 8), :]
                a = pr if a is None else a + pr
            outs.append(a)
        return jnp.concatenate(outs, axis=1), zf(outs[-1])

    def pair_body(p, _):
        z = z_v[...]
        last = p == HP - 1
        wk, wv = _split_pair(wuk_p[p]), _split_pair(wuv_p[p])
        _st(k_s, 0, jnp.dot(_ld(ckv_v, 0, S), wk, preferred_element_type=F32).astype(BF16))
        _st(v_s, 0, jnp.dot(_ld(ckv_v, 0, S), wv, preferred_element_type=F32).astype(BF16))

        rb = pl.multiple_of(p * TL, TL)
        dep, obs = None, []
        for k in range(TL // 8):
            ob, dep = local_attn(rb + k * 8, z, dep)
            if k == 0:
                v = g_v[pl.ds(rb, 24), :]
                dep = dep + pltpu.bitcast(_zero_after(z, jnp.broadcast_to(v[:, 0:1], v.shape)), F32)
            obs.append(ob)
        ob = jnp.concatenate(obs, axis=0)

        wqw = wq_p[p]
        wq = _split_pair(jnp.concatenate([wqw[:8] | _zero_after(z, ob[TL - 16:].astype(BF16)), wqw[8:]], axis=0))
        row = lax.broadcasted_iota(jnp.int32, (RG, TQ), 0)
        col = lax.broadcasted_iota(jnp.int32, (RG, TQ), 1)
        diag = col <= row + (TQ - RG)

        def rows(j):
            return [(j - j % G + b) * TQ + (j % G) * RG for b in range(G)]

        def geom(j):
            off = (j % G + 1) * RG % TQ
            return off, j - j % G + (0 if off else 1)

        def gather(ref, j, ld=lambda ref, r: ref[r:r + RG, :]):
            return jnp.concatenate([ld(ref, r) for r in rows(j)], axis=0)

        def head(h):
            return slice(h * D, (h + 1) * D)

        vbw = {}

        def qproj(j):
            xg = gather(x_v, j, lambda ref, r: _ld(ref, r, RG))
            if j == ORDER[1]:
                for h in range(2):
                    for i in range(RG // 2):
                        wrow = pltpu.bitcast(v_s[i:i + 1, head(h)], F32)
                        vbw[h, i] = pltpu.bitcast(jnp.broadcast_to(wrow, (TQ, D)).T, U32)
                top = _after(xg[:16, :128], _zero_after(z, *[x[TQ - 8:] for x in vbw.values()]))
                xg = jnp.concatenate([jnp.concatenate([top, xg[:16, 128:]], axis=1), xg[16:]], axis=0)
            _st(q_s, j * TQ, (jnp.dot(xg, wq, preferred_element_type=F32) * qscale).astype(BF16))

        def bout(rs, ks, cs):
            return jnp.dot(ob[rs, ks].astype(BF16), wop[ks, cs].astype(BF16), preferred_element_type=F32)

        due = {}

        def qk(step, j, hh):
            off, nc = geom(j)
            q = _ld(q_s, j * TQ, TQ, head(hh))
            for d in due.pop(step, ()):
                q = jnp.concatenate([q[:TQ - 16], _after(q[TQ - 16:], d)], axis=0)
            com = lax.dot_general(q, _ld(k_s, off, nc * TQ, head(hh)), NT, preferred_element_type=F32) if nc else None
            ext = {e: lax.dot_general(q[e * RG:], _ld(k_s, off + (nc + e - 1) * TQ, TQ, head(hh)), NT,
                                      preferred_element_type=F32) for e in reversed(range(1, G))}
            left = None
            if off:
                st = lax.dot_general(_ld(k_s, 0, off, head(hh)), _ld(q_s, j * TQ, TQ, head(hh)), NT,
                                     preferred_element_type=F32)
                left = jnp.concatenate([st, jnp.full((TQ - off, TQ), NEG, F32)], axis=0).T
            return com, ext, left

        deps = {"max": None, "sum": None, "pv": None}
        fill, early, late = [], [], []
        c0 = M - 128 * NCUT

        def softmax(parts):
            if len(parts) > MAXT:
                m, deps["max"] = _chain(jnp.maximum, parts[1:], z, deps["max"])
                m = jnp.maximum(m, parts[0])
            else:
                m = functools.reduce(jnp.maximum, parts[1:] + parts[:1])
            e = jnp.exp2(jnp.concatenate(parts, axis=1) - jnp.max(m, axis=1, keepdims=True))
            l = e
            if len(parts) > SUMT:
                l, deps["sum"] = _chain(jnp.add, [e[:, c:c + TQ] for c in range(0, e.shape[1], TQ)], z, deps["sum"])
            return e, jnp.sum(l, axis=1, keepdims=True)

        def softmax_pv(step, j, hh, sc):
            off, nc = geom(j)
            com, ext, left = sc
            es, ls = [], []
            for b in range(G):
                rs = slice(b * RG, (b + 1) * RG)
                parts = [left[rs]] if off else []
                parts += [com[rs, t * TQ:(t + 1) * TQ] for t in range(nc)]
                parts += [ext[e][(b - e) * RG:(b - e + 1) * RG] for e in range(1, b + 1)]
                parts[-1] = jnp.where(diag if nc + b else col <= row + (off - RG), parts[-1], NEG)
                e, l = softmax(parts)
                es.append(e)
                ls.append(l)
            w = es[0].shape[1]
            vpu = off == RG
            vs = [_ld(v_s, 0, TQ, head(hh))] if off and not vpu else []
            if nc:
                vs.append(_ld(v_s, off, nc * TQ, head(hh)))
            if vpu:
                tail = _after(es[-1][:, -TQ:], _zero_after(z, *[e[:, :TQ] for e in es]))
                es[-1] = jnp.concatenate([es[-1][:, :-TQ], tail], axis=1)
                fill.append(bout(slice(None), slice(len(fill) * 128, len(fill) * 128 + 128), slice(c0, c0 + 128)))
            o = [jnp.dot(jnp.concatenate([e[:, TQ * vpu:w] for e in es], axis=0).astype(BF16),
                         jnp.concatenate(vs, axis=0), preferred_element_type=F32)] if vs else []
            ox = [jnp.dot(jnp.concatenate([x[:, w + (e - 1) * TQ:w + e * TQ] for x in es[e:]], axis=0).astype(BF16),
                          _ld(v_s, off + (nc + e - 1) * TQ, TQ, head(hh)), preferred_element_type=F32)
                  for e in range(1, G)]
            if vpu:
                pt = jnp.concatenate([e[:, :off] for e in es], axis=0).T
                pb = [jnp.broadcast_to(pt[k:k + 1], (VG, TQ)) for k in range(off)]
                due.setdefault(step + 1 + hh + (j < G), []).append(_zero_after(z, pt))
                ot = []
                for r in reversed(range(0, D, VG)):
                    a = None
                    for k in range(off):
                        p8 = pb[k][:8] if deps["pv"] is None or k % 2 else _after(pb[k][:8], deps["pv"])
                        pr = ((_hi if k % 2 else _lo)(vbw[hh, k // 2])[r:r + VG]
                              * jnp.concatenate([p8] * (VG // 8), axis=0))
                        a = pr if a is None else a + pr
                        deps["pv"] = _zero_after(z, a)
                    ot.append(a)
                ov = jnp.concatenate(ot[::-1], axis=0).T
            og = [[x[b * RG:(b + 1) * RG] for x in o] + [ox[e - 1][(b - e) * RG:(b - e + 1) * RG] for e in range(1, b + 1)]
                  for b in range(G)]
            og = [functools.reduce(jnp.add, x) if x else 0.0 for x in og]
            if not vpu:
                return jnp.concatenate(og, axis=0) * (gather(g_v, j) * _recip(jnp.concatenate(ls, axis=0)))
            f = gather(g_v, j) * _recip(jnp.concatenate(ls, axis=0))
            due.setdefault(step + 2, []).append(_zero_after(z, *og[0 if o else 1:]))
            due.setdefault(step + 5, []).append(_zero_after(z, f))
            return f * jnp.concatenate([ov[b * RG:(b + 1) * RG] + x for b, x in enumerate(og)], axis=0)

        def oproj(j, o0, o1):
            y = gather(acc_v, j) + jnp.dot(jnp.concatenate([o0, o1], axis=1).astype(BF16),
                                           _ld(wo_v, p * (2 * D), 2 * D), preferred_element_type=F32)
            for b, r in enumerate(rows(j)):
                acc_v[r:r + RG, :] = y[b * RG:(b + 1) * RG]
                if r < S - TL:
                    o_st[r // TQ, r % TQ:r % TQ + RG, :] = y[b * RG:(b + 1) * RG].astype(BF16)
            j0 = j - j % G
            pl.when(last)(cp_o(j0, min(G, nq - 1 - j0), j % G * RG, RG).start)

        nq = S // TQ
        items = [(j, hh) for j in ORDER for hh in range(2)]
        n = len(items)
        s_vals, o_vals = {}, {}
        wop = jnp.concatenate([f(bwo_p[dp]) for dp in range(DH // 2) for f in (_lo, _hi)], axis=0)
        qproj(ORDER[0])
        for step in range(n + LOOK + OLAG):
            if step % 2 == 0 and 1 + step // 2 < nq:
                qproj(ORDER[1 + step // 2])
            if step < n:
                s_vals[step] = qk(step, *items[step])
            b = step - LOOK
            if 0 <= b < n:
                o_vals[b] = softmax_pv(step, *items[b], s_vals.pop(b))
            c = step - LOOK - OLAG
            if 0 <= c < n and c % 2 == 1:
                done = (items[c][0], o_vals.pop(c - 1), o_vals.pop(c))
                if done[0] % G:
                    oproj(*done)
                else:
                    late.append(done)
                    early.append(bout(slice(None), slice(None), slice(len(early) * 128, len(early) * 128 + 128)))
        for done in late:
            oproj(*done)

        early.append(bout(slice(None), slice(None), slice(len(early) * 128, c0)))
        yl = acc_v[pl.ds(rb, TL), :c0] + jnp.concatenate(early, axis=1)
        ya = acc_v[pl.ds(rb, TL), c0:]
        yr = [[ya[r:r + 16, c:c + 128] for r in range(0, TL, 16)] for c in range(0, M - c0, 128)]
        for t in fill:
            yr[0] = [yr[0][u] + t[u * 16:u * 16 + 16] for u in range(TL // 16)]
        for tile in range(len(fill), NT_M * NCUT):
            c, k = divmod(tile, NT_M)
            cuts = (0,) + CUTS.get(tile, ()) + (TL // 16,)
            for u0, u1 in zip(cuts[:-1], cuts[1:]):
                t = bout(slice(u0 * 16, u1 * 16), slice(k * 128, k * 128 + 128), slice(c0 + c * 128, c0 + c * 128 + 128))
                for u in range(u0, u1):
                    yr[c][u] = yr[c][u] + t[(u - u0) * 16:(u - u0 + 1) * 16]
        y = jnp.concatenate([yl] + [jnp.concatenate(v, axis=0) for v in yr], axis=1)
        acc_v[pl.ds(rb, TL), :] = y
        for ca, cb in zip(OCUT[:-1], OCUT[1:]):
            o_st[S // TQ - 1, :, ca:cb] = y[:, ca:cb].astype(BF16)
            pl.when(last)(cp_o(S // TQ - 1, 1, 0, TQ, ca, cb).start)
        return 0

    for cc in [w0a, x0a, x0b, w0b, w0c, cp_w(1), cp_g, xr] + [cp_w(k) for k in range(2, NT_M)] + a_early:
        cc.start()
    z_v[...] = jnp.zeros((8, 128), U32)
    for part in range(3):
        for t in range(NT_M):
            qkv_v[part, t, 0:PAD, :] = jnp.zeros((PAD, 128), F32)

    def phases():
        first_task()
        lax.fori_loop(1, NT_M, _scoped("bproj", bproj_body), 0)
        for cc in a_waits:
            cc.wait()
        lax.fori_loop(0, HP, _scoped("pair", pair_body), 0)

    def once(i, _):
        pl.when(i == 0)(phases)
        return 0

    lax.fori_loop(0, 2, once, 0)
    with _scope("ow"):
        cp_o(0, S // TQ, 0, TQ).wait()


def _kernel(*refs):
    dma = pltpu.SemaphoreType.DMA
    pl.run_scoped(functools.partial(_body, *refs), dma((4,)), dma((NT_M + 2,)), dma(()), dma(()))


@jax.jit
def pallas_gated_mix__compressed_kv_cla__sliding_local_dilated__prompt_kernel(
    A_x, A_c_kv, A_w_q, A_w_uk, A_w_uv, A_w_o, B_x, B_wqkv, B_wo, gate_w,
):
    del B_x
    x = A_x.reshape(S, M)
    ckv = A_c_kv.reshape(S, DC)
    wo = A_w_o.reshape(H * D, M)
    bwo = B_wo.reshape(H, DH, M)
    any_spec = pl.BlockSpec(memory_space=pl.ANY)
    out = pl.pallas_call(
        _kernel,
        out_shape=jax.ShapeDtypeStruct((S // TQ, TQ, M), BF16),
        in_specs=[any_spec] * 9,
        out_specs=any_spec,
        scratch_shapes=[
            pltpu.VMEM((S // 2, M), U32),
            pltpu.VMEM((S // 2, DC), U32),
            pltpu.VMEM((HP, M, D), U32),
            pltpu.VMEM((HP, DC, D), U32),
            pltpu.VMEM((HP, DC, D), U32),
            pltpu.VMEM((H * D // 2, M), U32),
            pltpu.VMEM((M, 3 * M), BF16),
            pltpu.VMEM((DH // 2, H, M), U32),
            pltpu.VMEM((3, DH * 24, 128), U32),
            pltpu.VMEM((64, 512), U32),
            pltpu.VMEM((3, NT_M, S + PAD, 128), F32),
            pltpu.VMEM((S, M), F32),
            pltpu.VMEM((S, 128), F32),
            pltpu.VMEM((8, 128), U32),
            pltpu.VMEM((S // 2, 2 * D), U32),
            pltpu.VMEM((S // 2, 2 * D), U32),
            pltpu.VMEM((S // 2, 2 * D), U32),
            pltpu.VMEM((S // TQ, TQ, M), BF16),
            pltpu.VMEM((2 * M,), BF16),
        ],
        compiler_params=pltpu.CompilerParams(vmem_limit_bytes=110 * 1024 * 1024),
    )(x, ckv, A_w_q, A_w_uk, A_w_uv, wo, B_wqkv, bwo, gate_w)
    return out.reshape(1, S, M)
```

```python
import contextlib
import functools

import jax
import jax.numpy as jnp
from jax import lax
import jax.experimental.pallas as pl
import jax.experimental.pallas.tpu as pltpu

S = 2048
M = 1024
DC = 512
H = 32
HP = H // 2
D = 128
DH = 32
W = 8
DIL = 2
PAD = 40
NT_M = M // 128
TQ = 128
TL = S // HP
XCUT = (0, 192, 512, 1792, S)
R0 = 256
FP = 33
FCH = 6
GR = 304
PITCH = 17
NA1 = 44
OCUT = (0, 512, 768, M)
LOOK = 2
OLAG = 7
SUMT = 4
MAXT = 8
LAQ = 2
G = 8
RG = TQ // G
ORDER = (8, 9, 2, 11, 12, 5, 14, 7, 0, 1, 10, 3, 4, 13, 6, 15)
NCUT = 4
CUTS = {4: (1,), 5: (1, 2), 9: (1,), 10: (1, 2), 13: (1, 2), 17: (1,), 18: (1,), 21: (1,), 23: (1,), 28: (1,),
        31: (5, 7)}
VG = 32
LOG2E = 1.4426950408889634
NEG = -1e9

F32 = jnp.float32
BF16 = jnp.bfloat16
U32 = jnp.uint32
NT = (((1,), (1,)), ((), ()))


_PROFILE = False


def _scope(name):
    return jax.named_scope(name) if _PROFILE else contextlib.nullcontext()


def _scoped(name, body):
    def f(i, c):
        with _scope(name):
            return body(i, c)
    return f


def _recip(l):
    r = pl.reciprocal(l, approx=True)
    return r * (2.0 - l * r)


def _lo(w):
    return pltpu.bitcast(w << 16, F32)


def _hi(w):
    return pltpu.bitcast(w & jnp.uint32(0xFFFF0000), F32)


def _split_pair(w):
    return jnp.concatenate([_lo(w), _hi(w)], axis=1).astype(BF16)


def _ld(ref, r0, n, cols=slice(None)):
    if isinstance(r0, int):
        rs = slice(r0 // 2, (r0 + n) // 2)
    else:
        rs = pl.ds(pl.multiple_of(lax.shift_right_logical(r0, 1), 8), n // 2)
    return pltpu.bitcast(ref[rs, cols], BF16)


def _st(ref, r0, val, cols=slice(None)):
    ref[r0 // 2:(r0 + val.shape[0]) // 2, cols] = pltpu.bitcast(val, U32)


def _zero_after(z, *vals):
    acc = None
    for v in vals:
        b = pltpu.bitcast(v, U32)
        for r in range(0, b.shape[0], 8):
            for c in range(0, b.shape[1], 128):
                t = b[r:r + 8, c:c + 128]
                acc = t if acc is None else acc | t
    return acc & z


def _after(v, dep):
    b = pltpu.bitcast(v, U32)
    return pltpu.bitcast(b | jnp.concatenate([dep] * (b.shape[0] // 8), axis=0), v.dtype)


def _chain(op, tiles, z, dep):
    a = functools.reduce(op, [tiles[0] if dep is None else _after(tiles[0], dep)] + tiles[1:])
    return a, _zero_after(z, a)


def _body(x_hbm, ckv_hbm, wq_hbm, wuk_hbm, wuv_hbm, wo_hbm, bqkv_hbm, bwo_hbm, gate_hbm,
          out_hbm,
          x_v, ckv_v, wq_p, wuk_p, wuv_p, wo_v, bqkv_v, bwo_p, wcur_v, wfst_v,
          qkv_v, acc_v, g_v, z_v, q_s, k_s, v_s, o_st, gate_v,
          sem_x, sem_w, sem_a, sem_o):
    def cp_x(sm, r0, r1, c0, c1):
        sl = (pl.ds(r0 // 2, (r1 - r0) // 2), pl.ds(c0, c1 - c0))
        return pltpu.make_async_copy(x_hbm.bitcast(U32).at[sl], x_v.at[sl], sem_x.at[sm])

    def cp_w(k, c0=0, c1=3 * M, sm=None):
        sl = (pl.ds(k * 128, 128), pl.ds(c0, c1 - c0))
        return pltpu.make_async_copy(bqkv_hbm.at[sl], bqkv_v.at[sl], sem_w.at[k if sm is None else sm])

    x0 = [cp_x(i, XCUT[i], XCUT[i + 1], 0, 128) for i in range(4)]
    xr = cp_x(4, 0, S, 128, M)
    w0 = [cp_w(0, 0, M // 2), cp_w(0, M // 2, M, NT_M), cp_w(0, M, 3 * M, NT_M + 1)]
    cp_g = pltpu.make_async_copy(gate_hbm, gate_v.at[pl.ds(0, M)], sem_x.at[5])

    def cp_pairs(src, dst):
        return [pltpu.make_async_copy(src.bitcast(U32).at[:, p, :], dst.at[p], sem_a) for p in range(HP)]

    a_early = cp_pairs(bwo_hbm, bwo_p) + [pltpu.make_async_copy(ckv_hbm.bitcast(U32), ckv_v, sem_a),
                                          pltpu.make_async_copy(wo_hbm.bitcast(U32), wo_v, sem_a)]
    a_late = cp_pairs(wuk_hbm, wuk_p) + cp_pairs(wuv_hbm, wuv_p) + cp_pairs(wq_hbm, wq_p)
    a_waits = [pltpu.make_async_copy(b, b, sem_a) for b in (ckv_v, wo_v, wuk_p, wuv_p, wq_p, bwo_p)]

    def cp_o(b0, nb, r0, n, c0=0, c1=M):
        sl = (pl.ds(b0, nb), pl.ds(r0, n), pl.ds(c0, c1 - c0))
        return pltpu.make_async_copy(o_st.at[sl], out_hbm.at[sl], sem_o)

    def prep(part, j, z=None, dep=None, cs=range(NT_M)):
        k0 = j * 128 if isinstance(j, int) else pl.multiple_of(j * 128, 128)
        for c in cs:
            src = bqkv_v[pl.ds(k0, 128), part * M + c * 128:part * M + (c + 1) * 128]
            if dep is not None:
                top = pltpu.bitcast(pltpu.bitcast(src[:16], U32) | dep, BF16)
                src = jnp.concatenate([top, src[16:]], axis=0)
            t = pltpu.bitcast(src.T, U32)
            for hp in range(2):
                a, b = t[32 * hp:32 * hp + 16], t[32 * hp + 16:32 * hp + 32]
                r = 2 * c + hp
                wcur_v[part, pl.ds(r, 16, stride=2 * PITCH), :] = (a & jnp.uint32(0xFFFF)) | (b << 16)
                wcur_v[part, pl.ds(PITCH + r, 16, stride=2 * PITCH), :] = (a >> 16) | (b & jnp.uint32(0xFFFF0000))
            if z is not None:
                dep = _zero_after(z, t[56:64])
        return dep

    def wrows(part, d0, d1):
        w = jnp.concatenate([wcur_v[part, d * PITCH:d * PITCH + HP, :] for d in range(d0, d1)], axis=0)
        return pltpu.bitcast(w, BF16)

    def first_tiles(part):
        for n in range(4):
            _st(wfst_v, 0, wrows(part, 4 * n, 4 * n + 4).T, slice(n * 128, (n + 1) * 128))

    def project(xk, part, first):
        if not first:
            return lax.dot_general(xk, wrows(part, 0, DH), NT, preferred_element_type=F32)
        return jnp.concatenate([jnp.dot(xk, _ld(wfst_v, 0, 128), preferred_element_type=F32),
                                lax.dot_general(xk, wrows(part, DH // 2, DH), NT, preferred_element_type=F32)], axis=1)

    def gate_rows(t, z, dep):
        gw = gate_v[0:M].astype(F32).reshape(1, M)
        g0 = jnp.minimum((t - 1) * GR, S - GR)
        for k in range(GR // 16):
            rr = pl.multiple_of(g0 + k * 16, 16)
            rw = pl.multiple_of(lax.shift_right_logical(rr, 1), 8)
            xb = x_v[pl.ds(rw, 8), :]
            if dep is not None:
                xb = xb | jnp.concatenate([dep] * NT_M, axis=1)
            xx = pltpu.bitcast(xb, BF16).astype(F32)
            zz = jnp.sum(xx * gw, axis=1, keepdims=True)
            g = jnp.broadcast_to(1.0 / (1.0 + jnp.exp(-zz)), (16, 128))
            g_v[pl.ds(rr, 16), :] = g
            acc_v[pl.ds(rr, 16), :] = jnp.zeros((16, M), F32)
            dep = _zero_after(z, g)

    def first_task():
        def piece(part, r0, r1, first):
            y = project(_ld(x_v, r0, r1 - r0, slice(0, 128)), part, first)
            for tt in range(NT_M):
                qkv_v[part, tt, PAD + r0:PAD + r1, :] = y[:, tt * 128:(tt + 1) * 128]

        def raw(r0, r1, c0, c1):
            acc_v[r0:r1, c0:c1] = jnp.dot(_ld(x_v, r0, r1 - r0, slice(0, 128)), bqkv_v[0:128, c0:c1],
                                          preferred_element_type=F32)

        def permute(z):
            deps = []

            def xp(v):
                if len(deps) >= FCH:
                    v = jnp.concatenate([_after(v[:8], deps[-FCH]), v[8:]], axis=0)
                t = v.T
                deps.append(_zero_after(z, t[120:128]))
                return t

            for rb in range(R0 // 128):
                for c in range(NT_M):
                    t = xp(acc_v[rb * 128:(rb + 1) * 128, c * 128:(c + 1) * 128])
                    for hh in range(4):
                        qkv_v[2, rb, pl.ds(PAD + 4 * c + hh, DH, stride=FP), :] = t[DH * hh:DH * (hh + 1)]
            for rb in range(R0 // 128):
                for tt in range(NT_M):
                    u = [qkv_v[2, rb, PAD + d * FP:PAD + d * FP + H, :] for d in range(4 * tt, 4 * tt + 4)]
                    qkv_v[0, tt, PAD + rb * 128:PAD + (rb + 1) * 128, :] = xp(jnp.concatenate(u, axis=0))

        with _scope("b0"):
            w0[0].wait()
            x0[0].wait()
            raw(0, XCUT[1], 0, M // 2)
            prep(0, 0, cs=range(NT_M // 2))
        with _scope("b1"):
            w0[1].wait()
            x0[1].wait()
            raw(XCUT[1], R0, 0, M // 2)
            raw(0, R0, M // 2, M)
            prep(0, 0, cs=range(NT_M // 2, NT_M))
            piece(0, R0, XCUT[2], False)
            first_tiles(0)
        with _scope("b2"):
            x0[2].wait()
            piece(0, XCUT[2], XCUT[3], True)
            permute(z_v[...])
        with _scope("b3"):
            x0[3].wait()
            w0[2].wait()
            cp_w(1).wait()
            z = z_v[...]
            piece(0, XCUT[3], S, True)
            prep(1, 0)
            piece(1, 0, S, False)
            prep(2, 0)
            dep = prep(0, 1, z)
            first_tiles(0)
            piece(2, 0, S, False)
            prep(1, 1, z, dep)
            prep(2, 1)
            for cc in a_late[:NA1]:
                cc.start()
        for cc in (xr, cp_g):
            cc.wait()
        for cc in a_late[NA1:]:
            cc.start()

    def bproj_body(t, _):
        @pl.when(t < NT_M - 1)
        def _():
            cp_w(t + 1).wait()

        z = z_v[...]
        u = jnp.minimum(t + 1, NT_M - 1)
        xw = x_v[:, pl.ds(pl.multiple_of(t * 128, 128), 128)]
        xk = pltpu.bitcast(xw | jnp.concatenate([z] * (S // 16), axis=0), BF16)
        dep = None
        for part in range(3):
            y = project(xk, part, part == 0)
            for tt in range(NT_M):
                qkv_v[part, tt, PAD:, :] = qkv_v[part, tt, PAD:, :] + y[:, tt * 128:(tt + 1) * 128]
            dep = prep(part, u, z, dep) if part < 2 else prep(part, u)
            if part == 0:
                first_tiles(0)
        gate_rows(t, z, None)
        return 0

    qscale = (D ** -0.5) * LOG2E
    bscale = (DH ** -0.5) * LOG2E

    def local_attn(r, z, dep):
        def zf(v):
            return pltpu.bitcast(_zero_after(z, v), F32)

        sc = jnp.full((8, 128), bscale, F32)
        if dep is not None:
            sc = sc + dep
        q = [qkv_v[0, t, pl.ds(PAD + r, 8), :] * sc for t in range(NT_M)]
        rowi = r + lax.broadcasted_iota(jnp.int32, (8, 128), 0)
        logits, raw = [], []
        for w in range(W):
            a = None if w < LAQ else zf(raw[w - LAQ])
            for t in range(NT_M):
                pr = q[t] * qkv_v[1, t, pl.ds(PAD + r - DIL * w, 8), :]
                a = pr if a is None else a + pr
            raw.append(a)
            a = a + pltpu.roll(a, 64, 1)
            a = a + pltpu.roll(a, 32, 1)
            logits.append(jnp.where(rowi >= DIL * w, a, NEG) if w > 0 else a)
        m = functools.reduce(jnp.maximum, logits)
        es = [jnp.exp2(lg - m) for lg in logits]
        l = functools.reduce(lambda a, b: a + b, es)
        f = (1.0 - g_v[pl.ds(r, 8), :]) * _recip(l)
        es = [e * f for e in es]
        outs = []
        for t in range(NT_M):
            a = None if t == 0 else zf(outs[t - 1])
            for w in range(W):
                pr = es[w] * qkv_v[2, t, pl.ds(PAD + r - DIL * w, 8), :]
                a = pr if a is None else a + pr
            outs.append(a)
        return jnp.concatenate(outs, axis=1), zf(outs[-1])

    def pair_body(p, _):
        z = z_v[...]
        last = p == HP - 1
        wk, wv = _split_pair(wuk_p[p]), _split_pair(wuv_p[p])
        _st(k_s, 0, jnp.dot(_ld(ckv_v, 0, S), wk, preferred_element_type=F32).astype(BF16))
        _st(v_s, 0, jnp.dot(_ld(ckv_v, 0, S), wv, preferred_element_type=F32).astype(BF16))

        rb = pl.multiple_of(p * TL, TL)
        dep, obs = None, []
        for k in range(TL // 8):
            ob, dep = local_attn(rb + k * 8, z, dep)
            if k == 0:
                v = g_v[pl.ds(rb, 24), :]
                dep = dep + pltpu.bitcast(_zero_after(z, jnp.broadcast_to(v[:, 0:1], v.shape)), F32)
            obs.append(ob)
        ob = jnp.concatenate(obs, axis=0)

        wqw = wq_p[p]
        wq = _split_pair(jnp.concatenate([wqw[:8] | _zero_after(z, ob[TL - 16:].astype(BF16)), wqw[8:]], axis=0))
        row = lax.broadcasted_iota(jnp.int32, (RG, TQ), 0)
        col = lax.broadcasted_iota(jnp.int32, (RG, TQ), 1)
        diag = col <= row + (TQ - RG)

        def rows(j):
            return [(j - j % G + b) * TQ + (j % G) * RG for b in range(G)]

        def geom(j):
            off = (j % G + 1) * RG % TQ
            return off, j - j % G + (0 if off else 1)

        def gather(ref, j, ld=lambda ref, r: ref[r:r + RG, :]):
            return jnp.concatenate([ld(ref, r) for r in rows(j)], axis=0)

        def head(h):
            return slice(h * D, (h + 1) * D)

        vbw = {}

        def qproj(j):
            xg = gather(x_v, j, lambda ref, r: _ld(ref, r, RG))
            if j == ORDER[1]:
                for h in range(2):
                    for i in range(RG // 2):
                        wrow = pltpu.bitcast(v_s[i:i + 1, head(h)], F32)
                        vbw[h, i] = pltpu.bitcast(jnp.broadcast_to(wrow, (TQ, D)).T, U32)
                top = _after(xg[:16, :128], _zero_after(z, *[x[TQ - 8:] for x in vbw.values()]))
                xg = jnp.concatenate([jnp.concatenate([top, xg[:16, 128:]], axis=1), xg[16:]], axis=0)
            _st(q_s, j * TQ, (jnp.dot(xg, wq, preferred_element_type=F32) * qscale).astype(BF16))

        def bout(rs, ks, cs):
            return jnp.dot(ob[rs, ks].astype(BF16), wop[ks, cs].astype(BF16), preferred_element_type=F32)

        due = {}

        def qk(step, j, hh):
            off, nc = geom(j)
            q = _ld(q_s, j * TQ, TQ, head(hh))
            for d in due.pop(step, ()):
                q = jnp.concatenate([q[:TQ - 16], _after(q[TQ - 16:], d)], axis=0)
            com = lax.dot_general(q, _ld(k_s, off, nc * TQ, head(hh)), NT, preferred_element_type=F32) if nc else None
            ext = {e: lax.dot_general(q[e * RG:], _ld(k_s, off + (nc + e - 1) * TQ, TQ, head(hh)), NT,
                                      preferred_element_type=F32) for e in reversed(range(1, G))}
            left = None
            if off:
                st = lax.dot_general(_ld(k_s, 0, off, head(hh)), _ld(q_s, j * TQ, TQ, head(hh)), NT,
                                     preferred_element_type=F32)
                left = jnp.concatenate([st, jnp.full((TQ - off, TQ), NEG, F32)], axis=0).T
            return com, ext, left

        deps = {"max": None, "sum": None, "pv": None}
        fill, early, late = [], [], []
        c0 = M - 128 * NCUT

        def softmax(parts):
            if len(parts) > MAXT:
                m, deps["max"] = _chain(jnp.maximum, parts[1:], z, deps["max"])
                m = jnp.maximum(m, parts[0])
            else:
                m = functools.reduce(jnp.maximum, parts[1:] + parts[:1])
            e = jnp.exp2(jnp.concatenate(parts, axis=1) - jnp.max(m, axis=1, keepdims=True))
            l = e
            if len(parts) > SUMT:
                l, deps["sum"] = _chain(jnp.add, [e[:, c:c + TQ] for c in range(0, e.shape[1], TQ)], z, deps["sum"])
            return e, jnp.sum(l, axis=1, keepdims=True)

        def softmax_pv(step, j, hh, sc):
            off, nc = geom(j)
            com, ext, left = sc
            es, ls = [], []
            for b in range(G):
                rs = slice(b * RG, (b + 1) * RG)
                parts = [left[rs]] if off else []
                parts += [com[rs, t * TQ:(t + 1) * TQ] for t in range(nc)]
                parts += [ext[e][(b - e) * RG:(b - e + 1) * RG] for e in range(1, b + 1)]
                parts[-1] = jnp.where(diag if nc + b else col <= row + (off - RG), parts[-1], NEG)
                e, l = softmax(parts)
                es.append(e)
                ls.append(l)
            w = es[0].shape[1]
            vpu = off == RG
            vs = [_ld(v_s, 0, TQ, head(hh))] if off and not vpu else []
            if nc:
                vs.append(_ld(v_s, off, nc * TQ, head(hh)))
            if vpu:
                tail = _after(es[-1][:, -TQ:], _zero_after(z, *[e[:, :TQ] for e in es]))
                es[-1] = jnp.concatenate([es[-1][:, :-TQ], tail], axis=1)
                fill.append(bout(slice(None), slice(len(fill) * 128, len(fill) * 128 + 128), slice(c0, c0 + 128)))
            o = [jnp.dot(jnp.concatenate([e[:, TQ * vpu:w] for e in es], axis=0).astype(BF16),
                         jnp.concatenate(vs, axis=0), preferred_element_type=F32)] if vs else []
            ox = [jnp.dot(jnp.concatenate([x[:, w + (e - 1) * TQ:w + e * TQ] for x in es[e:]], axis=0).astype(BF16),
                          _ld(v_s, off + (nc + e - 1) * TQ, TQ, head(hh)), preferred_element_type=F32)
                  for e in range(1, G)]
            if vpu:
                pt = jnp.concatenate([e[:, :off] for e in es], axis=0).T
                pb = [jnp.broadcast_to(pt[k:k + 1], (VG, TQ)) for k in range(off)]
                due.setdefault(step + 1 + hh + (j < G), []).append(_zero_after(z, pt))
                ot = []
                for r in reversed(range(0, D, VG)):
                    a = None
                    for k in range(off):
                        p8 = pb[k][:8] if deps["pv"] is None or k % 2 else _after(pb[k][:8], deps["pv"])
                        pr = ((_hi if k % 2 else _lo)(vbw[hh, k // 2])[r:r + VG]
                              * jnp.concatenate([p8] * (VG // 8), axis=0))
                        a = pr if a is None else a + pr
                        deps["pv"] = _zero_after(z, a)
                    ot.append(a)
                ov = jnp.concatenate(ot[::-1], axis=0).T
            og = [[x[b * RG:(b + 1) * RG] for x in o] + [ox[e - 1][(b - e) * RG:(b - e + 1) * RG] for e in range(1, b + 1)]
                  for b in range(G)]
            og = [functools.reduce(jnp.add, x) if x else 0.0 for x in og]
            if not vpu:
                return jnp.concatenate(og, axis=0) * (gather(g_v, j) * _recip(jnp.concatenate(ls, axis=0)))
            f = gather(g_v, j) * _recip(jnp.concatenate(ls, axis=0))
            due.setdefault(step + 2, []).append(_zero_after(z, *og[0 if o else 1:]))
            due.setdefault(step + 5, []).append(_zero_after(z, f))
            return f * jnp.concatenate([ov[b * RG:(b + 1) * RG] + x for b, x in enumerate(og)], axis=0)

        def oproj(j, o0, o1):
            y = gather(acc_v, j) + jnp.dot(jnp.concatenate([o0, o1], axis=1).astype(BF16),
                                           _ld(wo_v, p * (2 * D), 2 * D), preferred_element_type=F32)
            for b, r in enumerate(rows(j)):
                acc_v[r:r + RG, :] = y[b * RG:(b + 1) * RG]
                if r < S - TL:
                    o_st[r // TQ, r % TQ:r % TQ + RG, :] = y[b * RG:(b + 1) * RG].astype(BF16)
            j0 = j - j % G
            pl.when(last)(cp_o(j0, min(G, nq - 1 - j0), j % G * RG, RG).start)

        nq = S // TQ
        items = [(j, hh) for j in ORDER for hh in range(2)]
        n = len(items)
        s_vals, o_vals = {}, {}
        wop = jnp.concatenate([f(bwo_p[dp]) for dp in range(DH // 2) for f in (_lo, _hi)], axis=0)
        qproj(ORDER[0])
        for step in range(n + LOOK + OLAG):
            if step % 2 == 0 and 1 + step // 2 < nq:
                qproj(ORDER[1 + step // 2])
            if step < n:
                s_vals[step] = qk(step, *items[step])
            b = step - LOOK
            if 0 <= b < n:
                o_vals[b] = softmax_pv(step, *items[b], s_vals.pop(b))
            c = step - LOOK - OLAG
            if 0 <= c < n and c % 2 == 1:
                done = (items[c][0], o_vals.pop(c - 1), o_vals.pop(c))
                if done[0] % G:
                    oproj(*done)
                else:
                    late.append(done)
                    early.append(bout(slice(None), slice(None), slice(len(early) * 128, len(early) * 128 + 128)))
        for done in late:
            oproj(*done)

        early.append(bout(slice(None), slice(None), slice(len(early) * 128, c0)))
        yl = acc_v[pl.ds(rb, TL), :c0] + jnp.concatenate(early, axis=1)
        ya = acc_v[pl.ds(rb, TL), c0:]
        yr = [[ya[r:r + 16, c:c + 128] for r in range(0, TL, 16)] for c in range(0, M - c0, 128)]
        for t in fill:
            yr[0] = [yr[0][u] + t[u * 16:u * 16 + 16] for u in range(TL // 16)]
        for tile in range(len(fill), NT_M * NCUT):
            c, k = divmod(tile, NT_M)
            cuts = (0,) + CUTS.get(tile, ()) + (TL // 16,)
            for u0, u1 in zip(cuts[:-1], cuts[1:]):
                t = bout(slice(u0 * 16, u1 * 16), slice(k * 128, k * 128 + 128), slice(c0 + c * 128, c0 + c * 128 + 128))
                for u in range(u0, u1):
                    yr[c][u] = yr[c][u] + t[(u - u0) * 16:(u - u0 + 1) * 16]
        y = jnp.concatenate([yl] + [jnp.concatenate(v, axis=0) for v in yr], axis=1)
        acc_v[pl.ds(rb, TL), :] = y
        for ca, cb in zip(OCUT[:-1], OCUT[1:]):
            o_st[S // TQ - 1, :, ca:cb] = y[:, ca:cb].astype(BF16)
            pl.when(last)(cp_o(S // TQ - 1, 1, 0, TQ, ca, cb).start)
        return 0

    for cc in ([w0[0], x0[0], w0[1], x0[1], x0[2], x0[3], w0[2], cp_w(1), cp_g, xr]
               + [cp_w(k) for k in range(2, NT_M)] + a_early):
        cc.start()
    z_v[...] = jnp.zeros((8, 128), U32)
    for part in range(3):
        for t in range(NT_M):
            qkv_v[part, t, 0:PAD, :] = jnp.zeros((PAD, 128), F32)

    def phases():
        first_task()
        lax.fori_loop(1, NT_M, _scoped("bproj", bproj_body), 0)
        for cc in a_waits:
            cc.wait()
        lax.fori_loop(0, HP, _scoped("pair", pair_body), 0)

    def once(i, _):
        pl.when(i == 0)(phases)
        return 0

    lax.fori_loop(0, 2, once, 0)
    with _scope("ow"):
        cp_o(0, S // TQ, 0, TQ).wait()


def _kernel(*refs):
    dma = pltpu.SemaphoreType.DMA
    pl.run_scoped(functools.partial(_body, *refs), dma((6,)), dma((NT_M + 2,)), dma(()), dma(()))


@jax.jit
def pallas_gated_mix__compressed_kv_cla__sliding_local_dilated__prompt_kernel(
    A_x, A_c_kv, A_w_q, A_w_uk, A_w_uv, A_w_o, B_x, B_wqkv, B_wo, gate_w,
):
    del B_x
    x = A_x.reshape(S, M)
    ckv = A_c_kv.reshape(S, DC)
    wo = A_w_o.reshape(H * D, M)
    bwo = B_wo.reshape(H, DH, M)
    any_spec = pl.BlockSpec(memory_space=pl.ANY)
    out = pl.pallas_call(
        _kernel,
        out_shape=jax.ShapeDtypeStruct((S // TQ, TQ, M), BF16),
        in_specs=[any_spec] * 9,
        out_specs=any_spec,
        scratch_shapes=[
            pltpu.VMEM((S // 2, M), U32),
            pltpu.VMEM((S // 2, DC), U32),
            pltpu.VMEM((HP, M, D), U32),
            pltpu.VMEM((HP, DC, D), U32),
            pltpu.VMEM((HP, DC, D), U32),
            pltpu.VMEM((H * D // 2, M), U32),
            pltpu.VMEM((M, 3 * M), BF16),
            pltpu.VMEM((DH // 2, H, M), U32),
            pltpu.VMEM((3, DH * 24, 128), U32),
            pltpu.VMEM((64, 512), U32),
            pltpu.VMEM((3, NT_M, S + PAD, 128), F32),
            pltpu.VMEM((S, M), F32),
            pltpu.VMEM((S, 128), F32),
            pltpu.VMEM((8, 128), U32),
            pltpu.VMEM((S // 2, 2 * D), U32),
            pltpu.VMEM((S // 2, 2 * D), U32),
            pltpu.VMEM((S // 2, 2 * D), U32),
            pltpu.VMEM((S // TQ, TQ, M), BF16),
            pltpu.VMEM((2 * M,), BF16),
        ],
        compiler_params=pltpu.CompilerParams(vmem_limit_bytes=110 * 1024 * 1024),
    )(x, ckv, A_w_q, A_w_uk, A_w_uv, wo, B_wqkv, bwo, gate_w)
    return out.reshape(1, S, M)
```

```python
import contextlib
import functools

import jax
import jax.numpy as jnp
from jax import lax
import jax.experimental.pallas as pl
import jax.experimental.pallas.tpu as pltpu

S = 2048
M = 1024
DC = 512
H = 32
HP = H // 2
D = 128
DH = 32
W = 8
DIL = 2
PAD = 16
NT_M = M // 128
TQ = 128
TL = S // HP
XCUT = (0, 192, 512, 1792, S)
R0 = 256
FP = 33
FCH = 6
GR = 304
PITCH = 17
NA1 = 44
OCUT = (0, 512, 896, M)
LOOK = 2
OLAG = 7
SUMT = 5
MAXT = 8
LAQ = 2
G = 8
RG = TQ // G
ORDER = (8, 9, 2, 11, 12, 5, 14, 7, 0, 1, 10, 3, 4, 13, 6, 15)
NCUT = 4
CUTS = {1: (1, 2, 3), 4: (1,), 6: (1, 2), 9: (1, 2), 11: (1,), 13: (1,), 14: (1, 2), 17: (1,), 20: (1,), 21: (1,),
        24: (1,), 26: (1,), 28: (1,), 30: (7,), 31: (4, 6, 7)}
VO = 2 * RG
QK_ORD = {18: (2, 4, 3, 1, 6, 5, 7)}
PV_ORD = {16: (1, 6, 3, 4, 7, 2, 5), 17: (1, 5, 6, 4, 7, 2, 3)}
VG = 32
LOG2E = 1.4426950408889634
NEG = -1e9

F32 = jnp.float32
BF16 = jnp.bfloat16
U32 = jnp.uint32
NT = (((1,), (1,)), ((), ()))


_PROFILE = False


def _scope(name):
    return jax.named_scope(name) if _PROFILE else contextlib.nullcontext()


def _scoped(name, body):
    def f(i, c):
        with _scope(name):
            return body(i, c)
    return f


def _recip(l):
    r = pl.reciprocal(l, approx=True)
    return r * (2.0 - l * r)


def _lo(w):
    return pltpu.bitcast(w << 16, F32)


def _hi(w):
    return pltpu.bitcast(w & jnp.uint32(0xFFFF0000), F32)


def _split_pair(w):
    return jnp.concatenate([_lo(w), _hi(w)], axis=1).astype(BF16)


def _ld(ref, r0, n, cols=slice(None)):
    if isinstance(r0, int):
        rs = slice(r0 // 2, (r0 + n) // 2)
    else:
        rs = pl.ds(pl.multiple_of(lax.shift_right_logical(r0, 1), 8), n // 2)
    return pltpu.bitcast(ref[rs, cols], BF16)


def _st(ref, r0, val, cols=slice(None)):
    ref[r0 // 2:(r0 + val.shape[0]) // 2, cols] = pltpu.bitcast(val, U32)


def _zero_after(z, *vals):
    acc = None
    for v in vals:
        b = pltpu.bitcast(v, U32)
        for r in range(0, b.shape[0], 8):
            for c in range(0, b.shape[1], 128):
                t = b[r:r + 8, c:c + 128]
                acc = t if acc is None else acc | t
    return acc & z


def _after(v, dep):
    b = pltpu.bitcast(v, U32)
    return pltpu.bitcast(b | jnp.concatenate([dep] * (b.shape[0] // 8), axis=0), v.dtype)


def _chain(op, tiles, z, dep):
    a = functools.reduce(op, [tiles[0] if dep is None else _after(tiles[0], dep)] + tiles[1:])
    return a, _zero_after(z, a)


def _body(x_hbm, ckv_hbm, wq_hbm, wuk_hbm, wuv_hbm, wo_hbm, bqkv_hbm, bwo_hbm, gate_hbm,
          out_hbm,
          x_v, ckv_v, wq_p, wuk_p, wuv_p, wo_v, bqkv_v, bwo_p, wcur_v, wfst_v,
          qkv_v, acc_v, g_v, z_v, q_s, k_s, v_s, o_st, gate_v,
          sem_x, sem_w, sem_a, sem_o):
    def cp_x(sm, r0, r1, c0, c1):
        sl = (pl.ds(r0 // 2, (r1 - r0) // 2), pl.ds(c0, c1 - c0))
        return pltpu.make_async_copy(x_hbm.bitcast(U32).at[sl], x_v.at[sl], sem_x.at[sm])

    def cp_w(k, c0=0, c1=3 * M, sm=None):
        sl = (pl.ds(k * 128, 128), pl.ds(c0, c1 - c0))
        return pltpu.make_async_copy(bqkv_hbm.at[sl], bqkv_v.at[sl], sem_w.at[k if sm is None else sm])

    x0 = [cp_x(i, XCUT[i], XCUT[i + 1], 0, 128) for i in range(4)]
    xr = cp_x(4, 0, S, 128, M)
    w0 = [cp_w(0, 0, M // 2), cp_w(0, M // 2, M, NT_M), cp_w(0, M, 3 * M, NT_M + 1)]
    cp_g = pltpu.make_async_copy(gate_hbm, gate_v.at[pl.ds(0, M)], sem_x.at[5])

    def cp_pairs(src, dst):
        return [pltpu.make_async_copy(src.bitcast(U32).at[:, p, :], dst.at[p], sem_a) for p in range(HP)]

    a_early = cp_pairs(bwo_hbm, bwo_p) + [pltpu.make_async_copy(ckv_hbm.bitcast(U32), ckv_v, sem_a),
                                          pltpu.make_async_copy(wo_hbm.bitcast(U32), wo_v, sem_a)]
    a_late = cp_pairs(wuk_hbm, wuk_p) + cp_pairs(wuv_hbm, wuv_p) + cp_pairs(wq_hbm, wq_p)
    a_waits = [pltpu.make_async_copy(b, b, sem_a) for b in (ckv_v, wo_v, wuk_p, wuv_p, wq_p, bwo_p)]

    def cp_o(b0, nb, r0, n, c0=0, c1=M):
        sl = (pl.ds(b0, nb), pl.ds(r0, n), pl.ds(c0, c1 - c0))
        return pltpu.make_async_copy(o_st.at[sl], out_hbm.at[sl], sem_o)

    def prep(part, j, z=None, dep=None, cs=range(NT_M)):
        k0 = j * 128 if isinstance(j, int) else pl.multiple_of(j * 128, 128)
        for c in cs:
            src = bqkv_v[pl.ds(k0, 128), part * M + c * 128:part * M + (c + 1) * 128]
            if dep is not None:
                top = pltpu.bitcast(pltpu.bitcast(src[:16], U32) | dep, BF16)
                src = jnp.concatenate([top, src[16:]], axis=0)
            t = pltpu.bitcast(src.T, U32)
            for hp in range(2):
                a, b = t[32 * hp:32 * hp + 16], t[32 * hp + 16:32 * hp + 32]
                r = 2 * c + hp
                wcur_v[part, pl.ds(r, 16, stride=2 * PITCH), :] = (a & jnp.uint32(0xFFFF)) | (b << 16)
                wcur_v[part, pl.ds(PITCH + r, 16, stride=2 * PITCH), :] = (a >> 16) | (b & jnp.uint32(0xFFFF0000))
            if z is not None:
                dep = _zero_after(z, t[56:64])
        return dep

    def wrows(part, d0, d1):
        w = jnp.concatenate([wcur_v[part, d * PITCH:d * PITCH + HP, :] for d in range(d0, d1)], axis=0)
        return pltpu.bitcast(w, BF16)

    def first_tiles(part):
        for n in range(4):
            _st(wfst_v, 0, wrows(part, 4 * n, 4 * n + 4).T, slice(n * 128, (n + 1) * 128))

    def project(xk, part, first):
        if not first:
            return lax.dot_general(xk, wrows(part, 0, DH), NT, preferred_element_type=F32)
        return jnp.concatenate([jnp.dot(xk, _ld(wfst_v, 0, 128), preferred_element_type=F32),
                                lax.dot_general(xk, wrows(part, DH // 2, DH), NT, preferred_element_type=F32)], axis=1)

    def gate_rows(t, z, dep):
        gw = gate_v[0:M].astype(F32).reshape(1, M)
        g0 = jnp.minimum((t - 1) * GR, S - GR)
        for k in range(GR // 16):
            rr = pl.multiple_of(g0 + k * 16, 16)
            rw = pl.multiple_of(lax.shift_right_logical(rr, 1), 8)
            xb = x_v[pl.ds(rw, 8), :]
            if dep is not None:
                xb = xb | jnp.concatenate([dep] * NT_M, axis=1)
            xx = pltpu.bitcast(xb, BF16).astype(F32)
            zz = jnp.sum(xx * gw, axis=1, keepdims=True)
            g = jnp.broadcast_to(1.0 / (1.0 + jnp.exp(-zz)), (16, 128))
            g_v[pl.ds(rr, 16), :] = g
            acc_v[pl.ds(rr, 16), :] = jnp.zeros((16, M), F32)
            dep = _zero_after(z, g)

    def first_task():
        def piece(part, r0, r1, first):
            y = project(_ld(x_v, r0, r1 - r0, slice(0, 128)), part, first)
            for tt in range(NT_M):
                qkv_v[part, tt, PAD + r0:PAD + r1, :] = y[:, tt * 128:(tt + 1) * 128]

        def raw(r0, r1, c0, c1):
            acc_v[r0:r1, c0:c1] = jnp.dot(_ld(x_v, r0, r1 - r0, slice(0, 128)), bqkv_v[0:128, c0:c1],
                                          preferred_element_type=F32)

        def permute(z):
            deps = []

            def xp(v):
                if len(deps) >= FCH:
                    v = jnp.concatenate([_after(v[:8], deps[-FCH]), v[8:]], axis=0)
                t = v.T
                deps.append(_zero_after(z, t[120:128]))
                return t

            for rb in range(R0 // 128):
                for c in range(NT_M):
                    t = xp(acc_v[rb * 128:(rb + 1) * 128, c * 128:(c + 1) * 128])
                    for hh in range(4):
                        qkv_v[2, rb, pl.ds(PAD + 4 * c + hh, DH, stride=FP), :] = t[DH * hh:DH * (hh + 1)]
            for rb in range(R0 // 128):
                for tt in range(NT_M):
                    u = [qkv_v[2, rb, PAD + d * FP:PAD + d * FP + H, :] for d in range(4 * tt, 4 * tt + 4)]
                    qkv_v[0, tt, PAD + rb * 128:PAD + (rb + 1) * 128, :] = xp(jnp.concatenate(u, axis=0))

        with _scope("b0"):
            w0[0].wait()
            x0[0].wait()
            raw(0, XCUT[1], 0, M // 2)
            prep(0, 0, cs=range(NT_M // 2))
        with _scope("b1"):
            w0[1].wait()
            x0[1].wait()
            raw(XCUT[1], R0, 0, M // 2)
            raw(0, R0, M // 2, M)
            prep(0, 0, cs=range(NT_M // 2, NT_M))
            piece(0, R0, XCUT[2], False)
            first_tiles(0)
        with _scope("b2"):
            x0[2].wait()
            piece(0, XCUT[2], XCUT[3], True)
            permute(z_v[...])
        with _scope("b3"):
            x0[3].wait()
            w0[2].wait()
            cp_w(1).wait()
            z = z_v[...]
            piece(0, XCUT[3], S, True)
            prep(1, 0)
            piece(1, 0, S, False)
            prep(2, 0)
            dep = prep(0, 1, z)
            first_tiles(0)
            piece(2, 0, S, False)
            prep(1, 1, z, dep)
            prep(2, 1)
            for cc in a_late[:NA1]:
                cc.start()
        for cc in (xr, cp_g):
            cc.wait()
        for cc in a_late[NA1:]:
            cc.start()

    def bproj_body(t, _):
        @pl.when(t < NT_M - 1)
        def _():
            cp_w(t + 1).wait()

        z = z_v[...]
        u = jnp.minimum(t + 1, NT_M - 1)
        xw = x_v[:, pl.ds(pl.multiple_of(t * 128, 128), 128)]
        xk = pltpu.bitcast(xw | jnp.concatenate([z] * (S // 16), axis=0), BF16)
        dep = None
        for part in range(3):
            y = project(xk, part, part == 0)
            for tt in range(NT_M):
                qkv_v[part, tt, PAD:, :] = qkv_v[part, tt, PAD:, :] + y[:, tt * 128:(tt + 1) * 128]
            dep = prep(part, u, z, dep) if part < 2 else prep(part, u)
            if part == 0:
                first_tiles(0)
        gate_rows(t, z, None)
        return 0

    qscale = (D ** -0.5) * LOG2E
    bscale = (DH ** -0.5) * LOG2E

    def local_attn(r, z, dep):
        def zf(v):
            return pltpu.bitcast(_zero_after(z, v), F32)

        sc = jnp.full((8, 128), bscale, F32)
        if dep is not None:
            sc = sc + dep
        q = [qkv_v[0, t, pl.ds(PAD + r, 8), :] * sc for t in range(NT_M)]
        rowi = r + lax.broadcasted_iota(jnp.int32, (8, 128), 0)
        logits, raw = [], []
        for w in range(W):
            a = None if w < LAQ else zf(raw[w - LAQ])
            for t in range(NT_M):
                pr = q[t] * qkv_v[1, t, pl.ds(PAD + r - DIL * w, 8), :]
                a = pr if a is None else a + pr
            raw.append(a)
            a = a + pltpu.roll(a, 64, 1)
            a = a + pltpu.roll(a, 32, 1)
            logits.append(jnp.where(rowi >= DIL * w, a, NEG) if w > 0 else a)
        m = functools.reduce(jnp.maximum, logits)
        es = [jnp.exp2(lg - m) for lg in logits]
        l = functools.reduce(lambda a, b: a + b, es)
        f = (1.0 - g_v[pl.ds(r, 8), :]) * _recip(l)
        es = [e * f for e in es]
        outs = []
        for t in range(NT_M):
            a = None if t == 0 else zf(outs[t - 1])
            for w in range(W):
                pr = es[w] * qkv_v[2, t, pl.ds(PAD + r - DIL * w, 8), :]
                a = pr if a is None else a + pr
            outs.append(a)
        return jnp.concatenate(outs, axis=1), zf(outs[-1])

    def pair_body(p, _):
        z = z_v[...]
        last = p == HP - 1
        wk, wv = _split_pair(wuk_p[p]), _split_pair(wuv_p[p])
        _st(k_s, 0, jnp.dot(_ld(ckv_v, 0, S), wk, preferred_element_type=F32).astype(BF16))
        _st(v_s, 0, jnp.dot(_ld(ckv_v, 0, S), wv, preferred_element_type=F32).astype(BF16))

        rb = pl.multiple_of(p * TL, TL)
        dep, obs = None, []
        for k in range(TL // 8):
            ob, dep = local_attn(rb + k * 8, z, dep)
            if k == 0:
                v = g_v[pl.ds(rb, 24), :]
                dep = dep + pltpu.bitcast(_zero_after(z, jnp.broadcast_to(v[:, 0:1], v.shape)), F32)
            obs.append(ob)
        ob = jnp.concatenate(obs, axis=0)

        wqw = wq_p[p]
        wq = _split_pair(jnp.concatenate([wqw[:8] | _zero_after(z, ob[TL - 16:].astype(BF16)), wqw[8:]], axis=0))
        row = lax.broadcasted_iota(jnp.int32, (RG, TQ), 0)
        col = lax.broadcasted_iota(jnp.int32, (RG, TQ), 1)
        diag = col <= row + (TQ - RG)

        def rows(j):
            return [(j - j % G + b) * TQ + (j % G) * RG for b in range(G)]

        def geom(j):
            off = (j % G + 1) * RG % TQ
            return off, j - j % G + (0 if off else 1)

        def gather(ref, j, ld=lambda ref, r: ref[r:r + RG, :]):
            return jnp.concatenate([ld(ref, r) for r in rows(j)], axis=0)

        def head(h):
            return slice(h * D, (h + 1) * D)

        vbw = {}

        def qproj(j):
            xg = gather(x_v, j, lambda ref, r: _ld(ref, r, RG))
            if j == ORDER[1]:
                for h in range(2):
                    for i in range(VO // 2):
                        wrow = pltpu.bitcast(v_s[i:i + 1, head(h)], F32)
                        vbw[h, i] = pltpu.bitcast(jnp.broadcast_to(wrow, (TQ, D)).T, U32)
                top = _after(xg[:16, :128], _zero_after(z, *[x[TQ - 8:] for x in vbw.values()]))
                xg = jnp.concatenate([jnp.concatenate([top, xg[:16, 128:]], axis=1), xg[16:]], axis=0)
            _st(q_s, j * TQ, (jnp.dot(xg, wq, preferred_element_type=F32) * qscale).astype(BF16))

        def bout(rs, ks, cs):
            return jnp.dot(ob[rs, ks].astype(BF16), wop[ks, cs].astype(BF16), preferred_element_type=F32)

        due = {}

        def qk(step, j, hh):
            off, nc = geom(j)
            q = _ld(q_s, j * TQ, TQ, head(hh))
            for d in due.pop(step, ()):
                q = jnp.concatenate([q[:TQ - 16], _after(q[TQ - 16:], d)], axis=0)
            com = lax.dot_general(q, _ld(k_s, off, nc * TQ, head(hh)), NT, preferred_element_type=F32) if nc else None
            ext = {e: lax.dot_general(q[e * RG:], _ld(k_s, off + (nc + e - 1) * TQ, TQ, head(hh)), NT,
                                      preferred_element_type=F32) for e in QK_ORD.get(step, range(1, G))}
            left = None
            if off:
                st = lax.dot_general(_ld(k_s, 0, off, head(hh)), _ld(q_s, j * TQ, TQ, head(hh)), NT,
                                     preferred_element_type=F32)
                left = jnp.concatenate([st, jnp.full((TQ - off, TQ), NEG, F32)], axis=0).T
            return com, ext, left

        deps = {"max": None, "sum": None, "pv": None}
        fill = []
        c0 = M - 128 * NCUT

        def softmax(parts):
            if len(parts) > MAXT:
                m, deps["max"] = _chain(jnp.maximum, parts[1:], z, deps["max"])
                m = jnp.maximum(m, parts[0])
            else:
                m = functools.reduce(jnp.maximum, parts[1:] + parts[:1])
            e = jnp.exp2(jnp.concatenate(parts, axis=1) - jnp.max(m, axis=1, keepdims=True))
            l = e
            if len(parts) > SUMT:
                l, deps["sum"] = _chain(jnp.add, [e[:, c:c + TQ] for c in range(0, e.shape[1], TQ)], z, deps["sum"])
            return e, jnp.sum(l, axis=1, keepdims=True)

        def softmax_pv(step, j, hh, sc):
            off, nc = geom(j)
            com, ext, left = sc
            es, ls = [], []
            if hh == 0:
                deps["sum"] = None
            for b in range(G):
                rs = slice(b * RG, (b + 1) * RG)
                parts = [left[rs]] if off else []
                parts += [com[rs, t * TQ:(t + 1) * TQ] for t in range(nc)]
                parts += [ext[e][(b - e) * RG:(b - e + 1) * RG] for e in range(1, b + 1)]
                parts[-1] = jnp.where(diag if nc + b else col <= row + (off - RG), parts[-1], NEG)
                e, l = softmax(parts)
                es.append(e)
                ls.append(l)
            w = es[0].shape[1]
            vpu = 0 < off <= VO
            vs = [_ld(v_s, 0, TQ, head(hh))] if off and not vpu else []
            if nc:
                vs.append(_ld(v_s, off, nc * TQ, head(hh)))
            if vpu:
                fill.append(bout(slice(None), slice(len(fill) * 128, len(fill) * 128 + 128), slice(0, 128)))
            o = [jnp.dot(jnp.concatenate([e[:, TQ * vpu:w] for e in es], axis=0).astype(BF16),
                         jnp.concatenate(vs, axis=0), preferred_element_type=F32)] if vs else []
            ox = {e: jnp.dot(jnp.concatenate([x[:, w + (e - 1) * TQ:w + e * TQ] for x in es[e:]], axis=0).astype(BF16),
                             _ld(v_s, off + (nc + e - 1) * TQ, TQ, head(hh)), preferred_element_type=F32)
                  for e in PV_ORD.get(step - LOOK, range(1, G))}
            ov = []
            if vpu:
                pt = jnp.concatenate([e[:, :off] for e in es], axis=0).T
                pb = [jnp.broadcast_to(pt[k:k + 1], (VG, TQ)) for k in range(off)]
                due.setdefault(step + 1 + (j < G), []).append(_zero_after(z, pt))
                ot = []
                for r in reversed(range(0, D, VG)):
                    a = None
                    for k in range(off):
                        p8 = pb[k][:8] if deps["pv"] is None or k % 2 else _after(pb[k][:8], deps["pv"])
                        pr = ((_hi if k % 2 else _lo)(vbw[hh, k // 2])[r:r + VG]
                              * jnp.concatenate([p8] * (VG // 8), axis=0))
                        a = pr if a is None else a + pr
                        deps["pv"] = _zero_after(z, a)
                    ot.append(a)
                ov = [jnp.concatenate(ot[::-1], axis=0).T]
            og = [[x[b * RG:(b + 1) * RG] for x in o] + [ox[e][(b - e) * RG:(b - e + 1) * RG] for e in range(1, b + 1)]
                  + [x[b * RG:(b + 1) * RG] for x in ov] for b in range(G)]
            og = jnp.concatenate([functools.reduce(jnp.add, x) for x in og], axis=0)
            return og * (gather(g_v, j) * _recip(jnp.concatenate(ls, axis=0)))

        def oproj(j, o0, o1):
            y = gather(acc_v, j) + jnp.dot(jnp.concatenate([o0, o1], axis=1).astype(BF16),
                                           _ld(wo_v, p * (2 * D), 2 * D), preferred_element_type=F32)
            for b, r in enumerate(rows(j)):
                acc_v[r:r + RG, :] = y[b * RG:(b + 1) * RG]
                if r < S - TL:
                    o_st[r // TQ, r % TQ:r % TQ + RG, :] = y[b * RG:(b + 1) * RG].astype(BF16)
            j0 = j - j % G
            pl.when(last)(cp_o(j0, min(G, nq - 1 - j0), j % G * RG, RG).start)

        nq = S // TQ
        items = [(j, hh) for j in ORDER for hh in range(2)]
        n = len(items)
        s_vals, o_vals = {}, {}
        wop = jnp.concatenate([f(bwo_p[dp]) for dp in range(DH // 2) for f in (_lo, _hi)], axis=0)
        qproj(ORDER[0])
        for step in range(n + LOOK + OLAG):
            if step % 2 == 0 and 1 + step // 2 < nq:
                qproj(ORDER[1 + step // 2])
            if step < n:
                s_vals[step] = qk(step, *items[step])
            if step == LOOK:
                fill1 = [bout(slice(None), slice(k * 128, k * 128 + 128), slice(128, 256)) for k in range(4)]
            b = step - LOOK
            if 0 <= b < n:
                o_vals[b] = softmax_pv(step, *items[b], s_vals.pop(b))
            c = step - LOOK - OLAG
            if 0 <= c < n and c % 2 == 1:
                oproj(items[c][0], o_vals.pop(c - 1), o_vals.pop(c))

        def add16(ts):
            return jnp.concatenate([functools.reduce(jnp.add, [t[r:r + 16] for t in ts]) for r in range(0, TL, 16)],
                                   axis=0)

        assert len(fill) == NT_M
        early = [add16(fill), add16(fill1 + [bout(slice(None), slice(512, M), slice(128, 256))]),
                 bout(slice(None), slice(None), slice(256, c0))]
        yl = acc_v[pl.ds(rb, TL), :c0] + jnp.concatenate(early, axis=1)
        ya = acc_v[pl.ds(rb, TL), c0:]
        yr = [[ya[r:r + 16, c:c + 128] for r in range(0, TL, 16)] for c in range(0, M - c0, 128)]
        for tile in range(NT_M * NCUT):
            c, k = divmod(tile, NT_M)
            cuts = (0,) + CUTS.get(tile, ()) + (TL // 16,)
            for u0, u1 in zip(cuts[:-1], cuts[1:]):
                t = bout(slice(u0 * 16, u1 * 16), slice(k * 128, k * 128 + 128), slice(c0 + c * 128, c0 + c * 128 + 128))
                for u in range(u0, u1):
                    yr[c][u] = yr[c][u] + t[(u - u0) * 16:(u - u0 + 1) * 16]
        y = jnp.concatenate([yl] + [jnp.concatenate(v, axis=0) for v in yr], axis=1)
        acc_v[pl.ds(rb, TL), :] = y
        for ca, cb in zip(OCUT[:-1], OCUT[1:]):
            o_st[S // TQ - 1, :, ca:cb] = y[:, ca:cb].astype(BF16)
            pl.when(last)(cp_o(S // TQ - 1, 1, 0, TQ, ca, cb).start)
        return 0

    for cc in ([w0[0], x0[0], w0[1], x0[1], x0[2], x0[3], w0[2], cp_w(1), cp_g, xr]
               + [cp_w(k) for k in range(2, NT_M)] + a_early):
        cc.start()
    z_v[...] = jnp.zeros((8, 128), U32)
    for part in range(3):
        for t in range(NT_M):
            qkv_v[part, t, 0:PAD, :] = jnp.zeros((PAD, 128), F32)

    def phases():
        first_task()
        lax.fori_loop(1, NT_M, _scoped("bproj", bproj_body), 0)
        for cc in a_waits:
            cc.wait()
        lax.fori_loop(0, HP, _scoped("pair", pair_body), 0)

    def once(i, _):
        pl.when(i == 0)(phases)
        return 0

    lax.fori_loop(0, 2, once, 0)
    with _scope("ow"):
        cp_o(0, S // TQ, 0, TQ).wait()


def _kernel(*refs):
    dma = pltpu.SemaphoreType.DMA
    pl.run_scoped(functools.partial(_body, *refs), dma((6,)), dma((NT_M + 2,)), dma(()), dma(()))


@jax.jit
def pallas_gated_mix__compressed_kv_cla__sliding_local_dilated__prompt_kernel(
    A_x, A_c_kv, A_w_q, A_w_uk, A_w_uv, A_w_o, B_x, B_wqkv, B_wo, gate_w,
):
    del B_x
    x = A_x.reshape(S, M)
    ckv = A_c_kv.reshape(S, DC)
    wo = A_w_o.reshape(H * D, M)
    bwo = B_wo.reshape(H, DH, M)
    any_spec = pl.BlockSpec(memory_space=pl.ANY)
    out = pl.pallas_call(
        _kernel,
        out_shape=jax.ShapeDtypeStruct((S // TQ, TQ, M), BF16),
        in_specs=[any_spec] * 9,
        out_specs=any_spec,
        scratch_shapes=[
            pltpu.VMEM((S // 2, M), U32),
            pltpu.VMEM((S // 2, DC), U32),
            pltpu.VMEM((HP, M, D), U32),
            pltpu.VMEM((HP, DC, D), U32),
            pltpu.VMEM((HP, DC, D), U32),
            pltpu.VMEM((H * D // 2, M), U32),
            pltpu.VMEM((M, 3 * M), BF16),
            pltpu.VMEM((DH // 2, H, M), U32),
            pltpu.VMEM((3, DH * 24, 128), U32),
            pltpu.VMEM((64, 512), U32),
            pltpu.VMEM((3, NT_M, S + PAD, 128), F32),
            pltpu.VMEM((S, M), F32),
            pltpu.VMEM((S, 128), F32),
            pltpu.VMEM((8, 128), U32),
            pltpu.VMEM((S // 2, 2 * D), U32),
            pltpu.VMEM((S // 2, 2 * D), U32),
            pltpu.VMEM((S // 2, 2 * D), U32),
            pltpu.VMEM((S // TQ, TQ, M), BF16),
            pltpu.VMEM((2 * M,), BF16),
        ],
        compiler_params=pltpu.CompilerParams(vmem_limit_bytes=110 * 1024 * 1024),
    )(x, ckv, A_w_q, A_w_uk, A_w_uv, wo, B_wqkv, bwo, gate_w)
    return out.reshape(1, S, M)
```
